```python
import jax
import jax.numpy as jnp

def _softmax(x, axis=-1):
    return jax.nn.softmax(x, axis=axis)

def _gelu(x):
    return jax.nn.gelu(x, approximate=True)

def _silu(x):
    return jax.nn.silu(x)

def _sigmoid(x):
    return jax.nn.sigmoid(x)

def _layernorm(x, axis=-1, eps=1e-05):
    m = jnp.mean(x, axis=axis, keepdims=True)
    v = jnp.var(x, axis=axis, keepdims=True)
    return (x - m) / jnp.sqrt(v + eps)

def _scatter_add(tgt, idx, src, axis=0):
    return tgt.at[idx].add(src)

def _segment_sum(src, seg, n):
    return jax.ops.segment_sum(src, seg, n)

class _Rng:

    def __init__(self, key):
        self._k = key

    def _next(self):
        self._k, sub = jax.random.split(self._k)
        return sub

    def normal(self, shape):
        return jax.random.normal(self._next(), shape, dtype=jnp.bfloat16)

    def randint(self, lo, hi, shape):
        return jax.random.randint(self._next(), shape, lo, hi, dtype=jnp.int32)

    def uniform(self, shape, lo=0.0, hi=1.0):
        return jax.random.uniform(self._next(), shape, jnp.bfloat16, lo, hi)

    def permutation(self, n):
        return jax.random.permutation(self._next(), n)
kernel_name = 'gated_mix__ssm_conv_h3__memory_aug_recurrent_mem_tr__prompt'

def setup_inputs():
    _rng = _Rng(jax.random.key(int.from_bytes(__import__("os").urandom(4), "little")))
    _w = lambda a: (lambda t: t.astype(jnp.bfloat16) if jnp.issubdtype(t.dtype, jnp.floating) else t)(jnp.asarray(a))

    def _A_setup():
        B, S, D = (1, 2048, 1024)
        ks = 4
        return {'q': _w((lambda *s: _rng.normal(s) * 0.05)(B, S, D)), 'k': _w((lambda *s: _rng.normal(s) * 0.05)(B, S, D)), 'v': _w((lambda *s: _rng.normal(s) * 0.05)(B, S, D)), 'shift_k': _w((lambda *s: _rng.normal(s) * 0.05)(D, ks) * 0.5), 'ssm_k': _w((lambda *s: _rng.normal(s) * 0.05)(D, S) * (1.0 / S ** 0.5)), 'ssm_D': _w((lambda *s: _rng.normal(s) * 0.05)(D))}
    _A_in = _A_setup()

    def _B_setup():
        B, S, Dm = (1, 2048, 1024)
        H, Dh = (32, 128)
        M, seg = (8, 32)
        seg = min(seg, S)
        S = S // seg * seg
        return {'x': _w((lambda *s: _rng.normal(s) * 0.05)(B, S, Dm)), 'mem0': _w((lambda *s: _rng.normal(s) * 0.05)(B, M, Dm)), 'Wq': _w((lambda *s: _rng.normal(s) * 0.05)(Dm, H, Dh) * Dm ** (-0.5)), 'Wk': _w((lambda *s: _rng.normal(s) * 0.05)(Dm, H, Dh) * Dm ** (-0.5)), 'Wv': _w((lambda *s: _rng.normal(s) * 0.05)(Dm, H, Dh) * Dm ** (-0.5)), 'Wo': _w((lambda *s: _rng.normal(s) * 0.05)(H, Dh, Dm) * (H * Dh) ** (-0.5)), 'seg_len': seg}
    _B_in = _B_setup()
    return {'A_q': _A_in['q'], 'A_k': _A_in['k'], 'A_v': _A_in['v'], 'A_shift_k': _A_in['shift_k'], 'A_ssm_k': _A_in['ssm_k'], 'A_ssm_D': _A_in['ssm_D'], 'B_x': _B_in['x'], 'B_mem0': _B_in['mem0'], 'B_Wq': _B_in['Wq'], 'B_Wk': _B_in['Wk'], 'B_Wv': _B_in['Wv'], 'B_Wo': _B_in['Wo'], 'B_seg_len': _B_in['seg_len'], 'gate_w': _w((lambda *s: _rng.normal(s) * 0.05)(1024))}

def reference(A_q, A_k, A_v, A_shift_k, A_ssm_k, A_ssm_D, B_x, B_mem0, B_Wq, B_Wk, B_Wv, B_Wo, B_seg_len, gate_w):

    def _A_ref(q, k, v, shift_k, ssm_k, ssm_D):
        B, S, D = q.shape
        ks = shift_k.shape[-1]
        k_pad = jnp.pad(k, ((0, 0), (ks - 1, 0), (0, 0)))
        k_shift = jnp.zeros_like(k)
        for t in range(ks):
            k_shift = k_shift + k_pad[:, t:t + S, :] * shift_k[:, ks - 1 - t][None, None, :]
        kv = k_shift * v
        L = 2 * S
        kv_pad = jnp.pad(kv, ((0, 0), (0, S), (0, 0)))
        kf_pad = jnp.pad(ssm_k, ((0, 0), (0, S)))
        kv_f = (lambda x, axes=(-2, -1): jnp.fft.rfft2(x.astype(jnp.float32), axes=axes))(kv_pad[:, None, :, :], axes=(1, 2))
        kf_f = (lambda x, axes=(-2, -1): jnp.fft.rfft2(x.astype(jnp.float32), axes=axes))(kf_pad[:, None, :], axes=(1, 2))
        kf_f = (lambda x, *d: x.transpose(*d))(kf_f, 1, 2, 0)
        y_f = kv_f * kf_f[None, :, :, :]
        y = (lambda x, s, axes=(-2, -1): jnp.fft.irfft2(x, s=s, axes=axes).astype(jnp.bfloat16))(y_f, (1, L), axes=(1, 2))[:, 0, :S, :]
        y = y + kv * ssm_D[None, None, :]
        return q * y

    def _B_ref(x, mem0, Wq, Wk, Wv, Wo, seg_len):
        B, S, Dm = x.shape
        H, Dh = (Wq.shape[1], Wq.shape[2])
        M = mem0.shape[1]
        scale = Dh ** (-0.5)
        n_seg = S // seg_len
        L = M + seg_len
        idx = jnp.arange(L)
        mask = (idx[:, None] < M) | (idx[:, None] >= idx[None, :])
        mem = mem0
        outs = []
        for s in range(n_seg):
            xs = x[:, s * seg_len:(s + 1) * seg_len, :].copy()
            h = jnp.concatenate([mem, xs], axis=1)
            q = jnp.einsum('btd,dhe->bhte', h, Wq)
            k = jnp.einsum('btd,dhe->bhte', h, Wk)
            v = jnp.einsum('btd,dhe->bhte', h, Wv)
            scores = jnp.einsum('bhqe,bhke->bhqk', q, k) * scale
            scores = jnp.where(mask[None, None], scores, -1000000000.0)
            p = _softmax(scores, axis=-1)
            o = jnp.einsum('bhqk,bhke->bhqe', p, v)
            o = jnp.einsum('bhte,hed->btd', o, Wo)
            mem = o[:, :M, :].copy()
            outs.append(o[:, M:, :])
        return jnp.concatenate(outs, axis=1)
    x = A_q
    g = _sigmoid((x * gate_w).sum(-1, keepdims=True))
    a = _A_ref(x, A_k, A_v, A_shift_k, A_ssm_k, A_ssm_D)
    b = _B_ref(x, B_mem0, B_Wq, B_Wk, B_Wv, B_Wo, B_seg_len)
    return g * a + (1 - g) * b
```

```python
import functools

import numpy as np
import jax
import jax.numpy as jnp
from jax import lax
import jax.experimental.pallas as pl
import jax.experimental.pallas.tpu as pltpu

S, D, H, E, M, SEG = 2048, 1024, 32, 128, 8, 32
NSEG = S // SEG
NT = SEG - M
NP = H // 2
NCB = D // 128
C = 128
NCH = S // C
KS = 4
UNROLL = 2
bf16, f32, u32 = jnp.bfloat16, jnp.float32, jnp.uint32


def _dft_tables():
    t = np.arange(C, dtype=np.float64)
    rows = []
    for r in range(8):
        ev = 16 * r + np.arange(0, 16, 2)
        od = ev + 1
        for fn, fs in ((np.cos, ev), (np.cos, od), (np.sin, ev), (np.sin, od)):
            rows.append(fn(np.pi * (2 * fs[:, None] + 1) * t[None, :] / (2 * C)))
    f = np.concatenate(rows, axis=0)
    return f.astype(np.float32), (f.T / C).astype(np.float32)


def _fill_matrix():
    r = lax.broadcasted_iota(jnp.int32, (80, 80), 0)
    c = lax.broadcasted_iota(jnp.int32, (80, 80), 1)

    def head(i):
        return jnp.where(i < 64, i // 32, (i - 64) // 8)

    def idx(i):
        lo = i % 32
        main = jnp.where(lo < NT, lo + M, lo - NT)
        return jnp.where(i < 64, main, (i - 64) % 8 + NT + M)

    same = head(r) == head(c)
    ok = (idx(r) < M) | (idx(r) >= idx(c))
    return jnp.where(same, jnp.where(ok, 0.0, -1e9), -jnp.inf).astype(f32)


def _as_bf16(v):
    return pltpu.bitcast(v, bf16)


def _dot(a, b):
    return jnp.dot(a, b, preferred_element_type=f32)


def _dot_nt(a, b):
    return lax.dot_general(a, b, (((1,), (1,)), ((), ())), preferred_element_type=f32)


(SEM_XB, SEM_X, SEM_K, SEM_V, SEM_SSM, SEM_SHIFT, SEM_D, SEM_GW, SEM_MEM, SEM_F, SEM_G) = range(11)
SEM_W = 11
SEM_WO = SEM_W + 6
SEM_OUT = SEM_WO + 8
NSEM = SEM_OUT + 2


def _kernel(x_hbm, k_hbm, v_hbm, shift_hbm, ssm_hbm, d_hbm, mem_hbm, wq_hbm, wk_hbm, wv_hbm,
            wo_hbm, gw_hbm, f_hbm, g_hbm, out_hbm,
            wn_ref, wo_ref, x_ref, xb_ref, pre_ref, k_ref, v_ref, ssm_ref, u_ref, z_ref,
            fu_ref, fk_ref, kf_ref, f_ref, g_ref, fill_ref, shift_ref, wt_ref, d_ref, gw_ref,
            mem_ref, gate_ref, ost_ref, sems):
    w_hbm = (wq_hbm, wk_hbm, wv_hbm)

    def cp(src, dst, sem):
        return pltpu.make_async_copy(src, dst, sems.at[sem])

    cp_xb = cp(x_hbm.at[:, NT:SEG, :], x_ref.at[:, NT:SEG, :], SEM_XB)
    cp_x = cp(x_hbm.at[:, 0:NT, :], x_ref.at[:, 0:NT, :], SEM_X)
    cp_k = cp(k_hbm, k_ref, SEM_K)
    cp_v = cp(v_hbm, v_ref, SEM_V)
    cp_ssm = cp(ssm_hbm, ssm_ref, SEM_SSM)
    small = [cp(shift_hbm, shift_ref, SEM_SHIFT), cp(d_hbm, d_ref, SEM_D), cp(gw_hbm, gw_ref, SEM_GW),
             cp(mem_hbm, mem_ref, SEM_MEM), cp(f_hbm, f_ref, SEM_F), cp(g_hbm, g_ref, SEM_G)]
    wo32 = wo_hbm.bitcast(u32)
    cp_wo = [cp(wo32.at[:, n * 128:(n + 1) * 128], wo_ref.at[n], SEM_WO + n) for n in range(NCB)]

    def conv_prep(cb, r):
        lanes = pl.ds(pl.multiple_of(cb * 128, 128), 128)
        row0 = pl.multiple_of(r * 256, 256)
        prev0 = pl.multiple_of(jnp.maximum(row0 - 16, 0), 16)
        prev = k_ref[pl.ds(prev0, 16), lanes].astype(f32)[8:16]
        kf_ref[0:8, :] = jnp.where(r > 0, prev, 0.0)
        kf_ref[8:264, :] = k_ref[pl.ds(row0, 256), lanes].astype(f32)
        w = wt_ref[cb]
        ks = kf_ref[8:264, :] * w[0:1, :]
        for j in range(1, KS):
            ks = ks + kf_ref[8 - j:264 - j, :] * w[j:j + 1, :]
        kv = (ks * v_ref[pl.ds(row0, 256), lanes].astype(f32)).astype(bf16)
        u_ref[cb, pl.ds(pl.multiple_of(r * 128, 128), 128), :] = pltpu.bitcast(kv, u32)

    def conv_fwd(cb, r):
        fr = f_ref[pl.ds(pl.multiple_of(r * 32, 32), 32), :]
        rows = pl.ds(pl.multiple_of(cb * 128, 128), 128)
        prev = None
        for a in range(NCH):
            fu_ref[a] = _dot(fr, _as_bf16(u_ref[cb, a * 64:(a + 1) * 64, :]))
            kf = _dot_nt(fr, ssm_ref[rows, a * C:(a + 1) * C])
            if prev is None:
                fk_ref[a] = kf
            else:
                fk_ref[a] = jnp.concatenate([kf[0:8] + prev[16:24], kf[8:16] - prev[24:32],
                                             kf[16:24] - prev[0:8], kf[24:32] + prev[8:16]], axis=0)
            prev = kf

    def conv_mac(cb, r, a):
        p = q = None
        for c in range(a + 1):
            ua, ub = fu_ref[a - c, 0:16, :], fu_ref[a - c, 16:32, :]
            kc, kd = fk_ref[c, 0:16, :], fk_ref[c, 16:32, :]
            pp = ua * kc - ub * kd
            qq = ua * kd + ub * kc
            p = pp if p is None else p + pp
            q = qq if q is None else q + qq
        z = jnp.concatenate([p, q], axis=0).astype(bf16)
        z_ref[cb % 2, a, pl.ds(pl.multiple_of(r * 16, 16), 16), :] = pltpu.bitcast(z, u32)

    def conv_inv(a_ref, cb, dst, a):
        lanes = pl.ds(pl.multiple_of(cb * 128, 128), 128)
        y = _dot(g_ref[...], _as_bf16(z_ref[cb % 2, a]))
        kv = _as_bf16(u_ref[cb, pl.ds(pl.multiple_of(a * 64, 64), 64), :]).astype(f32)
        q = x_ref[pl.ds(a * 4, 4), :, lanes].astype(f32).reshape(C, 128)
        dv = d_ref[:, lanes].astype(f32)
        a_ref[dst, pl.ds(pl.multiple_of(a * C, C), C), :] = q * (y + kv * dv)

    def prologue(stage_ref):
        st3 = stage_ref.reshape(6 * D, 8, E)
        cp_w = [cp(w_hbm[g // 2].bitcast(u32).at[:, (g % 2) * 8:(g % 2) * 8 + 8, :],
                   st3.at[g * D:(g + 1) * D], SEM_W + g) for g in range(6)]
        cp_xb.start()
        cp_w[0].start()
        for c in small:
            c.start()
        fill_ref[...] = _fill_matrix()
        cp_xb.wait()

        def xb_build(it, c):
            s0 = pl.multiple_of(it * 8, 8)
            t = x_ref[pl.ds(s0, 8), NT:SEG, :].astype(f32).reshape(64, D).astype(bf16)
            xb_ref[pl.ds(pl.multiple_of(it * 32, 32), 32), :] = pltpu.bitcast(t, u32)
            return c
        lax.fori_loop(0, 8, xb_build, 0)
        for c in small:
            c.wait()
        eye = (lax.broadcasted_iota(jnp.int32, (8, KS), 0)
               == lax.broadcasted_iota(jnp.int32, (8, KS), 1)).astype(f32).astype(bf16)
        wt = _dot_nt(eye, shift_ref[...])
        for n in range(NCB):
            wt_ref[n] = wt[:, n * 128:(n + 1) * 128]

        later = {0: [cp_w[1], cp_k, cp_v], 1: [cp_w[2], cp_x], 2: [cp_w[3], cp_ssm],
                 3: [cp_w[4]] + cp_wo[0:4], 4: [cp_w[5]] + cp_wo[4:8], 5: []}

        def group(g, c):
            for gg in range(6):
                @pl.when(g == gg)
                def _():
                    cp_w[gg].wait()
                    for cc in later[gg]:
                        cc.start()
            sub = stage_ref.at[pl.ds(pl.multiple_of(g * (8 * D), 8 * D), 8 * D), :]

            def relayout(j):
                for blk in range(D // 256):
                    w = sub[pl.ds(blk * 2048 + j, 256, stride=8), :]
                    lo = pltpu.bitcast(w << 16, f32).astype(bf16)
                    hi = pltpu.bitcast(w & jnp.uint32(0xFFFF0000), f32).astype(bf16)
                    wn_ref[g * 16 + 2 * j, blk * 128:(blk + 1) * 128, :] = pltpu.bitcast(lo, u32)
                    wn_ref[g * 16 + 2 * j + 1, blk * 128:(blk + 1) * 128, :] = pltpu.bitcast(hi, u32)

            relayout(0)
            for j in range(8):
                if j + 1 < 8:
                    relayout(j + 1)
                xb = _as_bf16(xb_ref[...])
                r1 = _dot(xb, _as_bf16(wn_ref[g * 16 + 2 * j]))
                r2 = _dot(xb, _as_bf16(wn_ref[g * 16 + 2 * j + 1]))
                cc = jnp.concatenate([r1.reshape(NSEG, 8, E), r2.reshape(NSEG, 8, E)], axis=1).astype(bf16)
                pre_ref[g * 8 + j] = pltpu.bitcast(cc, u32)
            return c
        lax.fori_loop(0, 6, group, 0)

    pl.run_scoped(prologue, pltpu.VMEM((6 * 8 * D, E), u32))

    cp_k.wait()
    cp_v.wait()
    cp_x.wait()
    cp_ssm.wait()
    for c in cp_wo:
        c.wait()

    def prep0(r, c):
        conv_prep(0, r)
        return c
    lax.fori_loop(0, 8, prep0, 0)
    conv_fwd(0, 0)

    scale = E ** -0.5

    def main(odef_ref, b_ref, a_ref):
        def step(s, mem):
            cb = s // 8
            r = s % 8
            pcb = jnp.maximum(cb - 1, 0)
            pdst = jnp.where(cb > 0, cb - 1, NCB)
            conv_inv_prev = lambda a: conv_inv(a_ref, pcb, pdst, a)

            xs = x_ref[s].astype(f32)
            h32 = jnp.concatenate([xs[0:NT], mem], axis=0).astype(bf16)
            r0 = pl.multiple_of(s * 8, 8)

            conv_inv_prev(2 * r)
            conv_inv_prev(2 * r + 1)

            gl = jnp.sum(xs * gw_ref[...].astype(f32), axis=-1, keepdims=True)
            gate_ref[s] = jnp.broadcast_to(jax.nn.sigmoid(gl), (SEG, 128))

            def proj(m, j):
                r1 = _dot(h32, _as_bf16(wn_ref[m * H + 2 * j]))
                r2 = _dot(h32, _as_bf16(wn_ref[m * H + 2 * j + 1]))
                p = _as_bf16(pre_ref[m * NP + j, s]).astype(f32)
                return jnp.concatenate([r1, r2, p], axis=0).astype(bf16)

            def qk(q80, k80):
                fill = fill_ref[...]
                sc = jnp.where(fill == 0.0, _dot_nt(q80, k80) * scale, fill)
                p = jnp.exp(sc - jnp.max(sc, axis=-1, keepdims=True))
                den = jnp.sum(p, axis=-1, keepdims=True)
                rc = pl.reciprocal(den, approx=True)
                return p.astype(bf16), rc * (2.0 - den * rc)

            def pv(j, p, rden, v80):
                o80 = _dot(p, v80) * rden
                odef_ref[pl.ds(r0, 8), (2 * j) * E:(2 * j + 1) * E] = o80[64:72]
                odef_ref[pl.ds(r0, 8), (2 * j + 1) * E:(2 * j + 2) * E] = o80[72:80]
                return jnp.concatenate([o80[0:32], o80[32:64]], axis=1).astype(bf16)

            def wo_part(o, j0, j1, n, acc=None):
                for j in range(j0, j1):
                    d = _dot(o[j], _as_bf16(wo_ref[n, j * 128:(j + 1) * 128, :]))
                    acc = d if acc is None else d + acc
                return acc

            qs, ks, vs, ps, os_ = {}, {}, {}, {}, {}
            for j in range(NP):
                qs[j] = proj(0, j)
                if j >= 1:
                    ps[j - 1] = qk(qs[j - 1], ks[j - 1])
                if j >= 2:
                    os_[j - 2] = pv(j - 2, *ps[j - 2], vs[j - 2])
                ks[j] = proj(1, j)
                vs[j] = proj(2, j)
                conv_mac(cb, r, j)
            na = NP - 2
            acc = {}
            acc[0] = wo_part(os_, 0, na, 0)
            ps[NP - 1] = qk(qs[NP - 1], ks[NP - 1])
            os_[NP - 2] = pv(NP - 2, *ps[NP - 2], vs[NP - 2])
            acc[1] = wo_part(os_, 0, na, 1)
            acc[2] = wo_part(os_, 0, na, 2)
            os_[NP - 1] = pv(NP - 1, *ps[NP - 1], vs[NP - 1])
            conv_prep(jnp.minimum(cb + 1, NCB - 1), r)
            acc[3] = wo_part(os_, 0, na, 3)
            for n in range(4):
                acc[n] = wo_part(os_, na, NP, n, acc[n])
            for n in range(4, 8):
                acc[n] = wo_part(os_, 0, NP, n)
            sn = jnp.minimum(s + 1, NSEG - 1)
            conv_fwd(sn // 8, sn % 8)
            acc = jnp.concatenate([acc[n] for n in range(8)], axis=1)
            b_ref[s, 0:NT, :] = acc[0:NT]
            return acc[NT:SEG].astype(bf16).astype(f32)

        lax.fori_loop(0, NSEG, step, mem_ref[...].astype(f32), unroll=UNROLL)

        def out_copy(n):
            slot = n % 2
            return pltpu.make_async_copy(
                ost_ref.at[slot], out_hbm.at[:, :, pl.ds(pl.multiple_of(n * 128, 128), 128)],
                sems.at[SEM_OUT + slot])

        def fin(n, c):
            @pl.when(n >= 2)
            def _():
                out_copy(n - 2).wait()
            lanes = pl.ds(pl.multiple_of(n * 128, 128), 128)
            conv_inv(a_ref, NCB - 1, NCB - 1, 2 * n)
            conv_inv(a_ref, NCB - 1, NCB - 1, 2 * n + 1)
            bd = _dot(odef_ref[...].astype(bf16), _as_bf16(wo_ref[n]))
            b_ref[:, NT:SEG, lanes] = bd.reshape(NSEG, 8, 128)
            for blk in range(8):
                sg = slice(blk * 8, (blk + 1) * 8)
                b = b_ref[sg, :, lanes]
                a = a_ref[n, blk * 256:(blk + 1) * 256, :].reshape(8, SEG, 128)
                g = gate_ref[sg]
                ost_ref[n % 2, sg] = (g * a + (1.0 - g) * b).astype(bf16)
            out_copy(n).start()
            return c
        lax.fori_loop(0, NCB, fin, 0)
        out_copy(NCB - 2).wait()
        out_copy(NCB - 1).wait()

    pl.run_scoped(main, pltpu.VMEM((NSEG * 8, H * E), f32), pltpu.VMEM((NSEG, SEG, D), f32),
                  pltpu.VMEM((NCB + 1, S, 128), f32))


@jax.jit
def pallas_gated_mix__ssm_conv_h3__memory_aug_recurrent_mem_tr__prompt_kernel(
    A_q: jax.Array,
    A_k: jax.Array,
    A_v: jax.Array,
    A_shift_k: jax.Array,
    A_ssm_k: jax.Array,
    A_ssm_D: jax.Array,
    B_x: jax.Array,
    B_mem0: jax.Array,
    B_Wq: jax.Array,
    B_Wk: jax.Array,
    B_Wv: jax.Array,
    B_Wo: jax.Array,
    B_seg_len: jax.Array,
    gate_w: jax.Array,
):
    del B_x, B_seg_len
    f_tab, g_tab = _dft_tables()
    out = pl.pallas_call(
        _kernel,
        out_shape=jax.ShapeDtypeStruct((NSEG, SEG, D), bf16),
        in_specs=[pl.BlockSpec(memory_space=pl.ANY)] * 14,
        out_specs=pl.BlockSpec(memory_space=pl.ANY),
        scratch_shapes=[
            pltpu.VMEM((3 * H, D // 2, E), u32),
            pltpu.VMEM((NCB, H * E // 2, 128), u32),
            pltpu.VMEM((NSEG, SEG, D), bf16),
            pltpu.VMEM((NSEG * 4, D), u32),
            pltpu.VMEM((3 * NP, NSEG, 8, E), u32),
            pltpu.VMEM((S, D), bf16),
            pltpu.VMEM((S, D), bf16),
            pltpu.VMEM((D, S), bf16),
            pltpu.VMEM((NCB, S // 2, 128), u32),
            pltpu.VMEM((2, NCH, 128, 128), u32),
            pltpu.VMEM((NCH, 32, 128), f32),
            pltpu.VMEM((NCH, 32, 128), f32),
            pltpu.VMEM((264, 128), f32),
            pltpu.VMEM((256, 128), bf16),
            pltpu.VMEM((128, 256), bf16),
            pltpu.VMEM((80, 80), f32),
            pltpu.VMEM((D, KS), bf16),
            pltpu.VMEM((NCB, 8, 128), f32),
            pltpu.VMEM((1, D), bf16),
            pltpu.VMEM((1, D), bf16),
            pltpu.VMEM((M, D), bf16),
            pltpu.VMEM((NSEG, SEG, 128), f32),
            pltpu.VMEM((2, NSEG, SEG, 128), bf16),
            pltpu.SemaphoreType.DMA((NSEM,)),
        ],
        compiler_params=pltpu.CompilerParams(vmem_limit_bytes=120 * 2**20),
    )(A_q.reshape(NSEG, SEG, D), A_k.reshape(S, D), A_v.reshape(S, D), A_shift_k, A_ssm_k,
      A_ssm_D.reshape(1, D), B_mem0.reshape(M, D), B_Wq, B_Wk, B_Wv, B_Wo.reshape(H * E, D),
      gate_w.reshape(1, D), jnp.asarray(f_tab, bf16), jnp.asarray(g_tab, bf16))
    return out.reshape(1, S, D)
```

```python
import functools

import numpy as np
import jax
import jax.numpy as jnp
from jax import lax
import jax.experimental.pallas as pl
import jax.experimental.pallas.tpu as pltpu

S, D, H, E, M, SEG = 2048, 1024, 32, 128, 8, 32
NSEG = S // SEG
NT = SEG - M
NP = H // 2
NCB = D // 128
C = 128
NCH = S // C
KS = 4
UNROLL = 2
_DBG_STEPS = NSEG
bf16, f32, u32 = jnp.bfloat16, jnp.float32, jnp.uint32


def _dft_tables():
    t = np.arange(C, dtype=np.float64)
    rows = []
    for r in range(8):
        ev = 16 * r + np.arange(0, 16, 2)
        od = ev + 1
        for fn, fs in ((np.cos, ev), (np.sin, ev), (np.cos, od), (np.sin, od)):
            rows.append(fn(np.pi * (2 * fs[:, None] + 1) * t[None, :] / (2 * C)))
    f = np.concatenate(rows, axis=0)
    return f.astype(np.float32), (f.T / C).astype(np.float32)


def _fill_matrix():
    r = lax.broadcasted_iota(jnp.int32, (80, 80), 0)
    c = lax.broadcasted_iota(jnp.int32, (80, 80), 1)

    def head(i):
        return jnp.where(i < 64, i // 32, (i - 64) // 8)

    def idx(i):
        lo = i % 32
        main = jnp.where(lo < NT, lo + M, lo - NT)
        return jnp.where(i < 64, main, (i - 64) % 8 + NT + M)

    same = head(r) == head(c)
    ok = (idx(r) < M) | (idx(r) >= idx(c))
    return jnp.where(same, jnp.where(ok, 0.0, -1e9), -jnp.inf).astype(f32)


def _as_bf16(v):
    return pltpu.bitcast(v, bf16)


def _dot(a, b):
    return jnp.dot(a, b, preferred_element_type=f32)


def _dot_nt(a, b):
    return lax.dot_general(a, b, (((1,), (1,)), ((), ())), preferred_element_type=f32)


(SEM_XB, SEM_X, SEM_K, SEM_V, SEM_SSM, SEM_SHIFT, SEM_D, SEM_GW, SEM_MEM, SEM_F, SEM_G) = range(11)
SEM_W = 11
SEM_WO = SEM_W + 6
SEM_OUT = SEM_WO + 8
NSEM = SEM_OUT + 2


def _kernel(x_hbm, k_hbm, v_hbm, shift_hbm, ssm_hbm, d_hbm, mem_hbm, wq_hbm, wk_hbm, wv_hbm,
            wo_hbm, gw_hbm, f_hbm, g_hbm, out_hbm,
            wn_ref, wo_ref, x_ref, xb_ref, pre_ref, k_ref, v_ref, ssm_ref, u_ref, z_ref,
            fu_ref, fk_ref, kraw_ref, one_ref, kf_ref, f_ref, g_ref, fill_ref, shift_ref, wt_ref, d_ref, gw_ref,
            mem_ref, gate_ref, ost_ref, sems):
    w_hbm = (wq_hbm, wk_hbm, wv_hbm)

    def cp(src, dst, sem):
        return pltpu.make_async_copy(src, dst, sems.at[sem])

    cp_xb = cp(x_hbm.at[:, NT:SEG, :], x_ref.at[:, NT:SEG, :], SEM_XB)
    cp_x = cp(x_hbm.at[:, 0:NT, :], x_ref.at[:, 0:NT, :], SEM_X)
    cp_k = cp(k_hbm, k_ref, SEM_K)
    cp_v = cp(v_hbm, v_ref, SEM_V)
    cp_ssm = cp(ssm_hbm, ssm_ref, SEM_SSM)
    small = [cp(shift_hbm, shift_ref, SEM_SHIFT), cp(d_hbm, d_ref, SEM_D), cp(gw_hbm, gw_ref, SEM_GW),
             cp(mem_hbm, mem_ref, SEM_MEM), cp(f_hbm, f_ref, SEM_F), cp(g_hbm, g_ref, SEM_G)]
    wo32 = wo_hbm.bitcast(u32)
    cp_wo = [cp(wo32.at[:, n * 128:(n + 1) * 128], wo_ref.at[n], SEM_WO + n) for n in range(NCB)]

    def conv_prep(cb, i, slot):
        lanes = pl.ds(pl.multiple_of(cb * 128, 128), 128)
        row0 = pl.multiple_of(i * 32, 32)
        prev0 = pl.multiple_of(jnp.maximum(row0 - 16, 0), 16)
        prev = k_ref[pl.ds(prev0, 16), lanes].astype(f32)[8:16]
        kf_ref[slot, 0:8, :] = jnp.where(i > 0, prev, 0.0)
        kcur = k_ref[pl.ds(row0, 32), lanes].astype(f32)
        kf_ref[slot, 8:40, :] = kcur
        w = wt_ref[cb]
        ks = kcur * w[0:1, :]
        for j in range(1, KS):
            ks = ks + kf_ref[slot, 8 - j:40 - j, :] * w[j:j + 1, :]
        kv = (ks * v_ref[pl.ds(row0, 32), lanes].astype(f32)).astype(bf16)
        kv = pltpu.bitcast(kv, u32)
        u_ref[cb, pl.ds(pl.multiple_of(i * 16, 16), 16), :] = kv
        return kv[0:8] | kv[8:16]

    def combine(kf, prev):
        out = []
        for g in range(8):
            o = 32 * g
            out += [kf[o:o + 8] + prev[o + 8:o + 16], kf[o + 8:o + 16] - prev[o:o + 8],
                    kf[o + 16:o + 24] - prev[o + 24:o + 32], kf[o + 24:o + 32] + prev[o + 16:o + 24]]
        return jnp.concatenate(out, axis=0)

    def conv_fwd(cb, r):
        slot = cb % 2
        rows = pl.ds(pl.multiple_of(cb * 128, 128), 128)
        f = f_ref[...]
        kfs = []
        for a in (2 * r, 2 * r + 1):
            fu_ref[slot, a] = _dot(f, _as_bf16(u_ref[cb, pl.ds(pl.multiple_of(a * 64, 64), 64), :]))
            kfs.append(_dot_nt(f, ssm_ref[rows, pl.ds(pl.multiple_of(a * C, C), C)]))
        fk_ref[slot, 2 * r] = combine(kfs[0], jnp.where(r > 0, kraw_ref[...], 0.0))
        fk_ref[slot, 2 * r + 1] = combine(kfs[1], kfs[0])
        kraw_ref[...] = kfs[1]

    def conv_fwd_next(cb, r):
        conv_fwd(jnp.where(cb + 1 < NCB, cb + 1, NCB - 2), r)

    def conv_mac(cb, r, a, half):
        slot = cb % 2
        ro = pl.multiple_of(r * 32 + half * 16, 16)
        p = q = None
        for c in range(a + 1):
            u = fu_ref[slot, a - c, pl.ds(ro, 16), :]
            k = fk_ref[slot, c, pl.ds(ro, 16), :]
            ua, ub, kc, kd = u[0:8], u[8:16], k[0:8], k[8:16]
            p = (ua * kc if p is None else p + ua * kc) - ub * kd
            q = (ua * kd if q is None else q + ua * kd) + ub * kc
        z = pltpu.bitcast(jnp.concatenate([p, q], axis=0).astype(bf16), u32)
        z_ref[slot, a, pl.ds(pl.multiple_of(r * 16 + half * 8, 8), 8), :] = z
        return z

    def after(w, tok):
        if tok is None:
            return w
        return jnp.concatenate([jnp.where(one_ref[...] == 1, w[0:8], tok), w[8:]], axis=0)

    def conv_inv(a_ref, cb, dst, a):
        lanes = pl.ds(pl.multiple_of(cb * 128, 128), 128)
        y = _dot(g_ref[...], _as_bf16(z_ref[cb % 2, a]))
        kv = _as_bf16(u_ref[cb, pl.ds(pl.multiple_of(a * 64, 64), 64), :]).astype(f32)
        q = x_ref[pl.ds(a * 4, 4), :, lanes].astype(f32).reshape(C, 128)
        dv = d_ref[:, lanes].astype(f32)
        a_ref[dst, pl.ds(pl.multiple_of(a * C, C), C), :] = q * (y + kv * dv)

    def prologue(stage_ref):
        st3 = stage_ref.reshape(6 * D, 8, E)
        cp_w = [cp(w_hbm[g // 2].bitcast(u32).at[:, (g % 2) * 8:(g % 2) * 8 + 8, :],
                   st3.at[g * D:(g + 1) * D], SEM_W + g) for g in range(6)]
        cp_xb.start()
        cp_w[0].start()
        for c in small:
            c.start()
        fill_ref[...] = _fill_matrix()
        one_ref[...] = jnp.ones((8, 128), jnp.int32)
        cp_xb.wait()

        def xb_build(it, c):
            s0 = pl.multiple_of(it * 8, 8)
            t = x_ref[pl.ds(s0, 8), NT:SEG, :].astype(f32).reshape(64, D).astype(bf16)
            xb_ref[pl.ds(pl.multiple_of(it * 32, 32), 32), :] = pltpu.bitcast(t, u32)
            return c
        lax.fori_loop(0, 8, xb_build, 0)
        for c in small:
            c.wait()
        eye = (lax.broadcasted_iota(jnp.int32, (8, KS), 0)
               == lax.broadcasted_iota(jnp.int32, (8, KS), 1)).astype(f32).astype(bf16)
        wt = _dot_nt(eye, shift_ref[...])
        for n in range(NCB):
            wt_ref[n] = wt[:, n * 128:(n + 1) * 128]

        later = {0: [cp_w[1], cp_k, cp_v], 1: [cp_w[2], cp_x], 2: [cp_w[3], cp_ssm],
                 3: [cp_w[4]] + cp_wo[0:4], 4: [cp_w[5]] + cp_wo[4:8], 5: []}

        def group(g, c):
            for gg in range(6):
                @pl.when(g == gg)
                def _():
                    cp_w[gg].wait()
                    for cc in later[gg]:
                        cc.start()
            sub = stage_ref.at[pl.ds(pl.multiple_of(g * (8 * D), 8 * D), 8 * D), :]

            def relayout(j):
                for blk in range(D // 256):
                    w = sub[pl.ds(blk * 2048 + j, 256, stride=8), :]
                    lo = pltpu.bitcast(w << 16, f32).astype(bf16)
                    hi = pltpu.bitcast(w & jnp.uint32(0xFFFF0000), f32).astype(bf16)
                    wn_ref[g * 16 + 2 * j, blk * 128:(blk + 1) * 128, :] = pltpu.bitcast(lo, u32)
                    wn_ref[g * 16 + 2 * j + 1, blk * 128:(blk + 1) * 128, :] = pltpu.bitcast(hi, u32)

            relayout(0)
            for j in range(8):
                if j + 1 < 8:
                    relayout(j + 1)
                xb = _as_bf16(xb_ref[...])
                r1 = _dot(xb, _as_bf16(wn_ref[g * 16 + 2 * j]))
                r2 = _dot(xb, _as_bf16(wn_ref[g * 16 + 2 * j + 1]))
                cc = jnp.concatenate([r1.reshape(NSEG, 8, E), r2.reshape(NSEG, 8, E)], axis=1).astype(bf16)
                pre_ref[g * 8 + j] = pltpu.bitcast(cc, u32)
            return c
        lax.fori_loop(0, 6, group, 0)

    pl.run_scoped(prologue, pltpu.VMEM((6 * 8 * D, E), u32))

    cp_k.wait()
    cp_v.wait()
    cp_x.wait()
    cp_ssm.wait()
    for c in cp_wo:
        c.wait()

    def prep0(r, c):
        for i in range(8):
            conv_prep(0, 8 * r + i, i)
        conv_fwd(0, r)
        return c
    lax.fori_loop(0, 8, prep0, 0)

    scale = E ** -0.5

    def main(odef_ref, b_ref, a_ref):
        def step(s, mem):
            cb = s // 8
            r = s % 8
            pcb = jnp.maximum(cb - 1, 0)
            pdst = jnp.where(cb > 0, cb - 1, NCB)
            conv_inv_prev = lambda a: conv_inv(a_ref, pcb, pdst, a)

            xs = x_ref[s].astype(f32)
            h32 = jnp.concatenate([xs[0:NT], mem], axis=0).astype(bf16)
            r0 = pl.multiple_of(s * 8, 8)

            conv_inv_prev(2 * r)
            conv_inv_prev(2 * r + 1)

            gl = jnp.sum(xs * gw_ref[...].astype(f32), axis=-1, keepdims=True)
            gate_ref[s] = jnp.broadcast_to(jax.nn.sigmoid(gl), (SEG, 128))

            def proj(m, j, tok=None):
                r1 = _dot(h32, _as_bf16(after(wn_ref[m * H + 2 * j], tok)))
                r2 = _dot(h32, _as_bf16(wn_ref[m * H + 2 * j + 1]))
                p = _as_bf16(pre_ref[m * NP + j, s]).astype(f32)
                return jnp.concatenate([r1, r2, p], axis=0).astype(bf16)

            def qk(q80, k80):
                fill = fill_ref[...]
                sc = jnp.where(fill == 0.0, _dot_nt(q80, k80) * scale, fill)
                p = jnp.exp(sc - jnp.max(sc, axis=-1, keepdims=True))
                den = jnp.sum(p, axis=-1, keepdims=True)
                rc = pl.reciprocal(den, approx=True)
                return ((p * (rc * (2.0 - den * rc))).astype(bf16),)

            def pv(j, p, v80):
                o80 = _dot(p, v80)
                odef_ref[pl.ds(r0, 8), (2 * j) * E:(2 * j + 1) * E] = o80[64:72]
                odef_ref[pl.ds(r0, 8), (2 * j + 1) * E:(2 * j + 2) * E] = o80[72:80]
                return jnp.concatenate([o80[0:32], o80[32:64]], axis=1).astype(bf16)

            def wo_part(o, j0, j1, n, acc=None, toks=()):
                toks = dict(toks)
                for j in range(j0, j1):
                    d = _dot(o[j], _as_bf16(after(wo_ref[n, j * 128:(j + 1) * 128, :], toks.get(j))))
                    acc = d if acc is None else d + acc
                return acc

            ncb = jnp.minimum(cb + 1, NCB - 1)
            qs, ks, vs, ps, os_ = {}, {}, {}, {}, {}
            t0 = t1 = None
            for j in range(NP):
                qs[j] = proj(0, j, t0)
                if j >= 1:
                    ps[j - 1] = qk(qs[j - 1], ks[j - 1])
                ks[j] = proj(1, j)
                if j >= 2:
                    os_[j - 2] = pv(j - 2, *ps[j - 2], vs[j - 2])
                vs[j] = proj(2, j, t1)
                t0 = conv_mac(cb, r, j, 0)
                t1 = conv_mac(cb, r, NP - 1 - j, 1)
            na = NP - 2
            acc = {}
            ps[NP - 1] = qk(qs[NP - 1], ks[NP - 1])
            acc[0] = wo_part(os_, 0, na, 0, toks={0: t0})
            os_[NP - 2] = pv(NP - 2, *ps[NP - 2], vs[NP - 2])
            acc[1] = wo_part(os_, 0, na, 1, toks={0: t1})
            acc[2] = wo_part(os_, 0, na, 2)
            os_[NP - 1] = pv(NP - 1, *ps[NP - 1], vs[NP - 1])
            acc[3] = wo_part(os_, 0, na, 3)
            for n in range(4):
                acc[n] = wo_part(os_, na, NP, n, acc[n])
            tp = [conv_prep(ncb, 8 * r + i, i) for i in range(8)]
            for n in range(4, 8):
                acc[n] = wo_part(os_, 0, NP, n, toks={0: tp[2 * (n - 4)], 8: tp[2 * (n - 4) + 1]})
            conv_fwd_next(cb, r)
            acc = jnp.concatenate([acc[n] for n in range(8)], axis=1)
            b_ref[s, 0:NT, :] = acc[0:NT]
            return acc[NT:SEG].astype(bf16).astype(f32)

        lax.fori_loop(0, _DBG_STEPS, step, mem_ref[...].astype(f32), unroll=UNROLL)

        def out_copy(n):
            slot = n % 2
            return pltpu.make_async_copy(
                ost_ref.at[slot], out_hbm.at[:, :, pl.ds(pl.multiple_of(n * 128, 128), 128)],
                sems.at[SEM_OUT + slot])

        def fin(n, c):
            @pl.when(n >= 2)
            def _():
                out_copy(n - 2).wait()
            lanes = pl.ds(pl.multiple_of(n * 128, 128), 128)
            conv_inv(a_ref, NCB - 1, NCB - 1, 2 * n)
            conv_inv(a_ref, NCB - 1, NCB - 1, 2 * n + 1)
            bd = _dot(odef_ref[...].astype(bf16), _as_bf16(wo_ref[n]))
            b_ref[:, NT:SEG, lanes] = bd.reshape(NSEG, 8, 128)
            for blk in range(8):
                sg = slice(blk * 8, (blk + 1) * 8)
                b = b_ref[sg, :, lanes]
                a = a_ref[n, blk * 256:(blk + 1) * 256, :].reshape(8, SEG, 128)
                g = gate_ref[sg]
                ost_ref[n % 2, sg] = (g * a + (1.0 - g) * b).astype(bf16)
            out_copy(n).start()
            return c
        lax.fori_loop(0, NCB, fin, 0)
        out_copy(NCB - 2).wait()
        out_copy(NCB - 1).wait()

    pl.run_scoped(main, pltpu.VMEM((NSEG * 8, H * E), f32), pltpu.VMEM((NSEG, SEG, D), f32),
                  pltpu.VMEM((NCB + 1, S, 128), f32))


@jax.jit
def pallas_gated_mix__ssm_conv_h3__memory_aug_recurrent_mem_tr__prompt_kernel(
    A_q: jax.Array,
    A_k: jax.Array,
    A_v: jax.Array,
    A_shift_k: jax.Array,
    A_ssm_k: jax.Array,
    A_ssm_D: jax.Array,
    B_x: jax.Array,
    B_mem0: jax.Array,
    B_Wq: jax.Array,
    B_Wk: jax.Array,
    B_Wv: jax.Array,
    B_Wo: jax.Array,
    B_seg_len: jax.Array,
    gate_w: jax.Array,
):
    del B_x, B_seg_len
    f_tab, g_tab = _dft_tables()
    out = pl.pallas_call(
        _kernel,
        out_shape=jax.ShapeDtypeStruct((NSEG, SEG, D), bf16),
        in_specs=[pl.BlockSpec(memory_space=pl.ANY)] * 14,
        out_specs=pl.BlockSpec(memory_space=pl.ANY),
        scratch_shapes=[
            pltpu.VMEM((3 * H, D // 2, E), u32),
            pltpu.VMEM((NCB, H * E // 2, 128), u32),
            pltpu.VMEM((NSEG, SEG, D), bf16),
            pltpu.VMEM((NSEG * 4, D), u32),
            pltpu.VMEM((3 * NP, NSEG, 8, E), u32),
            pltpu.VMEM((S, D), bf16),
            pltpu.VMEM((S, D), bf16),
            pltpu.VMEM((D, S), bf16),
            pltpu.VMEM((NCB, S // 2, 128), u32),
            pltpu.VMEM((2, NCH, 128, 128), u32),
            pltpu.VMEM((2, NCH, 256, 128), f32),
            pltpu.VMEM((2, NCH, 256, 128), f32),
            pltpu.VMEM((256, 128), f32),
            pltpu.VMEM((8, 128), jnp.int32),
            pltpu.VMEM((8, 40, 128), f32),
            pltpu.VMEM((256, 128), bf16),
            pltpu.VMEM((128, 256), bf16),
            pltpu.VMEM((80, 80), f32),
            pltpu.VMEM((D, KS), bf16),
            pltpu.VMEM((NCB, 8, 128), f32),
            pltpu.VMEM((1, D), bf16),
            pltpu.VMEM((1, D), bf16),
            pltpu.VMEM((M, D), bf16),
            pltpu.VMEM((NSEG, SEG, 128), f32),
            pltpu.VMEM((2, NSEG, SEG, 128), bf16),
            pltpu.SemaphoreType.DMA((NSEM,)),
        ],
        compiler_params=pltpu.CompilerParams(vmem_limit_bytes=120 * 2**20),
    )(A_q.reshape(NSEG, SEG, D), A_k.reshape(S, D), A_v.reshape(S, D), A_shift_k, A_ssm_k,
      A_ssm_D.reshape(1, D), B_mem0.reshape(M, D), B_Wq, B_Wk, B_Wv, B_Wo.reshape(H * E, D),
      gate_w.reshape(1, D), jnp.asarray(f_tab, bf16), jnp.asarray(g_tab, bf16))
    return out.reshape(1, S, D)
```

```python
import numpy as np
import jax
import jax.numpy as jnp
from jax import lax
import jax.experimental.pallas as pl
import jax.experimental.pallas.tpu as pltpu

S, D, H, E, M, SEG = 2048, 1024, 32, 128, 8, 32
NSEG = S // SEG
NT = SEG - M
NP = H // 2
NCB = D // 128
C = 128
NCH = S // C
KS = 4
NG = 6
UNROLL = 2
_DBG_STEPS = NSEG
bf16, f32, u32 = jnp.bfloat16, jnp.float32, jnp.uint32


def _dft_tables():
    t = np.arange(C, dtype=np.float64)
    rows = []
    for r in range(8):
        ev = 16 * r + np.arange(0, 16, 2)
        od = ev + 1
        for fn, fs in ((np.cos, ev), (np.sin, ev), (np.cos, od), (np.sin, od)):
            rows.append(fn(np.pi * (2 * fs[:, None] + 1) * t[None, :] / (2 * C)))
    f = np.concatenate(rows, axis=0)
    return f.astype(np.float32), (f.T / C).astype(np.float32)


def _fill_matrix():
    r = lax.broadcasted_iota(jnp.int32, (80, 80), 0)
    c = lax.broadcasted_iota(jnp.int32, (80, 80), 1)

    def head(i):
        return jnp.where(i < 64, i // 32, (i - 64) // 8)

    def idx(i):
        lo = i % 32
        main = jnp.where(lo < NT, lo + M, lo - NT)
        return jnp.where(i < 64, main, (i - 64) % 8 + NT + M)

    same = head(r) == head(c)
    ok = (idx(r) < M) | (idx(r) >= idx(c))
    return jnp.where(same, jnp.where(ok, 0.0, -1e9), -jnp.inf).astype(f32)


def _as_bf16(v):
    return pltpu.bitcast(v, bf16)


def _dot(a, b):
    return jnp.dot(a, b, preferred_element_type=f32)


def _dot_nt(a, b):
    return lax.dot_general(a, b, (((1,), (1,)), ((), ())), preferred_element_type=f32)


(SEM_XB, SEM_X, SEM_K0, SEM_V0, SEM_KL, SEM_VL, SEM_SSM, SEM_WO, SEM_SHIFT, SEM_D, SEM_GW, SEM_MEM,
 SEM_F, SEM_G) = range(14)
SEM_W = 14
SEM_OUT = SEM_W + 2 * NG
NSEM = SEM_OUT + 2


def _kernel(x3_hbm, x_hbm, k_hbm, v_hbm, shift_hbm, ssm_hbm, d_hbm, mem_hbm, wq_hbm, wk_hbm, wv_hbm,
            wo_hbm, gw_hbm, f_hbm, g_hbm, out_hbm,
            wn_ref, wo_ref, x_ref, xr_ref, xb_ref, pre_ref, k_ref, v_ref, ssm_ref, u_ref, z_ref,
            fu_ref, fk_ref, kraw_ref, one_ref, kf_ref, f_ref, g_ref, fill_ref, shift_ref, wt_ref,
            d_ref, gw_ref, mem_ref, gate_ref, ost_ref, sems):
    w_hbm = (wq_hbm, wk_hbm, wv_hbm)

    def cp(src, dst, sem):
        return pltpu.make_async_copy(src, dst, sems.at[sem])

    def start_col_blocks(src_hbm, dst_ref, i0, i1, sem):
        src = src_hbm.bitcast(u32)
        for i in range(i0, i1):
            cp(src.at[:, i * 128:(i + 1) * 128], dst_ref.at[i], sem).start()

    def wait_all(dst, sem):
        cp(dst, dst, sem).wait()

    def conv_prep(cb, i, slot):
        row0 = pl.multiple_of(i * 16, 16)
        prev0 = pl.multiple_of(jnp.maximum(row0 - 8, 0), 8)
        prev = _as_bf16(k_ref[cb, pl.ds(prev0, 8), :]).astype(f32)[8:16]
        kf_ref[slot, 0:8, :] = jnp.where(i > 0, prev, 0.0)
        kcur = _as_bf16(k_ref[cb, pl.ds(row0, 16), :]).astype(f32)
        kf_ref[slot, 8:40, :] = kcur
        w = wt_ref[cb]
        ks = kcur * w[0:1, :]
        for j in range(1, KS):
            ks = ks + kf_ref[slot, 8 - j:40 - j, :] * w[j:j + 1, :]
        kv = (ks * _as_bf16(v_ref[cb, pl.ds(row0, 16), :]).astype(f32)).astype(bf16)
        kv = pltpu.bitcast(kv, u32)
        u_ref[cb, pl.ds(row0, 16), :] = kv
        return kv[0:8] | kv[8:16]

    def combine(kf, prev):
        out = []
        for g in range(8):
            o = 32 * g
            out += [kf[o:o + 8] + prev[o + 8:o + 16], kf[o + 8:o + 16] - prev[o:o + 8],
                    kf[o + 16:o + 24] - prev[o + 24:o + 32], kf[o + 24:o + 32] + prev[o + 16:o + 24]]
        return jnp.concatenate(out, axis=0)

    def conv_fwd(cb, r):
        slot = cb % 2
        rows = pl.ds(pl.multiple_of(cb * 64, 64), 64)
        f = f_ref[...]
        kfs = []
        for a in (2 * r, 2 * r + 1):
            fu_ref[slot, a] = _dot(f, _as_bf16(u_ref[cb, pl.ds(pl.multiple_of(a * 64, 64), 64), :]))
            kfs.append(_dot_nt(f, _as_bf16(ssm_ref[a, rows, :])))
        fk_ref[slot, 2 * r] = combine(kfs[0], jnp.where(r > 0, kraw_ref[...], 0.0))
        fk_ref[slot, 2 * r + 1] = combine(kfs[1], kfs[0])
        kraw_ref[...] = kfs[1]

    def conv_mac(slot, r, a, half, dep=None):
        ro = pl.multiple_of(r * 32, 32) + half * 16
        p = q = None
        for c in range(a + 1):
            u = fu_ref[slot, a - c, pl.ds(ro, 16), :]
            k = fk_ref[slot, c, pl.ds(ro, 16), :]
            ua, ub, kc, kd = u[0:8], u[8:16], k[0:8], k[8:16]
            if c == 0 and dep is not None:
                ua = jnp.where(one_ref[...] == 1, ua, pltpu.bitcast(dep, f32))
            p = (ua * kc if p is None else p + ua * kc) - ub * kd
            q = (ua * kd if q is None else q + ua * kd) + ub * kc
        z = pltpu.bitcast(jnp.concatenate([p, q], axis=0).astype(bf16), u32)
        z_ref[slot, a, pl.ds(pl.multiple_of(r * 16, 16) + half * 8, 8), :] = z
        return z

    def conv_inv(a_ref, cb, slot, dst, a):
        rows = pl.ds(pl.multiple_of(a * 64, 64), 64)
        y = _dot(g_ref[...], _as_bf16(z_ref[slot, a]))
        kv = _as_bf16(u_ref[cb, rows, :]).astype(f32)
        q = _as_bf16(x_ref[cb, rows, :]).astype(f32)
        a_ref[dst, pl.ds(pl.multiple_of(a * C, C), C), :] = q * (y + kv * wt_ref[cb, KS:KS + 1, :])

    def after(w, tok):
        if tok is None:
            return w
        return jnp.concatenate([jnp.where(one_ref[...] == 1, w[0:8], tok), w[8:]], axis=0)

    def prologue(stage_ref):
        st3 = stage_ref.reshape(NG * D, 8, E)

        def start_w(g):
            src = w_hbm[g // 2].bitcast(u32)
            for hf in range(2):
                r0 = (g % 2) * 8 + hf * 4
                cp(src.at[:, r0:r0 + 4, :], st3.at[g * D:(g + 1) * D, hf * 4:hf * 4 + 4, :],
                   SEM_W + 2 * g + hf).start()

        def wait_w(g, hf):
            wait_all(st3.at[pl.ds(g * D, D), hf * 4:hf * 4 + 4, :], SEM_W + 2 * g + hf)

        small = [cp(shift_hbm, shift_ref, SEM_SHIFT), cp(d_hbm, d_ref, SEM_D), cp(gw_hbm, gw_ref, SEM_GW),
                 cp(mem_hbm, mem_ref, SEM_MEM), cp(f_hbm, f_ref, SEM_F), cp(g_hbm, g_ref, SEM_G)]
        cp_xb = cp(x3_hbm.at[:, NT:SEG, :], xr_ref, SEM_XB)
        cp_xb.start()
        start_w(0)
        for c in small:
            c.start()
        for g in range(1, NG):
            start_w(g)
        start_col_blocks(wo_hbm, wo_ref, 0, NCB, SEM_WO)
        start_col_blocks(x_hbm, x_ref, 0, NCB, SEM_X)
        start_col_blocks(k_hbm, k_ref, 0, 1, SEM_K0)
        start_col_blocks(v_hbm, v_ref, 0, 1, SEM_V0)
        start_col_blocks(ssm_hbm, ssm_ref, 0, NCH, SEM_SSM)
        start_col_blocks(k_hbm, k_ref, 1, NCB, SEM_KL)
        start_col_blocks(v_hbm, v_ref, 1, NCB, SEM_VL)
        fill_ref[...] = _fill_matrix()
        one_ref[...] = jnp.ones((8, 128), jnp.int32)
        cp_xb.wait()

        def xb_build(it, c):
            s0 = pl.multiple_of(it * 8, 8)
            t = xr_ref[pl.ds(s0, 8)].astype(f32).reshape(64, D).astype(bf16)
            xb_ref[pl.ds(pl.multiple_of(it * 32, 32), 32), :] = pltpu.bitcast(t, u32)
            return c
        lax.fori_loop(0, 8, xb_build, 0)

        def group(g, c):
            sub = stage_ref.at[pl.ds(pl.multiple_of(g * (8 * D), 8 * D), 8 * D), :]

            def relayout(j):
                toks = []
                for blk in range(D // 256):
                    w = sub[pl.ds(blk * 2048 + j, 256, stride=8), :]
                    lo = pltpu.bitcast(pltpu.bitcast(w << 16, f32).astype(bf16), u32)
                    hi = pltpu.bitcast(pltpu.bitcast(w & jnp.uint32(0xFFFF0000), f32).astype(bf16), u32)
                    wn_ref[g * 16 + 2 * j, blk * 128:(blk + 1) * 128, :] = lo
                    wn_ref[g * 16 + 2 * j + 1, blk * 128:(blk + 1) * 128, :] = hi
                    t = lo | hi
                    tok = t[0:8]
                    for i in range(1, 16):
                        tok = tok | t[8 * i:8 * i + 8]
                    toks.append(tok)
                return toks

            wait_w(g, 0)
            relayout(0)
            for j in range(8):
                if j == 3:
                    wait_w(g, 1)
                xb = _as_bf16(xb_ref[...])
                w1, w2 = wn_ref[g * 16 + 2 * j], wn_ref[g * 16 + 2 * j + 1]
                toks = relayout(j + 1) if j + 1 < 8 else None
                if j == 2:
                    w1 = jnp.concatenate([after(w1[0:256], toks[0]), after(w1[256:], toks[1])], axis=0)
                    w2 = jnp.concatenate([after(w2[0:256], toks[2]), after(w2[256:], toks[3])], axis=0)
                r1 = _dot(xb, _as_bf16(w1))
                r2 = _dot(xb, _as_bf16(w2))
                cc = jnp.concatenate([r1.reshape(NSEG, 8, E), r2.reshape(NSEG, 8, E)], axis=1).astype(bf16)
                pre_ref[:, g * 8 + j] = pltpu.bitcast(cc, u32)
            return c
        lax.fori_loop(0, NG, group, 0)
        for c in small:
            c.wait()

    pl.run_scoped(prologue, pltpu.VMEM((NG * 8 * D, E), u32))

    sh = shift_ref[...].astype(f32)
    dv = d_ref[...].astype(f32)
    for n in range(NCB):
        wt_ref[n, 0:KS, :] = sh[:, n * 128:(n + 1) * 128]
        wt_ref[n, KS:KS + 1, :] = dv[n:n + 1, :]
    wait_all(wo_ref, SEM_WO)
    wait_all(x_ref, SEM_X)
    wait_all(k_ref.at[0:1], SEM_K0)
    wait_all(v_ref.at[0:1], SEM_V0)
    wait_all(ssm_ref, SEM_SSM)

    scale = E ** -0.5

    def main(odef_ref, b_ref, a_ref):
        def step(s, mem):
            cb = s // 8
            r = s % 8
            icb = jnp.maximum(cb - 2, 0)
            idst = jnp.where(cb >= 2, cb - 2, NCB)
            mslot = (cb + 1) % 2

            xrows = pl.ds(pl.multiple_of(s * 16, 16), 16)
            xs = [_as_bf16(x_ref[n, xrows, :]).astype(f32) for n in range(NCB)]
            h32 = jnp.concatenate([jnp.concatenate(xs, axis=1)[0:NT], mem], axis=0).astype(bf16)
            r0 = pl.multiple_of(s * 8, 8)

            conv_inv(a_ref, icb, cb % 2, idst, 2 * r)
            conv_inv(a_ref, icb, cb % 2, idst, 2 * r + 1)

            gw = gw_ref[...].astype(f32)
            gl = xs[0] * gw[0:1, :]
            for n in range(1, NCB):
                gl = gl + xs[n] * gw[n:n + 1, :]
            gl = jnp.sum(gl, axis=-1, keepdims=True)
            gate_ref[s] = jnp.broadcast_to(jax.nn.sigmoid(gl), (SEG, 128))

            def proj(m, j, tok=None):
                r1 = _dot(h32, _as_bf16(after(wn_ref[m * H + 2 * j], tok)))
                r2 = _dot(h32, _as_bf16(wn_ref[m * H + 2 * j + 1]))
                p = _as_bf16(pre_ref[s, m * NP + j]).astype(f32)
                return jnp.concatenate([r1, r2, p], axis=0).astype(bf16)

            def qk(q80, k80):
                fill = fill_ref[...]
                sc = jnp.where(fill == 0.0, _dot_nt(q80, k80) * scale, fill)
                p = jnp.exp(sc - jnp.max(sc, axis=-1, keepdims=True))
                den = jnp.sum(p, axis=-1, keepdims=True)
                rc = pl.reciprocal(den, approx=True)
                return (p * (rc * (2.0 - den * rc))).astype(bf16)

            def pv(j, p, v80):
                o80 = _dot(p, v80)
                odef_ref[pl.ds(r0, 8), (2 * j) * E:(2 * j + 1) * E] = o80[64:72]
                odef_ref[pl.ds(r0, 8), (2 * j + 1) * E:(2 * j + 2) * E] = o80[72:80]
                return jnp.concatenate([o80[0:32], o80[32:64]], axis=1).astype(bf16)

            def wo_part(o, j0, j1, n, acc=None, toks=()):
                toks = dict(toks)
                for j in range(j0, j1):
                    d = _dot(o[j], _as_bf16(after(wo_ref[n, j * 128:(j + 1) * 128, :], toks.get(j))))
                    acc = d if acc is None else d + acc
                return acc

            qs, ks, vs, ps, os_ = {}, {}, {}, {}, {}
            t0 = t1 = None
            for j in range(NP):
                qs[j] = proj(0, j, t0)
                if j >= 1:
                    ps[j - 1] = qk(qs[j - 1], ks[j - 1])
                ks[j] = proj(1, j)
                if j >= 2:
                    os_[j - 2] = pv(j - 2, ps[j - 2], vs[j - 2])
                vs[j] = proj(2, j, t1)
                t0 = conv_mac(mslot, r, j, 0)
                t1 = conv_mac(mslot, r, NP - 1 - j, 1)
            na = NP - 2
            acc = {}
            acc[0] = wo_part(os_, 0, 8, 0, toks={0: t0})
            ps[NP - 1] = qk(qs[NP - 1], ks[NP - 1])
            acc[0] = wo_part(os_, 8, na, 0, acc[0])
            os_[NP - 2] = pv(NP - 2, ps[NP - 2], vs[NP - 2])
            acc[1] = wo_part(os_, 0, na, 1, toks={0: t1})
            acc[2] = wo_part(os_, 0, na, 2)
            os_[NP - 1] = pv(NP - 1, ps[NP - 1], vs[NP - 1])
            acc[3] = wo_part(os_, 0, na, 3)
            for n in range(4):
                acc[n] = wo_part(os_, na, NP, n, acc[n])
            tp = [conv_prep(cb, 8 * r + i, i) for i in range(8)]
            for n in range(4, 8):
                acc[n] = wo_part(os_, 0, NP, n, toks={0: tp[2 * (n - 4)], 8: tp[2 * (n - 4) + 1]})
            conv_fwd(cb, r)
            for n in range(NCB):
                b_ref[n, s, 0:NT, :] = acc[n][0:NT]
            return jnp.concatenate([acc[n][NT:SEG] for n in range(NCB)], axis=1).astype(bf16).astype(f32)

        def steps(i, mem):
            @pl.when(i == 8 // UNROLL)
            def _():
                wait_all(k_ref.at[1:NCB], SEM_KL)
                wait_all(v_ref.at[1:NCB], SEM_VL)
            for t in range(UNROLL):
                mem = step(i * UNROLL + t, mem)
            return mem

        lax.fori_loop(0, _DBG_STEPS // UNROLL, steps, mem_ref[...].astype(f32))

        def out_copy(n):
            slot = n % 2
            return pltpu.make_async_copy(
                ost_ref.at[slot], out_hbm.at[:, :, pl.ds(pl.multiple_of(n * 128, 128), 128)],
                sems.at[SEM_OUT + slot])

        def fin(n, c):
            @pl.when(n >= 2)
            def _():
                out_copy(n - 2).wait()
            icb = NCB - 2 + n // 4
            for i in range(4):
                conv_inv(a_ref, icb, icb % 2, icb, 4 * (n % 4) + i)
            toks = []
            for rr in range(2):
                r = 2 * (n % 4) + rr
                for a in range(NCH):
                    t = conv_mac((NCB - 1) % 2, r, a, 0, None if a % 4 == 0 else t)
                    t = conv_mac((NCB - 1) % 2, r, NCH - 1 - a, 1, t)
                    if a % 4 == 3:
                        toks.append(t)
            bd = None
            for kb in range(8):
                w = after(wo_ref[n, kb * 256:(kb + 1) * 256, :], toks[kb - 1] if kb > 0 else None)
                d = _dot(odef_ref[:, kb * 512:(kb + 1) * 512].astype(bf16), _as_bf16(w))
                bd = d if bd is None else d + bd
            b_ref[n, :, NT:SEG, :] = bd.reshape(NSEG, 8, 128)
            for blk in range(8):
                sg = slice(blk * 8, (blk + 1) * 8)
                b = b_ref[n, sg]
                a = a_ref[n, blk * 256:(blk + 1) * 256, :].reshape(8, SEG, 128)
                g = gate_ref[sg]
                ost_ref[n % 2, sg] = (g * a + (1.0 - g) * b).astype(bf16)
            out_copy(n).start()
            return c
        lax.fori_loop(0, NCB, fin, 0)
        out_copy(NCB - 2).wait()
        out_copy(NCB - 1).wait()

    pl.run_scoped(main, pltpu.VMEM((NSEG * 8, H * E), f32), pltpu.VMEM((NCB, NSEG, SEG, 128), f32),
                  pltpu.VMEM((NCB + 1, S, 128), f32))


@jax.jit
def pallas_gated_mix__ssm_conv_h3__memory_aug_recurrent_mem_tr__prompt_kernel(
    A_q: jax.Array,
    A_k: jax.Array,
    A_v: jax.Array,
    A_shift_k: jax.Array,
    A_ssm_k: jax.Array,
    A_ssm_D: jax.Array,
    B_x: jax.Array,
    B_mem0: jax.Array,
    B_Wq: jax.Array,
    B_Wk: jax.Array,
    B_Wv: jax.Array,
    B_Wo: jax.Array,
    B_seg_len: jax.Array,
    gate_w: jax.Array,
):
    del B_x, B_seg_len
    f_tab, g_tab = _dft_tables()
    out = pl.pallas_call(
        _kernel,
        out_shape=jax.ShapeDtypeStruct((NSEG, SEG, D), bf16),
        in_specs=[pl.BlockSpec(memory_space=pl.ANY)] * 15,
        out_specs=pl.BlockSpec(memory_space=pl.ANY),
        scratch_shapes=[
            pltpu.VMEM((3 * H, D // 2, E), u32),
            pltpu.VMEM((NCB, H * E // 2, 128), u32),
            pltpu.VMEM((NCB, S // 2, 128), u32),
            pltpu.VMEM((NSEG, M, D), bf16),
            pltpu.VMEM((NSEG * 4, D), u32),
            pltpu.VMEM((NSEG, 3 * NP, 8, E), u32),
            pltpu.VMEM((NCB, S // 2, 128), u32),
            pltpu.VMEM((NCB, S // 2, 128), u32),
            pltpu.VMEM((NCH, D // 2, 128), u32),
            pltpu.VMEM((NCB, S // 2, 128), u32),
            pltpu.VMEM((2, NCH, 128, 128), u32),
            pltpu.VMEM((2, NCH, 256, 128), f32),
            pltpu.VMEM((2, NCH, 256, 128), f32),
            pltpu.VMEM((256, 128), f32),
            pltpu.VMEM((8, 128), jnp.int32),
            pltpu.VMEM((8, 40, 128), f32),
            pltpu.VMEM((256, 128), bf16),
            pltpu.VMEM((128, 256), bf16),
            pltpu.VMEM((80, 80), f32),
            pltpu.VMEM((KS, D), bf16),
            pltpu.VMEM((NCB, 8, 128), f32),
            pltpu.VMEM((NCB, 128), bf16),
            pltpu.VMEM((NCB, 128), bf16),
            pltpu.VMEM((M, D), bf16),
            pltpu.VMEM((NSEG, SEG, 128), f32),
            pltpu.VMEM((2, NSEG, SEG, 128), bf16),
            pltpu.SemaphoreType.DMA((NSEM,)),
        ],
        compiler_params=pltpu.CompilerParams(vmem_limit_bytes=120 * 2**20),
    )(A_q.reshape(NSEG, SEG, D), A_q.reshape(S, D), A_k.reshape(S, D), A_v.reshape(S, D), A_shift_k.T,
      A_ssm_k, A_ssm_D.reshape(NCB, 128), B_mem0.reshape(M, D), B_Wq, B_Wk, B_Wv,
      B_Wo.reshape(H * E, D), gate_w.reshape(NCB, 128), jnp.asarray(f_tab, bf16), jnp.asarray(g_tab, bf16))
    return out.reshape(1, S, D)
```

```python
import numpy as np
import jax
import jax.numpy as jnp
from jax import lax
import jax.experimental.pallas as pl
import jax.experimental.pallas.tpu as pltpu

S, D, H, E, M, SEG = 2048, 1024, 32, 128, 8, 32
NSEG = S // SEG
NT = SEG - M
NP = H // 2
NCB = D // 128
C = 128
NCH = S // C
KS = 4
NG = 6
UNROLL = 2
_DBG_STEPS = NSEG
bf16, f32, u32 = jnp.bfloat16, jnp.float32, jnp.uint32


def _dft_tables():
    t = np.arange(C, dtype=np.float64)
    rows = []
    for r in range(8):
        ev = 16 * r + np.arange(0, 16, 2)
        od = ev + 1
        for fn, fs in ((np.cos, ev), (np.sin, ev), (np.cos, od), (np.sin, od)):
            rows.append(fn(np.pi * (2 * fs[:, None] + 1) * t[None, :] / (2 * C)))
    f = np.concatenate(rows, axis=0)
    return f.astype(np.float32), (f.T / C).astype(np.float32)


def _fill_matrix():
    r = lax.broadcasted_iota(jnp.int32, (80, 80), 0)
    c = lax.broadcasted_iota(jnp.int32, (80, 80), 1)

    def head(i):
        return jnp.where(i < 64, i // 32, (i - 64) // 8)

    def idx(i):
        lo = i % 32
        main = jnp.where(lo < NT, lo + M, lo - NT)
        return jnp.where(i < 64, main, (i - 64) % 8 + NT + M)

    same = head(r) == head(c)
    ok = (idx(r) < M) | (idx(r) >= idx(c))
    return jnp.where(same, jnp.where(ok, 0.0, -1e9), -jnp.inf).astype(f32)


def _as_bf16(v):
    return pltpu.bitcast(v, bf16)


def _dot(a, b):
    return jnp.dot(a, b, preferred_element_type=f32)


def _dot_nt(a, b):
    return lax.dot_general(a, b, (((1,), (1,)), ((), ())), preferred_element_type=f32)


(SEM_XB, SEM_X, SEM_K0, SEM_V0, SEM_KL, SEM_VL, SEM_SSM, SEM_WO, SEM_SHIFT, SEM_D, SEM_GW, SEM_MEM,
 SEM_F, SEM_G) = range(14)
SEM_W = 14
SEM_OUT = SEM_W + 2 * NG
NSEM = SEM_OUT + 2


def _kernel(x3_hbm, x_hbm, k_hbm, v_hbm, shift_hbm, ssm_hbm, d_hbm, mem_hbm, wq_hbm, wk_hbm, wv_hbm,
            wo_hbm, gw_hbm, f_hbm, g_hbm, out_hbm,
            wn_ref, wo_ref, x_ref, xr_ref, xb_ref, pre_ref, k_ref, v_ref, ssm_ref, u_ref, z_ref,
            fu_ref, fk_ref, kraw_ref, one_ref, kf_ref, f_ref, g_ref, fill_ref, shift_ref, wt_ref,
            d_ref, gw_ref, mem_ref, gate_ref, ost_ref, sems):
    w_hbm = (wq_hbm, wk_hbm, wv_hbm)

    def cp(src, dst, sem):
        return pltpu.make_async_copy(src, dst, sems.at[sem])

    def start_col_blocks(src_hbm, dst_ref, i0, i1, sem):
        src = src_hbm.bitcast(u32)
        for i in range(i0, i1):
            cp(src.at[:, i * 128:(i + 1) * 128], dst_ref.at[i], sem).start()

    def wait_all(dst, sem):
        cp(dst, dst, sem).wait()

    def conv_prep(cb, i, slot):
        row0 = pl.multiple_of(i * 16, 16)
        prev0 = pl.multiple_of(jnp.maximum(row0 - 8, 0), 8)
        prev = _as_bf16(k_ref[cb, pl.ds(prev0, 8), :]).astype(f32)[8:16]
        kf_ref[slot, 0:8, :] = jnp.where(i > 0, prev, 0.0)
        kcur = _as_bf16(k_ref[cb, pl.ds(row0, 16), :]).astype(f32)
        kf_ref[slot, 8:40, :] = kcur
        w = wt_ref[cb]
        ks = kcur * w[0:1, :]
        for j in range(1, KS):
            ks = ks + kf_ref[slot, 8 - j:40 - j, :] * w[j:j + 1, :]
        kv = (ks * _as_bf16(v_ref[cb, pl.ds(row0, 16), :]).astype(f32)).astype(bf16)
        kv = pltpu.bitcast(kv, u32)
        u_ref[cb, pl.ds(row0, 16), :] = kv
        return kv[0:8] | kv[8:16]

    def combine(kf, prev):
        out = []
        for g in range(8):
            o = 32 * g
            out += [kf[o:o + 8] + prev[o + 8:o + 16], kf[o + 8:o + 16] - prev[o:o + 8],
                    kf[o + 16:o + 24] - prev[o + 24:o + 32], kf[o + 24:o + 32] + prev[o + 16:o + 24]]
        return jnp.concatenate(out, axis=0)

    def conv_fwd(cb, r):
        slot = cb % 2
        rows = pl.ds(pl.multiple_of(cb * 64, 64), 64)
        f = f_ref[...]
        kfs = []
        for a in (2 * r, 2 * r + 1):
            fu_ref[slot, a] = _dot(f, _as_bf16(u_ref[cb, pl.ds(pl.multiple_of(a * 64, 64), 64), :]))
            kfs.append(_dot_nt(f, _as_bf16(ssm_ref[a, rows, :])))
        fk_ref[slot, 2 * r] = combine(kfs[0], jnp.where(r > 0, kraw_ref[...], 0.0))
        fk_ref[slot, 2 * r + 1] = combine(kfs[1], kfs[0])
        kraw_ref[...] = kfs[1]

    def conv_mac(slot, r, a, half, dep=None):
        ro = pl.multiple_of(r * 32, 32) + half * 16
        p = q = None
        for c in range(a + 1):
            u = fu_ref[slot, a - c, pl.ds(ro, 16), :]
            k = fk_ref[slot, c, pl.ds(ro, 16), :]
            ua, ub, kc, kd = u[0:8], u[8:16], k[0:8], k[8:16]
            if c == 0 and dep is not None:
                ua = jnp.where(one_ref[...] == 1, ua, pltpu.bitcast(dep, f32))
            p = (ua * kc if p is None else p + ua * kc) - ub * kd
            q = (ua * kd if q is None else q + ua * kd) + ub * kc
        z = pltpu.bitcast(jnp.concatenate([p, q], axis=0).astype(bf16), u32)
        z_ref[slot, a, pl.ds(pl.multiple_of(r * 16, 16) + half * 8, 8), :] = z
        return z

    def conv_inv(a_ref, cb, slot, dst, a):
        rows = pl.ds(pl.multiple_of(a * 64, 64), 64)
        y = _dot(g_ref[...], _as_bf16(z_ref[slot, a]))
        kv = _as_bf16(u_ref[cb, rows, :]).astype(f32)
        q = _as_bf16(x_ref[cb, rows, :]).astype(f32)
        a_ref[dst, pl.ds(pl.multiple_of(a * C, C), C), :] = q * (y + kv * wt_ref[cb, KS:KS + 1, :])

    def after(w, tok):
        if tok is None:
            return w
        return jnp.concatenate([jnp.where(one_ref[...] == 1, w[0:8], tok), w[8:]], axis=0)

    def prologue(stage_ref):
        st3 = stage_ref.reshape(NG * D, 8, E)

        def start_w(g):
            src = w_hbm[g // 2].bitcast(u32)
            for hf in range(2):
                r0 = (g % 2) * 8 + hf * 4
                cp(src.at[:, r0:r0 + 4, :], st3.at[g * D:(g + 1) * D, hf * 4:hf * 4 + 4, :],
                   SEM_W + 2 * g + hf).start()

        def wait_w(g, hf):
            wait_all(st3.at[pl.ds(g * D, D), hf * 4:hf * 4 + 4, :], SEM_W + 2 * g + hf)

        small = [cp(shift_hbm, shift_ref, SEM_SHIFT), cp(d_hbm, d_ref, SEM_D), cp(gw_hbm, gw_ref, SEM_GW),
                 cp(mem_hbm, mem_ref, SEM_MEM), cp(f_hbm, f_ref, SEM_F), cp(g_hbm, g_ref, SEM_G)]
        cp_xb = cp(x3_hbm.at[:, NT:SEG, :], xr_ref, SEM_XB)
        cp_xb.start()
        start_w(0)
        for c in small:
            c.start()
        for g in range(1, NG):
            start_w(g)
        start_col_blocks(wo_hbm, wo_ref, 0, NCB, SEM_WO)
        start_col_blocks(x_hbm, x_ref, 0, NCB, SEM_X)
        start_col_blocks(k_hbm, k_ref, 0, 1, SEM_K0)
        start_col_blocks(v_hbm, v_ref, 0, 1, SEM_V0)
        start_col_blocks(ssm_hbm, ssm_ref, 0, NCH, SEM_SSM)
        start_col_blocks(k_hbm, k_ref, 1, NCB, SEM_KL)
        start_col_blocks(v_hbm, v_ref, 1, NCB, SEM_VL)
        fill_ref[...] = _fill_matrix()
        one_ref[...] = jnp.ones((8, 128), jnp.int32)
        cp_xb.wait()

        def xb_build(it, c):
            s0 = pl.multiple_of(it * 8, 8)
            t = xr_ref[pl.ds(s0, 8)].astype(f32).reshape(64, D).astype(bf16)
            xb_ref[pl.ds(pl.multiple_of(it * 32, 32), 32), :] = pltpu.bitcast(t, u32)
            return c
        lax.fori_loop(0, 8, xb_build, 0)

        def group(g, c):
            sub = stage_ref.at[pl.ds(pl.multiple_of(g * (8 * D), 8 * D), 8 * D), :]

            def relayout(j):
                toks = []
                for blk in range(D // 256):
                    w = sub[pl.ds(blk * 2048 + j, 256, stride=8), :]
                    lo = pltpu.bitcast(pltpu.bitcast(w << 16, f32).astype(bf16), u32)
                    hi = pltpu.bitcast(pltpu.bitcast(w & jnp.uint32(0xFFFF0000), f32).astype(bf16), u32)
                    wn_ref[g * 16 + 2 * j, blk * 128:(blk + 1) * 128, :] = lo
                    wn_ref[g * 16 + 2 * j + 1, blk * 128:(blk + 1) * 128, :] = hi
                    t = lo | hi
                    tok = t[0:8]
                    for i in range(1, 16):
                        tok = tok | t[8 * i:8 * i + 8]
                    toks.append(tok)
                return toks

            wait_w(g, 0)
            relayout(0)
            for j in range(8):
                if j == 3:
                    wait_w(g, 1)
                xb = _as_bf16(xb_ref[...])
                w1, w2 = wn_ref[g * 16 + 2 * j], wn_ref[g * 16 + 2 * j + 1]
                toks = relayout(j + 1) if j + 1 < 8 else None
                if j == 2:
                    w1 = jnp.concatenate([after(w1[0:256], toks[0]), after(w1[256:], toks[1])], axis=0)
                    w2 = jnp.concatenate([after(w2[0:256], toks[2]), after(w2[256:], toks[3])], axis=0)
                r1 = _dot(xb, _as_bf16(w1))
                r2 = _dot(xb, _as_bf16(w2))
                cc = jnp.concatenate([r1.reshape(NSEG, 8, E), r2.reshape(NSEG, 8, E)], axis=1).astype(bf16)
                pre_ref[:, g * 8 + j] = pltpu.bitcast(cc, u32)
            return c
        lax.fori_loop(0, NG, group, 0)
        for c in small:
            c.wait()

    pl.run_scoped(prologue, pltpu.VMEM((NG * 8 * D, E), u32))

    sh = shift_ref[...].astype(f32)
    dv = d_ref[...].astype(f32)
    for n in range(NCB):
        wt_ref[n, 0:KS, :] = sh[:, n * 128:(n + 1) * 128]
        wt_ref[n, KS:KS + 1, :] = dv[n:n + 1, :]
    wait_all(wo_ref, SEM_WO)
    wait_all(x_ref, SEM_X)
    wait_all(k_ref.at[0:1], SEM_K0)
    wait_all(v_ref.at[0:1], SEM_V0)
    wait_all(ssm_ref, SEM_SSM)

    scale = E ** -0.5

    def main(odef_ref, b_ref, a_ref):
        def step(s, mem):
            cb = s // 8
            r = s % 8
            icb = jnp.maximum(cb - 2, 0)
            idst = jnp.where(cb >= 2, cb - 2, NCB)
            mslot = (cb + 1) % 2

            xrows = pl.ds(pl.multiple_of(s * 16, 16), 16)
            xs = [_as_bf16(x_ref[n, xrows, :]).astype(f32) for n in range(NCB)]
            h32 = jnp.concatenate([jnp.concatenate(xs, axis=1)[0:NT], mem], axis=0).astype(bf16)
            r0 = pl.multiple_of(s * 8, 8)

            conv_inv(a_ref, icb, cb % 2, idst, 2 * r)
            conv_inv(a_ref, icb, cb % 2, idst, 2 * r + 1)

            gw = gw_ref[...].astype(f32)
            gl = xs[0] * gw[0:1, :]
            for n in range(1, NCB):
                gl = gl + xs[n] * gw[n:n + 1, :]
            gl = jnp.sum(gl, axis=-1, keepdims=True)
            gate_ref[s] = jnp.broadcast_to(jax.nn.sigmoid(gl), (SEG, 128))

            def proj(m, j, tok=None):
                r1 = _dot(h32, _as_bf16(after(wn_ref[m * H + 2 * j], tok)))
                r2 = _dot(h32, _as_bf16(wn_ref[m * H + 2 * j + 1]))
                p = _as_bf16(pre_ref[s, m * NP + j]).astype(f32)
                r = jnp.concatenate([r1, r2, p], axis=0)
                return r if m == 0 else r.astype(bf16)

            def split_rows(dot, lhs, rhs, split):
                if not split:
                    return dot(lhs.astype(bf16), rhs)
                return jnp.concatenate([dot(lhs[0:48].astype(bf16), rhs), dot(lhs[48:80].astype(bf16), rhs)], axis=0)

            def qk(q80, k80, split=False):
                fill = fill_ref[...]
                sc = jnp.where(fill == 0.0, split_rows(_dot_nt, q80, k80, split) * scale, fill)
                p = jnp.exp(sc - jnp.max(sc, axis=-1, keepdims=True))
                den = jnp.sum(p, axis=-1, keepdims=True)
                rc = pl.reciprocal(den, approx=True)
                return p * (rc * (2.0 - den * rc))

            def pv(j, p, v80, split=False):
                o80 = split_rows(_dot, p, v80, split)
                odef_ref[pl.ds(r0, 8), (2 * j) * E:(2 * j + 1) * E] = o80[64:72]
                odef_ref[pl.ds(r0, 8), (2 * j + 1) * E:(2 * j + 2) * E] = o80[72:80]
                return jnp.concatenate([o80[0:32], o80[32:64]], axis=1).astype(bf16)

            def wo_part(o, j0, j1, n, acc=None, toks=()):
                toks = dict(toks)
                for j in range(j0, j1):
                    d = _dot(o[j], _as_bf16(after(wo_ref[n, j * 128:(j + 1) * 128, :], toks.get(j))))
                    acc = d if acc is None else d + acc
                return acc

            qs, ks, vs, ps, os_ = {}, {}, {}, {}, {}
            tk = [None] * 4
            for j in range(0, NP, 2):
                qs[j] = proj(0, j, tk[0])
                ks[j] = proj(1, j)
                qs[j + 1] = proj(0, j + 1, tk[1])
                ks[j + 1] = proj(1, j + 1, tk[2])
                vs[j] = proj(2, j)
                vs[j + 1] = proj(2, j + 1, tk[3])
                ps[j] = qk(qs[j], ks[j], j == 0)
                ps[j + 1] = qk(qs[j + 1], ks[j + 1], j == 0)
                if j >= 2:
                    os_[j - 2] = pv(j - 2, ps[j - 2], vs[j - 2])
                    os_[j - 1] = pv(j - 1, ps[j - 1], vs[j - 1])
                tk = [conv_mac(mslot, r, j, 0), conv_mac(mslot, r, NP - 1 - j, 1),
                      conv_mac(mslot, r, j + 1, 0), conv_mac(mslot, r, NP - 2 - j, 1)]
            na = NP - 2
            acc = {}
            acc[0] = wo_part(os_, 0, na, 0, toks={0: tk[0], 8: tk[1]})
            acc[1] = wo_part(os_, 0, na, 1, toks={0: tk[2], 8: tk[3]})
            acc[2] = wo_part(os_, 0, na, 2)
            os_[NP - 2] = pv(NP - 2, ps[NP - 2], vs[NP - 2], True)
            os_[NP - 1] = pv(NP - 1, ps[NP - 1], vs[NP - 1], True)
            acc[3] = wo_part(os_, 0, na, 3)
            for n in range(4):
                acc[n] = wo_part(os_, na, NP, n, acc[n])
            tp = [conv_prep(cb, 8 * r + i, i) for i in range(8)]
            for n in range(4, 8):
                acc[n] = wo_part(os_, 0, NP, n, toks={0: tp[2 * (n - 4)], 8: tp[2 * (n - 4) + 1]})
            conv_fwd(cb, r)
            for n in range(NCB):
                b_ref[n, s, 0:NT, :] = acc[n][0:NT]
            return jnp.concatenate([acc[n][NT:SEG] for n in range(NCB)], axis=1).astype(bf16).astype(f32)

        def steps(i, mem):
            @pl.when(i == 8 // UNROLL)
            def _():
                wait_all(k_ref.at[1:NCB], SEM_KL)
                wait_all(v_ref.at[1:NCB], SEM_VL)
            for t in range(UNROLL):
                mem = step(i * UNROLL + t, mem)
            return mem

        lax.fori_loop(0, _DBG_STEPS // UNROLL, steps, mem_ref[...].astype(f32))

        def out_copy(n):
            slot = n % 2
            return pltpu.make_async_copy(
                ost_ref.at[slot], out_hbm.at[:, :, pl.ds(pl.multiple_of(n * 128, 128), 128)],
                sems.at[SEM_OUT + slot])

        def fin(n, c):
            @pl.when(n >= 2)
            def _():
                out_copy(n - 2).wait()
            icb = NCB - 2 + n // 4
            for i in range(4):
                conv_inv(a_ref, icb, icb % 2, icb, 4 * (n % 4) + i)
            toks = []
            for rr in range(2):
                r = 2 * (n % 4) + rr
                for a in range(NCH):
                    t = conv_mac((NCB - 1) % 2, r, a, 0, None if a % 4 == 0 else t)
                    t = conv_mac((NCB - 1) % 2, r, NCH - 1 - a, 1, t)
                    if a % 4 == 3:
                        toks.append(t)
            bd = None
            for kb in range(8):
                w = after(wo_ref[n, kb * 256:(kb + 1) * 256, :], toks[kb - 1] if kb > 0 else None)
                d = _dot(odef_ref[:, kb * 512:(kb + 1) * 512].astype(bf16), _as_bf16(w))
                bd = d if bd is None else d + bd
            b_ref[n, :, NT:SEG, :] = bd.reshape(NSEG, 8, 128)
            for blk in range(8):
                sg = slice(blk * 8, (blk + 1) * 8)
                b = b_ref[n, sg]
                a = a_ref[n, blk * 256:(blk + 1) * 256, :].reshape(8, SEG, 128)
                g = gate_ref[sg]
                ost_ref[n % 2, sg] = (g * a + (1.0 - g) * b).astype(bf16)
            out_copy(n).start()
            return c
        lax.fori_loop(0, NCB, fin, 0)
        out_copy(NCB - 2).wait()
        out_copy(NCB - 1).wait()

    pl.run_scoped(main, pltpu.VMEM((NSEG * 8, H * E), f32), pltpu.VMEM((NCB, NSEG, SEG, 128), f32),
                  pltpu.VMEM((NCB + 1, S, 128), f32))


@jax.jit
def pallas_gated_mix__ssm_conv_h3__memory_aug_recurrent_mem_tr__prompt_kernel(
    A_q: jax.Array,
    A_k: jax.Array,
    A_v: jax.Array,
    A_shift_k: jax.Array,
    A_ssm_k: jax.Array,
    A_ssm_D: jax.Array,
    B_x: jax.Array,
    B_mem0: jax.Array,
    B_Wq: jax.Array,
    B_Wk: jax.Array,
    B_Wv: jax.Array,
    B_Wo: jax.Array,
    B_seg_len: jax.Array,
    gate_w: jax.Array,
):
    del B_x, B_seg_len
    f_tab, g_tab = _dft_tables()
    out = pl.pallas_call(
        _kernel,
        out_shape=jax.ShapeDtypeStruct((NSEG, SEG, D), bf16),
        in_specs=[pl.BlockSpec(memory_space=pl.ANY)] * 15,
        out_specs=pl.BlockSpec(memory_space=pl.ANY),
        scratch_shapes=[
            pltpu.VMEM((3 * H, D // 2, E), u32),
            pltpu.VMEM((NCB, H * E // 2, 128), u32),
            pltpu.VMEM((NCB, S // 2, 128), u32),
            pltpu.VMEM((NSEG, M, D), bf16),
            pltpu.VMEM((NSEG * 4, D), u32),
            pltpu.VMEM((NSEG, 3 * NP, 8, E), u32),
            pltpu.VMEM((NCB, S // 2, 128), u32),
            pltpu.VMEM((NCB, S // 2, 128), u32),
            pltpu.VMEM((NCH, D // 2, 128), u32),
            pltpu.VMEM((NCB, S // 2, 128), u32),
            pltpu.VMEM((2, NCH, 128, 128), u32),
            pltpu.VMEM((2, NCH, 256, 128), f32),
            pltpu.VMEM((2, NCH, 256, 128), f32),
            pltpu.VMEM((256, 128), f32),
            pltpu.VMEM((8, 128), jnp.int32),
            pltpu.VMEM((8, 40, 128), f32),
            pltpu.VMEM((256, 128), bf16),
            pltpu.VMEM((128, 256), bf16),
            pltpu.VMEM((80, 80), f32),
            pltpu.VMEM((KS, D), bf16),
            pltpu.VMEM((NCB, 8, 128), f32),
            pltpu.VMEM((NCB, 128), bf16),
            pltpu.VMEM((NCB, 128), bf16),
            pltpu.VMEM((M, D), bf16),
            pltpu.VMEM((NSEG, SEG, 128), f32),
            pltpu.VMEM((2, NSEG, SEG, 128), bf16),
            pltpu.SemaphoreType.DMA((NSEM,)),
        ],
        compiler_params=pltpu.CompilerParams(vmem_limit_bytes=120 * 2**20),
    )(A_q.reshape(NSEG, SEG, D), A_q.reshape(S, D), A_k.reshape(S, D), A_v.reshape(S, D), A_shift_k.T,
      A_ssm_k, A_ssm_D.reshape(NCB, 128), B_mem0.reshape(M, D), B_Wq, B_Wk, B_Wv,
      B_Wo.reshape(H * E, D), gate_w.reshape(NCB, 128), jnp.asarray(f_tab, bf16), jnp.asarray(g_tab, bf16))
    return out.reshape(1, S, D)
```

```python
import numpy as np
import jax
import jax.numpy as jnp
from jax import lax
import jax.experimental.pallas as pl
import jax.experimental.pallas.tpu as pltpu

S, D, H, E, M, SEG = 2048, 1024, 32, 128, 8, 32
NSEG = S // SEG
NT = SEG - M
NP = H // 2
NCB = D // 128
C = 128
NCH = S // C
KS = 4
NG = 6
UNROLL = 2
CFG = dict(mac0=0, macsp=15, maclag=16, macrel=False, prep0=448, prepsp=8, preplag=0, preprel=False,
           split0=True, split1=True, nw=3, order=((0, 0), (1, 0), (0, 1), (1, 1), (2, 0), (2, 1)))
_DBG_STEPS = NSEG
bf16, f32, u32 = jnp.bfloat16, jnp.float32, jnp.uint32


def _dft_tables():
    t = np.arange(C, dtype=np.float64)
    rows = []
    for r in range(8):
        ev = 16 * r + np.arange(0, 16, 2)
        od = ev + 1
        for fn, fs in ((np.cos, ev), (np.sin, ev), (np.cos, od), (np.sin, od)):
            rows.append(fn(np.pi * (2 * fs[:, None] + 1) * t[None, :] / (2 * C)))
    f = np.concatenate(rows, axis=0)
    return f.astype(np.float32), (f.T / C).astype(np.float32)


def _fill_matrix():
    r = lax.broadcasted_iota(jnp.int32, (80, 80), 0)
    c = lax.broadcasted_iota(jnp.int32, (80, 80), 1)

    def head(i):
        return jnp.where(i < 64, i // 32, (i - 64) // 8)

    def idx(i):
        lo = i % 32
        main = jnp.where(lo < NT, lo + M, lo - NT)
        return jnp.where(i < 64, main, (i - 64) % 8 + NT + M)

    same = head(r) == head(c)
    ok = (idx(r) < M) | (idx(r) >= idx(c))
    return jnp.where(same, jnp.where(ok, 0.0, -1e9), -jnp.inf).astype(f32)


def _as_bf16(v):
    return pltpu.bitcast(v, bf16)


def _dot(a, b):
    return jnp.dot(a, b, preferred_element_type=f32)


def _dot_nt(a, b):
    return lax.dot_general(a, b, (((1,), (1,)), ((), ())), preferred_element_type=f32)


(SEM_XB, SEM_X, SEM_K0, SEM_V0, SEM_KL, SEM_VL, SEM_SSM, SEM_WO, SEM_SHIFT, SEM_D, SEM_GW, SEM_MEM,
 SEM_F, SEM_G) = range(14)
SEM_W = 14
SEM_OUT = SEM_W + 2 * NG
NSEM = SEM_OUT + 2


def _kernel(x3_hbm, x_hbm, k_hbm, v_hbm, shift_hbm, ssm_hbm, d_hbm, mem_hbm, wq_hbm, wk_hbm, wv_hbm,
            wo_hbm, gw_hbm, f_hbm, g_hbm, out_hbm,
            wn_ref, wo_ref, x_ref, xr_ref, xb_ref, pre_ref, k_ref, v_ref, ssm_ref, u_ref, z_ref,
            fu_ref, fk_ref, kraw_ref, one_ref, kf_ref, f_ref, g_ref, fill_ref, shift_ref, wt_ref,
            d_ref, gw_ref, mem_ref, gate_ref, ost_ref, sems):
    w_hbm = (wq_hbm, wk_hbm, wv_hbm)

    def cp(src, dst, sem):
        return pltpu.make_async_copy(src, dst, sems.at[sem])

    def start_col_blocks(src_hbm, dst_ref, i0, i1, sem):
        src = src_hbm.bitcast(u32)
        for i in range(i0, i1):
            cp(src.at[:, i * 128:(i + 1) * 128], dst_ref.at[i], sem).start()

    def wait_all(dst, sem):
        cp(dst, dst, sem).wait()

    def conv_prep(cb, i, slot, dep=None):
        row0 = pl.multiple_of(i * 16, 16)
        prev0 = pl.multiple_of(jnp.maximum(row0 - 8, 0), 8)
        prev = _as_bf16(k_ref[cb, pl.ds(prev0, 8), :]).astype(f32)[8:16]
        prev = jnp.where(i > 0, prev, 0.0)
        kraw = k_ref[cb, pl.ds(row0, 16), :]
        if dep is not None:
            kraw = jnp.where(jnp.concatenate([one_ref[...]] * 2, axis=0) == 1, kraw,
                             jnp.concatenate([dep] * 2, axis=0))
        kcur = _as_bf16(kraw).astype(f32)
        kk = jnp.concatenate([prev, kcur], axis=0)
        w = wt_ref[cb]
        ks = kcur * w[0:1, :]
        for j in range(1, KS):
            ks = ks + pltpu.roll(kk, j, axis=0)[8:40] * w[j:j + 1, :]
        kv = (ks * _as_bf16(v_ref[cb, pl.ds(row0, 16), :]).astype(f32)).astype(bf16)
        kv = pltpu.bitcast(kv, u32)
        u_ref[cb, pl.ds(row0, 16), :] = kv
        return kv[0:8] | kv[8:16]

    def combine(kf, prev):
        out = []
        for g in range(8):
            o = 32 * g
            out += [kf[o:o + 8] + prev[o + 8:o + 16], kf[o + 8:o + 16] - prev[o:o + 8],
                    kf[o + 16:o + 24] - prev[o + 24:o + 32], kf[o + 24:o + 32] + prev[o + 16:o + 24]]
        return jnp.concatenate(out, axis=0)

    def conv_fwd(cb, r):
        slot = cb % 2
        rows = pl.ds(pl.multiple_of(cb * 64, 64), 64)
        f = f_ref[...]
        kfs = []
        for a in (2 * r, 2 * r + 1):
            fu_ref[slot, a] = _dot(f, _as_bf16(u_ref[cb, pl.ds(pl.multiple_of(a * 64, 64), 64), :]))
            kfs.append(_dot_nt(f, _as_bf16(ssm_ref[a, rows, :])))
        fk_ref[slot, 2 * r] = combine(kfs[0], jnp.where(r > 0, kraw_ref[...], 0.0))
        fk_ref[slot, 2 * r + 1] = combine(kfs[1], kfs[0])
        kraw_ref[...] = kfs[1]

    def conv_mac(slot, r, a, half, dep=None):
        ro = pl.multiple_of(r * 32, 32) + half * 16
        p = q = None
        for c in range(a + 1):
            u = fu_ref[slot, a - c, pl.ds(ro, 16), :]
            k = fk_ref[slot, c, pl.ds(ro, 16), :]
            ua, ub, kc, kd = u[0:8], u[8:16], k[0:8], k[8:16]
            if c == 0 and dep is not None:
                ua = jnp.where(one_ref[...] == 1, ua, pltpu.bitcast(dep, f32))
            p = (ua * kc if p is None else p + ua * kc) - ub * kd
            q = (ua * kd if q is None else q + ua * kd) + ub * kc
        z = pltpu.bitcast(jnp.concatenate([p, q], axis=0).astype(bf16), u32)
        z_ref[slot, a, pl.ds(pl.multiple_of(r * 16, 16) + half * 8, 8), :] = z
        return z

    def conv_inv(a_ref, cb, slot, dst, a):
        rows = pl.ds(pl.multiple_of(a * 64, 64), 64)
        y = _dot(g_ref[...], _as_bf16(z_ref[slot, a]))
        kv = _as_bf16(u_ref[cb, rows, :]).astype(f32)
        q = _as_bf16(x_ref[cb, rows, :]).astype(f32)
        a_ref[dst, pl.ds(pl.multiple_of(a * C, C), C), :] = q * (y + kv * wt_ref[cb, KS:KS + 1, :])

    def after(w, tok):
        if tok is None:
            return w
        return jnp.concatenate([jnp.where(one_ref[...] == 1, w[0:8], tok), w[8:]], axis=0)

    def prologue(stage_ref):
        st3 = stage_ref.reshape(NG * D, 8, E)

        def start_w(g):
            src = w_hbm[g // 2].bitcast(u32)
            for hf in range(2):
                r0 = (g % 2) * 8 + hf * 4
                cp(src.at[:, r0:r0 + 4, :], st3.at[g * D:(g + 1) * D, hf * 4:hf * 4 + 4, :],
                   SEM_W + 2 * g + hf).start()

        def wait_w(g, hf):
            wait_all(st3.at[pl.ds(g * D, D), hf * 4:hf * 4 + 4, :], SEM_W + 2 * g + hf)

        small = [cp(shift_hbm, shift_ref, SEM_SHIFT), cp(d_hbm, d_ref, SEM_D), cp(gw_hbm, gw_ref, SEM_GW),
                 cp(mem_hbm, mem_ref, SEM_MEM), cp(f_hbm, f_ref, SEM_F), cp(g_hbm, g_ref, SEM_G)]
        cp_xb = cp(x3_hbm.at[:, NT:SEG, :], xr_ref, SEM_XB)
        cp_xb.start()
        start_w(0)
        for c in small:
            c.start()
        for g in range(1, NG):
            start_w(g)
        start_col_blocks(wo_hbm, wo_ref, 0, NCB, SEM_WO)
        start_col_blocks(x_hbm, x_ref, 0, NCB, SEM_X)
        start_col_blocks(k_hbm, k_ref, 0, 1, SEM_K0)
        start_col_blocks(v_hbm, v_ref, 0, 1, SEM_V0)
        start_col_blocks(ssm_hbm, ssm_ref, 0, NCH, SEM_SSM)
        start_col_blocks(k_hbm, k_ref, 1, NCB, SEM_KL)
        start_col_blocks(v_hbm, v_ref, 1, NCB, SEM_VL)
        fill_ref[...] = _fill_matrix()
        one_ref[...] = jnp.ones((8, 128), jnp.int32)
        cp_xb.wait()

        def xb_build(it, c):
            s0 = pl.multiple_of(it * 8, 8)
            t = xr_ref[pl.ds(s0, 8)].astype(f32).reshape(64, D).astype(bf16)
            xb_ref[pl.ds(pl.multiple_of(it * 32, 32), 32), :] = pltpu.bitcast(t, u32)
            return c
        lax.fori_loop(0, 8, xb_build, 0)

        def group(g, c):
            sub = stage_ref.at[pl.ds(pl.multiple_of(g * (8 * D), 8 * D), 8 * D), :]

            def relayout(j):
                toks = []
                for blk in range(D // 256):
                    w = sub[pl.ds(blk * 2048 + j, 256, stride=8), :]
                    lo = pltpu.bitcast(pltpu.bitcast(w << 16, f32).astype(bf16), u32)
                    hi = pltpu.bitcast(pltpu.bitcast(w & jnp.uint32(0xFFFF0000), f32).astype(bf16), u32)
                    wn_ref[g * 16 + 2 * j, blk * 128:(blk + 1) * 128, :] = lo
                    wn_ref[g * 16 + 2 * j + 1, blk * 128:(blk + 1) * 128, :] = hi
                    t = lo | hi
                    tok = t[0:8]
                    for i in range(1, 16):
                        tok = tok | t[8 * i:8 * i + 8]
                    toks.append(tok)
                return toks

            wait_w(g, 0)
            relayout(0)
            for j in range(8):
                if j == 3:
                    wait_w(g, 1)
                xb = _as_bf16(xb_ref[...])
                w1, w2 = wn_ref[g * 16 + 2 * j], wn_ref[g * 16 + 2 * j + 1]
                toks = relayout(j + 1) if j + 1 < 8 else None
                if j == 2:
                    w1 = jnp.concatenate([after(w1[0:256], toks[0]), after(w1[256:], toks[1])], axis=0)
                    w2 = jnp.concatenate([after(w2[0:256], toks[2]), after(w2[256:], toks[3])], axis=0)
                r1 = _dot(xb, _as_bf16(w1))
                r2 = _dot(xb, _as_bf16(w2))
                cc = jnp.concatenate([r1.reshape(NSEG, 8, E), r2.reshape(NSEG, 8, E)], axis=1).astype(bf16)
                pre_ref[:, g * 8 + j] = pltpu.bitcast(cc, u32)
            return c
        lax.fori_loop(0, NG, group, 0)
        for c in small:
            c.wait()

    pl.run_scoped(prologue, pltpu.VMEM((NG * 8 * D, E), u32))

    sh = shift_ref[...].astype(f32)
    dv = d_ref[...].astype(f32)
    for n in range(NCB):
        wt_ref[n, 0:KS, :] = sh[:, n * 128:(n + 1) * 128]
        wt_ref[n, KS:KS + 1, :] = dv[n:n + 1, :]
    wait_all(wo_ref, SEM_WO)
    wait_all(x_ref, SEM_X)
    wait_all(k_ref.at[0:1], SEM_K0)
    wait_all(v_ref.at[0:1], SEM_V0)
    wait_all(ssm_ref, SEM_SSM)

    scale = E ** -0.5

    def main(odef_ref, b_ref, a_ref):
        def step(s, mem):
            cb = s // 8
            r = s % 8
            icb = jnp.maximum(cb - 2, 0)
            idst = jnp.where(cb >= 2, cb - 2, NCB)
            mslot = (cb + 1) % 2

            xrows = pl.ds(pl.multiple_of(s * 16, 16), 16)
            xs = [_as_bf16(x_ref[n, xrows, :]).astype(f32) for n in range(NCB)]
            h32 = jnp.concatenate([jnp.concatenate(xs, axis=1)[0:NT], mem], axis=0).astype(bf16)
            r0 = pl.multiple_of(s * 8, 8)

            conv_inv(a_ref, icb, cb % 2, idst, 2 * r)
            conv_inv(a_ref, icb, cb % 2, idst, 2 * r + 1)

            gw = gw_ref[...].astype(f32)
            gl = xs[0] * gw[0:1, :]
            for n in range(1, NCB):
                gl = gl + xs[n] * gw[n:n + 1, :]
            gl = jnp.sum(gl, axis=-1, keepdims=True)
            gate_ref[s] = jnp.broadcast_to(jax.nn.sigmoid(gl), (SEG, 128))

            cfg = CFG
            jobs = []
            units = []
            for a in range(NCH):
                units += [(a, 0), (NCH - 1 - a, 1)]
            for i, (ua, uh) in enumerate(units):
                jobs.append((cfg["mac0"] + int(i * cfg["macsp"]), cfg["maclag"], cfg["macrel"],
                             lambda dep, ua=ua, uh=uh: conv_mac(mslot, r, ua, uh, dep)))
            for i in range(8):
                jobs.append((cfg["prep0"] + int(i * cfg["prepsp"]), cfg["preplag"], cfg["preprel"],
                             lambda dep, i=i: conv_prep(cb, 8 * r + i, i, dep)))
            state = dict(count=0, due={})

            def sdot(lhs, w, acc=None, weight=1):
                c = state["count"]
                toks = [t for cc in range(c, c + weight) for t in state["due"].pop(cc, [])]
                nt = w.shape[0] // 64
                if toks:
                    tiles = [w[64 * i:64 * (i + 1)] for i in range(nt)]
                    for i, t in enumerate(toks):
                        tiles[i % nt] = after(tiles[i % nt], t)
                    w = jnp.concatenate(tiles, axis=0)
                d = _dot(lhs, _as_bf16(w))
                d = d if acc is None else d + acc
                for (st, lag, rel, fn) in jobs:
                    if c <= st < c + weight:
                        tok = fn(pltpu.bitcast(d[0:8], u32) if rel else None)
                        state["due"].setdefault(max(st + lag, c + weight), []).append(tok)
                state["count"] = c + weight
                return d

            def proj(m, j):
                r1 = sdot(h32, wn_ref[m * H + 2 * j], weight=4)
                r2 = sdot(h32, wn_ref[m * H + 2 * j + 1], weight=4)
                p = _as_bf16(pre_ref[s, m * NP + j]).astype(f32)
                r = jnp.concatenate([r1, r2, p], axis=0)
                return r if m == 0 else r.astype(bf16)

            def split_rows(dot, lhs, rhs, split):
                if not split:
                    return dot(lhs.astype(bf16), rhs)
                return jnp.concatenate([dot(lhs[0:48].astype(bf16), rhs), dot(lhs[48:80].astype(bf16), rhs)], axis=0)

            def qk(q80, k80, split=False):
                fill = fill_ref[...]
                sc = jnp.where(fill == 0.0, split_rows(_dot_nt, q80, k80, split) * scale, fill)
                p = jnp.exp(sc - jnp.max(sc, axis=-1, keepdims=True))
                den = jnp.sum(p, axis=-1, keepdims=True)
                rc = pl.reciprocal(den, approx=True)
                return p * (rc * (2.0 - den * rc))

            def pv(j, p, v80, split=False):
                o80 = split_rows(_dot, p, v80, split)
                odef_ref[pl.ds(r0, 8), (2 * j) * E:(2 * j + 1) * E] = o80[64:72]
                odef_ref[pl.ds(r0, 8), (2 * j + 1) * E:(2 * j + 2) * E] = o80[72:80]
                return jnp.concatenate([o80[0:32], o80[32:64]], axis=1).astype(bf16)

            def wo_part(o, j0, j1, n, acc=None):
                for j in range(j0, j1):
                    acc = sdot(o[j], wo_ref[n, j * 128:(j + 1) * 128, :], acc)
                return acc

            qs, ks, vs, ps, os_ = {}, {}, {}, {}, {}
            for j in range(0, NP, 2):
                for m, jj in cfg["order"]:
                    (qs, ks, vs)[m][j + jj] = proj(m, j + jj)
                ps[j] = qk(qs[j], ks[j], j == 0 and cfg["split0"])
                ps[j + 1] = qk(qs[j + 1], ks[j + 1], j == 0 and cfg["split0"])
                if j >= 2:
                    os_[j - 2] = pv(j - 2, ps[j - 2], vs[j - 2])
                    os_[j - 1] = pv(j - 1, ps[j - 1], vs[j - 1])
            na = NP - 2
            acc = {}
            nw = cfg["nw"]
            for n in range(nw):
                acc[n] = wo_part(os_, 0, na, n)
            os_[NP - 2] = pv(NP - 2, ps[NP - 2], vs[NP - 2], cfg["split1"])
            os_[NP - 1] = pv(NP - 1, ps[NP - 1], vs[NP - 1], cfg["split1"])
            acc[nw] = wo_part(os_, 0, na, nw)
            for n in range(nw + 1):
                acc[n] = wo_part(os_, na, NP, n, acc[n])
            for n in range(nw + 1, 8):
                acc[n] = wo_part(os_, 0, NP, n)
            assert state["count"] == 512 and not state["due"], state
            conv_fwd(cb, r)
            for n in range(NCB):
                b_ref[n, s, 0:NT, :] = acc[n][0:NT]
            return jnp.concatenate([acc[n][NT:SEG] for n in range(NCB)], axis=1).astype(bf16).astype(f32)

        def steps(i, mem):
            @pl.when(i == 8 // UNROLL)
            def _():
                wait_all(k_ref.at[1:NCB], SEM_KL)
                wait_all(v_ref.at[1:NCB], SEM_VL)
            for t in range(UNROLL):
                mem = step(i * UNROLL + t, mem)
            return mem

        lax.fori_loop(0, _DBG_STEPS // UNROLL, steps, mem_ref[...].astype(f32))

        def out_copy(n):
            slot = n % 2
            return pltpu.make_async_copy(
                ost_ref.at[slot], out_hbm.at[:, :, pl.ds(pl.multiple_of(n * 128, 128), 128)],
                sems.at[SEM_OUT + slot])

        def fin(n, c):
            @pl.when(n >= 2)
            def _():
                out_copy(n - 2).wait()
            icb = NCB - 2 + n // 4
            for i in range(4):
                conv_inv(a_ref, icb, icb % 2, icb, 4 * (n % 4) + i)
            toks = []
            for rr in range(2):
                r = 2 * (n % 4) + rr
                for a in range(NCH):
                    t = conv_mac((NCB - 1) % 2, r, a, 0, None if a % 4 == 0 else t)
                    t = conv_mac((NCB - 1) % 2, r, NCH - 1 - a, 1, t)
                    if a % 4 == 3:
                        toks.append(t)
            bd = None
            for kb in range(8):
                w = after(wo_ref[n, kb * 256:(kb + 1) * 256, :], toks[kb - 1] if kb > 0 else None)
                d = _dot(odef_ref[:, kb * 512:(kb + 1) * 512].astype(bf16), _as_bf16(w))
                bd = d if bd is None else d + bd
            b_ref[n, :, NT:SEG, :] = bd.reshape(NSEG, 8, 128)
            for blk in range(8):
                sg = slice(blk * 8, (blk + 1) * 8)
                b = b_ref[n, sg]
                a = a_ref[n, blk * 256:(blk + 1) * 256, :].reshape(8, SEG, 128)
                g = gate_ref[sg]
                ost_ref[n % 2, sg] = (g * a + (1.0 - g) * b).astype(bf16)
            out_copy(n).start()
            return c
        lax.fori_loop(0, NCB, fin, 0)
        out_copy(NCB - 2).wait()
        out_copy(NCB - 1).wait()

    pl.run_scoped(main, pltpu.VMEM((NSEG * 8, H * E), f32), pltpu.VMEM((NCB, NSEG, SEG, 128), f32),
                  pltpu.VMEM((NCB + 1, S, 128), f32))


@jax.jit
def pallas_gated_mix__ssm_conv_h3__memory_aug_recurrent_mem_tr__prompt_kernel(
    A_q: jax.Array,
    A_k: jax.Array,
    A_v: jax.Array,
    A_shift_k: jax.Array,
    A_ssm_k: jax.Array,
    A_ssm_D: jax.Array,
    B_x: jax.Array,
    B_mem0: jax.Array,
    B_Wq: jax.Array,
    B_Wk: jax.Array,
    B_Wv: jax.Array,
    B_Wo: jax.Array,
    B_seg_len: jax.Array,
    gate_w: jax.Array,
):
    del B_x, B_seg_len
    f_tab, g_tab = _dft_tables()
    out = pl.pallas_call(
        _kernel,
        out_shape=jax.ShapeDtypeStruct((NSEG, SEG, D), bf16),
        in_specs=[pl.BlockSpec(memory_space=pl.ANY)] * 15,
        out_specs=pl.BlockSpec(memory_space=pl.ANY),
        scratch_shapes=[
            pltpu.VMEM((3 * H, D // 2, E), u32),
            pltpu.VMEM((NCB, H * E // 2, 128), u32),
            pltpu.VMEM((NCB, S // 2, 128), u32),
            pltpu.VMEM((NSEG, M, D), bf16),
            pltpu.VMEM((NSEG * 4, D), u32),
            pltpu.VMEM((NSEG, 3 * NP, 8, E), u32),
            pltpu.VMEM((NCB, S // 2, 128), u32),
            pltpu.VMEM((NCB, S // 2, 128), u32),
            pltpu.VMEM((NCH, D // 2, 128), u32),
            pltpu.VMEM((NCB, S // 2, 128), u32),
            pltpu.VMEM((2, NCH, 128, 128), u32),
            pltpu.VMEM((2, NCH, 256, 128), f32),
            pltpu.VMEM((2, NCH, 256, 128), f32),
            pltpu.VMEM((256, 128), f32),
            pltpu.VMEM((8, 128), jnp.int32),
            pltpu.VMEM((8, 40, 128), f32),
            pltpu.VMEM((256, 128), bf16),
            pltpu.VMEM((128, 256), bf16),
            pltpu.VMEM((80, 80), f32),
            pltpu.VMEM((KS, D), bf16),
            pltpu.VMEM((NCB, 8, 128), f32),
            pltpu.VMEM((NCB, 128), bf16),
            pltpu.VMEM((NCB, 128), bf16),
            pltpu.VMEM((M, D), bf16),
            pltpu.VMEM((NSEG, SEG, 128), f32),
            pltpu.VMEM((2, NSEG, SEG, 128), bf16),
            pltpu.SemaphoreType.DMA((NSEM,)),
        ],
        compiler_params=pltpu.CompilerParams(vmem_limit_bytes=120 * 2**20),
    )(A_q.reshape(NSEG, SEG, D), A_q.reshape(S, D), A_k.reshape(S, D), A_v.reshape(S, D), A_shift_k.T,
      A_ssm_k, A_ssm_D.reshape(NCB, 128), B_mem0.reshape(M, D), B_Wq, B_Wk, B_Wv,
      B_Wo.reshape(H * E, D), gate_w.reshape(NCB, 128), jnp.asarray(f_tab, bf16), jnp.asarray(g_tab, bf16))
    return out.reshape(1, S, D)
```

```python
import numpy as np
import jax
import jax.numpy as jnp
from jax import lax
import jax.experimental.pallas as pl
import jax.experimental.pallas.tpu as pltpu

S, D, H, E, M, SEG = 2048, 1024, 32, 128, 8, 32
NSEG = S // SEG
NT = SEG - M
NP = H // 2
NCB = D // 128
C = 128
NCH = S // C
KS = 4
KPAD = 32
NG = 6
UNROLL = 2
CFG = dict(mac0=0, macsp=15, maclag=16, macrel=False,
           split0=True, split1=True, nw=3, order=((0, 0), (1, 0), (0, 1), (1, 1), (2, 0), (2, 1)))
_DBG_STEPS = NSEG
bf16, f32, u32 = jnp.bfloat16, jnp.float32, jnp.uint32


def _dft_tables():
    t = np.arange(C, dtype=np.float64)
    rows = []
    for r in range(8):
        ev = 16 * r + np.arange(0, 16, 2)
        od = ev + 1
        for fn, fs in ((np.cos, ev), (np.sin, ev), (np.cos, od), (np.sin, od)):
            rows.append(fn(np.pi * (2 * fs[:, None] + 1) * t[None, :] / (2 * C)))
    f = np.concatenate(rows, axis=0)
    return f.astype(np.float32), (f.T / C).astype(np.float32)


def _fill_matrix():
    r = lax.broadcasted_iota(jnp.int32, (80, 80), 0)
    c = lax.broadcasted_iota(jnp.int32, (80, 80), 1)

    def head(i):
        return jnp.where(i < 64, i // 32, (i - 64) // 8)

    def idx(i):
        lo = i % 32
        main = jnp.where(lo < NT, lo + M, lo - NT)
        return jnp.where(i < 64, main, (i - 64) % 8 + NT + M)

    same = head(r) == head(c)
    ok = (idx(r) < M) | (idx(r) >= idx(c))
    return jnp.where(same, jnp.where(ok, 0.0, -1e9), -jnp.inf).astype(f32)


def _as_bf16(v):
    return pltpu.bitcast(v, bf16)


def _dot(a, b):
    return jnp.dot(a, b, preferred_element_type=f32)


def _dot_nt(a, b):
    return lax.dot_general(a, b, (((1,), (1,)), ((), ())), preferred_element_type=f32)


(SEM_XB, SEM_X, SEM_SSM0, SEM_SSM1, SEM_WO, SEM_SHIFT, SEM_D, SEM_GW, SEM_MEM, SEM_F, SEM_G) = range(11)
SEM_K = 11
SEM_V = SEM_K + 4
SEM_W = SEM_V + 4
SEM_OUT = SEM_W + 2 * NG
NSEM = SEM_OUT + 2


def _kernel(x3_hbm, x_hbm, k_hbm, v_hbm, shift_hbm, ssm_hbm, d_hbm, mem_hbm, wq_hbm, wk_hbm, wv_hbm,
            wo_hbm, gw_hbm, f_hbm, g_hbm, out_hbm,
            wn_ref, wo_ref, x_ref, xr_ref, xb_ref, pre_ref, k_ref, v_ref, ssm_ref, u_ref, z_ref,
            fu_ref, fk_ref, kraw_ref, one_ref, f_ref, g_ref, fill_ref, shift_ref, wt_ref,
            d_ref, gw_ref, mem_ref, gate_ref, ost_ref, sems):
    w_hbm = (wq_hbm, wk_hbm, wv_hbm)

    def cp(src, dst, sem):
        return pltpu.make_async_copy(src, dst, sems.at[sem])

    def start_col_blocks(src_hbm, dst_ref, i0, i1, sem, row0=0):
        src = src_hbm.bitcast(u32)
        for i in range(i0, i1):
            cp(src.at[:, i * 128:(i + 1) * 128], dst_ref.at[i, row0:], sem).start()

    def wait_all(dst, sem):
        cp(dst, dst, sem).wait()

    def even(p):
        return pltpu.bitcast(p << 16, f32)

    def odd(p):
        return pltpu.bitcast(p & jnp.uint32(0xFFFF0000), f32)

    def conv_prep(cb, i, dep=None):
        r0 = KPAD + 8 * i
        p0 = k_ref[cb, r0:r0 + 8, :]
        if dep is not None:
            p0 = jnp.where(one_ref[...] == 1, p0, dep)
        p1 = k_ref[cb, r0 - 1:r0 + 7, :]
        p2 = k_ref[cb, r0 - 2:r0 + 6, :]
        pv = v_ref[cb, 8 * i:8 * i + 8, :]
        w = wt_ref[cb]
        w0, w1, w2, w3 = w[0:1, :], w[1:2, :], w[2:3, :], w[3:4, :]
        e0, o0, e1, o1, o2 = even(p0), odd(p0), even(p1), odd(p1), odd(p2)
        ke = ((e0 * w0 + o1 * w1) + e1 * w2) + o2 * w3
        ko = ((o0 * w0 + e0 * w1) + o1 * w2) + e1 * w3
        re = pltpu.bitcast((ke * even(pv)).astype(bf16).astype(f32), u32)
        ro = pltpu.bitcast((ko * odd(pv)).astype(bf16).astype(f32), u32)
        kv = (re >> 16) | ro
        u_ref[cb, 8 * i:8 * i + 8, :] = kv
        return kv

    def combine(kf, prev):
        out = []
        for g in range(8):
            o = 32 * g
            out += [kf[o:o + 8] + prev[o + 8:o + 16], kf[o + 8:o + 16] - prev[o:o + 8],
                    kf[o + 16:o + 24] - prev[o + 24:o + 32], kf[o + 24:o + 32] + prev[o + 16:o + 24]]
        return jnp.concatenate(out, axis=0)

    def conv_fwd(cb, r):
        slot = cb % 2
        rows = pl.ds(pl.multiple_of(cb * 64, 64), 64)
        f = f_ref[...]
        kfs = []
        for a in (2 * r, 2 * r + 1):
            fu_ref[slot, a] = _dot(f, _as_bf16(u_ref[cb, pl.ds(pl.multiple_of(a * 64, 64), 64), :]))
            kfs.append(_dot_nt(f, _as_bf16(ssm_ref[a, rows, :])))
        fk_ref[slot, 2 * r] = combine(kfs[0], jnp.where(r > 0, kraw_ref[...], 0.0))
        fk_ref[slot, 2 * r + 1] = combine(kfs[1], kfs[0])
        kraw_ref[...] = kfs[1]

    def conv_mac(slot, r, a, half, dep=None):
        ro = pl.multiple_of(r * 32, 32) + half * 16
        p = q = None
        for c in range(a + 1):
            u = fu_ref[slot, a - c, pl.ds(ro, 16), :]
            k = fk_ref[slot, c, pl.ds(ro, 16), :]
            ua, ub, kc, kd = u[0:8], u[8:16], k[0:8], k[8:16]
            if c == 0 and dep is not None:
                ua = jnp.where(one_ref[...] == 1, ua, pltpu.bitcast(dep, f32))
            p = (ua * kc if p is None else p + ua * kc) - ub * kd
            q = (ua * kd if q is None else q + ua * kd) + ub * kc
        z = pltpu.bitcast(jnp.concatenate([p, q], axis=0).astype(bf16), u32)
        z_ref[slot, a, pl.ds(pl.multiple_of(r * 16, 16) + half * 8, 8), :] = z
        return z

    def conv_inv(a_ref, cb, slot, dst, a):
        rows = pl.ds(pl.multiple_of(a * 64, 64), 64)
        y = _dot(g_ref[...], _as_bf16(z_ref[slot, a]))
        kv = _as_bf16(u_ref[cb, rows, :]).astype(f32)
        q = _as_bf16(x_ref[cb, rows, :]).astype(f32)
        a_ref[dst, pl.ds(pl.multiple_of(a * C, C), C), :] = q * (y + kv * wt_ref[cb, KS:KS + 1, :])

    def after(w, tok):
        if tok is None:
            return w
        return jnp.concatenate([jnp.where(one_ref[...] == 1, w[0:8], tok), w[8:]], axis=0)

    def prologue(stage_ref):
        st3 = stage_ref.reshape(NG * D, 8, E)

        def start_w(g):
            src = w_hbm[g // 2].bitcast(u32)
            for hf in range(2):
                r0 = (g % 2) * 8 + hf * 4
                cp(src.at[:, r0:r0 + 4, :], st3.at[g * D:(g + 1) * D, hf * 4:hf * 4 + 4, :],
                   SEM_W + 2 * g + hf).start()

        def wait_w(g, hf):
            wait_all(st3.at[pl.ds(g * D, D), hf * 4:hf * 4 + 4, :], SEM_W + 2 * g + hf)

        taps = [cp(shift_hbm, shift_ref, SEM_SHIFT), cp(d_hbm, d_ref, SEM_D)]
        small = [cp(gw_hbm, gw_ref, SEM_GW), cp(mem_hbm, mem_ref, SEM_MEM), cp(f_hbm, f_ref, SEM_F),
                 cp(g_hbm, g_ref, SEM_G)]
        cp_xb = cp(x3_hbm.at[:, NT:SEG, :], xr_ref, SEM_XB)
        for c in taps:
            c.start()
        cp_xb.start()
        start_w(0)
        for g in range(1, NG):
            start_w(g)
            if g <= 4:
                start_col_blocks(k_hbm, k_ref, 2 * g - 2, 2 * g, SEM_K + g - 1, row0=KPAD)
                start_col_blocks(v_hbm, v_ref, 2 * g - 2, 2 * g, SEM_V + g - 1)
        for c in small:
            c.start()
        start_col_blocks(wo_hbm, wo_ref, 0, NCB, SEM_WO)
        start_col_blocks(x_hbm, x_ref, 0, NCB, SEM_X)
        start_col_blocks(ssm_hbm, ssm_ref, 0, 2 * UNROLL, SEM_SSM0)
        start_col_blocks(ssm_hbm, ssm_ref, 2 * UNROLL, NCH, SEM_SSM1)
        fill_ref[...] = _fill_matrix()
        one_ref[...] = jnp.ones((8, 128), jnp.int32)
        k_ref[:, KPAD - 8:KPAD, :] = jnp.zeros((NCB + 1, 8, 128), u32)
        for c in taps:
            c.wait()
        sh = shift_ref[...].astype(f32)
        dv = d_ref[...].astype(f32)
        for n in range(NCB):
            wt_ref[n, 0:KS, :] = sh[:, n * 128:(n + 1) * 128]
            wt_ref[n, KS:KS + 1, :] = dv[n:n + 1, :]
        cp_xb.wait()

        def xb_build(it, c):
            s0 = pl.multiple_of(it * 8, 8)
            t = xr_ref[pl.ds(s0, 8)].astype(f32).reshape(64, D).astype(bf16)
            xb_ref[pl.ds(pl.multiple_of(it * 32, 32), 32), :] = pltpu.bitcast(t, u32)
            return c
        lax.fori_loop(0, 8, xb_build, 0)

        def group(g, c):
            sub = stage_ref.at[pl.ds(pl.multiple_of(g * (8 * D), 8 * D), 8 * D), :]

            def relayout(j):
                toks = []
                for blk in range(D // 256):
                    w = sub[pl.ds(blk * 2048 + j, 256, stride=8), :]
                    lo = pltpu.bitcast(even(w).astype(bf16), u32)
                    hi = pltpu.bitcast(odd(w).astype(bf16), u32)
                    wn_ref[g * 16 + 2 * j, blk * 128:(blk + 1) * 128, :] = lo
                    wn_ref[g * 16 + 2 * j + 1, blk * 128:(blk + 1) * 128, :] = hi
                    t = lo | hi
                    tok = t[0:8]
                    for i in range(1, 16):
                        tok = tok | t[8 * i:8 * i + 8]
                    toks.append(tok)
                return toks

            has_kv = jnp.logical_and(g >= 1, g <= 4)

            def prep_chain(k):
                cb = jnp.where(has_kv, 2 * g - 2 + k // 8, NCB)
                t = None
                for i in range(16):
                    t = conv_prep(cb, (k % 8) * 16 + i, t)
                return t

            wait_w(g, 0)
            relayout(0)
            for j in range(8):
                if j == 3:
                    wait_w(g, 1)

                    @pl.when(has_kv)
                    def _():
                        wait_all(k_ref.at[pl.ds(2 * g - 2, 2), KPAD:], SEM_K + g - 1)
                        wait_all(v_ref.at[pl.ds(2 * g - 2, 2)], SEM_V + g - 1)
                xb = _as_bf16(xb_ref[...])
                w1, w2 = wn_ref[g * 16 + 2 * j], wn_ref[g * 16 + 2 * j + 1]
                toks = relayout(j + 1) if j + 1 < 8 else None
                if j >= 4:
                    toks = [prep_chain(4 * (j - 4) + i) for i in range(4)]
                if j == 2 or j >= 4:
                    w1 = jnp.concatenate([after(w1[0:256], toks[0]), after(w1[256:], toks[1])], axis=0)
                    w2 = jnp.concatenate([after(w2[0:256], toks[2]), after(w2[256:], toks[3])], axis=0)
                r1 = _dot(xb, _as_bf16(w1))
                r2 = _dot(xb, _as_bf16(w2))
                cc = jnp.concatenate([r1.reshape(NSEG, 8, E), r2.reshape(NSEG, 8, E)], axis=1).astype(bf16)
                pre_ref[:, g * 8 + j] = pltpu.bitcast(cc, u32)
            return c
        lax.fori_loop(0, NG, group, 0)
        for c in small:
            c.wait()

    pl.run_scoped(prologue, pltpu.VMEM((NG * 8 * D, E), u32))

    wait_all(wo_ref, SEM_WO)
    wait_all(x_ref, SEM_X)
    wait_all(ssm_ref.at[0:2 * UNROLL], SEM_SSM0)

    scale = E ** -0.5

    def main(odef_ref, b_ref, a_ref):
        def step(s, mem):
            cb = s // 8
            r = s % 8
            icb = jnp.maximum(cb - 2, 0)
            idst = jnp.where(cb >= 2, cb - 2, NCB)
            mslot = (cb + 1) % 2

            xrows = pl.ds(pl.multiple_of(s * 16, 16), 16)
            xs = [_as_bf16(x_ref[n, xrows, :]).astype(f32) for n in range(NCB)]
            h32 = jnp.concatenate([jnp.concatenate(xs, axis=1)[0:NT], mem], axis=0).astype(bf16)
            r0 = pl.multiple_of(s * 8, 8)

            conv_inv(a_ref, icb, cb % 2, idst, 2 * r)
            conv_inv(a_ref, icb, cb % 2, idst, 2 * r + 1)

            gw = gw_ref[...].astype(f32)
            gl = xs[0] * gw[0:1, :]
            for n in range(1, NCB):
                gl = gl + xs[n] * gw[n:n + 1, :]
            gl = jnp.sum(gl, axis=-1, keepdims=True)
            gate_ref[s] = jnp.broadcast_to(jax.nn.sigmoid(gl), (SEG, 128))

            cfg = CFG
            jobs = []
            units = []
            for a in range(NCH):
                units += [(a, 0), (NCH - 1 - a, 1)]
            for i, (ua, uh) in enumerate(units):
                jobs.append((cfg["mac0"] + int(i * cfg["macsp"]), cfg["maclag"], cfg["macrel"],
                             lambda dep, ua=ua, uh=uh: conv_mac(mslot, r, ua, uh, dep)))
            state = dict(count=0, due={})

            def sdot(lhs, w, acc=None, weight=1):
                c = state["count"]
                toks = [t for cc in range(c, c + weight) for t in state["due"].pop(cc, [])]
                nt = w.shape[0] // 64
                if toks:
                    tiles = [w[64 * i:64 * (i + 1)] for i in range(nt)]
                    for i, t in enumerate(toks):
                        tiles[i % nt] = after(tiles[i % nt], t)
                    w = jnp.concatenate(tiles, axis=0)
                d = _dot(lhs, _as_bf16(w))
                d = d if acc is None else d + acc
                for (st, lag, rel, fn) in jobs:
                    if c <= st < c + weight:
                        tok = fn(pltpu.bitcast(d[0:8], u32) if rel else None)
                        state["due"].setdefault(max(st + lag, c + weight), []).append(tok)
                state["count"] = c + weight
                return d

            def proj(m, j):
                r1 = sdot(h32, wn_ref[m * H + 2 * j], weight=4)
                r2 = sdot(h32, wn_ref[m * H + 2 * j + 1], weight=4)
                p = _as_bf16(pre_ref[s, m * NP + j]).astype(f32)
                r = jnp.concatenate([r1, r2, p], axis=0)
                return r if m == 0 else r.astype(bf16)

            def split_rows(dot, lhs, rhs, split):
                if not split:
                    return dot(lhs.astype(bf16), rhs)
                return jnp.concatenate([dot(lhs[0:48].astype(bf16), rhs), dot(lhs[48:80].astype(bf16), rhs)], axis=0)

            def qk(q80, k80, split=False):
                fill = fill_ref[...]
                sc = jnp.where(fill == 0.0, split_rows(_dot_nt, q80, k80, split) * scale, fill)
                p = jnp.exp(sc - jnp.max(sc, axis=-1, keepdims=True))
                den = jnp.sum(p, axis=-1, keepdims=True)
                rc = pl.reciprocal(den, approx=True)
                return p * (rc * (2.0 - den * rc))

            def pv(j, p, v80, split=False):
                o80 = split_rows(_dot, p, v80, split)
                odef_ref[pl.ds(r0, 8), (2 * j) * E:(2 * j + 1) * E] = o80[64:72]
                odef_ref[pl.ds(r0, 8), (2 * j + 1) * E:(2 * j + 2) * E] = o80[72:80]
                return jnp.concatenate([o80[0:32], o80[32:64]], axis=1).astype(bf16)

            def wo_part(o, j0, j1, n, acc=None):
                for j in range(j0, j1):
                    acc = sdot(o[j], wo_ref[n, j * 128:(j + 1) * 128, :], acc)
                return acc

            qs, ks, vs, ps, os_ = {}, {}, {}, {}, {}
            for j in range(0, NP, 2):
                for m, jj in cfg["order"]:
                    (qs, ks, vs)[m][j + jj] = proj(m, j + jj)
                ps[j] = qk(qs[j], ks[j], j == 0 and cfg["split0"])
                ps[j + 1] = qk(qs[j + 1], ks[j + 1], j == 0 and cfg["split0"])
                if j >= 2:
                    os_[j - 2] = pv(j - 2, ps[j - 2], vs[j - 2])
                    os_[j - 1] = pv(j - 1, ps[j - 1], vs[j - 1])
            na = NP - 2
            acc = {}
            nw = cfg["nw"]
            for n in range(nw):
                acc[n] = wo_part(os_, 0, na, n)
            os_[NP - 2] = pv(NP - 2, ps[NP - 2], vs[NP - 2], cfg["split1"])
            os_[NP - 1] = pv(NP - 1, ps[NP - 1], vs[NP - 1], cfg["split1"])
            acc[nw] = wo_part(os_, 0, na, nw)
            for n in range(nw + 1):
                acc[n] = wo_part(os_, na, NP, n, acc[n])
            for n in range(nw + 1, 8):
                acc[n] = wo_part(os_, 0, NP, n)
            assert state["count"] == 512 and not state["due"], state
            conv_fwd(cb, r)
            for n in range(NCB):
                b_ref[n, s, 0:NT, :] = acc[n][0:NT]
            return jnp.concatenate([acc[n][NT:SEG] for n in range(NCB)], axis=1).astype(bf16).astype(f32)

        def steps(i, mem):
            @pl.when(i == 1)
            def _():
                wait_all(ssm_ref.at[2 * UNROLL:NCH], SEM_SSM1)
            for t in range(UNROLL):
                mem = step(i * UNROLL + t, mem)
            return mem

        lax.fori_loop(0, _DBG_STEPS // UNROLL, steps, mem_ref[...].astype(f32))

        def out_copy(n):
            slot = n % 2
            return pltpu.make_async_copy(
                ost_ref.at[slot], out_hbm.at[:, :, pl.ds(pl.multiple_of(n * 128, 128), 128)],
                sems.at[SEM_OUT + slot])

        def fin(n, c):
            @pl.when(n >= 2)
            def _():
                out_copy(n - 2).wait()
            icb = NCB - 2 + n // 4
            for i in range(4):
                conv_inv(a_ref, icb, icb % 2, icb, 4 * (n % 4) + i)
            toks = []
            for rr in range(2):
                r = 2 * (n % 4) + rr
                for a in range(NCH):
                    t = conv_mac((NCB - 1) % 2, r, a, 0, None if a % 4 == 0 else t)
                    t = conv_mac((NCB - 1) % 2, r, NCH - 1 - a, 1, t)
                    if a % 4 == 3:
                        toks.append(t)
            bd = None
            for kb in range(8):
                w = after(wo_ref[n, kb * 256:(kb + 1) * 256, :], toks[kb - 1] if kb > 0 else None)
                d = _dot(odef_ref[:, kb * 512:(kb + 1) * 512].astype(bf16), _as_bf16(w))
                bd = d if bd is None else d + bd
            b_ref[n, :, NT:SEG, :] = bd.reshape(NSEG, 8, 128)
            for blk in range(8):
                sg = slice(blk * 8, (blk + 1) * 8)
                b = b_ref[n, sg]
                a = a_ref[n, blk * 256:(blk + 1) * 256, :].reshape(8, SEG, 128)
                g = gate_ref[sg]
                ost_ref[n % 2, sg] = (g * a + (1.0 - g) * b).astype(bf16)
            out_copy(n).start()
            return c
        lax.fori_loop(0, NCB, fin, 0)
        out_copy(NCB - 2).wait()
        out_copy(NCB - 1).wait()

    pl.run_scoped(main, pltpu.VMEM((NSEG * 8, H * E), f32), pltpu.VMEM((NCB, NSEG, SEG, 128), f32),
                  pltpu.VMEM((NCB + 1, S, 128), f32))


@jax.jit
def pallas_gated_mix__ssm_conv_h3__memory_aug_recurrent_mem_tr__prompt_kernel(
    A_q: jax.Array,
    A_k: jax.Array,
    A_v: jax.Array,
    A_shift_k: jax.Array,
    A_ssm_k: jax.Array,
    A_ssm_D: jax.Array,
    B_x: jax.Array,
    B_mem0: jax.Array,
    B_Wq: jax.Array,
    B_Wk: jax.Array,
    B_Wv: jax.Array,
    B_Wo: jax.Array,
    B_seg_len: jax.Array,
    gate_w: jax.Array,
):
    del B_x, B_seg_len
    f_tab, g_tab = _dft_tables()
    out = pl.pallas_call(
        _kernel,
        out_shape=jax.ShapeDtypeStruct((NSEG, SEG, D), bf16),
        in_specs=[pl.BlockSpec(memory_space=pl.ANY)] * 15,
        out_specs=pl.BlockSpec(memory_space=pl.ANY),
        scratch_shapes=[
            pltpu.VMEM((3 * H, D // 2, E), u32),
            pltpu.VMEM((NCB, H * E // 2, 128), u32),
            pltpu.VMEM((NCB, S // 2, 128), u32),
            pltpu.VMEM((NSEG, M, D), bf16),
            pltpu.VMEM((NSEG * 4, D), u32),
            pltpu.VMEM((NSEG, 3 * NP, 8, E), u32),
            pltpu.VMEM((NCB + 1, KPAD + S // 2, 128), u32),
            pltpu.VMEM((NCB + 1, S // 2, 128), u32),
            pltpu.VMEM((NCH, D // 2, 128), u32),
            pltpu.VMEM((NCB + 1, S // 2, 128), u32),
            pltpu.VMEM((2, NCH, 128, 128), u32),
            pltpu.VMEM((2, NCH, 256, 128), f32),
            pltpu.VMEM((2, NCH, 256, 128), f32),
            pltpu.VMEM((256, 128), f32),
            pltpu.VMEM((8, 128), jnp.int32),
            pltpu.VMEM((256, 128), bf16),
            pltpu.VMEM((128, 256), bf16),
            pltpu.VMEM((80, 80), f32),
            pltpu.VMEM((KS, D), bf16),
            pltpu.VMEM((NCB + 1, 8, 128), f32),
            pltpu.VMEM((NCB, 128), bf16),
            pltpu.VMEM((NCB, 128), bf16),
            pltpu.VMEM((M, D), bf16),
            pltpu.VMEM((NSEG, SEG, 128), f32),
            pltpu.VMEM((2, NSEG, SEG, 128), bf16),
            pltpu.SemaphoreType.DMA((NSEM,)),
        ],
        compiler_params=pltpu.CompilerParams(vmem_limit_bytes=120 * 2**20),
    )(A_q.reshape(NSEG, SEG, D), A_q.reshape(S, D), A_k.reshape(S, D), A_v.reshape(S, D), A_shift_k.T,
      A_ssm_k, A_ssm_D.reshape(NCB, 128), B_mem0.reshape(M, D), B_Wq, B_Wk, B_Wv,
      B_Wo.reshape(H * E, D), gate_w.reshape(NCB, 128), jnp.asarray(f_tab, bf16), jnp.asarray(g_tab, bf16))
    return out.reshape(1, S, D)
```

```python
import numpy as np
import jax
import jax.numpy as jnp
from jax import lax
import jax.experimental.pallas as pl
import jax.experimental.pallas.tpu as pltpu

S, D, H, E, M, SEG = 2048, 1024, 32, 128, 8, 32
NSEG = S // SEG
NT = SEG - M
NP = H // 2
NCB = D // 128
C = 128
NCH = S // C
KS = 4
KPAD = 32
NG = 6
UNROLL = 4
CFG = dict(inv=((), (0, 1, 2, 3), (4, 5), (6, 7)), fwd=((), (), (), (0, 1, 2, 3)), dues=[48 * p + o for p in range(8) for o in (32, 36, 40, 44)], maclag=4, relfrom=99,
           split0=True, split1=True, nw=3, order=((0, 0), (1, 0), (0, 1), (1, 1), (2, 0), (2, 1)))
_DBG_STEPS = NSEG
bf16, f32, u32 = jnp.bfloat16, jnp.float32, jnp.uint32


def _dft_tables():
    t = np.arange(C, dtype=np.float64)
    rows = []
    for r in range(8):
        ev = 16 * r + np.arange(0, 16, 2)
        od = ev + 1
        for fn, fs in ((np.cos, ev), (np.sin, ev), (np.cos, od), (np.sin, od)):
            rows.append(fn(np.pi * (2 * fs[:, None] + 1) * t[None, :] / (2 * C)))
    f = np.concatenate(rows, axis=0)
    return f.astype(np.float32), (f.T / C).astype(np.float32)


def _fill_matrix():
    r = lax.broadcasted_iota(jnp.int32, (80, 80), 0)
    c = lax.broadcasted_iota(jnp.int32, (80, 80), 1)

    def head(i):
        return jnp.where(i < 64, i // 32, (i - 64) // 8)

    def idx(i):
        lo = i % 32
        main = jnp.where(lo < NT, lo + M, lo - NT)
        return jnp.where(i < 64, main, (i - 64) % 8 + NT + M)

    same = head(r) == head(c)
    ok = (idx(r) < M) | (idx(r) >= idx(c))
    return jnp.where(same, jnp.where(ok, 0.0, -1e9), -jnp.inf).astype(f32)


def _as_bf16(v):
    return pltpu.bitcast(v, bf16)


def _dot(a, b):
    return jnp.dot(a, b, preferred_element_type=f32)


def _dot_nt(a, b):
    return lax.dot_general(a, b, (((1,), (1,)), ((), ())), preferred_element_type=f32)


(SEM_XB, SEM_X, SEM_SSM0, SEM_SSM1, SEM_WO, SEM_SHIFT, SEM_D, SEM_GW, SEM_MEM, SEM_F, SEM_G) = range(11)
SEM_K = 11
SEM_V = SEM_K + 4
SEM_W = SEM_V + 4
SEM_OUT = SEM_W + 2 * NG
NSEM = SEM_OUT + 2


def _kernel(x3_hbm, x_hbm, k_hbm, v_hbm, shift_hbm, ssm_hbm, d_hbm, mem_hbm, wq_hbm, wk_hbm, wv_hbm,
            wo_hbm, gw_hbm, f_hbm, g_hbm, out_hbm,
            wn_ref, wo_ref, x_ref, xr_ref, xb_ref, pre_ref, k_ref, v_ref, ssm_ref, u_ref, z_ref,
            fu_ref, fk_ref, kraw_ref, one_ref, f_ref, g_ref, fill_ref, shift_ref, wt_ref,
            d_ref, gw_ref, mem_ref, gate_ref, ost_ref, sems):
    w_hbm = (wq_hbm, wk_hbm, wv_hbm)

    def cp(src, dst, sem):
        return pltpu.make_async_copy(src, dst, sems.at[sem])

    def start_col_blocks(src_hbm, dst_ref, i0, i1, sem, row0=0):
        src = src_hbm.bitcast(u32)
        for i in range(i0, i1):
            cp(src.at[:, i * 128:(i + 1) * 128], dst_ref.at[i, row0:], sem).start()

    def wait_all(dst, sem):
        cp(dst, dst, sem).wait()

    def even(p):
        return pltpu.bitcast(p << 16, f32)

    def odd(p):
        return pltpu.bitcast(p & jnp.uint32(0xFFFF0000), f32)

    def conv_prep(cb, i, dep=None):
        r0 = KPAD + 8 * i
        p0 = k_ref[cb, r0:r0 + 8, :]
        if dep is not None:
            p0 = jnp.where(one_ref[...] == 1, p0, dep)
        p1 = k_ref[cb, r0 - 1:r0 + 7, :]
        p2 = k_ref[cb, r0 - 2:r0 + 6, :]
        pv = v_ref[cb, 8 * i:8 * i + 8, :]
        w = wt_ref[cb]
        w0, w1, w2, w3 = w[0:1, :], w[1:2, :], w[2:3, :], w[3:4, :]
        e0, o0, e1, o1, o2 = even(p0), odd(p0), even(p1), odd(p1), odd(p2)
        ke = ((e0 * w0 + o1 * w1) + e1 * w2) + o2 * w3
        ko = ((o0 * w0 + e0 * w1) + o1 * w2) + e1 * w3
        re = pltpu.bitcast((ke * even(pv)).astype(bf16).astype(f32), u32)
        ro = pltpu.bitcast((ko * odd(pv)).astype(bf16).astype(f32), u32)
        kv = (re >> 16) | ro
        u_ref[cb, 8 * i:8 * i + 8, :] = kv
        return kv

    def combine(kf, prev):
        out = []
        for g in range(8):
            o = 32 * g
            out += [kf[o:o + 8] + prev[o + 8:o + 16], kf[o + 8:o + 16] - prev[o:o + 8],
                    kf[o + 16:o + 24] - prev[o + 24:o + 32], kf[o + 24:o + 32] + prev[o + 16:o + 24]]
        return jnp.concatenate(out, axis=0)

    def conv_fwd(cb, r):
        slot = cb % 2
        rows = pl.ds(pl.multiple_of(cb * 64, 64), 64)
        f = f_ref[...]
        kfs = []
        for a in (2 * r, 2 * r + 1):
            fu_ref[slot, a] = _dot(f, _as_bf16(u_ref[cb, pl.ds(pl.multiple_of(a * 64, 64), 64), :]))
            kfs.append(_dot_nt(f, _as_bf16(ssm_ref[a, rows, :])))
        fk_ref[slot, 2 * r] = combine(kfs[0], jnp.where(r > 0, kraw_ref[...], 0.0))
        fk_ref[slot, 2 * r + 1] = combine(kfs[1], kfs[0])
        kraw_ref[...] = kfs[1]

    def conv_mac(slot, r, a, half, dep=None):
        ro = pl.multiple_of(r * 32, 32) + half * 16
        p = q = None
        for c in range(a + 1):
            u = fu_ref[slot, a - c, pl.ds(ro, 16), :]
            k = fk_ref[slot, c, pl.ds(ro, 16), :]
            ua, ub, kc, kd = u[0:8], u[8:16], k[0:8], k[8:16]
            if c == 0 and dep is not None:
                ua = jnp.where(one_ref[...] == 1, ua, pltpu.bitcast(dep, f32))
            p = (ua * kc if p is None else p + ua * kc) - ub * kd
            q = (ua * kd if q is None else q + ua * kd) + ub * kc
        z = pltpu.bitcast(jnp.concatenate([p, q], axis=0).astype(bf16), u32)
        z_ref[slot, a, pl.ds(pl.multiple_of(r * 16, 16) + half * 8, 8), :] = z
        return z

    def conv_inv(a_ref, cb, slot, dst, a):
        rows = pl.ds(pl.multiple_of(a * 64, 64), 64)
        y = _dot(g_ref[...], _as_bf16(z_ref[slot, a]))
        kv = _as_bf16(u_ref[cb, rows, :]).astype(f32)
        q = _as_bf16(x_ref[cb, rows, :]).astype(f32)
        a_ref[dst, pl.ds(pl.multiple_of(a * C, C), C), :] = q * (y + kv * wt_ref[cb, KS:KS + 1, :])

    def after(w, tok):
        if tok is None:
            return w
        return jnp.concatenate([jnp.where(one_ref[...] == 1, w[0:8], tok), w[8:]], axis=0)

    def prologue(stage_ref):
        st3 = stage_ref.reshape(NG * D, 8, E)

        def start_w(g):
            src = w_hbm[g // 2].bitcast(u32)
            for hf in range(2):
                r0 = (g % 2) * 8 + hf * 4
                cp(src.at[:, r0:r0 + 4, :], st3.at[g * D:(g + 1) * D, hf * 4:hf * 4 + 4, :],
                   SEM_W + 2 * g + hf).start()

        def wait_w(g, hf):
            wait_all(st3.at[pl.ds(g * D, D), hf * 4:hf * 4 + 4, :], SEM_W + 2 * g + hf)

        taps = [cp(shift_hbm, shift_ref, SEM_SHIFT), cp(d_hbm, d_ref, SEM_D)]
        small = [cp(gw_hbm, gw_ref, SEM_GW), cp(mem_hbm, mem_ref, SEM_MEM), cp(f_hbm, f_ref, SEM_F),
                 cp(g_hbm, g_ref, SEM_G)]
        cp_xb = cp(x3_hbm.at[:, NT:SEG, :], xr_ref, SEM_XB)
        for c in taps:
            c.start()
        cp_xb.start()
        start_w(0)
        for g in range(1, NG):
            start_w(g)
            if g <= 4:
                start_col_blocks(k_hbm, k_ref, 2 * g - 2, 2 * g, SEM_K + g - 1, row0=KPAD)
                start_col_blocks(v_hbm, v_ref, 2 * g - 2, 2 * g, SEM_V + g - 1)
        for c in small:
            c.start()
        start_col_blocks(wo_hbm, wo_ref, 0, NCB, SEM_WO)
        start_col_blocks(x_hbm, x_ref, 0, NCB, SEM_X)
        start_col_blocks(ssm_hbm, ssm_ref, 0, 2 * UNROLL, SEM_SSM0)
        start_col_blocks(ssm_hbm, ssm_ref, 2 * UNROLL, NCH, SEM_SSM1)
        fill_ref[...] = _fill_matrix()
        one_ref[...] = jnp.ones((8, 128), jnp.int32)
        k_ref[:, KPAD - 8:KPAD, :] = jnp.zeros((NCB + 1, 8, 128), u32)
        for c in taps:
            c.wait()
        sh = shift_ref[...].astype(f32)
        dv = d_ref[...].astype(f32)
        for n in range(NCB):
            wt_ref[n, 0:KS, :] = sh[:, n * 128:(n + 1) * 128]
            wt_ref[n, KS:KS + 1, :] = dv[n:n + 1, :]
        cp_xb.wait()

        def xb_build(it, c):
            s0 = pl.multiple_of(it * 8, 8)
            t = xr_ref[pl.ds(s0, 8)].astype(f32).reshape(64, D).astype(bf16)
            xb_ref[pl.ds(pl.multiple_of(it * 32, 32), 32), :] = pltpu.bitcast(t, u32)
            return c
        lax.fori_loop(0, 8, xb_build, 0)

        def group(g, c):
            sub = stage_ref.at[pl.ds(pl.multiple_of(g * (8 * D), 8 * D), 8 * D), :]

            def relayout(j, chain=False):
                toks, t = [], None
                nd = 16 if chain else 256
                for blk in range(D // nd):
                    w = sub[pl.ds(blk * 8 * nd + j, nd, stride=8), :]
                    if chain and blk % 16 != 0:
                        w = after(w, t)
                    lo = pltpu.bitcast(even(w).astype(bf16), u32)
                    hi = pltpu.bitcast(odd(w).astype(bf16), u32)
                    rows = slice(blk * nd // 2, (blk + 1) * nd // 2)
                    wn_ref[g * 16 + 2 * j, rows, :] = lo
                    wn_ref[g * 16 + 2 * j + 1, rows, :] = hi
                    if chain:
                        t = lo | hi
                        if blk % 16 == 15:
                            toks.append(t)
                return toks

            has_kv = jnp.logical_and(g >= 1, g <= 4)

            def prep_chain(k):
                cb = jnp.where(has_kv, 2 * g - 2 + k // 8, NCB)
                t = None
                for i in range(16):
                    t = conv_prep(cb, (k % 8) * 16 + i, t)
                return t

            wait_w(g, 0)
            relayout(0)
            for j in range(8):
                if j == 3:
                    wait_w(g, 1)

                    @pl.when(has_kv)
                    def _():
                        wait_all(k_ref.at[pl.ds(2 * g - 2, 2), KPAD:], SEM_K + g - 1)
                        wait_all(v_ref.at[pl.ds(2 * g - 2, 2)], SEM_V + g - 1)
                xb = _as_bf16(xb_ref[...])
                w1, w2 = wn_ref[g * 16 + 2 * j], wn_ref[g * 16 + 2 * j + 1]
                toks = relayout(j + 1, j == 2) if j + 1 < 8 else None
                if j >= 4:
                    toks = [prep_chain(4 * (j - 4) + i) for i in range(4)]
                if j == 2 or j >= 4:
                    w1 = jnp.concatenate([after(w1[0:256], toks[0]), after(w1[256:], toks[1])], axis=0)
                    w2 = jnp.concatenate([after(w2[0:256], toks[2]), after(w2[256:], toks[3])], axis=0)
                r1 = _dot(xb, _as_bf16(w1))
                r2 = _dot(xb, _as_bf16(w2))
                cc = jnp.concatenate([r1.reshape(NSEG, 8, E), r2.reshape(NSEG, 8, E)], axis=1).astype(bf16)
                pre_ref[:, g * 8 + j] = pltpu.bitcast(cc, u32)
            return c
        lax.fori_loop(0, NG, group, 0)
        for c in small:
            c.wait()

    pl.run_scoped(prologue, pltpu.VMEM((NG * 8 * D, E), u32))

    wait_all(wo_ref, SEM_WO)
    wait_all(x_ref, SEM_X)
    wait_all(ssm_ref.at[0:2 * UNROLL], SEM_SSM0)

    scale = E ** -0.5

    def main(odef_ref, b_ref, a_ref):
        def step(s, mem, t):
            cfg = CFG
            cb = s // 8
            r = s % 8
            icb = jnp.maximum(cb - 2, 0)
            idst = jnp.where(cb >= 2, cb - 2, NCB)
            mslot = (cb + 1) % 2

            xrows = pl.ds(pl.multiple_of(s * 16, 16), 16)
            xs = [_as_bf16(x_ref[n, xrows, :]).astype(f32) for n in range(NCB)]
            h32 = jnp.concatenate([jnp.concatenate(xs, axis=1)[0:NT], mem], axis=0).astype(bf16)
            r0 = pl.multiple_of(s * 8, 8)

            for a in cfg["inv"][t]:
                conv_inv(a_ref, icb, cb % 2, idst, 2 * (r - t) + a)

            gw = gw_ref[...].astype(f32)
            gl = xs[0] * gw[0:1, :]
            for n in range(1, NCB):
                gl = gl + xs[n] * gw[n:n + 1, :]
            gl = jnp.sum(gl, axis=-1, keepdims=True)
            gate_ref[s] = jnp.broadcast_to(jax.nn.sigmoid(gl), (SEG, 128))

            jobs = []
            units = []
            for a in range(NCH):
                units += [(a, 0), (NCH - 1 - a, 1)]
            for i, (ua, uh) in enumerate(units):
                due = cfg["dues"][i]
                start = max(due - cfg["maclag"], 0)
                jobs.append((start, due - start, t >= cfg["relfrom"],
                             lambda dep, ua=ua, uh=uh: conv_mac(mslot, r, ua, uh, dep)))
            state = dict(count=0, due={})

            def sdot(lhs, w, acc=None, weight=1):
                c = state["count"]
                toks = [t for cc in range(c, c + weight) for t in state["due"].pop(cc, [])]
                nt = w.shape[0] // 64
                if toks:
                    tiles = [w[64 * i:64 * (i + 1)] for i in range(nt)]
                    for i, t in enumerate(toks):
                        tiles[i % nt] = after(tiles[i % nt], t)
                    w = jnp.concatenate(tiles, axis=0)
                d = _dot(lhs, _as_bf16(w))
                d = d if acc is None else d + acc
                for (st, lag, rel, fn) in jobs:
                    if c <= st < c + weight:
                        tok = fn(pltpu.bitcast(d[0:8], u32) if rel else None)
                        state["due"].setdefault(max(st + lag, c + weight), []).append(tok)
                state["count"] = c + weight
                return d

            def proj(m, j):
                r1 = sdot(h32, wn_ref[m * H + 2 * j], weight=4)
                r2 = sdot(h32, wn_ref[m * H + 2 * j + 1], weight=4)
                p = _as_bf16(pre_ref[s, m * NP + j]).astype(f32)
                r = jnp.concatenate([r1, r2, p], axis=0)
                return r if m == 0 else r.astype(bf16)

            def split_rows(dot, lhs, rhs, split):
                if not split:
                    return dot(lhs.astype(bf16), rhs)
                return jnp.concatenate([dot(lhs[0:48].astype(bf16), rhs), dot(lhs[48:80].astype(bf16), rhs)], axis=0)

            def qk(q80, k80, split=False):
                fill = fill_ref[...]
                sc = jnp.where(fill == 0.0, split_rows(_dot_nt, q80, k80, split) * scale, fill)
                p = jnp.exp(sc - jnp.max(sc, axis=-1, keepdims=True))
                den = jnp.sum(p, axis=-1, keepdims=True)
                rc = pl.reciprocal(den, approx=True)
                return p * (rc * (2.0 - den * rc))

            def pv(j, p, v80, split=False):
                o80 = split_rows(_dot, p, v80, split)
                odef_ref[pl.ds(r0, 8), (2 * j) * E:(2 * j + 1) * E] = o80[64:72]
                odef_ref[pl.ds(r0, 8), (2 * j + 1) * E:(2 * j + 2) * E] = o80[72:80]
                return jnp.concatenate([o80[0:32], o80[32:64]], axis=1).astype(bf16)

            def wo_part(o, j0, j1, n, acc=None):
                for j in range(j0, j1):
                    acc = sdot(o[j], wo_ref[n, j * 128:(j + 1) * 128, :], acc)
                return acc

            qs, ks, vs, ps, os_ = {}, {}, {}, {}, {}
            for j in range(0, NP, 2):
                for m, jj in cfg["order"]:
                    (qs, ks, vs)[m][j + jj] = proj(m, j + jj)
                ps[j] = qk(qs[j], ks[j], j == 0 and cfg["split0"])
                ps[j + 1] = qk(qs[j + 1], ks[j + 1], j == 0 and cfg["split0"])
                if j >= 2:
                    os_[j - 2] = pv(j - 2, ps[j - 2], vs[j - 2])
                    os_[j - 1] = pv(j - 1, ps[j - 1], vs[j - 1])
            na = NP - 2
            acc = {}
            nw = cfg["nw"]
            for n in range(nw):
                acc[n] = wo_part(os_, 0, na, n)
            os_[NP - 2] = pv(NP - 2, ps[NP - 2], vs[NP - 2], cfg["split1"])
            os_[NP - 1] = pv(NP - 1, ps[NP - 1], vs[NP - 1], cfg["split1"])
            acc[nw] = wo_part(os_, 0, na, nw)
            for n in range(nw + 1):
                acc[n] = wo_part(os_, na, NP, n, acc[n])
            for n in range(nw + 1, 8):
                acc[n] = wo_part(os_, 0, NP, n)
            assert state["count"] == 512 and not state["due"], state
            for tt in cfg["fwd"][t]:
                conv_fwd(cb, r - t + tt)
            for n in range(NCB):
                b_ref[n, s, 0:NT, :] = acc[n][0:NT]
            return jnp.concatenate([acc[n][NT:SEG] for n in range(NCB)], axis=1).astype(bf16).astype(f32)

        def steps(i, mem):
            @pl.when(i == 1)
            def _():
                wait_all(ssm_ref.at[2 * UNROLL:NCH], SEM_SSM1)
            for t in range(UNROLL):
                mem = step(i * UNROLL + t, mem, t)
            return mem

        lax.fori_loop(0, _DBG_STEPS // UNROLL, steps, mem_ref[...].astype(f32))

        def out_copy(n):
            slot = n % 2
            return pltpu.make_async_copy(
                ost_ref.at[slot], out_hbm.at[:, :, pl.ds(pl.multiple_of(n * 128, 128), 128)],
                sems.at[SEM_OUT + slot])

        def fin(n, c):
            @pl.when(n >= 2)
            def _():
                out_copy(n - 2).wait()
            icb = NCB - 2 + n // 4
            for i in range(4):
                conv_inv(a_ref, icb, icb % 2, icb, 4 * (n % 4) + i)
            toks = []
            for rr in range(2):
                r = 2 * (n % 4) + rr
                for a in range(NCH):
                    t = conv_mac((NCB - 1) % 2, r, a, 0, None if a % 4 == 0 else t)
                    t = conv_mac((NCB - 1) % 2, r, NCH - 1 - a, 1, t)
                    if a % 4 == 3:
                        toks.append(t)
            bd = None
            for kb in range(8):
                w = after(wo_ref[n, kb * 256:(kb + 1) * 256, :], toks[kb - 1] if kb > 0 else None)
                d = _dot(odef_ref[:, kb * 512:(kb + 1) * 512].astype(bf16), _as_bf16(w))
                bd = d if bd is None else d + bd
            b_ref[n, :, NT:SEG, :] = bd.reshape(NSEG, 8, 128)
            for blk in range(8):
                sg = slice(blk * 8, (blk + 1) * 8)
                b = b_ref[n, sg]
                a = a_ref[n, blk * 256:(blk + 1) * 256, :].reshape(8, SEG, 128)
                g = gate_ref[sg]
                ost_ref[n % 2, sg] = (g * a + (1.0 - g) * b).astype(bf16)
            out_copy(n).start()
            return c
        lax.fori_loop(0, NCB, fin, 0)
        out_copy(NCB - 2).wait()
        out_copy(NCB - 1).wait()

    pl.run_scoped(main, pltpu.VMEM((NSEG * 8, H * E), f32), pltpu.VMEM((NCB, NSEG, SEG, 128), f32),
                  pltpu.VMEM((NCB + 1, S, 128), f32))


@jax.jit
def pallas_gated_mix__ssm_conv_h3__memory_aug_recurrent_mem_tr__prompt_kernel(
    A_q: jax.Array,
    A_k: jax.Array,
    A_v: jax.Array,
    A_shift_k: jax.Array,
    A_ssm_k: jax.Array,
    A_ssm_D: jax.Array,
    B_x: jax.Array,
    B_mem0: jax.Array,
    B_Wq: jax.Array,
    B_Wk: jax.Array,
    B_Wv: jax.Array,
    B_Wo: jax.Array,
    B_seg_len: jax.Array,
    gate_w: jax.Array,
):
    del B_x, B_seg_len
    f_tab, g_tab = _dft_tables()
    out = pl.pallas_call(
        _kernel,
        out_shape=jax.ShapeDtypeStruct((NSEG, SEG, D), bf16),
        in_specs=[pl.BlockSpec(memory_space=pl.ANY)] * 15,
        out_specs=pl.BlockSpec(memory_space=pl.ANY),
        scratch_shapes=[
            pltpu.VMEM((3 * H, D // 2, E), u32),
            pltpu.VMEM((NCB, H * E // 2, 128), u32),
            pltpu.VMEM((NCB, S // 2, 128), u32),
            pltpu.VMEM((NSEG, M, D), bf16),
            pltpu.VMEM((NSEG * 4, D), u32),
            pltpu.VMEM((NSEG, 3 * NP, 8, E), u32),
            pltpu.VMEM((NCB + 1, KPAD + S // 2, 128), u32),
            pltpu.VMEM((NCB + 1, S // 2, 128), u32),
            pltpu.VMEM((NCH, D // 2, 128), u32),
            pltpu.VMEM((NCB + 1, S // 2, 128), u32),
            pltpu.VMEM((2, NCH, 128, 128), u32),
            pltpu.VMEM((2, NCH, 256, 128), f32),
            pltpu.VMEM((2, NCH, 256, 128), f32),
            pltpu.VMEM((256, 128), f32),
            pltpu.VMEM((8, 128), jnp.int32),
            pltpu.VMEM((256, 128), bf16),
            pltpu.VMEM((128, 256), bf16),
            pltpu.VMEM((80, 80), f32),
            pltpu.VMEM((KS, D), bf16),
            pltpu.VMEM((NCB + 1, 8, 128), f32),
            pltpu.VMEM((NCB, 128), bf16),
            pltpu.VMEM((NCB, 128), bf16),
            pltpu.VMEM((M, D), bf16),
            pltpu.VMEM((NSEG, SEG, 128), f32),
            pltpu.VMEM((2, NSEG, SEG, 128), bf16),
            pltpu.SemaphoreType.DMA((NSEM,)),
        ],
        compiler_params=pltpu.CompilerParams(vmem_limit_bytes=120 * 2**20),
    )(A_q.reshape(NSEG, SEG, D), A_q.reshape(S, D), A_k.reshape(S, D), A_v.reshape(S, D), A_shift_k.T,
      A_ssm_k, A_ssm_D.reshape(NCB, 128), B_mem0.reshape(M, D), B_Wq, B_Wk, B_Wv,
      B_Wo.reshape(H * E, D), gate_w.reshape(NCB, 128), jnp.asarray(f_tab, bf16), jnp.asarray(g_tab, bf16))
    return out.reshape(1, S, D)
```

```python
import numpy as np
import jax
import jax.numpy as jnp
from jax import lax
import jax.experimental.pallas as pl
import jax.experimental.pallas.tpu as pltpu

S, D, H, E, M, SEG = 2048, 1024, 32, 128, 8, 32
NSEG = S // SEG
NT = SEG - M
NP = H // 2
NCB = D // 128
C = 128
NCH = S // C
LOG2E = 1.4426950408889634
KS = 4
KPAD = 32
NG = 6
UNROLL = 4
CFG = dict(inv=((), (0, 1, 2, 3), (4, 5), (6, 7)), fwd=((), (), (), (0, 1, 2, 3)), dues=[12, 16, 20, 24, 28, 32, 36, 40, 44] + [48 * p + 40 for p in range(1, 8)] + [444 + 4 * i for i in range(16)], maclag=4, relfrom=99, gate=436,
           split0=True, split1=True, nw=3, order=((0, 0), (1, 0), (0, 1), (1, 1), (2, 0), (2, 1)))
_DBG_STEPS = NSEG
bf16, f32, u32 = jnp.bfloat16, jnp.float32, jnp.uint32


def _dft_tables():
    t = np.arange(C, dtype=np.float64)
    rows = []
    for r in range(8):
        ev = 16 * r + np.arange(0, 16, 2)
        od = ev + 1
        for fn, fs in ((np.cos, ev), (np.sin, ev), (np.cos, od), (np.sin, od)):
            rows.append(fn(np.pi * (2 * fs[:, None] + 1) * t[None, :] / (2 * C)))
    f = np.concatenate(rows, axis=0)
    return f.astype(bf16), (f.T / C).astype(bf16)


def _fill_matrix():
    r = lax.broadcasted_iota(jnp.int32, (80, 128), 0)
    c = lax.broadcasted_iota(jnp.int32, (80, 128), 1)

    def head(i):
        return jnp.where(i < 64, i // 32, (i - 64) // 8)

    def idx(i):
        lo = i % 32
        main = jnp.where(lo < NT, lo + M, lo - NT)
        return jnp.where(i < 64, main, (i - 64) % 8 + NT + M)

    same = (head(r) == head(c)) & (c < 80)
    ok = (idx(r) < M) | (idx(r) >= idx(c))
    return jnp.where(same, jnp.where(ok, 0.0, -1e9 * E ** 0.5), -jnp.inf).astype(f32)


def _as_bf16(v):
    return pltpu.bitcast(v, bf16)


def _dot(a, b):
    return jnp.dot(a, b, preferred_element_type=f32)


def _dot_nt(a, b):
    return lax.dot_general(a, b, (((1,), (1,)), ((), ())), preferred_element_type=f32)


(SEM_XB, SEM_X, SEM_SSM0, SEM_SSM1, SEM_WO, SEM_SHIFT, SEM_D, SEM_GW, SEM_MEM, SEM_F, SEM_G) = range(11)
SEM_K = 11
SEM_V = SEM_K + 4
SEM_W = SEM_V + 4
SEM_OUT = SEM_W + NG + 1
NSEM = SEM_OUT + 2


def _kernel(x3_hbm, x_hbm, k_hbm, v_hbm, shift_hbm, ssm_hbm, d_hbm, mem_hbm, wq_hbm, wk_hbm, wv_hbm,
            wo_hbm, gw_hbm, f_hbm, g_hbm, out_hbm,
            wn_ref, wo_ref, x_ref, xr_ref, xb_ref, pre_ref, k_ref, v_ref, ssm_ref, u_ref, z_ref,
            fu_ref, fk_ref, kraw_ref, one_ref, f_ref, g_ref, fill_ref, shift_ref, wt_ref,
            d_ref, gw_ref, mem_ref, gate_ref, ost_ref, sems):
    w_hbm = (wq_hbm, wk_hbm, wv_hbm)

    def cp(src, dst, sem):
        return pltpu.make_async_copy(src, dst, sems.at[sem])

    def start_col_blocks(src_hbm, dst_ref, i0, i1, sem, row0=0):
        src = src_hbm.bitcast(u32)
        for i in range(i0, i1):
            cp(src.at[:, i * 128:(i + 1) * 128], dst_ref.at[i, row0:], sem).start()

    def wait_all(dst, sem):
        cp(dst, dst, sem).wait()

    def even(p):
        return pltpu.bitcast(p << 16, f32)

    def odd(p):
        return pltpu.bitcast(p & jnp.uint32(0xFFFF0000), f32)

    def conv_prep(cb, i, dep=None):
        r0 = KPAD + 8 * i
        p0 = k_ref[cb, r0:r0 + 8, :]
        if dep is not None:
            p0 = jnp.where(one_ref[...] == 1, p0, dep)
        p1 = k_ref[cb, r0 - 1:r0 + 7, :]
        p2 = k_ref[cb, r0 - 2:r0 + 6, :]
        pv = v_ref[cb, 8 * i:8 * i + 8, :]
        w = wt_ref[cb]
        w0, w1, w2, w3 = w[0:1, :], w[1:2, :], w[2:3, :], w[3:4, :]
        e0, o0, e1, o1, o2 = even(p0), odd(p0), even(p1), odd(p1), odd(p2)
        ke = ((e0 * w0 + o1 * w1) + e1 * w2) + o2 * w3
        ko = ((o0 * w0 + e0 * w1) + o1 * w2) + e1 * w3
        re = pltpu.bitcast((ke * even(pv)).astype(bf16).astype(f32), u32)
        ro = pltpu.bitcast((ko * odd(pv)).astype(bf16).astype(f32), u32)
        kv = (re >> 16) | ro
        u_ref[cb, 8 * i:8 * i + 8, :] = kv
        return kv

    def combine(kf, prev):
        out = []
        for g in range(8):
            o = 32 * g
            out += [kf[o:o + 8] + prev[o + 8:o + 16], kf[o + 8:o + 16] - prev[o:o + 8],
                    kf[o + 16:o + 24] - prev[o + 24:o + 32], kf[o + 24:o + 32] + prev[o + 16:o + 24]]
        return jnp.concatenate(out, axis=0)

    def conv_fwd(cb, r):
        slot = cb % 2
        rows = pl.ds(pl.multiple_of(cb * 64, 64), 64)
        f = f_ref[...]
        kfs = []
        for a in (2 * r, 2 * r + 1):
            fu_ref[slot, a] = _dot(f, _as_bf16(u_ref[cb, pl.ds(pl.multiple_of(a * 64, 64), 64), :]))
            kfs.append(_dot_nt(f, _as_bf16(ssm_ref[a, rows, :])))
        fk_ref[slot, 2 * r] = combine(kfs[0], jnp.where(r > 0, kraw_ref[...], 0.0))
        fk_ref[slot, 2 * r + 1] = combine(kfs[1], kfs[0])
        kraw_ref[...] = kfs[1]

    def conv_mac(slot, r, a, half, dep=None):
        ro = pl.multiple_of(r * 32, 32) + half * 16
        p = q = None
        for c in range(a + 1):
            u = fu_ref[slot, a - c, pl.ds(ro, 16), :]
            k = fk_ref[slot, c, pl.ds(ro, 16), :]
            ua, ub, kc, kd = u[0:8], u[8:16], k[0:8], k[8:16]
            if c == 0 and dep is not None:
                ua = jnp.where(one_ref[...] == 1, ua, pltpu.bitcast(dep, f32))
            p = (ua * kc if p is None else p + ua * kc) - ub * kd
            q = (ua * kd if q is None else q + ua * kd) + ub * kc
        z = pltpu.bitcast(jnp.concatenate([p, q], axis=0).astype(bf16), u32)
        z_ref[slot, a, pl.ds(pl.multiple_of(r * 16, 16) + half * 8, 8), :] = z
        return z

    def conv_inv(a_ref, cb, slot, dst, a):
        rows = pl.ds(pl.multiple_of(a * 64, 64), 64)
        y = _dot(g_ref[...], _as_bf16(z_ref[slot, a]))
        kv = _as_bf16(u_ref[cb, rows, :]).astype(f32)
        q = _as_bf16(x_ref[cb, rows, :]).astype(f32)
        a_ref[dst, pl.ds(pl.multiple_of(a * C, C), C), :] = q * (y + kv * wt_ref[cb, KS:KS + 1, :])

    def after(w, tok):
        if tok is None:
            return w
        return jnp.concatenate([jnp.where(one_ref[...] == 1, w[0:8], tok), w[8:]], axis=0)

    def prologue(stage_ref):
        st3 = stage_ref.reshape((NG + 1) * D, 8, E)
        w0 = wq_hbm.bitcast(u32)
        cp_w0a = cp(w0.at[:, 0:4, :], st3.at[0:D, 0:4, :], SEM_W)
        cp_w0b = cp(w0.at[:, 4:8, :], st3.at[NG * D:(NG + 1) * D, 4:8, :], SEM_W + NG)

        def start_w(g):
            r0 = (g % 2) * 8
            cp(w_hbm[g // 2].bitcast(u32).at[:, r0:r0 + 8, :], st3.at[g * D:(g + 1) * D], SEM_W + g).start()

        taps = [cp(shift_hbm, shift_ref, SEM_SHIFT), cp(d_hbm, d_ref, SEM_D)]
        small = [cp(gw_hbm, gw_ref, SEM_GW), cp(mem_hbm, mem_ref, SEM_MEM), cp(f_hbm, f_ref, SEM_F),
                 cp(g_hbm, g_ref, SEM_G)]
        cp_xb = cp(x3_hbm.at[:, NT:SEG, :], xr_ref, SEM_XB)
        for c in taps:
            c.start()
        cp_xb.start()
        cp_w0a.start()
        cp_w0b.start()
        for g in range(1, NG):
            start_w(g)
            if g <= 4:
                start_col_blocks(k_hbm, k_ref, 2 * g - 2, 2 * g, SEM_K + g - 1, row0=KPAD)
                start_col_blocks(v_hbm, v_ref, 2 * g - 2, 2 * g, SEM_V + g - 1)
        for c in small:
            c.start()
        start_col_blocks(wo_hbm, wo_ref, 0, NCB, SEM_WO)
        start_col_blocks(x_hbm, x_ref, 0, NCB, SEM_X)
        start_col_blocks(ssm_hbm, ssm_ref, 0, 2 * UNROLL, SEM_SSM0)
        start_col_blocks(ssm_hbm, ssm_ref, 2 * UNROLL, NCH, SEM_SSM1)
        fill_ref[...] = _fill_matrix()
        one_ref[...] = jnp.ones((8, 128), jnp.int32)
        k_ref[:, KPAD - 8:KPAD, :] = jnp.zeros((NCB + 1, 8, 128), u32)
        wt_ref[...] = jnp.zeros(wt_ref.shape, f32)
        kraw_ref[...] = jnp.zeros(kraw_ref.shape, f32)

        def clear(a, c):
            rows = pl.ds(pl.multiple_of(a * 64, 64), 64)
            k_ref[NCB, pl.ds(pl.multiple_of(KPAD + a * 64, 32), 64), :] = jnp.zeros((64, 128), u32)
            v_ref[NCB, rows, :] = jnp.zeros((64, 128), u32)
            fu_ref[1, a] = jnp.zeros((256, 128), f32)
            fk_ref[1, a] = jnp.zeros((256, 128), f32)
            z_ref[0, a] = jnp.zeros((128, 128), u32)
            return c
        lax.fori_loop(0, NCH, clear, 0)
        for c in taps:
            c.wait()
        sh = shift_ref[...].astype(f32)
        dv = d_ref[...].astype(f32)
        for n in range(NCB):
            wt_ref[n, 0:KS, :] = sh[:, n * 128:(n + 1) * 128]
            wt_ref[n, KS:KS + 1, :] = dv[n:n + 1, :]
        cp_xb.wait()

        def xb_build(it, c):
            s0 = pl.multiple_of(it * 8, 8)
            t = xr_ref[pl.ds(s0, 8)].astype(f32).reshape(64, D).astype(bf16)
            xb_ref[pl.ds(pl.multiple_of(it * 32, 32), 32), :] = pltpu.bitcast(t, u32)
            return c
        lax.fori_loop(0, 8, xb_build, 0)

        def group(g, c):
            def region(i):
                return stage_ref.at[pl.ds(pl.multiple_of(i * (8 * D), 8 * D), 8 * D), :]
            subs = (region(g), region(jnp.where(g == 0, NG, g)))

            def relayout(j, chain=False):
                toks, t = [], None
                nd = 16 if chain else 256
                for blk in range(D // nd):
                    w = subs[j // 4][pl.ds(blk * 8 * nd + j, nd, stride=8), :]
                    if chain and blk % 16 != 0:
                        w = after(w, t)
                    lo = pltpu.bitcast(even(w).astype(bf16), u32)
                    hi = pltpu.bitcast(odd(w).astype(bf16), u32)
                    rows = slice(blk * nd // 2, (blk + 1) * nd // 2)
                    wn_ref[g * 16 + 2 * j, rows, :] = lo
                    wn_ref[g * 16 + 2 * j + 1, rows, :] = hi
                    if chain:
                        t = lo | hi
                        if blk % 16 == 15:
                            toks.append(t)
                return toks

            has_kv = jnp.logical_and(g >= 1, g <= 4)

            def prep_chain(k):
                cb = jnp.where(has_kv, 2 * g - 2 + k // 8, NCB)
                t = None
                for i in range(16):
                    t = conv_prep(cb, (k % 8) * 16 + i, t)
                return t

            @pl.when(g > 0)
            def _():
                wait_all(st3.at[pl.ds(g * D, D)], SEM_W + g)
            relayout(0)
            for j in range(8):
                if j == 3:
                    @pl.when(g == 0)
                    def _():
                        cp_w0b.wait()

                    @pl.when(has_kv)
                    def _():
                        wait_all(k_ref.at[pl.ds(2 * g - 2, 2), KPAD:], SEM_K + g - 1)
                        wait_all(v_ref.at[pl.ds(2 * g - 2, 2)], SEM_V + g - 1)
                xb = _as_bf16(xb_ref[...])
                w1, w2 = wn_ref[g * 16 + 2 * j], wn_ref[g * 16 + 2 * j + 1]
                toks = relayout(j + 1, j == 2) if j + 1 < 8 else None
                if j >= 4:
                    toks = [prep_chain(4 * (j - 4) + i) for i in range(4)]
                if j == 2 or j >= 4:
                    w1 = jnp.concatenate([after(w1[0:256], toks[0]), after(w1[256:], toks[1])], axis=0)
                    w2 = jnp.concatenate([after(w2[0:256], toks[2]), after(w2[256:], toks[3])], axis=0)
                r1 = _dot(xb, _as_bf16(w1))
                r2 = _dot(xb, _as_bf16(w2))
                cc = jnp.concatenate([r1.reshape(NSEG, 8, E), r2.reshape(NSEG, 8, E)], axis=1).astype(bf16)
                pre_ref[:, g * 8 + j] = pltpu.bitcast(cc, u32)
            return c
        cp_w0a.wait()
        lax.fori_loop(0, NG, group, 0)
        for c in small:
            c.wait()

    pl.run_scoped(prologue, pltpu.VMEM(((NG + 1) * 8 * D, E), u32))

    wait_all(wo_ref, SEM_WO)
    wait_all(x_ref, SEM_X)
    wait_all(ssm_ref.at[0:2 * UNROLL], SEM_SSM0)

    scale = E ** -0.5

    def main(odef_ref, b_ref, a_ref):
        def step(s, mem, t):
            cfg = CFG
            cb = s // 8
            r = s % 8
            icb = jnp.maximum(cb - 2, 0)
            idst = jnp.where(cb >= 2, cb - 2, NCB)
            mslot = (cb + 1) % 2

            xrows = pl.ds(pl.multiple_of(s * 16, 16), 16)
            xs = [_as_bf16(x_ref[n, xrows, :]).astype(f32) for n in range(NCB)]
            h32 = jnp.concatenate([jnp.concatenate(xs, axis=1)[0:NT], mem], axis=0).astype(bf16)
            r0 = pl.multiple_of(s * 8, 8)

            for a in cfg["inv"][t]:
                conv_inv(a_ref, icb, cb % 2, idst, 2 * (r - t) + a)

            def gate(dep):
                gw = gw_ref[...].astype(f32)
                gl = None
                for n in range(NCB):
                    xg = _as_bf16(x_ref[n, xrows, :]).astype(f32) * gw[n:n + 1, :]
                    gl = xg if gl is None else gl + xg
                g = jnp.broadcast_to(jax.nn.sigmoid(jnp.sum(gl, axis=-1, keepdims=True)), (SEG, 128))
                gate_ref[s] = g
                g = pltpu.bitcast(g, u32)
                return (g[0:8] | g[8:16]) | (g[16:24] | g[24:32])

            jobs = []
            units = []
            for a in range(NCH):
                units += [(a, 0), (NCH - 1 - a, 1)]
            for i, (ua, uh) in enumerate(units):
                due = cfg["dues"][i]
                start = max(due - cfg["maclag"], 0)
                jobs.append((start, due - start, t >= cfg["relfrom"],
                             lambda dep, ua=ua, uh=uh: conv_mac(mslot, r, ua, uh, dep)))
            jobs.append((cfg["gate"], 4, False, gate))
            state = dict(count=0, due={})

            def sdot(lhs, w, acc=None, weight=1):
                c = state["count"]
                toks = [t for cc in range(c, c + weight) for t in state["due"].pop(cc, [])]
                nt = w.shape[0] // 64
                if toks:
                    tiles = [w[64 * i:64 * (i + 1)] for i in range(nt)]
                    for i, t in enumerate(toks):
                        tiles[i % nt] = after(tiles[i % nt], t)
                    w = jnp.concatenate(tiles, axis=0)
                d = _dot(lhs, _as_bf16(w))
                d = d if acc is None else d + acc
                for (st, lag, rel, fn) in jobs:
                    if c <= st < c + weight:
                        tok = fn(pltpu.bitcast(d[0:8], u32) if rel else None)
                        state["due"].setdefault(max(st + lag, c + weight), []).append(tok)
                state["count"] = c + weight
                return d

            def proj(m, j):
                r1 = sdot(h32, wn_ref[m * H + 2 * j], weight=4)
                r2 = sdot(h32, wn_ref[m * H + 2 * j + 1], weight=4)
                p = _as_bf16(pre_ref[s, m * NP + j]).astype(f32)
                if m == 0:
                    return jnp.concatenate([r1, r2, p], axis=0)
                return jnp.concatenate([r1, r2, p, jnp.zeros((48, E), f32)], axis=0).astype(bf16)

            def split_rows(dot, lhs, rhs, split):
                if not split:
                    return dot(lhs.astype(bf16), rhs)
                return jnp.concatenate([dot(lhs[0:48].astype(bf16), rhs), dot(lhs[48:80].astype(bf16), rhs)], axis=0)

            def qk(q80, k80, split=False):
                fill = fill_ref[...]
                sc = jnp.where(fill == 0.0, split_rows(_dot_nt, q80, k80, split), fill)
                p = jnp.exp2((sc - jnp.max(sc, axis=-1, keepdims=True)) * (scale * LOG2E))
                den = jnp.sum(p, axis=-1, keepdims=True)
                rc = pl.reciprocal(den, approx=True)
                return p * (rc * (2.0 - den * rc))

            def pv(j, p, v80, split=False):
                o80 = split_rows(_dot, p, v80, split)
                odef_ref[pl.ds(r0, 8), (2 * j) * E:(2 * j + 1) * E] = o80[64:72]
                odef_ref[pl.ds(r0, 8), (2 * j + 1) * E:(2 * j + 2) * E] = o80[72:80]
                return jnp.concatenate([o80[0:32], o80[32:64]], axis=1).astype(bf16)

            def wo_part(o, j0, j1, n, acc=None):
                for j in range(j0, j1):
                    acc = sdot(o[j], wo_ref[n, j * 128:(j + 1) * 128, :], acc)
                return acc

            qs, ks, vs, ps, os_ = {}, {}, {}, {}, {}
            for j in range(0, NP, 2):
                for m, jj in cfg["order"]:
                    (qs, ks, vs)[m][j + jj] = proj(m, j + jj)
                ps[j] = qk(qs[j], ks[j], j == 0 and cfg["split0"])
                ps[j + 1] = qk(qs[j + 1], ks[j + 1], j == 0 and cfg["split0"])
                if j >= 2:
                    os_[j - 2] = pv(j - 2, ps[j - 2], vs[j - 2])
                    os_[j - 1] = pv(j - 1, ps[j - 1], vs[j - 1])
            na = NP - 2
            acc = {}
            nw = cfg["nw"]
            for n in range(nw):
                acc[n] = wo_part(os_, 0, na, n)
            os_[NP - 2] = pv(NP - 2, ps[NP - 2], vs[NP - 2], cfg["split1"])
            os_[NP - 1] = pv(NP - 1, ps[NP - 1], vs[NP - 1], cfg["split1"])
            acc[nw] = wo_part(os_, 0, na, nw)
            for n in range(nw + 1):
                acc[n] = wo_part(os_, na, NP, n, acc[n])
            for n in range(nw + 1, 8):
                acc[n] = wo_part(os_, 0, NP, n)
            assert state["count"] == 512 and not state["due"], state
            for tt in cfg["fwd"][t]:
                conv_fwd(cb, r - t + tt)
            for n in range(NCB):
                b_ref[n, s, 0:NT, :] = acc[n][0:NT]
            return jnp.concatenate([acc[n][NT:SEG] for n in range(NCB)], axis=1).astype(bf16).astype(f32)

        def steps(i, mem):
            @pl.when(i == 1)
            def _():
                wait_all(ssm_ref.at[2 * UNROLL:NCH], SEM_SSM1)
            for t in range(UNROLL):
                mem = step(i * UNROLL + t, mem, t)
            return mem

        lax.fori_loop(0, _DBG_STEPS // UNROLL, steps, mem_ref[...].astype(f32))

        def out_copy(n):
            slot = n % 2
            return pltpu.make_async_copy(
                ost_ref.at[slot], out_hbm.at[:, :, pl.ds(pl.multiple_of(n * 128, 128), 128)],
                sems.at[SEM_OUT + slot])

        def fin(n, c):
            @pl.when(n >= 2)
            def _():
                out_copy(n - 2).wait()
            icb = NCB - 2 + n // 4
            for i in range(4):
                conv_inv(a_ref, icb, icb % 2, icb, 4 * (n % 4) + i)
            toks = []
            for rr in range(2):
                r = 2 * (n % 4) + rr
                for a in range(NCH):
                    t = conv_mac((NCB - 1) % 2, r, a, 0, None if a % 4 == 0 else t)
                    t = conv_mac((NCB - 1) % 2, r, NCH - 1 - a, 1, t)
                    if a % 4 == 3:
                        toks.append(t)
            bd = None
            for kb in range(8):
                w = after(wo_ref[n, kb * 256:(kb + 1) * 256, :], toks[kb - 1] if kb > 0 else None)
                d = _dot(odef_ref[:, kb * 512:(kb + 1) * 512].astype(bf16), _as_bf16(w))
                bd = d if bd is None else d + bd
            b_ref[n, :, NT:SEG, :] = bd.reshape(NSEG, 8, 128)
            for blk in range(8):
                sg = slice(blk * 8, (blk + 1) * 8)
                b = b_ref[n, sg]
                a = a_ref[n, blk * 256:(blk + 1) * 256, :].reshape(8, SEG, 128)
                g = gate_ref[sg]
                ost_ref[n % 2, sg] = (g * a + (1.0 - g) * b).astype(bf16)
            out_copy(n).start()
            return c
        lax.fori_loop(0, NCB, fin, 0)
        out_copy(NCB - 2).wait()
        out_copy(NCB - 1).wait()

    pl.run_scoped(main, pltpu.VMEM((NSEG * 8, H * E), f32), pltpu.VMEM((NCB, NSEG, SEG, 128), f32),
                  pltpu.VMEM((NCB + 1, S, 128), f32))


@jax.jit
def pallas_gated_mix__ssm_conv_h3__memory_aug_recurrent_mem_tr__prompt_kernel(
    A_q: jax.Array,
    A_k: jax.Array,
    A_v: jax.Array,
    A_shift_k: jax.Array,
    A_ssm_k: jax.Array,
    A_ssm_D: jax.Array,
    B_x: jax.Array,
    B_mem0: jax.Array,
    B_Wq: jax.Array,
    B_Wk: jax.Array,
    B_Wv: jax.Array,
    B_Wo: jax.Array,
    B_seg_len: jax.Array,
    gate_w: jax.Array,
):
    del B_x, B_seg_len
    f_tab, g_tab = _dft_tables()
    out = pl.pallas_call(
        _kernel,
        out_shape=jax.ShapeDtypeStruct((NSEG, SEG, D), bf16),
        in_specs=[pl.BlockSpec(memory_space=pl.ANY)] * 15,
        out_specs=pl.BlockSpec(memory_space=pl.ANY),
        scratch_shapes=[
            pltpu.VMEM((3 * H, D // 2, E), u32),
            pltpu.VMEM((NCB, H * E // 2, 128), u32),
            pltpu.VMEM((NCB, S // 2, 128), u32),
            pltpu.VMEM((NSEG, M, D), bf16),
            pltpu.VMEM((NSEG * 4, D), u32),
            pltpu.VMEM((NSEG, 3 * NP, 8, E), u32),
            pltpu.VMEM((NCB + 1, KPAD + S // 2, 128), u32),
            pltpu.VMEM((NCB + 1, S // 2, 128), u32),
            pltpu.VMEM((NCH, D // 2, 128), u32),
            pltpu.VMEM((NCB + 1, S // 2, 128), u32),
            pltpu.VMEM((2, NCH, 128, 128), u32),
            pltpu.VMEM((2, NCH, 256, 128), f32),
            pltpu.VMEM((2, NCH, 256, 128), f32),
            pltpu.VMEM((256, 128), f32),
            pltpu.VMEM((8, 128), jnp.int32),
            pltpu.VMEM((256, 128), bf16),
            pltpu.VMEM((128, 256), bf16),
            pltpu.VMEM((80, 128), f32),
            pltpu.VMEM((KS, D), bf16),
            pltpu.VMEM((NCB + 1, 8, 128), f32),
            pltpu.VMEM((NCB, 128), bf16),
            pltpu.VMEM((NCB, 128), bf16),
            pltpu.VMEM((M, D), bf16),
            pltpu.VMEM((NSEG, SEG, 128), f32),
            pltpu.VMEM((2, NSEG, SEG, 128), bf16),
            pltpu.SemaphoreType.DMA((NSEM,)),
        ],
        compiler_params=pltpu.CompilerParams(vmem_limit_bytes=120 * 2**20),
    )(A_q.reshape(NSEG, SEG, D), A_q.reshape(S, D), A_k.reshape(S, D), A_v.reshape(S, D), A_shift_k.T,
      A_ssm_k, A_ssm_D.reshape(NCB, 128), B_mem0.reshape(M, D), B_Wq, B_Wk, B_Wv,
      B_Wo.reshape(H * E, D), gate_w.reshape(NCB, 128), f_tab, g_tab)
    return out.reshape(1, S, D)
```

```python
import functools

import numpy as np
import jax
import jax.numpy as jnp
from jax import lax
import jax.experimental.pallas as pl
import jax.experimental.pallas.tpu as pltpu

S, D, H, E, M, SEG = 2048, 1024, 32, 128, 8, 32
NSEG = S // SEG
NT = SEG - M
NP = H // 2
NCB = D // 128
C = 128
NCH = S // C
LOG2E = 1.4426950408889634
KS = 4
NZ = 8
KPAD = 32
NG = 6
UNROLL = 4
CFG = dict(dues=[12, 16, 20, 24, 28, 32, 36, 40, 44] + [48 * p + 40 for p in range(1, 8)] + [444 + 4 * i for i in range(16)], maclag=4, gate=436,
           split0=True, split1=True, nw=3, order=((0, 0), (1, 0), (0, 1), (1, 1), (2, 0), (2, 1)))
_DBG_STEPS = NSEG
bf16, f32, u32 = jnp.bfloat16, jnp.float32, jnp.uint32


def _dft_tables():
    t = np.arange(C, dtype=np.float64)
    rows = []
    for r in range(8):
        ev = 16 * r + np.arange(0, 16, 2)
        od = ev + 1
        for fn, fs in ((np.cos, ev), (np.sin, ev), (np.cos, od), (np.sin, od)):
            rows.append(fn(np.pi * (2 * fs[:, None] + 1) * t[None, :] / (2 * C)))
    f = np.concatenate(rows, axis=0)
    return f.astype(bf16), (f.T / C).astype(bf16)


def _fill_matrix():
    r = lax.broadcasted_iota(jnp.int32, (80, 128), 0)
    c = lax.broadcasted_iota(jnp.int32, (80, 128), 1)

    def head(i):
        return jnp.where(i < 64, i // 32, (i - 64) // 8)

    def idx(i):
        lo = i % 32
        main = jnp.where(lo < NT, lo + M, lo - NT)
        return jnp.where(i < 64, main, (i - 64) % 8 + NT + M)

    same = (head(r) == head(c)) & (c < 80)
    ok = (idx(r) < M) | (idx(r) >= idx(c))
    return jnp.where(same, jnp.where(ok, 0.0, -1e9 * E ** 0.5), -jnp.inf).astype(f32)


def _as_bf16(v):
    return pltpu.bitcast(v, bf16)


def _dot(a, b):
    return jnp.dot(a, b, preferred_element_type=f32)


def _dot_nt(a, b):
    return lax.dot_general(a, b, (((1,), (1,)), ((), ())), preferred_element_type=f32)


(SEM_XB, SEM_X, SEM_SSM0, SEM_SSM1, SEM_WO, SEM_SHIFT, SEM_D, SEM_GW, SEM_MEM, SEM_F, SEM_G) = range(11)
SEM_K = 11
SEM_V = SEM_K + 4
SEM_W = SEM_V + 4
SEM_OUT = SEM_W + NG + 1
NSEM = SEM_OUT + 2


def _kernel(x3_hbm, x_hbm, k_hbm, v_hbm, shift_hbm, ssm_hbm, d_hbm, mem_hbm, wq_hbm, wk_hbm, wv_hbm,
            wo_hbm, gw_hbm, f_hbm, g_hbm, out_hbm,
            wn_ref, wo_ref, x_ref, xr_ref, xb_ref, pre_ref, k_ref, v_ref, ssm_ref, u_ref,
            fu_ref, fk_ref, kraw_ref, one_ref, f_ref, g_ref, fill_ref, shift_ref, wt_ref,
            d_ref, gw_ref, mem_ref, gate_ref, ost_ref, sems):
    w_hbm = (wq_hbm, wk_hbm, wv_hbm)

    def cp(src, dst, sem):
        return pltpu.make_async_copy(src, dst, sems.at[sem])

    def start_col_blocks(src_hbm, dst_ref, i0, i1, sem, row0=0):
        src = src_hbm.bitcast(u32)
        for i in range(i0, i1):
            cp(src.at[:, i * 128:(i + 1) * 128], dst_ref.at[i, row0:], sem).start()

    def wait_all(dst, sem):
        cp(dst, dst, sem).wait()

    def even(p):
        return pltpu.bitcast(p << 16, f32)

    def odd(p):
        return pltpu.bitcast(p & jnp.uint32(0xFFFF0000), f32)

    def conv_prep(cb, i, dep=None):
        r0 = KPAD + 8 * i
        p0 = k_ref[cb, r0:r0 + 8, :]
        if dep is not None:
            p0 = jnp.where(one_ref[...] == 1, p0, dep)
        p1 = k_ref[cb, r0 - 1:r0 + 7, :]
        p2 = k_ref[cb, r0 - 2:r0 + 6, :]
        pv = v_ref[cb, 8 * i:8 * i + 8, :]
        w = wt_ref[cb]
        w0, w1, w2, w3 = w[0:1, :], w[1:2, :], w[2:3, :], w[3:4, :]
        e0, o0, e1, o1, o2 = even(p0), odd(p0), even(p1), odd(p1), odd(p2)
        ke = ((e0 * w0 + o1 * w1) + e1 * w2) + o2 * w3
        ko = ((o0 * w0 + e0 * w1) + o1 * w2) + e1 * w3
        re = pltpu.bitcast((ke * even(pv)).astype(bf16).astype(f32), u32)
        ro = pltpu.bitcast((ko * odd(pv)).astype(bf16).astype(f32), u32)
        kv = (re >> 16) | ro
        u_ref[cb, 8 * i:8 * i + 8, :] = kv
        return kv

    def combine(kf, prev):
        out = []
        for g in range(8):
            o = 32 * g
            out += [kf[o:o + 8] + prev[o + 8:o + 16], kf[o + 8:o + 16] - prev[o:o + 8],
                    kf[o + 16:o + 24] - prev[o + 24:o + 32], kf[o + 24:o + 32] + prev[o + 16:o + 24]]
        return jnp.concatenate(out, axis=0)

    def conv_fwd(cb, r):
        slot = cb % 2
        rows = pl.ds(pl.multiple_of(cb * 64, 64), 64)
        f = f_ref[...]
        kfs = []
        for a in (2 * r, 2 * r + 1):
            fu_ref[slot, NZ + a] = _dot(f, _as_bf16(u_ref[cb, pl.ds(pl.multiple_of(a * 64, 64), 64), :]))
            kfs.append(_dot_nt(f, _as_bf16(ssm_ref[a, rows, :])))
        fk_ref[slot, 2 * r] = combine(kfs[0], jnp.where(r > 0, kraw_ref[...], 0.0))
        fk_ref[slot, 2 * r + 1] = combine(kfs[1], kfs[0])
        kraw_ref[...] = kfs[1]

    def conv_mac(slot, a, nterms, pos, dep=None):
        rows = slice(pos * 16, pos * 16 + 16)
        p = q = None
        for c in range(nterms):
            u = fu_ref[slot, NZ + a - c, rows, :]
            k = fk_ref[slot, c, rows, :]
            ua, ub, kc, kd = u[0:8], u[8:16], k[0:8], k[8:16]
            if c == 0 and dep is not None:
                ua = jnp.where(one_ref[...] == 1, ua, pltpu.bitcast(dep, f32))
            p = (ua * kc if p is None else p + ua * kc) - ub * kd
            q = (ua * kd if q is None else q + ua * kd) + ub * kc
        return pltpu.bitcast(jnp.concatenate([p, q], axis=0).astype(bf16), u32)

    def conv_inv(a_ref, cb, dst, a, zs):
        rows = pl.ds(pl.multiple_of(a * 64, 64), 64)
        y = _dot(g_ref[...], _as_bf16(jnp.concatenate(zs, axis=0)))
        kv = _as_bf16(u_ref[cb, rows, :]).astype(f32)
        q = _as_bf16(x_ref[cb, rows, :]).astype(f32)
        a_ref[dst, pl.ds(pl.multiple_of(a * C, C), C), :] = q * (y + kv * wt_ref[cb, KS:KS + 1, :])

    def after(w, tok):
        if tok is None:
            return w
        return jnp.concatenate([jnp.where(one_ref[...] == 1, w[0:8], tok), w[8:]], axis=0)

    def prologue(stage_ref):
        st3 = stage_ref.reshape((NG + 1) * D, 8, E)
        w0 = wq_hbm.bitcast(u32)
        cp_w0a = cp(w0.at[:, 0:4, :], st3.at[0:D, 0:4, :], SEM_W)
        cp_w0b = cp(w0.at[:, 4:8, :], st3.at[NG * D:(NG + 1) * D, 4:8, :], SEM_W + NG)

        def start_w(g):
            r0 = (g % 2) * 8
            cp(w_hbm[g // 2].bitcast(u32).at[:, r0:r0 + 8, :], st3.at[g * D:(g + 1) * D], SEM_W + g).start()

        taps = [cp(shift_hbm, shift_ref, SEM_SHIFT), cp(d_hbm, d_ref, SEM_D)]
        small = [cp(gw_hbm, gw_ref, SEM_GW), cp(mem_hbm, mem_ref, SEM_MEM), cp(f_hbm, f_ref, SEM_F),
                 cp(g_hbm, g_ref, SEM_G)]
        cp_xb = cp(x3_hbm.at[:, NT:SEG, :], xr_ref, SEM_XB)
        for c in taps:
            c.start()
        cp_xb.start()
        cp_w0a.start()
        cp_w0b.start()
        for g in range(1, NG):
            start_w(g)
            if g <= 4:
                start_col_blocks(k_hbm, k_ref, 2 * g - 2, 2 * g, SEM_K + g - 1, row0=KPAD)
                start_col_blocks(v_hbm, v_ref, 2 * g - 2, 2 * g, SEM_V + g - 1)
        for c in small:
            c.start()
        start_col_blocks(wo_hbm, wo_ref, 0, NCB, SEM_WO)
        start_col_blocks(x_hbm, x_ref, 0, NCB, SEM_X)
        start_col_blocks(ssm_hbm, ssm_ref, 0, 2 * UNROLL, SEM_SSM0)
        start_col_blocks(ssm_hbm, ssm_ref, 2 * UNROLL, NCH, SEM_SSM1)
        fill_ref[...] = _fill_matrix()
        one_ref[...] = jnp.ones((8, 128), jnp.int32)
        k_ref[:, KPAD - 8:KPAD, :] = jnp.zeros((NCB + 1, 8, 128), u32)
        wt_ref[...] = jnp.zeros(wt_ref.shape, f32)
        kraw_ref[...] = jnp.zeros(kraw_ref.shape, f32)

        def clear(a, c):
            rows = pl.ds(pl.multiple_of(a * 64, 64), 64)
            k_ref[NCB, pl.ds(pl.multiple_of(KPAD + a * 64, 32), 64), :] = jnp.zeros((64, 128), u32)
            v_ref[NCB, rows, :] = jnp.zeros((64, 128), u32)
            fu_ref[1, NZ + a] = jnp.zeros((256, 128), f32)
            fk_ref[1, a] = jnp.zeros((256, 128), f32)
            fu_ref[a // NZ, a % NZ] = jnp.zeros((256, 128), f32)
            return c
        lax.fori_loop(0, NCH, clear, 0)
        for c in taps:
            c.wait()
        sh = shift_ref[...].astype(f32)
        dv = d_ref[...].astype(f32)
        for n in range(NCB):
            wt_ref[n, 0:KS, :] = sh[:, n * 128:(n + 1) * 128]
            wt_ref[n, KS:KS + 1, :] = dv[n:n + 1, :]
        cp_xb.wait()

        def xb_build(it, c):
            s0 = pl.multiple_of(it * 8, 8)
            t = xr_ref[pl.ds(s0, 8)].astype(f32).reshape(64, D).astype(bf16)
            xb_ref[pl.ds(pl.multiple_of(it * 32, 32), 32), :] = pltpu.bitcast(t, u32)
            return c
        lax.fori_loop(0, 8, xb_build, 0)

        def group(g, c):
            def region(i):
                return stage_ref.at[pl.ds(pl.multiple_of(i * (8 * D), 8 * D), 8 * D), :]
            subs = (region(g), region(jnp.where(g == 0, NG, g)))

            def relayout(j, chain=False):
                toks, t = [], None
                nd = 16 if chain else 256
                for blk in range(D // nd):
                    w = subs[j // 4][pl.ds(blk * 8 * nd + j, nd, stride=8), :]
                    if chain and blk % 16 != 0:
                        w = after(w, t)
                    lo = pltpu.bitcast(even(w).astype(bf16), u32)
                    hi = pltpu.bitcast(odd(w).astype(bf16), u32)
                    rows = slice(blk * nd // 2, (blk + 1) * nd // 2)
                    wn_ref[g * 16 + 2 * j, rows, :] = lo
                    wn_ref[g * 16 + 2 * j + 1, rows, :] = hi
                    if chain:
                        t = lo | hi
                        if blk % 16 == 15:
                            toks.append(t)
                return toks

            has_kv = jnp.logical_and(g >= 1, g <= 4)

            def prep_chain(k):
                cb = jnp.where(has_kv, 2 * g - 2 + k // 8, NCB)
                t = None
                for i in range(16):
                    t = conv_prep(cb, (k % 8) * 16 + i, t)
                return t

            @pl.when(g > 0)
            def _():
                wait_all(st3.at[pl.ds(g * D, D)], SEM_W + g)
            relayout(0)
            for j in range(8):
                if j == 3:
                    @pl.when(g == 0)
                    def _():
                        cp_w0b.wait()

                    @pl.when(has_kv)
                    def _():
                        wait_all(k_ref.at[pl.ds(2 * g - 2, 2), KPAD:], SEM_K + g - 1)
                        wait_all(v_ref.at[pl.ds(2 * g - 2, 2)], SEM_V + g - 1)
                xb = _as_bf16(xb_ref[...])
                w1, w2 = wn_ref[g * 16 + 2 * j], wn_ref[g * 16 + 2 * j + 1]
                toks = relayout(j + 1, j == 2) if j + 1 < 8 else None
                if j >= 4:
                    toks = [prep_chain(4 * (j - 4) + i) for i in range(4)]
                if j == 2 or j >= 4:
                    w1 = jnp.concatenate([after(w1[0:256], toks[0]), after(w1[256:], toks[1])], axis=0)
                    w2 = jnp.concatenate([after(w2[0:256], toks[2]), after(w2[256:], toks[3])], axis=0)
                r1 = _dot(xb, _as_bf16(w1))
                r2 = _dot(xb, _as_bf16(w2))
                cc = jnp.concatenate([r1.reshape(NSEG, 8, E), r2.reshape(NSEG, 8, E)], axis=1).astype(bf16)
                pre_ref[:, g * 8 + j] = pltpu.bitcast(cc, u32)
            return c
        cp_w0a.wait()
        lax.fori_loop(0, NG, group, 0)
        for c in small:
            c.wait()

    pl.run_scoped(prologue, pltpu.VMEM(((NG + 1) * 8 * D, E), u32))

    wait_all(wo_ref, SEM_WO)
    wait_all(x_ref, SEM_X)
    wait_all(ssm_ref.at[0:2 * UNROLL], SEM_SSM0)

    scale = E ** -0.5

    def main(odef_ref, b_ref, a_ref):
        def step(s, mem, t):
            cfg = CFG
            cb = s // 8
            r = s % 8
            icb = jnp.maximum(cb - 1, 0)
            idst = jnp.where(cb >= 1, cb - 1, NCB)
            mslot = (cb + 1) % 2
            nh = 8 // UNROLL
            chunks = ((nh * t + r // UNROLL, nh * t + nh), (NCH - 1 - nh * t - r // UNROLL, NCH - nh * t))
            zs = ({}, {})

            xrows = pl.ds(pl.multiple_of(s * 16, 16), 16)
            xs = [_as_bf16(x_ref[n, xrows, :]).astype(f32) for n in range(NCB)]
            h32 = jnp.concatenate([jnp.concatenate(xs, axis=1)[0:NT], mem], axis=0).astype(bf16)
            r0 = pl.multiple_of(s * 8, 8)

            def gate(dep):
                gw = gw_ref[...].astype(f32)
                gl = None
                for n in range(NCB):
                    xg = _as_bf16(x_ref[n, xrows, :]).astype(f32) * gw[n:n + 1, :]
                    gl = xg if gl is None else gl + xg
                g = jnp.broadcast_to(jax.nn.sigmoid(jnp.sum(gl, axis=-1, keepdims=True)), (SEG, 128))
                gate_ref[s] = g
                g = pltpu.bitcast(g, u32)
                return (g[0:8] | g[8:16]) | (g[16:24] | g[24:32])

            jobs = []

            def mac_job(dep, w, pos):
                zs[w][pos] = conv_mac(mslot, chunks[w][0], chunks[w][1], pos, dep)
                return zs[w][pos]

            for i in range(32):
                due = cfg["dues"][i]
                start = max(due - cfg["maclag"], 0)
                jobs.append((start, due - start, False, functools.partial(mac_job, w=i % 2, pos=i // 2)))
            jobs.append((cfg["gate"], 4, False, gate))
            state = dict(count=0, due={})

            def sdot(lhs, w, acc=None, weight=1):
                c = state["count"]
                toks = [t for cc in range(c, c + weight) for t in state["due"].pop(cc, [])]
                nt = w.shape[0] // 64
                if toks:
                    tiles = [w[64 * i:64 * (i + 1)] for i in range(nt)]
                    for i, t in enumerate(toks):
                        tiles[i % nt] = after(tiles[i % nt], t)
                    w = jnp.concatenate(tiles, axis=0)
                d = _dot(lhs, _as_bf16(w))
                d = d if acc is None else d + acc
                for (st, lag, rel, fn) in jobs:
                    if c <= st < c + weight:
                        tok = fn(pltpu.bitcast(d[0:8], u32) if rel else None)
                        state["due"].setdefault(max(st + lag, c + weight), []).append(tok)
                state["count"] = c + weight
                return d

            def proj(m, j):
                r1 = sdot(h32, wn_ref[m * H + 2 * j], weight=4)
                r2 = sdot(h32, wn_ref[m * H + 2 * j + 1], weight=4)
                p = _as_bf16(pre_ref[s, m * NP + j]).astype(f32)
                if m == 0:
                    return jnp.concatenate([r1, r2, p], axis=0)
                return jnp.concatenate([r1, r2, p, jnp.zeros((48, E), f32)], axis=0).astype(bf16)

            def split_rows(dot, lhs, rhs, split):
                if not split:
                    return dot(lhs.astype(bf16), rhs)
                return jnp.concatenate([dot(lhs[0:48].astype(bf16), rhs), dot(lhs[48:80].astype(bf16), rhs)], axis=0)

            def qk(q80, k80, split=False):
                fill = fill_ref[...]
                sc = jnp.where(fill == 0.0, split_rows(_dot_nt, q80, k80, split), fill)
                p = jnp.exp2((sc - jnp.max(sc, axis=-1, keepdims=True)) * (scale * LOG2E))
                den = jnp.sum(p, axis=-1, keepdims=True)
                rc = pl.reciprocal(den, approx=True)
                return p * (rc * (2.0 - den * rc))

            def pv(j, p, v80, split=False):
                o80 = split_rows(_dot, p, v80, split)
                odef_ref[pl.ds(r0, 8), (2 * j) * E:(2 * j + 1) * E] = o80[64:72]
                odef_ref[pl.ds(r0, 8), (2 * j + 1) * E:(2 * j + 2) * E] = o80[72:80]
                return jnp.concatenate([o80[0:32], o80[32:64]], axis=1).astype(bf16)

            def wo_part(o, j0, j1, n, acc=None):
                for j in range(j0, j1):
                    acc = sdot(o[j], wo_ref[n, j * 128:(j + 1) * 128, :], acc)
                return acc

            qs, ks, vs, ps, os_ = {}, {}, {}, {}, {}
            for j in range(0, NP, 2):
                for m, jj in cfg["order"]:
                    (qs, ks, vs)[m][j + jj] = proj(m, j + jj)
                ps[j] = qk(qs[j], ks[j], j == 0 and cfg["split0"])
                ps[j + 1] = qk(qs[j + 1], ks[j + 1], j == 0 and cfg["split0"])
                if j >= 2:
                    os_[j - 2] = pv(j - 2, ps[j - 2], vs[j - 2])
                    os_[j - 1] = pv(j - 1, ps[j - 1], vs[j - 1])
            na = NP - 2
            acc = {}
            nw = cfg["nw"]
            for n in range(nw):
                acc[n] = wo_part(os_, 0, na, n)
            os_[NP - 2] = pv(NP - 2, ps[NP - 2], vs[NP - 2], cfg["split1"])
            os_[NP - 1] = pv(NP - 1, ps[NP - 1], vs[NP - 1], cfg["split1"])
            acc[nw] = wo_part(os_, 0, na, nw)
            for n in range(nw + 1):
                acc[n] = wo_part(os_, na, NP, n, acc[n])
            for n in range(nw + 1, 8):
                acc[n] = wo_part(os_, 0, NP, n)
            assert state["count"] == 512 and not state["due"], state
            for w in range(2):
                conv_inv(a_ref, icb, idst, chunks[w][0], [zs[w][pos] for pos in range(16)])
            if t == UNROLL - 1:
                for tt in range(UNROLL):
                    conv_fwd(cb, r - t + tt)
            for n in range(NCB):
                b_ref[n, s, 0:NT, :] = acc[n][0:NT]
            return jnp.concatenate([acc[n][NT:SEG] for n in range(NCB)], axis=1).astype(bf16).astype(f32)

        def steps(i, mem):
            @pl.when(i == 1)
            def _():
                wait_all(ssm_ref.at[2 * UNROLL:NCH], SEM_SSM1)
            for t in range(UNROLL):
                mem = step(i * UNROLL + t, mem, t)
            return mem

        lax.fori_loop(0, _DBG_STEPS // UNROLL, steps, mem_ref[...].astype(f32))

        def out_copy(n):
            slot = n % 2
            return pltpu.make_async_copy(
                ost_ref.at[slot], out_hbm.at[:, :, pl.ds(pl.multiple_of(n * 128, 128), 128)],
                sems.at[SEM_OUT + slot])

        def fin(n, c):
            @pl.when(n >= 2)
            def _():
                out_copy(n - 2).wait()
            zs, toks, t = ([], []), [], None
            for pos in range(16):
                if pos % 3 == 0:
                    t = None
                for w in range(2):
                    t = conv_mac((NCB - 1) % 2, n + 8 * w, 8 + 8 * w, pos, t)
                    zs[w].append(t)
                if pos % 3 == 2 or pos == 15:
                    toks.append(t)
            bd = None
            for kb in range(8):
                if kb == 7:
                    for w in range(2):
                        conv_inv(a_ref, NCB - 1, NCB - 1, n + 8 * w, zs[w])
                w = after(wo_ref[n, kb * 256:(kb + 1) * 256, :], toks[kb - 1] if 0 < kb <= len(toks) else None)
                d = _dot(odef_ref[:, kb * 512:(kb + 1) * 512].astype(bf16), _as_bf16(w))
                bd = d if bd is None else d + bd
            b_ref[n, :, NT:SEG, :] = bd.reshape(NSEG, 8, 128)
            for blk in range(8):
                sg = slice(blk * 8, (blk + 1) * 8)
                b = b_ref[n, sg]
                a = a_ref[n, blk * 256:(blk + 1) * 256, :].reshape(8, SEG, 128)
                g = gate_ref[sg]
                ost_ref[n % 2, sg] = (g * a + (1.0 - g) * b).astype(bf16)
            out_copy(n).start()
            return c
        lax.fori_loop(0, NCB, fin, 0)
        out_copy(NCB - 2).wait()
        out_copy(NCB - 1).wait()

    pl.run_scoped(main, pltpu.VMEM((NSEG * 8, H * E), f32), pltpu.VMEM((NCB, NSEG, SEG, 128), f32),
                  pltpu.VMEM((NCB + 1, S, 128), f32))


@jax.jit
def pallas_gated_mix__ssm_conv_h3__memory_aug_recurrent_mem_tr__prompt_kernel(
    A_q: jax.Array,
    A_k: jax.Array,
    A_v: jax.Array,
    A_shift_k: jax.Array,
    A_ssm_k: jax.Array,
    A_ssm_D: jax.Array,
    B_x: jax.Array,
    B_mem0: jax.Array,
    B_Wq: jax.Array,
    B_Wk: jax.Array,
    B_Wv: jax.Array,
    B_Wo: jax.Array,
    B_seg_len: jax.Array,
    gate_w: jax.Array,
):
    del B_x, B_seg_len
    f_tab, g_tab = _dft_tables()
    out = pl.pallas_call(
        _kernel,
        out_shape=jax.ShapeDtypeStruct((NSEG, SEG, D), bf16),
        in_specs=[pl.BlockSpec(memory_space=pl.ANY)] * 15,
        out_specs=pl.BlockSpec(memory_space=pl.ANY),
        scratch_shapes=[
            pltpu.VMEM((3 * H, D // 2, E), u32),
            pltpu.VMEM((NCB, H * E // 2, 128), u32),
            pltpu.VMEM((NCB, S // 2, 128), u32),
            pltpu.VMEM((NSEG, M, D), bf16),
            pltpu.VMEM((NSEG * 4, D), u32),
            pltpu.VMEM((NSEG, 3 * NP, 8, E), u32),
            pltpu.VMEM((NCB + 1, KPAD + S // 2, 128), u32),
            pltpu.VMEM((NCB + 1, S // 2, 128), u32),
            pltpu.VMEM((NCH, D // 2, 128), u32),
            pltpu.VMEM((NCB + 1, S // 2, 128), u32),
            pltpu.VMEM((2, NZ + NCH, 256, 128), f32),
            pltpu.VMEM((2, NCH, 256, 128), f32),
            pltpu.VMEM((256, 128), f32),
            pltpu.VMEM((8, 128), jnp.int32),
            pltpu.VMEM((256, 128), bf16),
            pltpu.VMEM((128, 256), bf16),
            pltpu.VMEM((80, 128), f32),
            pltpu.VMEM((KS, D), bf16),
            pltpu.VMEM((NCB + 1, 8, 128), f32),
            pltpu.VMEM((NCB, 128), bf16),
            pltpu.VMEM((NCB, 128), bf16),
            pltpu.VMEM((M, D), bf16),
            pltpu.VMEM((NSEG, SEG, 128), f32),
            pltpu.VMEM((2, NSEG, SEG, 128), bf16),
            pltpu.SemaphoreType.DMA((NSEM,)),
        ],
        compiler_params=pltpu.CompilerParams(vmem_limit_bytes=120 * 2**20),
    )(A_q.reshape(NSEG, SEG, D), A_q.reshape(S, D), A_k.reshape(S, D), A_v.reshape(S, D), A_shift_k.T,
      A_ssm_k, A_ssm_D.reshape(NCB, 128), B_mem0.reshape(M, D), B_Wq, B_Wk, B_Wv,
      B_Wo.reshape(H * E, D), gate_w.reshape(NCB, 128), f_tab, g_tab)
    return out.reshape(1, S, D)
```

```python
import functools

import numpy as np
import jax
import jax.numpy as jnp
from jax import lax
import jax.experimental.pallas as pl
import jax.experimental.pallas.tpu as pltpu

S, D, H, E, M, SEG = 2048, 1024, 32, 128, 8, 32
NSEG = S // SEG
NT = SEG - M
NP = H // 2
NCB = D // 128
C = 128
NCH = S // C
LOG2E = 1.4426950408889634
KS = 4
NZ = 8
KPAD = 32
NG = 6
UNROLL = 4
CFG = dict(fgrp=4, finv=4, dues=[12, 16, 20, 24, 28, 32, 36, 40, 44] + [48 * p + 40 for p in range(1, 8)] + [444 + 4 * i for i in range(16)], maclag=4, gate=436,
           split0=True, split1=True, nw=3, order=((0, 0), (1, 0), (0, 1), (1, 1), (2, 0), (2, 1)))
_DBG_STEPS = NSEG
bf16, f32, u32 = jnp.bfloat16, jnp.float32, jnp.uint32


def _dft_tables():
    t = np.arange(C, dtype=np.float64)
    rows = []
    for r in range(8):
        ev = 16 * r + np.arange(0, 16, 2)
        od = ev + 1
        for fn, fs in ((np.cos, ev), (np.sin, ev), (np.cos, od), (np.sin, od)):
            rows.append(fn(np.pi * (2 * fs[:, None] + 1) * t[None, :] / (2 * C)))
    f = np.concatenate(rows, axis=0)
    return f.astype(bf16), (f.T / C).astype(bf16)


def _fill_matrix():
    r = lax.broadcasted_iota(jnp.int32, (80, 128), 0)
    c = lax.broadcasted_iota(jnp.int32, (80, 128), 1)

    def head(i):
        return jnp.where(i < 64, i // 32, (i - 64) // 8)

    def idx(i):
        lo = i % 32
        main = jnp.where(lo < NT, lo + M, lo - NT)
        return jnp.where(i < 64, main, (i - 64) % 8 + NT + M)

    same = (head(r) == head(c)) & (c < 80)
    ok = (idx(r) < M) | (idx(r) >= idx(c))
    return jnp.where(same, jnp.where(ok, 0.0, -1e9 * E ** 0.5), -jnp.inf).astype(f32)


def _as_bf16(v):
    return pltpu.bitcast(v, bf16)


def _dot(a, b):
    return jnp.dot(a, b, preferred_element_type=f32)


def _dot_nt(a, b):
    return lax.dot_general(a, b, (((1,), (1,)), ((), ())), preferred_element_type=f32)


SEM_TAPS, SEM_SMALL, SEM_XB, SEM_WO, SEM_X, SEM_SSM0, SEM_SSM1 = range(7)
SEM_K = 7
SEM_V = SEM_K + 4
SEM_W = SEM_V + 4
SEM_OUT = SEM_W + NG + 1
NSEM = SEM_OUT + 2


def _kernel(x3_hbm, x_hbm, k_hbm, v_hbm, shift_hbm, ssm_hbm, d_hbm, mem_hbm, wq_hbm, wk_hbm, wv_hbm,
            wo_hbm, gw_hbm, f_hbm, g_hbm, out_hbm,
            wn_ref, wo_ref, x_ref, xr_ref, xb_ref, pre_ref, k_ref, v_ref, ssm_ref, u_ref,
            fu_ref, fk_ref, kraw_ref, one_ref, f_ref, g_ref, fill_ref, shift_ref, wt_ref,
            d_ref, gw_ref, mem_ref, gate_ref, ost_ref, sems):
    w_hbm = (wq_hbm, wk_hbm, wv_hbm)

    def cp(src, dst, sem):
        return pltpu.make_async_copy(src, dst, sems.at[sem])

    def start_col_blocks(src_hbm, dst_ref, i0, i1, sem, row0=0):
        src = src_hbm.bitcast(u32)
        for i in range(i0, i1):
            cp(src.at[:, i * 128:(i + 1) * 128], dst_ref.at[i, row0:], sem).start()

    def wait_all(dst, sem):
        cp(dst, dst, sem).wait()

    def even(p):
        return pltpu.bitcast(p << 16, f32)

    def odd(p):
        return pltpu.bitcast(p & jnp.uint32(0xFFFF0000), f32)

    def conv_prep(cb, i, dep=None):
        r0 = KPAD + 8 * i
        p0 = k_ref[cb, r0:r0 + 8, :]
        if dep is not None:
            p0 = jnp.where(one_ref[...] == 1, p0, dep)
        p1 = k_ref[cb, r0 - 1:r0 + 7, :]
        p2 = k_ref[cb, r0 - 2:r0 + 6, :]
        pv = v_ref[cb, 8 * i:8 * i + 8, :]
        w = wt_ref[cb]
        w0, w1, w2, w3 = w[0:1, :], w[1:2, :], w[2:3, :], w[3:4, :]
        e0, o0, e1, o1, o2 = even(p0), odd(p0), even(p1), odd(p1), odd(p2)
        ke = ((e0 * w0 + o1 * w1) + e1 * w2) + o2 * w3
        ko = ((o0 * w0 + e0 * w1) + o1 * w2) + e1 * w3
        re = pltpu.bitcast((ke * even(pv)).astype(bf16).astype(f32), u32)
        ro = pltpu.bitcast((ko * odd(pv)).astype(bf16).astype(f32), u32)
        kv = (re >> 16) | ro
        u_ref[cb, 8 * i:8 * i + 8, :] = kv
        return kv

    def combine(kf, prev):
        out = []
        for g in range(8):
            o = 32 * g
            out += [kf[o:o + 8] + prev[o + 8:o + 16], kf[o + 8:o + 16] - prev[o:o + 8],
                    kf[o + 16:o + 24] - prev[o + 24:o + 32], kf[o + 24:o + 32] + prev[o + 16:o + 24]]
        return jnp.concatenate(out, axis=0)

    def conv_fwd(cb, r):
        slot = cb % 2
        rows = pl.ds(pl.multiple_of(cb * 64, 64), 64)
        f = f_ref[...]
        kfs = []
        for a in (2 * r, 2 * r + 1):
            fu_ref[slot, NZ + a] = _dot(f, _as_bf16(u_ref[cb, pl.ds(pl.multiple_of(a * 64, 64), 64), :]))
            kfs.append(_dot_nt(f, _as_bf16(ssm_ref[a, rows, :])))
        fk_ref[slot, 2 * r] = combine(kfs[0], jnp.where(r > 0, kraw_ref[...], 0.0))
        fk_ref[slot, 2 * r + 1] = combine(kfs[1], kfs[0])
        kraw_ref[...] = kfs[1]

    def conv_mac(slot, a, nterms, pos, dep=None):
        rows = slice(pos * 16, pos * 16 + 16)
        p = q = None
        for c in range(nterms):
            u = fu_ref[slot, NZ + a - c, rows, :]
            k = fk_ref[slot, c, rows, :]
            ua, ub, kc, kd = u[0:8], u[8:16], k[0:8], k[8:16]
            if c == 0 and dep is not None:
                ua = jnp.where(one_ref[...] == 1, ua, pltpu.bitcast(dep, f32))
            p = (ua * kc if p is None else p + ua * kc) - ub * kd
            q = (ua * kd if q is None else q + ua * kd) + ub * kc
        return pltpu.bitcast(jnp.concatenate([p, q], axis=0).astype(bf16), u32)

    def conv_inv(a_ref, cb, dst, a, zs):
        rows = pl.ds(pl.multiple_of(a * 64, 64), 64)
        y = _dot(g_ref[...], _as_bf16(jnp.concatenate(zs, axis=0)))
        kv = _as_bf16(u_ref[cb, rows, :]).astype(f32)
        q = _as_bf16(x_ref[cb, rows, :]).astype(f32)
        a_ref[dst, pl.ds(pl.multiple_of(a * C, C), C), :] = q * (y + kv * wt_ref[cb, KS:KS + 1, :])

    def after(w, tok):
        if tok is None:
            return w
        return jnp.concatenate([jnp.where(one_ref[...] == 1, w[0:8], tok), w[8:]], axis=0)

    def prologue(stage_ref):
        st3 = stage_ref.reshape((NG + 1) * D, 8, E)
        w0 = wq_hbm.bitcast(u32)
        cp_w0a = cp(w0.at[:, 0:4, :], st3.at[0:D, 0:4, :], SEM_W)
        cp_w0b = cp(w0.at[:, 4:8, :], st3.at[NG * D:(NG + 1) * D, 4:8, :], SEM_W + NG)

        def start_w(g):
            r0 = (g % 2) * 8
            cp(w_hbm[g // 2].bitcast(u32).at[:, r0:r0 + 8, :], st3.at[g * D:(g + 1) * D], SEM_W + g).start()

        taps = [cp(shift_hbm, shift_ref, SEM_TAPS), cp(d_hbm, d_ref, SEM_TAPS)]
        small = [cp(gw_hbm, gw_ref, SEM_SMALL), cp(mem_hbm, mem_ref, SEM_SMALL), cp(f_hbm, f_ref, SEM_SMALL),
                 cp(g_hbm, g_ref, SEM_SMALL)]
        cp_xb = cp(x3_hbm.at[:, NT:SEG, :], xr_ref, SEM_XB)
        for c in taps:
            c.start()
        cp_xb.start()
        cp_w0a.start()
        cp_w0b.start()
        for g in range(1, NG):
            start_w(g)
            if g <= 4:
                start_col_blocks(k_hbm, k_ref, 2 * g - 2, 2 * g, SEM_K + g - 1, row0=KPAD)
                start_col_blocks(v_hbm, v_ref, 2 * g - 2, 2 * g, SEM_V + g - 1)
        for c in small:
            c.start()
        start_col_blocks(wo_hbm, wo_ref, 0, NCB, SEM_WO)
        start_col_blocks(x_hbm, x_ref, 0, NCB, SEM_X)
        start_col_blocks(ssm_hbm, ssm_ref, 0, 2 * UNROLL, SEM_SSM0)
        start_col_blocks(ssm_hbm, ssm_ref, 2 * UNROLL, NCH, SEM_SSM1)
        fill_ref[...] = _fill_matrix()
        one_ref[...] = jnp.ones((8, 128), jnp.int32)
        k_ref[:, KPAD - 8:KPAD, :] = jnp.zeros((NCB + 1, 8, 128), u32)
        wt_ref[...] = jnp.zeros(wt_ref.shape, f32)
        kraw_ref[...] = jnp.zeros(kraw_ref.shape, f32)

        def clear(a, c):
            rows = pl.ds(pl.multiple_of(a * 64, 64), 64)
            k_ref[NCB, pl.ds(pl.multiple_of(KPAD + a * 64, 32), 64), :] = jnp.zeros((64, 128), u32)
            v_ref[NCB, rows, :] = jnp.zeros((64, 128), u32)
            fu_ref[1, NZ + a] = jnp.zeros((256, 128), f32)
            fk_ref[1, a] = jnp.zeros((256, 128), f32)
            fu_ref[a // NZ, a % NZ] = jnp.zeros((256, 128), f32)
            return c
        lax.fori_loop(0, NCH, clear, 0)
        for c in taps:
            c.wait()
        sh = shift_ref[...].astype(f32)
        dv = d_ref[...].astype(f32)
        for n in range(NCB):
            wt_ref[n, 0:KS, :] = sh[:, n * 128:(n + 1) * 128]
            wt_ref[n, KS:KS + 1, :] = dv[n:n + 1, :]
        cp_xb.wait()

        def xb_build(it, c):
            s0 = pl.multiple_of(it * 8, 8)
            t = xr_ref[pl.ds(s0, 8)].astype(f32).reshape(64, D).astype(bf16)
            xb_ref[pl.ds(pl.multiple_of(it * 32, 32), 32), :] = pltpu.bitcast(t, u32)
            return c
        lax.fori_loop(0, 8, xb_build, 0)

        def group(g, c):
            def region(i):
                return stage_ref.at[pl.ds(pl.multiple_of(i * (8 * D), 8 * D), 8 * D), :]
            subs = (region(g), region(jnp.where(g == 0, NG, g)))

            def relayout(j, chain=False):
                toks, t = [], None
                nd = 16 if chain else 256
                for blk in range(D // nd):
                    w = subs[j // 4][pl.ds(blk * 8 * nd + j, nd, stride=8), :]
                    if chain and blk % 16 != 0:
                        w = after(w, t)
                    lo = pltpu.bitcast(even(w).astype(bf16), u32)
                    hi = pltpu.bitcast(odd(w).astype(bf16), u32)
                    rows = slice(blk * nd // 2, (blk + 1) * nd // 2)
                    wn_ref[g * 16 + 2 * j, rows, :] = lo
                    wn_ref[g * 16 + 2 * j + 1, rows, :] = hi
                    if chain:
                        t = lo | hi
                        if blk % 16 == 15:
                            toks.append(t)
                return toks

            has_kv = jnp.logical_and(g >= 1, g <= 4)

            def prep_chain(k):
                cb = jnp.where(has_kv, 2 * g - 2 + k // 8, NCB)
                t = None
                for i in range(16):
                    t = conv_prep(cb, (k % 8) * 16 + i, t)
                return t

            @pl.when(g > 0)
            def _():
                wait_all(st3.at[pl.ds(g * D, D)], SEM_W + g)
            relayout(0)
            for j in range(8):
                if j == 3:
                    @pl.when(g == 0)
                    def _():
                        cp_w0b.wait()

                    @pl.when(has_kv)
                    def _():
                        wait_all(k_ref.at[pl.ds(2 * g - 2, 2), KPAD:], SEM_K + g - 1)
                        wait_all(v_ref.at[pl.ds(2 * g - 2, 2)], SEM_V + g - 1)
                xb = _as_bf16(xb_ref[...])
                w1, w2 = wn_ref[g * 16 + 2 * j], wn_ref[g * 16 + 2 * j + 1]
                toks = relayout(j + 1, j == 2) if j + 1 < 8 else None
                if j >= 4:
                    toks = [prep_chain(4 * (j - 4) + i) for i in range(4)]
                if j == 2 or j >= 4:
                    w1 = jnp.concatenate([after(w1[0:256], toks[0]), after(w1[256:], toks[1])], axis=0)
                    w2 = jnp.concatenate([after(w2[0:256], toks[2]), after(w2[256:], toks[3])], axis=0)
                r1 = _dot(xb, _as_bf16(w1))
                r2 = _dot(xb, _as_bf16(w2))
                cc = jnp.concatenate([r1.reshape(NSEG, 8, E), r2.reshape(NSEG, 8, E)], axis=1).astype(bf16)
                pre_ref[:, g * 8 + j] = pltpu.bitcast(cc, u32)
            return c
        cp_w0a.wait()
        lax.fori_loop(0, NG, group, 0)
        for c in small:
            c.wait()

    pl.run_scoped(prologue, pltpu.VMEM(((NG + 1) * 8 * D, E), u32))

    wait_all(wo_ref, SEM_WO)
    wait_all(x_ref, SEM_X)
    wait_all(ssm_ref.at[0:2 * UNROLL], SEM_SSM0)

    scale = E ** -0.5

    def main(odef_ref, b_ref, a_ref):
        def step(s, mem, t):
            cfg = CFG
            cb = s // 8
            r = s % 8
            icb = jnp.maximum(cb - 1, 0)
            idst = jnp.where(cb >= 1, cb - 1, NCB)
            mslot = (cb + 1) % 2
            nh = 8 // UNROLL
            chunks = ((nh * t + r // UNROLL, nh * t + nh), (NCH - 1 - nh * t - r // UNROLL, NCH - nh * t))
            zs = ({}, {})

            xrows = pl.ds(pl.multiple_of(s * 16, 16), 16)
            xs = [_as_bf16(x_ref[n, xrows, :]).astype(f32) for n in range(NCB)]
            h32 = jnp.concatenate([jnp.concatenate(xs, axis=1)[0:NT], mem], axis=0).astype(bf16)
            r0 = pl.multiple_of(s * 8, 8)

            def gate(dep):
                gw = gw_ref[...].astype(f32)
                gl = None
                for n in range(NCB):
                    xg = _as_bf16(x_ref[n, xrows, :]).astype(f32) * gw[n:n + 1, :]
                    gl = xg if gl is None else gl + xg
                g = jnp.broadcast_to(jax.nn.sigmoid(jnp.sum(gl, axis=-1, keepdims=True)), (SEG, 128))
                gate_ref[s] = g
                g = pltpu.bitcast(g, u32)
                return (g[0:8] | g[8:16]) | (g[16:24] | g[24:32])

            jobs = []

            def mac_job(dep, w, pos):
                zs[w][pos] = conv_mac(mslot, chunks[w][0], chunks[w][1], pos, dep)
                return zs[w][pos]

            for i in range(32):
                due = cfg["dues"][i]
                start = max(due - cfg["maclag"], 0)
                jobs.append((start, due - start, False, functools.partial(mac_job, w=i % 2, pos=i // 2)))
            jobs.append((cfg["gate"], 4, False, gate))
            state = dict(count=0, due={})

            def sdot(lhs, w, acc=None, weight=1):
                c = state["count"]
                toks = [t for cc in range(c, c + weight) for t in state["due"].pop(cc, [])]
                nt = w.shape[0] // 64
                if toks:
                    tiles = [w[64 * i:64 * (i + 1)] for i in range(nt)]
                    for i, t in enumerate(toks):
                        tiles[i % nt] = after(tiles[i % nt], t)
                    w = jnp.concatenate(tiles, axis=0)
                d = _dot(lhs, _as_bf16(w))
                d = d if acc is None else d + acc
                for (st, lag, rel, fn) in jobs:
                    if c <= st < c + weight:
                        tok = fn(pltpu.bitcast(d[0:8], u32) if rel else None)
                        state["due"].setdefault(max(st + lag, c + weight), []).append(tok)
                state["count"] = c + weight
                return d

            def proj(m, j):
                r1 = sdot(h32, wn_ref[m * H + 2 * j], weight=4)
                r2 = sdot(h32, wn_ref[m * H + 2 * j + 1], weight=4)
                p = _as_bf16(pre_ref[s, m * NP + j]).astype(f32)
                if m == 0:
                    return jnp.concatenate([r1, r2, p], axis=0)
                return jnp.concatenate([r1, r2, p, jnp.zeros((48, E), f32)], axis=0).astype(bf16)

            def split_rows(dot, lhs, rhs, split):
                if not split:
                    return dot(lhs.astype(bf16), rhs)
                return jnp.concatenate([dot(lhs[0:48].astype(bf16), rhs), dot(lhs[48:80].astype(bf16), rhs)], axis=0)

            def qk(q80, k80, split=False):
                fill = fill_ref[...]
                sc = jnp.where(fill == 0.0, split_rows(_dot_nt, q80, k80, split), fill)
                p = jnp.exp2((sc - jnp.max(sc, axis=-1, keepdims=True)) * (scale * LOG2E))
                den = jnp.sum(p, axis=-1, keepdims=True)
                rc = pl.reciprocal(den, approx=True)
                return p * (rc * (2.0 - den * rc))

            def pv(j, p, v80, split=False):
                o80 = split_rows(_dot, p, v80, split)
                odef_ref[pl.ds(r0, 8), (2 * j) * E:(2 * j + 1) * E] = o80[64:72]
                odef_ref[pl.ds(r0, 8), (2 * j + 1) * E:(2 * j + 2) * E] = o80[72:80]
                return jnp.concatenate([o80[0:32], o80[32:64]], axis=1).astype(bf16)

            def wo_part(o, j0, j1, n, acc=None):
                for j in range(j0, j1):
                    acc = sdot(o[j], wo_ref[n, j * 128:(j + 1) * 128, :], acc)
                return acc

            qs, ks, vs, ps, os_ = {}, {}, {}, {}, {}
            for j in range(0, NP, 2):
                for m, jj in cfg["order"]:
                    (qs, ks, vs)[m][j + jj] = proj(m, j + jj)
                ps[j] = qk(qs[j], ks[j], j == 0 and cfg["split0"])
                ps[j + 1] = qk(qs[j + 1], ks[j + 1], j == 0 and cfg["split0"])
                if j >= 2:
                    os_[j - 2] = pv(j - 2, ps[j - 2], vs[j - 2])
                    os_[j - 1] = pv(j - 1, ps[j - 1], vs[j - 1])
            na = NP - 2
            acc = {}
            nw = cfg["nw"]
            for n in range(nw):
                acc[n] = wo_part(os_, 0, na, n)
            os_[NP - 2] = pv(NP - 2, ps[NP - 2], vs[NP - 2], cfg["split1"])
            os_[NP - 1] = pv(NP - 1, ps[NP - 1], vs[NP - 1], cfg["split1"])
            acc[nw] = wo_part(os_, 0, na, nw)
            for n in range(nw + 1):
                acc[n] = wo_part(os_, na, NP, n, acc[n])
            for n in range(nw + 1, 8):
                acc[n] = wo_part(os_, 0, NP, n)
            assert state["count"] == 512 and not state["due"], state
            for w in range(2):
                conv_inv(a_ref, icb, idst, chunks[w][0], [zs[w][pos] for pos in range(16)])
            if t == UNROLL - 1:
                for tt in range(UNROLL):
                    conv_fwd(cb, r - t + tt)
            for n in range(NCB):
                b_ref[n, s, 0:NT, :] = acc[n][0:NT]
            return jnp.concatenate([acc[n][NT:SEG] for n in range(NCB)], axis=1).astype(bf16).astype(f32)

        def steps(i, mem):
            @pl.when(i == 1)
            def _():
                wait_all(ssm_ref.at[2 * UNROLL:NCH], SEM_SSM1)
            for t in range(UNROLL):
                mem = step(i * UNROLL + t, mem, t)
            return mem

        lax.fori_loop(0, _DBG_STEPS // UNROLL, steps, mem_ref[...].astype(f32))

        def out_copy(n):
            slot = n % 2
            return pltpu.make_async_copy(
                ost_ref.at[slot], out_hbm.at[:, :, pl.ds(pl.multiple_of(n * 128, 128), 128)],
                sems.at[SEM_OUT + slot])

        def fin(n, c):
            @pl.when(n >= 2)
            def _():
                out_copy(n - 2).wait()
            zs, toks, t = ([], []), [], None
            for pos in range(16):
                if pos % CFG["fgrp"] == 0:
                    t = None
                for w in range(2):
                    t = conv_mac((NCB - 1) % 2, n + 8 * w, 8 + 8 * w, pos, t)
                    zs[w].append(t)
                if pos % CFG["fgrp"] == CFG["fgrp"] - 1:
                    toks.append(t)
            bd = None
            for kb in range(8):
                if kb == CFG["finv"]:
                    for w in range(2):
                        conv_inv(a_ref, NCB - 1, NCB - 1, n + 8 * w, zs[w])
                w = after(wo_ref[n, kb * 256:(kb + 1) * 256, :], toks[kb - 1] if 0 < kb <= len(toks) else None)
                d = _dot(odef_ref[:, kb * 512:(kb + 1) * 512].astype(bf16), _as_bf16(w))
                bd = d if bd is None else d + bd
            b_ref[n, :, NT:SEG, :] = bd.reshape(NSEG, 8, 128)
            for blk in range(8):
                sg = slice(blk * 8, (blk + 1) * 8)
                b = b_ref[n, sg]
                a = a_ref[n, blk * 256:(blk + 1) * 256, :].reshape(8, SEG, 128)
                g = gate_ref[sg]
                ost_ref[n % 2, sg] = (g * a + (1.0 - g) * b).astype(bf16)
            out_copy(n).start()
            return c
        lax.fori_loop(0, NCB, fin, 0)
        out_copy(NCB - 2).wait()
        out_copy(NCB - 1).wait()

    pl.run_scoped(main, pltpu.VMEM((NSEG * 8, H * E), f32), pltpu.VMEM((NCB, NSEG, SEG, 128), f32),
                  pltpu.VMEM((NCB + 1, S, 128), f32))


@jax.jit
def pallas_gated_mix__ssm_conv_h3__memory_aug_recurrent_mem_tr__prompt_kernel(
    A_q: jax.Array,
    A_k: jax.Array,
    A_v: jax.Array,
    A_shift_k: jax.Array,
    A_ssm_k: jax.Array,
    A_ssm_D: jax.Array,
    B_x: jax.Array,
    B_mem0: jax.Array,
    B_Wq: jax.Array,
    B_Wk: jax.Array,
    B_Wv: jax.Array,
    B_Wo: jax.Array,
    B_seg_len: jax.Array,
    gate_w: jax.Array,
):
    del B_x, B_seg_len
    f_tab, g_tab = _dft_tables()
    out = pl.pallas_call(
        _kernel,
        out_shape=jax.ShapeDtypeStruct((NSEG, SEG, D), bf16),
        in_specs=[pl.BlockSpec(memory_space=pl.ANY)] * 15,
        out_specs=pl.BlockSpec(memory_space=pl.ANY),
        scratch_shapes=[
            pltpu.VMEM((3 * H, D // 2, E), u32),
            pltpu.VMEM((NCB, H * E // 2, 128), u32),
            pltpu.VMEM((NCB, S // 2, 128), u32),
            pltpu.VMEM((NSEG, M, D), bf16),
            pltpu.VMEM((NSEG * 4, D), u32),
            pltpu.VMEM((NSEG, 3 * NP, 8, E), u32),
            pltpu.VMEM((NCB + 1, KPAD + S // 2, 128), u32),
            pltpu.VMEM((NCB + 1, S // 2, 128), u32),
            pltpu.VMEM((NCH, D // 2, 128), u32),
            pltpu.VMEM((NCB + 1, S // 2, 128), u32),
            pltpu.VMEM((2, NZ + NCH, 256, 128), f32),
            pltpu.VMEM((2, NCH, 256, 128), f32),
            pltpu.VMEM((256, 128), f32),
            pltpu.VMEM((8, 128), jnp.int32),
            pltpu.VMEM((256, 128), bf16),
            pltpu.VMEM((128, 256), bf16),
            pltpu.VMEM((80, 128), f32),
            pltpu.VMEM((KS, D), bf16),
            pltpu.VMEM((NCB + 1, 8, 128), f32),
            pltpu.VMEM((NCB, 128), bf16),
            pltpu.VMEM((NCB, 128), bf16),
            pltpu.VMEM((M, D), bf16),
            pltpu.VMEM((NSEG, SEG, 128), f32),
            pltpu.VMEM((2, NSEG, SEG, 128), bf16),
            pltpu.SemaphoreType.DMA((NSEM,)),
        ],
        compiler_params=pltpu.CompilerParams(vmem_limit_bytes=120 * 2**20),
    )(A_q.reshape(NSEG, SEG, D), A_q.reshape(S, D), A_k.reshape(S, D), A_v.reshape(S, D), A_shift_k.T,
      A_ssm_k, A_ssm_D.reshape(NCB, 128), B_mem0.reshape(M, D), B_Wq, B_Wk, B_Wv,
      B_Wo.reshape(H * E, D), gate_w.reshape(NCB, 128), f_tab, g_tab)
    return out.reshape(1, S, D)
```

```python
import functools

import numpy as np
import jax
import jax.numpy as jnp
from jax import lax
import jax.experimental.pallas as pl
import jax.experimental.pallas.tpu as pltpu

S, D, H, E, M, SEG = 2048, 1024, 32, 128, 8, 32
NSEG = S // SEG
NT = SEG - M
NP = H // 2
NCB = D // 128
C = 128
NCH = S // C
LOG2E = 1.4426950408889634
KS = 4
NZ = 8
KPAD = 32
NG = 6
NQ = 4
DQ = D // NQ
UNROLL = 4
CFG = dict(fgrp=4, finv=4, dues=[12, 16, 20, 24, 28, 32, 36, 40, 44] + [48 * p + 40 for p in range(1, 8)] + [444 + 4 * i for i in range(16)], maclag=4, gate=436,
           split0=True, split1=True, nw=3, order=((0, 0), (1, 0), (0, 1), (1, 1), (2, 0), (2, 1)))
_DBG_STEPS = NSEG
bf16, f32, u32 = jnp.bfloat16, jnp.float32, jnp.uint32


def _dft_tables():
    t = np.arange(C, dtype=np.float64)
    rows = []
    for r in range(8):
        ev = 16 * r + np.arange(0, 16, 2)
        od = ev + 1
        for fn, fs in ((np.cos, ev), (np.sin, ev), (np.cos, od), (np.sin, od)):
            rows.append(fn(np.pi * (2 * fs[:, None] + 1) * t[None, :] / (2 * C)))
    f = np.concatenate(rows, axis=0)
    return f.astype(bf16), (f.T / C).astype(bf16)


def _fill_matrix():
    r = lax.broadcasted_iota(jnp.int32, (80, 128), 0)
    c = lax.broadcasted_iota(jnp.int32, (80, 128), 1)

    def head(i):
        return jnp.where(i < 64, i // 32, (i - 64) // 8)

    def idx(i):
        lo = i % 32
        main = jnp.where(lo < NT, lo + M, lo - NT)
        return jnp.where(i < 64, main, (i - 64) % 8 + NT + M)

    same = (head(r) == head(c)) & (c < 80)
    ok = (idx(r) < M) | (idx(r) >= idx(c))
    return jnp.where(same, jnp.where(ok, 0.0, -1e9 * E ** 0.5), -jnp.inf).astype(f32)


def _as_bf16(v):
    return pltpu.bitcast(v, bf16)


def _dot(a, b):
    return jnp.dot(a, b, preferred_element_type=f32)


def _dot_nt(a, b):
    return lax.dot_general(a, b, (((1,), (1,)), ((), ())), preferred_element_type=f32)


SEM_SMALL, SEM_WO, SEM_X, SEM_SSM0, SEM_SSM1 = range(5)
SEM_XB = 5
SEM_W0 = SEM_XB + NQ
SEM_K = SEM_W0 + NQ
SEM_V = SEM_K + 4
SEM_W = SEM_V + 4
SEM_OUT = SEM_W + NG
NSEM = SEM_OUT + 2


def _kernel(x3_hbm, x_hbm, k_hbm, v_hbm, shift_hbm, ssm_hbm, d_hbm, mem_hbm, wq_hbm, wk_hbm, wv_hbm,
            wo_hbm, gw_hbm, f_hbm, g_hbm, out_hbm,
            wn_ref, wo_ref, x_ref, xr_ref, xb_ref, pre_ref, k_ref, v_ref, ssm_ref, u_ref,
            fu_ref, fk_ref, kraw_ref, one_ref, f_ref, g_ref, fill_ref, shift_ref, wt_ref,
            d_ref, gw_ref, mem_ref, gate_ref, ost_ref, sems):
    w_hbm = (wq_hbm, wk_hbm, wv_hbm)

    def cp(src, dst, sem):
        return pltpu.make_async_copy(src, dst, sems.at[sem])

    def start_col_blocks(src_hbm, dst_ref, i0, i1, sem, row0=0):
        src = src_hbm.bitcast(u32)
        for i in range(i0, i1):
            cp(src.at[:, i * 128:(i + 1) * 128], dst_ref.at[i, row0:], sem).start()

    def start_ssm(r0, r1, sem):
        src = ssm_hbm.bitcast(u32)
        for a in range(NCH):
            cp(src.at[r0:r1, a * C:(a + 1) * C], ssm_ref.at[a, r0:r1], sem).start()

    def wait_all(dst, sem):
        cp(dst, dst, sem).wait()

    def even(p):
        return pltpu.bitcast(p << 16, f32)

    def odd(p):
        return pltpu.bitcast(p & jnp.uint32(0xFFFF0000), f32)

    def conv_prep(cb, i, dep=None):
        r0 = KPAD + 8 * i
        p0 = k_ref[cb, r0:r0 + 8, :]
        if dep is not None:
            p0 = jnp.where(one_ref[...] == 1, p0, dep)
        p1 = k_ref[cb, r0 - 1:r0 + 7, :]
        p2 = k_ref[cb, r0 - 2:r0 + 6, :]
        pv = v_ref[cb, 8 * i:8 * i + 8, :]
        w = wt_ref[cb]
        w0, w1, w2, w3 = w[0:1, :], w[1:2, :], w[2:3, :], w[3:4, :]
        e0, o0, e1, o1, o2 = even(p0), odd(p0), even(p1), odd(p1), odd(p2)
        ke = ((e0 * w0 + o1 * w1) + e1 * w2) + o2 * w3
        ko = ((o0 * w0 + e0 * w1) + o1 * w2) + e1 * w3
        re = pltpu.bitcast((ke * even(pv)).astype(bf16).astype(f32), u32)
        ro = pltpu.bitcast((ko * odd(pv)).astype(bf16).astype(f32), u32)
        kv = (re >> 16) | ro
        u_ref[cb, 8 * i:8 * i + 8, :] = kv
        return kv

    def combine(kf, prev):
        out = []
        for g in range(8):
            o = 32 * g
            out += [kf[o:o + 8] + prev[o + 8:o + 16], kf[o + 8:o + 16] - prev[o:o + 8],
                    kf[o + 16:o + 24] - prev[o + 24:o + 32], kf[o + 24:o + 32] + prev[o + 16:o + 24]]
        return jnp.concatenate(out, axis=0)

    def conv_fwd(cb, r):
        slot = cb % 2
        rows = pl.ds(pl.multiple_of(cb * 64, 64), 64)
        f = f_ref[...]
        kfs = []
        for a in (2 * r, 2 * r + 1):
            fu_ref[slot, NZ + a] = _dot(f, _as_bf16(u_ref[cb, pl.ds(pl.multiple_of(a * 64, 64), 64), :]))
            kfs.append(_dot_nt(f, _as_bf16(ssm_ref[a, rows, :])))
        fk_ref[slot, 2 * r] = combine(kfs[0], jnp.where(r > 0, kraw_ref[...], 0.0))
        fk_ref[slot, 2 * r + 1] = combine(kfs[1], kfs[0])
        kraw_ref[...] = kfs[1]

    def conv_mac(slot, a, nterms, pos, dep=None):
        rows = slice(pos * 16, pos * 16 + 16)
        p = q = None
        for c in range(nterms):
            u = fu_ref[slot, NZ + a - c, rows, :]
            k = fk_ref[slot, c, rows, :]
            ua, ub, kc, kd = u[0:8], u[8:16], k[0:8], k[8:16]
            if c == 0 and dep is not None:
                ua = jnp.where(one_ref[...] == 1, ua, pltpu.bitcast(dep, f32))
            p = (ua * kc if p is None else p + ua * kc) - ub * kd
            q = (ua * kd if q is None else q + ua * kd) + ub * kc
        return pltpu.bitcast(jnp.concatenate([p, q], axis=0).astype(bf16), u32)

    def conv_inv(a_ref, cb, dst, a, zs):
        rows = pl.ds(pl.multiple_of(a * 64, 64), 64)
        y = _dot(g_ref[...], _as_bf16(jnp.concatenate(zs, axis=0)))
        kv = _as_bf16(u_ref[cb, rows, :]).astype(f32)
        q = _as_bf16(x_ref[cb, rows, :]).astype(f32)
        a_ref[dst, pl.ds(pl.multiple_of(a * C, C), C), :] = q * (y + kv * wt_ref[cb, KS:KS + 1, :])

    def after(w, tok):
        if tok is None:
            return w
        return jnp.concatenate([jnp.where(one_ref[...] == 1, w[0:8], tok), w[8:]], axis=0)

    def prologue(stage_ref, acc_ref):
        st3 = stage_ref.reshape((NG + 1) * D, 8, E)
        w0 = wq_hbm.bitcast(u32)
        cp_w0b = cp(w0.at[:, 4:8, :], st3.at[NG * D:(NG + 1) * D, 4:8, :], SEM_W)

        def start_w(g):
            r0 = (g % 2) * 8
            cp(w_hbm[g // 2].bitcast(u32).at[:, r0:r0 + 8, :], st3.at[g * D:(g + 1) * D], SEM_W + g).start()

        small = [cp(shift_hbm, shift_ref, SEM_SMALL), cp(d_hbm, d_ref, SEM_SMALL), cp(gw_hbm, gw_ref, SEM_SMALL),
                 cp(mem_hbm, mem_ref, SEM_SMALL), cp(f_hbm, f_ref, SEM_SMALL), cp(g_hbm, g_ref, SEM_SMALL)]
        for q in range(NQ):
            cp(x3_hbm.at[:, NT:SEG, q * DQ:(q + 1) * DQ], xr_ref.at[q], SEM_XB + q).start()
            cp(w0.at[q * DQ:(q + 1) * DQ, 0:4, :], st3.at[q * DQ:(q + 1) * DQ, 0:4, :], SEM_W0 + q).start()
        for c in small:
            c.start()
        cp_w0b.start()
        for g in range(1, NG):
            start_w(g)
            if g >= 2:
                start_col_blocks(k_hbm, k_ref, 2 * g - 4, 2 * g - 2, SEM_K + g - 2, row0=KPAD)
                start_col_blocks(v_hbm, v_ref, 2 * g - 4, 2 * g - 2, SEM_V + g - 2)
        start_col_blocks(wo_hbm, wo_ref, 0, NCB, SEM_WO)
        start_col_blocks(x_hbm, x_ref, 0, NCB, SEM_X)
        fill_ref[...] = _fill_matrix()
        one_ref[...] = jnp.ones((8, 128), jnp.int32)
        k_ref[:, KPAD - 8:KPAD, :] = jnp.zeros((NCB + 1, 8, 128), u32)
        wt_ref[...] = jnp.zeros(wt_ref.shape, f32)
        kraw_ref[...] = jnp.zeros(kraw_ref.shape, f32)
        fu_ref[0, NZ - 1] = jnp.zeros((256, 128), f32)

        def clear(a, c):
            rows = pl.ds(pl.multiple_of(a * 64, 64), 64)
            k_ref[NCB, pl.ds(pl.multiple_of(KPAD + a * 64, 32), 64), :] = jnp.zeros((64, 128), u32)
            v_ref[NCB, rows, :] = jnp.zeros((64, 128), u32)
            fu_ref[1, NZ + a] = jnp.zeros((256, 128), f32)
            fk_ref[1, a] = jnp.zeros((256, 128), f32)
            fu_ref[1, a // 2, pl.ds(pl.multiple_of((a % 2) * 128, 128), 128), :] = jnp.zeros((128, 128), f32)
            acc_ref[a // 2, pl.ds(pl.multiple_of((a % 2) * 256, 256), 256), :] = jnp.zeros((256, 128), f32)
            return c
        lax.fori_loop(0, NCH, clear, 0)

        def region(i):
            return stage_ref.at[pl.ds(pl.multiple_of(i * (8 * D), 8 * D), 8 * D), :]

        def unpack_pair(w):
            return pltpu.bitcast(even(w).astype(bf16), u32), pltpu.bitcast(odd(w).astype(bf16), u32)

        def relayout(g, sub, j, chain=False):
            toks, t = [], None
            nd = 16 if chain else 256
            for blk in range(D // nd):
                w = sub[pl.ds(blk * 8 * nd + j, nd, stride=8), :]
                if chain and blk % 16 != 0:
                    w = after(w, t)
                lo, hi = unpack_pair(w)
                rows = slice(blk * nd // 2, (blk + 1) * nd // 2)
                wn_ref[g * 16 + 2 * j, rows, :] = lo
                wn_ref[g * 16 + 2 * j + 1, rows, :] = hi
                if chain:
                    t = lo | hi
                    if blk % 16 == 15:
                        toks.append(t)
            return toks

        def store_pre(idx, r1, r2):
            cc = jnp.concatenate([r1.reshape(NSEG, 8, E), r2.reshape(NSEG, 8, E)], axis=1).astype(bf16)
            pre_ref[:, idx] = pltpu.bitcast(cc, u32)

        def first(q, c):
            wait_all(xr_ref.at[q], SEM_XB + q)
            wait_all(st3.at[pl.ds(q * DQ, DQ), 0:4, :], SEM_W0 + q)
            xq = pltpu.bitcast(xr_ref[q].astype(f32).reshape(NSEG * M, DQ).astype(bf16), u32)
            xb_ref[q] = xq
            sub = stage_ref.at[pl.ds(pl.multiple_of(q * (8 * DQ), 8 * DQ), 8 * DQ), :]
            rows = pl.ds(pl.multiple_of(q * (DQ // 2), DQ // 2), DQ // 2)
            for j in range(4):
                rs = []
                for h, w in zip((2 * j, 2 * j + 1), unpack_pair(sub[pl.ds(j, DQ, stride=8), :])):
                    wn_ref[h, rows, :] = w
                    r = _dot(_as_bf16(xq), _as_bf16(w)) + acc_ref[h]
                    acc_ref[h] = r
                    rs.append(r)
                store_pre(j, *rs)
            return c
        lax.fori_loop(0, NQ, first, 0)
        start_ssm(0, 64, SEM_SSM0)

        for c in small:
            c.wait()
        sh = shift_ref[...].astype(f32)
        dv = d_ref[...].astype(f32)
        for n in range(NCB):
            wt_ref[n, 0:KS, :] = sh[:, n * 128:(n + 1) * 128]
            wt_ref[n, KS:KS + 1, :] = dv[n:n + 1, :]
        cp_w0b.wait()
        relayout(0, region(NG), 4)

        def pair(g, j, toks):
            xb = _as_bf16(jnp.concatenate([xb_ref[q] for q in range(NQ)], axis=1))
            rs = []
            for i in range(2):
                w = wn_ref[g * 16 + 2 * j + i]
                tiles = [w[64 * k:64 * (k + 1)] for k in range(8)]
                for rnd in range(2):
                    for k, t in enumerate(toks[2 * i + rnd]):
                        tiles[4 * rnd + k] = after(tiles[4 * rnd + k], t)
                rs.append(_dot(xb, _as_bf16(jnp.concatenate(tiles, axis=0))))
            store_pre(g * 8 + j, *rs)

        def group(g, c):
            @pl.when(g > 0)
            def _():
                wait_all(st3.at[pl.ds(g * D, D)], SEM_W + g)

                @pl.when(g >= 2)
                def _():
                    wait_all(k_ref.at[pl.ds(2 * g - 4, 2), KPAD:], SEM_K + g - 2)
                    wait_all(v_ref.at[pl.ds(2 * g - 4, 2)], SEM_V + g - 2)
                cbs = [jnp.where(g >= 2, 2 * g - 4 + i, NCB) for i in range(2)]
                toks = [[] for _ in range(16)]
                for k in range(15):
                    t = None
                    for i in range(k * 256 // 15, (k + 1) * 256 // 15):
                        t = conv_prep(cbs[i // 128], i % 128, t)
                    toks[k + 1].append(t)
                sub = region(g)
                relayout(g, sub, 0)
                for j in range(4):
                    rt = relayout(g, sub, j + 1, chain=(j == 3))
                    for i, t in enumerate(rt):
                        toks[12 + i].append(t)
                    pair(g, j, toks[4 * j:4 * j + 4])

            sub = region(jnp.where(g == 0, NG, g))
            for j in range(4, 8):
                if j + 1 < 8:
                    relayout(g, sub, j + 1)
                pair(g, j, [[]] * 4)
            return c
        lax.fori_loop(0, NG, group, 0)

    pl.run_scoped(prologue, pltpu.VMEM(((NG + 1) * 8 * D, E), u32), pltpu.VMEM((8, NSEG * M, E), f32))

    start_ssm(64, D // 2, SEM_SSM1)
    wait_all(wo_ref, SEM_WO)
    wait_all(x_ref, SEM_X)
    wait_all(ssm_ref.at[:, 0:64], SEM_SSM0)

    scale = E ** -0.5

    def main(odef_ref, b_ref, a_ref):
        def step(s, mem, t):
            cfg = CFG
            cb = s // 8
            r = s % 8
            icb = jnp.maximum(cb - 1, 0)
            idst = jnp.where(cb >= 1, cb - 1, NCB)
            mslot = (cb + 1) % 2
            nh = 8 // UNROLL
            chunks = ((nh * t + r // UNROLL, nh * t + nh), (NCH - 1 - nh * t - r // UNROLL, NCH - nh * t))
            zs = ({}, {})

            xrows = pl.ds(pl.multiple_of(s * 16, 16), 16)
            xs = [_as_bf16(x_ref[n, xrows, :]).astype(f32) for n in range(NCB)]
            h32 = jnp.concatenate([jnp.concatenate(xs, axis=1)[0:NT], mem], axis=0).astype(bf16)
            r0 = pl.multiple_of(s * 8, 8)

            def gate(dep):
                gw = gw_ref[...].astype(f32)
                gl = None
                for n in range(NCB):
                    xg = _as_bf16(x_ref[n, xrows, :]).astype(f32) * gw[n:n + 1, :]
                    gl = xg if gl is None else gl + xg
                g = jnp.broadcast_to(jax.nn.sigmoid(jnp.sum(gl, axis=-1, keepdims=True)), (SEG, 128))
                gate_ref[s] = g
                g = pltpu.bitcast(g, u32)
                return (g[0:8] | g[8:16]) | (g[16:24] | g[24:32])

            jobs = []

            def mac_job(dep, w, pos):
                zs[w][pos] = conv_mac(mslot, chunks[w][0], chunks[w][1], pos, dep)
                return zs[w][pos]

            for i in range(32):
                due = cfg["dues"][i]
                start = max(due - cfg["maclag"], 0)
                jobs.append((start, due - start, False, functools.partial(mac_job, w=i % 2, pos=i // 2)))
            jobs.append((cfg["gate"], 4, False, gate))
            state = dict(count=0, due={})

            def sdot(lhs, w, acc=None, weight=1):
                c = state["count"]
                toks = [t for cc in range(c, c + weight) for t in state["due"].pop(cc, [])]
                nt = w.shape[0] // 64
                if toks:
                    tiles = [w[64 * i:64 * (i + 1)] for i in range(nt)]
                    for i, t in enumerate(toks):
                        tiles[i % nt] = after(tiles[i % nt], t)
                    w = jnp.concatenate(tiles, axis=0)
                d = _dot(lhs, _as_bf16(w))
                d = d if acc is None else d + acc
                for (st, lag, rel, fn) in jobs:
                    if c <= st < c + weight:
                        tok = fn(pltpu.bitcast(d[0:8], u32) if rel else None)
                        state["due"].setdefault(max(st + lag, c + weight), []).append(tok)
                state["count"] = c + weight
                return d

            def proj(m, j):
                r1 = sdot(h32, wn_ref[m * H + 2 * j], weight=4)
                r2 = sdot(h32, wn_ref[m * H + 2 * j + 1], weight=4)
                p = _as_bf16(pre_ref[s, m * NP + j]).astype(f32)
                if m == 0:
                    return jnp.concatenate([r1, r2, p], axis=0)
                return jnp.concatenate([r1, r2, p, jnp.zeros((48, E), f32)], axis=0).astype(bf16)

            def split_rows(dot, lhs, rhs, split):
                if not split:
                    return dot(lhs.astype(bf16), rhs)
                return jnp.concatenate([dot(lhs[0:48].astype(bf16), rhs), dot(lhs[48:80].astype(bf16), rhs)], axis=0)

            def qk(q80, k80, split=False):
                fill = fill_ref[...]
                sc = jnp.where(fill == 0.0, split_rows(_dot_nt, q80, k80, split), fill)
                p = jnp.exp2((sc - jnp.max(sc, axis=-1, keepdims=True)) * (scale * LOG2E))
                den = jnp.sum(p, axis=-1, keepdims=True)
                rc = pl.reciprocal(den, approx=True)
                return p * (rc * (2.0 - den * rc))

            def pv(j, p, v80, split=False):
                o80 = split_rows(_dot, p, v80, split)
                odef_ref[pl.ds(r0, 8), (2 * j) * E:(2 * j + 1) * E] = o80[64:72]
                odef_ref[pl.ds(r0, 8), (2 * j + 1) * E:(2 * j + 2) * E] = o80[72:80]
                return jnp.concatenate([o80[0:32], o80[32:64]], axis=1).astype(bf16)

            def wo_part(o, j0, j1, n, acc=None):
                for j in range(j0, j1):
                    acc = sdot(o[j], wo_ref[n, j * 128:(j + 1) * 128, :], acc)
                return acc

            qs, ks, vs, ps, os_ = {}, {}, {}, {}, {}
            for j in range(0, NP, 2):
                for m, jj in cfg["order"]:
                    (qs, ks, vs)[m][j + jj] = proj(m, j + jj)
                ps[j] = qk(qs[j], ks[j], j == 0 and cfg["split0"])
                ps[j + 1] = qk(qs[j + 1], ks[j + 1], j == 0 and cfg["split0"])
                if j >= 2:
                    os_[j - 2] = pv(j - 2, ps[j - 2], vs[j - 2])
                    os_[j - 1] = pv(j - 1, ps[j - 1], vs[j - 1])
            na = NP - 2
            acc = {}
            nw = cfg["nw"]
            for n in range(nw):
                acc[n] = wo_part(os_, 0, na, n)
            os_[NP - 2] = pv(NP - 2, ps[NP - 2], vs[NP - 2], cfg["split1"])
            os_[NP - 1] = pv(NP - 1, ps[NP - 1], vs[NP - 1], cfg["split1"])
            acc[nw] = wo_part(os_, 0, na, nw)
            for n in range(nw + 1):
                acc[n] = wo_part(os_, na, NP, n, acc[n])
            for n in range(nw + 1, 8):
                acc[n] = wo_part(os_, 0, NP, n)
            assert state["count"] == 512 and not state["due"], state
            for w in range(2):
                conv_inv(a_ref, icb, idst, chunks[w][0], [zs[w][pos] for pos in range(16)])
            if t == UNROLL - 1:
                for tt in range(UNROLL):
                    conv_fwd(cb, r - t + tt)
            for n in range(NCB):
                b_ref[n, s, 0:NT, :] = acc[n][0:NT]
            return jnp.concatenate([acc[n][NT:SEG] for n in range(NCB)], axis=1).astype(bf16).astype(f32)

        def steps(i, mem):
            @pl.when(i == 8 // UNROLL)
            def _():
                wait_all(ssm_ref.at[:, 64:], SEM_SSM1)
            for t in range(UNROLL):
                mem = step(i * UNROLL + t, mem, t)
            return mem

        lax.fori_loop(0, _DBG_STEPS // UNROLL, steps, mem_ref[...].astype(f32))

        def out_copy(n):
            slot = n % 2
            return pltpu.make_async_copy(
                ost_ref.at[slot], out_hbm.at[:, :, pl.ds(pl.multiple_of(n * 128, 128), 128)],
                sems.at[SEM_OUT + slot])

        def fin(n, c):
            @pl.when(n >= 2)
            def _():
                out_copy(n - 2).wait()
            zs, toks, t = ([], []), [], None
            for pos in range(16):
                if pos % CFG["fgrp"] == 0:
                    t = None
                for w in range(2):
                    t = conv_mac((NCB - 1) % 2, n + 8 * w, 8 + 8 * w, pos, t)
                    zs[w].append(t)
                if pos % CFG["fgrp"] == CFG["fgrp"] - 1:
                    toks.append(t)
            bd = None
            for kb in range(8):
                if kb == CFG["finv"]:
                    for w in range(2):
                        conv_inv(a_ref, NCB - 1, NCB - 1, n + 8 * w, zs[w])
                w = after(wo_ref[n, kb * 256:(kb + 1) * 256, :], toks[kb - 1] if 0 < kb <= len(toks) else None)
                d = _dot(odef_ref[:, kb * 512:(kb + 1) * 512].astype(bf16), _as_bf16(w))
                bd = d if bd is None else d + bd
            b_ref[n, :, NT:SEG, :] = bd.reshape(NSEG, 8, 128)
            for blk in range(8):
                sg = slice(blk * 8, (blk + 1) * 8)
                b = b_ref[n, sg]
                a = a_ref[n, blk * 256:(blk + 1) * 256, :].reshape(8, SEG, 128)
                g = gate_ref[sg]
                ost_ref[n % 2, sg] = (g * a + (1.0 - g) * b).astype(bf16)
            out_copy(n).start()
            return c
        lax.fori_loop(0, NCB, fin, 0)
        out_copy(NCB - 2).wait()
        out_copy(NCB - 1).wait()

    pl.run_scoped(main, pltpu.VMEM((NSEG * 8, H * E), f32), pltpu.VMEM((NCB, NSEG, SEG, 128), f32),
                  pltpu.VMEM((NCB + 1, S, 128), f32))


@jax.jit
def pallas_gated_mix__ssm_conv_h3__memory_aug_recurrent_mem_tr__prompt_kernel(
    A_q: jax.Array,
    A_k: jax.Array,
    A_v: jax.Array,
    A_shift_k: jax.Array,
    A_ssm_k: jax.Array,
    A_ssm_D: jax.Array,
    B_x: jax.Array,
    B_mem0: jax.Array,
    B_Wq: jax.Array,
    B_Wk: jax.Array,
    B_Wv: jax.Array,
    B_Wo: jax.Array,
    B_seg_len: jax.Array,
    gate_w: jax.Array,
):
    del B_x, B_seg_len
    f_tab, g_tab = _dft_tables()
    out = pl.pallas_call(
        _kernel,
        out_shape=jax.ShapeDtypeStruct((NSEG, SEG, D), bf16),
        in_specs=[pl.BlockSpec(memory_space=pl.ANY)] * 15,
        out_specs=pl.BlockSpec(memory_space=pl.ANY),
        scratch_shapes=[
            pltpu.VMEM((3 * H, D // 2, E), u32),
            pltpu.VMEM((NCB, H * E // 2, 128), u32),
            pltpu.VMEM((NCB, S // 2, 128), u32),
            pltpu.VMEM((NQ, NSEG, M, DQ), bf16),
            pltpu.VMEM((NQ, NSEG * 4, DQ), u32),
            pltpu.VMEM((NSEG, 3 * NP, 8, E), u32),
            pltpu.VMEM((NCB + 1, KPAD + S // 2, 128), u32),
            pltpu.VMEM((NCB + 1, S // 2, 128), u32),
            pltpu.VMEM((NCH, D // 2, 128), u32),
            pltpu.VMEM((NCB + 1, S // 2, 128), u32),
            pltpu.VMEM((2, NZ + NCH, 256, 128), f32),
            pltpu.VMEM((2, NCH, 256, 128), f32),
            pltpu.VMEM((256, 128), f32),
            pltpu.VMEM((8, 128), jnp.int32),
            pltpu.VMEM((256, 128), bf16),
            pltpu.VMEM((128, 256), bf16),
            pltpu.VMEM((80, 128), f32),
            pltpu.VMEM((KS, D), bf16),
            pltpu.VMEM((NCB + 1, 8, 128), f32),
            pltpu.VMEM((NCB, 128), bf16),
            pltpu.VMEM((NCB, 128), bf16),
            pltpu.VMEM((M, D), bf16),
            pltpu.VMEM((NSEG, SEG, 128), f32),
            pltpu.VMEM((2, NSEG, SEG, 128), bf16),
            pltpu.SemaphoreType.DMA((NSEM,)),
        ],
        compiler_params=pltpu.CompilerParams(vmem_limit_bytes=120 * 2**20),
    )(A_q.reshape(NSEG, SEG, D), A_q.reshape(S, D), A_k.reshape(S, D), A_v.reshape(S, D), A_shift_k.T,
      A_ssm_k, A_ssm_D.reshape(NCB, 128), B_mem0.reshape(M, D), B_Wq, B_Wk, B_Wv,
      B_Wo.reshape(H * E, D), gate_w.reshape(NCB, 128), f_tab, g_tab)
    return out.reshape(1, S, D)
```

```python
import functools

import numpy as np
import jax
import jax.numpy as jnp
from jax import lax
import jax.experimental.pallas as pl
import jax.experimental.pallas.tpu as pltpu

S, D, H, E, M, SEG = 2048, 1024, 32, 128, 8, 32
NSEG = S // SEG
NT = SEG - M
NP = H // 2
NCB = D // 128
C = 128
NCH = S // C
LOG2E = 1.4426950408889634
KS = 4
NZ = 8
KPAD = 32
NG = 6
NQ = 4
DQ = D // NQ
UNROLL = 4
CFG = dict(rl=8, fgrp=4, finv=4, dues=[12, 16, 20, 24, 28, 32, 36, 40, 44] + [48 * p + 40 for p in range(1, 8)] + [444 + 4 * i for i in range(16)], maclag=4, gate=436,
           split=((32, 32, 32, 32),) * 4, nw=3, order=((0, 0), (1, 0), (0, 1), (1, 1), (2, 0), (2, 1)))
_DBG_STEPS = NSEG
bf16, f32, u32 = jnp.bfloat16, jnp.float32, jnp.uint32


def _dft_tables():
    t = np.arange(C, dtype=np.float64)
    rows = []
    for r in range(8):
        ev = 16 * r + np.arange(0, 16, 2)
        od = ev + 1
        for fn, fs in ((np.cos, ev), (np.sin, ev), (np.cos, od), (np.sin, od)):
            rows.append(fn(np.pi * (2 * fs[:, None] + 1) * t[None, :] / (2 * C)))
    f = np.concatenate(rows, axis=0)
    return f.astype(bf16), (f.T / C).astype(bf16)


def _fill_matrix():
    r = lax.broadcasted_iota(jnp.int32, (80, 128), 0)
    c = lax.broadcasted_iota(jnp.int32, (80, 128), 1)

    def head(i):
        return jnp.where(i < 64, i // 32, (i - 64) // 8)

    def idx(i):
        lo = i % 32
        main = jnp.where(lo < NT, lo + M, lo - NT)
        return jnp.where(i < 64, main, (i - 64) % 8 + NT + M)

    same = (head(r) == head(c)) & (c < 80)
    ok = (idx(r) < M) | (idx(r) >= idx(c))
    return jnp.where(same, jnp.where(ok, 0.0, -1e9 * E ** 0.5), -jnp.inf).astype(f32)


def _as_bf16(v):
    return pltpu.bitcast(v, bf16)


def _dot(a, b):
    return jnp.dot(a, b, preferred_element_type=f32)


def _dot_nt(a, b):
    return lax.dot_general(a, b, (((1,), (1,)), ((), ())), preferred_element_type=f32)


SEM_SMALL, SEM_WO, SEM_X, SEM_SSM0, SEM_SSM1 = range(5)
SEM_XB = 5
SEM_W0 = SEM_XB + NQ
SEM_K = SEM_W0 + NQ
SEM_V = SEM_K + 4
SEM_W = SEM_V + 4
SEM_OUT = SEM_W + NG
NSEM = SEM_OUT + 2


def _kernel(x3_hbm, x_hbm, k_hbm, v_hbm, shift_hbm, ssm_hbm, d_hbm, mem_hbm, wq_hbm, wk_hbm, wv_hbm,
            wo_hbm, gw_hbm, f_hbm, g_hbm, out_hbm,
            wn_ref, wo_ref, x_ref, xr_ref, xb_ref, pre_ref, k_ref, v_ref, ssm_ref, u_ref,
            fu_ref, fk_ref, kraw_ref, one_ref, f_ref, g_ref, fill_ref, shift_ref, wt_ref,
            d_ref, gw_ref, mem_ref, gate_ref, ost_ref, sems):
    w_hbm = (wq_hbm, wk_hbm, wv_hbm)

    def cp(src, dst, sem):
        return pltpu.make_async_copy(src, dst, sems.at[sem])

    def start_col_blocks(src_hbm, dst_ref, i0, i1, sem, row0=0):
        src = src_hbm.bitcast(u32)
        for i in range(i0, i1):
            cp(src.at[:, i * 128:(i + 1) * 128], dst_ref.at[i, row0:], sem).start()

    def start_ssm(r0, r1, sem):
        src = ssm_hbm.bitcast(u32)
        for a in range(NCH):
            cp(src.at[r0:r1, a * C:(a + 1) * C], ssm_ref.at[a, r0:r1], sem).start()

    def wait_all(dst, sem):
        cp(dst, dst, sem).wait()

    def even(p):
        return pltpu.bitcast(p << 16, f32)

    def odd(p):
        return pltpu.bitcast(p & jnp.uint32(0xFFFF0000), f32)

    def conv_prep(cb, i, dep=None):
        r0 = KPAD + 8 * i
        p0 = k_ref[cb, r0:r0 + 8, :]
        if dep is not None:
            p0 = jnp.where(one_ref[...] == 1, p0, dep)
        p1 = k_ref[cb, r0 - 1:r0 + 7, :]
        p2 = k_ref[cb, r0 - 2:r0 + 6, :]
        pv = v_ref[cb, 8 * i:8 * i + 8, :]
        w = wt_ref[cb]
        w0, w1, w2, w3 = w[0:1, :], w[1:2, :], w[2:3, :], w[3:4, :]
        e0, o0, e1, o1, o2 = even(p0), odd(p0), even(p1), odd(p1), odd(p2)
        ke = ((e0 * w0 + o1 * w1) + e1 * w2) + o2 * w3
        ko = ((o0 * w0 + e0 * w1) + o1 * w2) + e1 * w3
        re = pltpu.bitcast((ke * even(pv)).astype(bf16).astype(f32), u32)
        ro = pltpu.bitcast((ko * odd(pv)).astype(bf16).astype(f32), u32)
        kv = (re >> 16) | ro
        u_ref[cb, 8 * i:8 * i + 8, :] = kv
        return kv

    def combine(kf, prev):
        out = []
        for g in range(8):
            o = 32 * g
            out += [kf[o:o + 8] + prev[o + 8:o + 16], kf[o + 8:o + 16] - prev[o:o + 8],
                    kf[o + 16:o + 24] - prev[o + 24:o + 32], kf[o + 24:o + 32] + prev[o + 16:o + 24]]
        return jnp.concatenate(out, axis=0)

    def conv_fwd(cb, r):
        slot = cb % 2
        rows = pl.ds(pl.multiple_of(cb * 64, 64), 64)
        f = f_ref[...]
        kfs = []
        for a in (2 * r, 2 * r + 1):
            fu_ref[slot, NZ + a] = _dot(f, _as_bf16(u_ref[cb, pl.ds(pl.multiple_of(a * 64, 64), 64), :]))
            kfs.append(_dot_nt(f, _as_bf16(ssm_ref[a, rows, :])))
        fk_ref[slot, 2 * r] = combine(kfs[0], jnp.where(r > 0, kraw_ref[...], 0.0))
        fk_ref[slot, 2 * r + 1] = combine(kfs[1], kfs[0])
        kraw_ref[...] = kfs[1]

    def conv_mac(slot, a, nterms, pos, dep=None):
        rows = slice(pos * 16, pos * 16 + 16)
        p = q = None
        for c in range(nterms):
            u = fu_ref[slot, NZ + a - c, rows, :]
            k = fk_ref[slot, c, rows, :]
            ua, ub, kc, kd = u[0:8], u[8:16], k[0:8], k[8:16]
            if c == 0 and dep is not None:
                ua = jnp.where(one_ref[...] == 1, ua, pltpu.bitcast(dep, f32))
            p = (ua * kc if p is None else p + ua * kc) - ub * kd
            q = (ua * kd if q is None else q + ua * kd) + ub * kc
        return pltpu.bitcast(jnp.concatenate([p, q], axis=0).astype(bf16), u32)

    def conv_inv(a_ref, cb, dst, a, zs):
        rows = pl.ds(pl.multiple_of(a * 64, 64), 64)
        y = _dot(g_ref[...], _as_bf16(jnp.concatenate(zs, axis=0)))
        kv = _as_bf16(u_ref[cb, rows, :]).astype(f32)
        q = _as_bf16(x_ref[cb, rows, :]).astype(f32)
        a_ref[dst, pl.ds(pl.multiple_of(a * C, C), C), :] = q * (y + kv * wt_ref[cb, KS:KS + 1, :])

    def after(w, tok):
        if tok is None:
            return w
        return jnp.concatenate([jnp.where(one_ref[...] == 1, w[0:8], tok), w[8:]], axis=0)

    def prologue(stage_ref, acc_ref):
        st3 = stage_ref.reshape((NG + 1) * D, 8, E)
        w0 = wq_hbm.bitcast(u32)
        cp_w0b = cp(w0.at[:, 4:8, :], st3.at[NG * D:(NG + 1) * D, 4:8, :], SEM_W)

        def start_w(g):
            r0 = (g % 2) * 8
            cp(w_hbm[g // 2].bitcast(u32).at[:, r0:r0 + 8, :], st3.at[g * D:(g + 1) * D], SEM_W + g).start()

        small = [cp(shift_hbm, shift_ref, SEM_SMALL), cp(d_hbm, d_ref, SEM_SMALL), cp(gw_hbm, gw_ref, SEM_SMALL),
                 cp(mem_hbm, mem_ref, SEM_SMALL), cp(f_hbm, f_ref, SEM_SMALL), cp(g_hbm, g_ref, SEM_SMALL)]
        for q in range(NQ):
            cp(x3_hbm.at[:, NT:SEG, q * DQ:(q + 1) * DQ], xr_ref.at[q], SEM_XB + q).start()
            cp(w0.at[q * DQ:(q + 1) * DQ, 0:4, :], st3.at[q * DQ:(q + 1) * DQ, 0:4, :], SEM_W0 + q).start()
        for c in small:
            c.start()
        cp_w0b.start()
        for g in range(1, NG):
            start_w(g)
            if g >= 2:
                start_col_blocks(k_hbm, k_ref, 2 * g - 4, 2 * g - 2, SEM_K + g - 2, row0=KPAD)
                start_col_blocks(v_hbm, v_ref, 2 * g - 4, 2 * g - 2, SEM_V + g - 2)
        start_col_blocks(wo_hbm, wo_ref, 0, NCB, SEM_WO)
        start_col_blocks(x_hbm, x_ref, 0, NCB, SEM_X)
        fill_ref[...] = _fill_matrix()
        one_ref[...] = jnp.ones((8, 128), jnp.int32)
        k_ref[:, KPAD - 8:KPAD, :] = jnp.zeros((NCB + 1, 8, 128), u32)
        wt_ref[...] = jnp.zeros(wt_ref.shape, f32)
        kraw_ref[...] = jnp.zeros(kraw_ref.shape, f32)
        fu_ref[0, NZ - 1] = jnp.zeros((256, 128), f32)

        def clear(a, c):
            rows = pl.ds(pl.multiple_of(a * 64, 64), 64)
            k_ref[NCB, pl.ds(pl.multiple_of(KPAD + a * 64, 32), 64), :] = jnp.zeros((64, 128), u32)
            v_ref[NCB, rows, :] = jnp.zeros((64, 128), u32)
            fu_ref[1, NZ + a] = jnp.zeros((256, 128), f32)
            fk_ref[1, a] = jnp.zeros((256, 128), f32)
            fu_ref[1, a // 2, pl.ds(pl.multiple_of((a % 2) * 128, 128), 128), :] = jnp.zeros((128, 128), f32)
            acc_ref[a // 2, pl.ds(pl.multiple_of((a % 2) * 256, 256), 256), :] = jnp.zeros((256, 128), f32)
            return c
        lax.fori_loop(0, NCH, clear, 0)

        def region(i):
            return stage_ref.at[pl.ds(pl.multiple_of(i * (8 * D), 8 * D), 8 * D), :]

        def unpack_pair(w):
            return pltpu.bitcast(even(w).astype(bf16), u32), pltpu.bitcast(odd(w).astype(bf16), u32)

        def relayout(g, sub, j, chain=False):
            toks, t = [], None
            nd = 16 if chain else 256
            for blk in range(D // nd):
                w = sub[pl.ds(blk * 8 * nd + j, nd, stride=8), :]
                if chain and blk % CFG["rl"] != 0:
                    w = after(w, t)
                lo, hi = unpack_pair(w)
                rows = slice(blk * nd // 2, (blk + 1) * nd // 2)
                wn_ref[g * 16 + 2 * j, rows, :] = lo
                wn_ref[g * 16 + 2 * j + 1, rows, :] = hi
                if chain:
                    t = lo | hi
                    if blk % CFG["rl"] == CFG["rl"] - 1:
                        toks.append(t)
            return toks

        def store_pre(idx, r1, r2):
            cc = jnp.concatenate([r1.reshape(NSEG, 8, E), r2.reshape(NSEG, 8, E)], axis=1).astype(bf16)
            pre_ref[:, idx] = pltpu.bitcast(cc, u32)

        def first(q, c):
            wait_all(xr_ref.at[q], SEM_XB + q)
            wait_all(st3.at[pl.ds(q * DQ, DQ), 0:4, :], SEM_W0 + q)
            xq = pltpu.bitcast(xr_ref[q].astype(f32).reshape(NSEG * M, DQ).astype(bf16), u32)
            xb_ref[q] = xq
            sub = stage_ref.at[pl.ds(pl.multiple_of(q * (8 * DQ), 8 * DQ), 8 * DQ), :]
            rows = pl.ds(pl.multiple_of(q * (DQ // 2), DQ // 2), DQ // 2)
            for j in range(4):
                rs = []
                for h, w in zip((2 * j, 2 * j + 1), unpack_pair(sub[pl.ds(j, DQ, stride=8), :])):
                    wn_ref[h, rows, :] = w
                    r = _dot(_as_bf16(xq), _as_bf16(w)) + acc_ref[h]
                    acc_ref[h] = r
                    rs.append(r)
                store_pre(j, *rs)
            return c
        lax.fori_loop(0, NQ, first, 0)
        start_ssm(0, 64, SEM_SSM0)

        for c in small:
            c.wait()
        sh = shift_ref[...].astype(f32)
        dv = d_ref[...].astype(f32)
        for n in range(NCB):
            wt_ref[n, 0:KS, :] = sh[:, n * 128:(n + 1) * 128]
            wt_ref[n, KS:KS + 1, :] = dv[n:n + 1, :]
        cp_w0b.wait()
        relayout(0, region(NG), 4)

        def pair(g, j, toks):
            xb = _as_bf16(jnp.concatenate([xb_ref[q] for q in range(NQ)], axis=1))
            rs = []
            for i in range(2):
                w = wn_ref[g * 16 + 2 * j + i]
                tiles = [w[64 * k:64 * (k + 1)] for k in range(8)]
                for rnd in range(2):
                    for k, t in enumerate(toks[2 * i + rnd]):
                        tiles[4 * rnd + k] = after(tiles[4 * rnd + k], t)
                rs.append(_dot(xb, _as_bf16(jnp.concatenate(tiles, axis=0))))
            store_pre(g * 8 + j, *rs)

        def group(g, c):
            @pl.when(g > 0)
            def _():
                wait_all(st3.at[pl.ds(g * D, D)], SEM_W + g)

                @pl.when(g >= 2)
                def _():
                    wait_all(k_ref.at[pl.ds(2 * g - 4, 2), KPAD:], SEM_K + g - 2)
                    wait_all(v_ref.at[pl.ds(2 * g - 4, 2)], SEM_V + g - 2)
                cbs = [jnp.where(g >= 2, 2 * g - 4 + i, NCB) for i in range(2)]
                toks = [[] for _ in range(16)]
                for k in range(15):
                    t = None
                    for i in range(k * 256 // 15, (k + 1) * 256 // 15):
                        t = conv_prep(cbs[i // 128], i % 128, t)
                    toks[k + 1].append(t)
                sub = region(g)
                relayout(g, sub, 0)
                rt = relayout(g, sub, 4, chain=True)
                for i, t in enumerate(rt):
                    toks[16 - len(rt) + i].append(t)
                for j in range(4):
                    if j < 3:
                        relayout(g, sub, j + 1)
                    pair(g, j, toks[4 * j:4 * j + 4])

            sub = region(jnp.where(g == 0, NG, g))
            for j in range(4, 8):
                if j + 1 < 8:
                    relayout(g, sub, j + 1)
                pair(g, j, [[]] * 4)
            return c
        lax.fori_loop(0, NG, group, 0)

    pl.run_scoped(prologue, pltpu.VMEM(((NG + 1) * 8 * D, E), u32), pltpu.VMEM((8, NSEG * M, E), f32))

    start_ssm(64, D // 2, SEM_SSM1)
    wait_all(wo_ref, SEM_WO)
    wait_all(x_ref, SEM_X)
    wait_all(ssm_ref.at[:, 0:64], SEM_SSM0)

    scale = E ** -0.5

    def main(odef_ref, b_ref, a_ref):
        def step(s, mem, t):
            cfg = CFG
            cb = s // 8
            r = s % 8
            icb = jnp.maximum(cb - 1, 0)
            idst = jnp.where(cb >= 1, cb - 1, NCB)
            mslot = (cb + 1) % 2
            nh = 8 // UNROLL
            chunks = ((nh * t + r // UNROLL, nh * t + nh), (NCH - 1 - nh * t - r // UNROLL, NCH - nh * t))
            zs = ({}, {})

            xrows = pl.ds(pl.multiple_of(s * 16, 16), 16)
            xs = [_as_bf16(x_ref[n, xrows, :]).astype(f32) for n in range(NCB)]
            h32 = jnp.concatenate([jnp.concatenate(xs, axis=1)[0:NT], mem], axis=0).astype(bf16)
            r0 = pl.multiple_of(s * 8, 8)

            def gate(dep):
                gw = gw_ref[...].astype(f32)
                gl = None
                for n in range(NCB):
                    xg = _as_bf16(x_ref[n, xrows, :]).astype(f32) * gw[n:n + 1, :]
                    gl = xg if gl is None else gl + xg
                g = jnp.broadcast_to(jax.nn.sigmoid(jnp.sum(gl, axis=-1, keepdims=True)), (SEG, 128))
                gate_ref[s] = g
                g = pltpu.bitcast(g, u32)
                return (g[0:8] | g[8:16]) | (g[16:24] | g[24:32])

            jobs = []

            def mac_job(dep, w, pos):
                zs[w][pos] = conv_mac(mslot, chunks[w][0], chunks[w][1], pos, dep)
                return zs[w][pos]

            for i in range(32):
                due = cfg["dues"][i]
                start = max(due - cfg["maclag"], 0)
                jobs.append((start, due - start, False, functools.partial(mac_job, w=i % 2, pos=i // 2)))
            jobs.append((cfg["gate"], 4, False, gate))
            state = dict(count=0, due={})

            def sdot(lhs, w, acc=None, weight=1):
                c = state["count"]
                toks = [t for cc in range(c, c + weight) for t in state["due"].pop(cc, [])]
                nt = w.shape[0] // 64
                if toks:
                    tiles = [w[64 * i:64 * (i + 1)] for i in range(nt)]
                    for i, t in enumerate(toks):
                        tiles[i % nt] = after(tiles[i % nt], t)
                    w = jnp.concatenate(tiles, axis=0)
                d = _dot(lhs, _as_bf16(w))
                d = d if acc is None else d + acc
                for (st, lag, rel, fn) in jobs:
                    if c <= st < c + weight:
                        tok = fn(pltpu.bitcast(d[0:8], u32) if rel else None)
                        state["due"].setdefault(max(st + lag, c + weight), []).append(tok)
                state["count"] = c + weight
                return d

            def proj(m, j):
                r1 = sdot(h32, wn_ref[m * H + 2 * j], weight=4)
                r2 = sdot(h32, wn_ref[m * H + 2 * j + 1], weight=4)
                p = _as_bf16(pre_ref[s, m * NP + j]).astype(f32)
                if m == 0:
                    return jnp.concatenate([r1, r2, p], axis=0)
                return jnp.concatenate([r1, r2, p, jnp.zeros((48, E), f32)], axis=0).astype(bf16)

            def split_rows(dot, lhs, rhs, split):
                if not split:
                    return dot(lhs.astype(bf16), rhs)
                return jnp.concatenate([dot(lhs[0:split].astype(bf16), rhs), dot(lhs[split:].astype(bf16), rhs)], axis=0)

            def qk(q80, k80, split=False):
                fill = fill_ref[...]
                sc = jnp.where(fill == 0.0, split_rows(_dot_nt, q80, k80, split), fill)
                p = jnp.exp2((sc - jnp.max(sc, axis=-1, keepdims=True)) * (scale * LOG2E))
                den = jnp.sum(p, axis=-1, keepdims=True)
                rc = pl.reciprocal(den, approx=True)
                return p * (rc * (2.0 - den * rc))

            def pv(j, p, v80, split=False):
                o80 = split_rows(_dot, p, v80, split)
                odef_ref[pl.ds(r0, 8), (2 * j) * E:(2 * j + 1) * E] = o80[64:72]
                odef_ref[pl.ds(r0, 8), (2 * j + 1) * E:(2 * j + 2) * E] = o80[72:80]
                return jnp.concatenate([o80[0:32], o80[32:64]], axis=1).astype(bf16)

            def wo_part(o, j0, j1, n, acc=None):
                for j in range(j0, j1):
                    acc = sdot(o[j], wo_ref[n, j * 128:(j + 1) * 128, :], acc)
                return acc

            qs, ks, vs, ps, os_ = {}, {}, {}, {}, {}
            for j in range(0, NP, 2):
                for m, jj in cfg["order"]:
                    (qs, ks, vs)[m][j + jj] = proj(m, j + jj)
                ps[j] = qk(qs[j], ks[j], j == 0 and cfg["split"][t][0])
                ps[j + 1] = qk(qs[j + 1], ks[j + 1], j == 0 and cfg["split"][t][1])
                if j >= 2:
                    os_[j - 2] = pv(j - 2, ps[j - 2], vs[j - 2])
                    os_[j - 1] = pv(j - 1, ps[j - 1], vs[j - 1])
            na = NP - 2
            acc = {}
            nw = cfg["nw"]
            for n in range(nw):
                acc[n] = wo_part(os_, 0, na, n)
            os_[NP - 2] = pv(NP - 2, ps[NP - 2], vs[NP - 2], cfg["split"][t][2])
            os_[NP - 1] = pv(NP - 1, ps[NP - 1], vs[NP - 1], cfg["split"][t][3])
            acc[nw] = wo_part(os_, 0, na, nw)
            for n in range(nw + 1):
                acc[n] = wo_part(os_, na, NP, n, acc[n])
            for n in range(nw + 1, 8):
                acc[n] = wo_part(os_, 0, NP, n)
            assert state["count"] == 512 and not state["due"], state
            for w in range(2):
                conv_inv(a_ref, icb, idst, chunks[w][0], [zs[w][pos] for pos in range(16)])
            if t == UNROLL - 1:
                for tt in range(UNROLL):
                    conv_fwd(cb, r - t + tt)
            for n in range(NCB):
                b_ref[n, s, 0:NT, :] = acc[n][0:NT]
            return jnp.concatenate([acc[n][NT:SEG] for n in range(NCB)], axis=1).astype(bf16).astype(f32)

        def steps(i, mem):
            @pl.when(i == 8 // UNROLL)
            def _():
                wait_all(ssm_ref.at[:, 64:], SEM_SSM1)
            for t in range(UNROLL):
                mem = step(i * UNROLL + t, mem, t)
            return mem

        lax.fori_loop(0, _DBG_STEPS // UNROLL, steps, mem_ref[...].astype(f32))

        def out_copy(n):
            slot = n % 2
            return pltpu.make_async_copy(
                ost_ref.at[slot], out_hbm.at[:, :, pl.ds(pl.multiple_of(n * 128, 128), 128)],
                sems.at[SEM_OUT + slot])

        def fin(n, c):
            @pl.when(n >= 2)
            def _():
                out_copy(n - 2).wait()
            zs, toks, t = ([], []), [], None
            for pos in range(16):
                if pos % CFG["fgrp"] == 0:
                    t = None
                for w in range(2):
                    t = conv_mac((NCB - 1) % 2, n + 8 * w, 8 + 8 * w, pos, t)
                    zs[w].append(t)
                if pos % CFG["fgrp"] == CFG["fgrp"] - 1:
                    toks.append(t)
            bd = None
            for kb in range(8):
                if kb == CFG["finv"]:
                    for w in range(2):
                        conv_inv(a_ref, NCB - 1, NCB - 1, n + 8 * w, zs[w])
                w = after(wo_ref[n, kb * 256:(kb + 1) * 256, :], toks[kb - 1] if 0 < kb <= len(toks) else None)
                d = _dot(odef_ref[:, kb * 512:(kb + 1) * 512].astype(bf16), _as_bf16(w))
                bd = d if bd is None else d + bd
            b_ref[n, :, NT:SEG, :] = bd.reshape(NSEG, 8, 128)
            for blk in range(8):
                sg = slice(blk * 8, (blk + 1) * 8)
                b = b_ref[n, sg]
                a = a_ref[n, blk * 256:(blk + 1) * 256, :].reshape(8, SEG, 128)
                g = gate_ref[sg]
                ost_ref[n % 2, sg] = (g * a + (1.0 - g) * b).astype(bf16)
            out_copy(n).start()
            return c
        lax.fori_loop(0, NCB, fin, 0)
        out_copy(NCB - 2).wait()
        out_copy(NCB - 1).wait()

    pl.run_scoped(main, pltpu.VMEM((NSEG * 8, H * E), f32), pltpu.VMEM((NCB, NSEG, SEG, 128), f32),
                  pltpu.VMEM((NCB + 1, S, 128), f32))


@jax.jit
def pallas_gated_mix__ssm_conv_h3__memory_aug_recurrent_mem_tr__prompt_kernel(
    A_q: jax.Array,
    A_k: jax.Array,
    A_v: jax.Array,
    A_shift_k: jax.Array,
    A_ssm_k: jax.Array,
    A_ssm_D: jax.Array,
    B_x: jax.Array,
    B_mem0: jax.Array,
    B_Wq: jax.Array,
    B_Wk: jax.Array,
    B_Wv: jax.Array,
    B_Wo: jax.Array,
    B_seg_len: jax.Array,
    gate_w: jax.Array,
):
    del B_x, B_seg_len
    f_tab, g_tab = _dft_tables()
    out = pl.pallas_call(
        _kernel,
        out_shape=jax.ShapeDtypeStruct((NSEG, SEG, D), bf16),
        in_specs=[pl.BlockSpec(memory_space=pl.ANY)] * 15,
        out_specs=pl.BlockSpec(memory_space=pl.ANY),
        scratch_shapes=[
            pltpu.VMEM((3 * H, D // 2, E), u32),
            pltpu.VMEM((NCB, H * E // 2, 128), u32),
            pltpu.VMEM((NCB, S // 2, 128), u32),
            pltpu.VMEM((NQ, NSEG, M, DQ), bf16),
            pltpu.VMEM((NQ, NSEG * 4, DQ), u32),
            pltpu.VMEM((NSEG, 3 * NP, 8, E), u32),
            pltpu.VMEM((NCB + 1, KPAD + S // 2, 128), u32),
            pltpu.VMEM((NCB + 1, S // 2, 128), u32),
            pltpu.VMEM((NCH, D // 2, 128), u32),
            pltpu.VMEM((NCB + 1, S // 2, 128), u32),
            pltpu.VMEM((2, NZ + NCH, 256, 128), f32),
            pltpu.VMEM((2, NCH, 256, 128), f32),
            pltpu.VMEM((256, 128), f32),
            pltpu.VMEM((8, 128), jnp.int32),
            pltpu.VMEM((256, 128), bf16),
            pltpu.VMEM((128, 256), bf16),
            pltpu.VMEM((80, 128), f32),
            pltpu.VMEM((KS, D), bf16),
            pltpu.VMEM((NCB + 1, 8, 128), f32),
            pltpu.VMEM((NCB, 128), bf16),
            pltpu.VMEM((NCB, 128), bf16),
            pltpu.VMEM((M, D), bf16),
            pltpu.VMEM((NSEG, SEG, 128), f32),
            pltpu.VMEM((2, NSEG, SEG, 128), bf16),
            pltpu.SemaphoreType.DMA((NSEM,)),
        ],
        compiler_params=pltpu.CompilerParams(vmem_limit_bytes=120 * 2**20),
    )(A_q.reshape(NSEG, SEG, D), A_q.reshape(S, D), A_k.reshape(S, D), A_v.reshape(S, D), A_shift_k.T,
      A_ssm_k, A_ssm_D.reshape(NCB, 128), B_mem0.reshape(M, D), B_Wq, B_Wk, B_Wv,
      B_Wo.reshape(H * E, D), gate_w.reshape(NCB, 128), f_tab, g_tab)
    return out.reshape(1, S, D)
```

```python
import functools

import numpy as np
import jax
import jax.numpy as jnp
from jax import lax
import jax.experimental.pallas as pl
import jax.experimental.pallas.tpu as pltpu

S, D, H, E, M, SEG = 2048, 1024, 32, 128, 8, 32
NSEG = S // SEG
NT = SEG - M
NP = H // 2
NCB = D // 128
C = 128
NCH = S // C
LOG2E = 1.4426950408889634
KS = 4
NZ = 8
KPAD = 32
NG = 6
NQ = 8
DQ = D // NQ
UNROLL = 4
CFG = dict(kq0=True, npt=28, fgrp=4, finv=4, dues=[12, 16, 20, 24, 28, 32, 36, 40, 44] + [48 * p + 40 for p in range(1, 8)] + [444 + 4 * i for i in range(16)], maclag=4, gate=436,
           split=((32, 32, 32, 32),) * 4, nw=3, order=((0, 0), (1, 0), (0, 1), (1, 1), (2, 0), (2, 1)))
_DBG_STEPS = NSEG
bf16, f32, u32 = jnp.bfloat16, jnp.float32, jnp.uint32


def _dft_tables():
    t = np.arange(C, dtype=np.float64)
    rows = []
    for r in range(8):
        ev = 16 * r + np.arange(0, 16, 2)
        od = ev + 1
        for fn, fs in ((np.cos, ev), (np.sin, ev), (np.cos, od), (np.sin, od)):
            rows.append(fn(np.pi * (2 * fs[:, None] + 1) * t[None, :] / (2 * C)))
    f = np.concatenate(rows, axis=0)
    return f.astype(bf16), (f.T / C).astype(bf16)


def _fill_matrix():
    r = lax.broadcasted_iota(jnp.int32, (80, 128), 0)
    c = lax.broadcasted_iota(jnp.int32, (80, 128), 1)

    def head(i):
        return jnp.where(i < 64, i // 32, (i - 64) // 8)

    def idx(i):
        lo = i % 32
        main = jnp.where(lo < NT, lo + M, lo - NT)
        return jnp.where(i < 64, main, (i - 64) % 8 + NT + M)

    same = (head(r) == head(c)) & (c < 80)
    ok = (idx(r) < M) | (idx(r) >= idx(c))
    return jnp.where(same, jnp.where(ok, 0.0, -1e9 * E ** 0.5), -jnp.inf).astype(f32)


def _as_bf16(v):
    return pltpu.bitcast(v, bf16)


def _dot(a, b):
    return jnp.dot(a, b, preferred_element_type=f32)


def _dot_nt(a, b):
    return lax.dot_general(a, b, (((1,), (1,)), ((), ())), preferred_element_type=f32)


SEM_SMALL, SEM_WO, SEM_X, SEM_SSM0, SEM_SSM1 = range(5)
SEM_Q = 5
SEM_K = SEM_Q + NQ
SEM_V = SEM_K + 4
SEM_W = SEM_V + 4
SEM_OUT = SEM_W + NG - 1
NSEM = SEM_OUT + 2


def _kernel(x3_hbm, x_hbm, k_hbm, v_hbm, shift_hbm, ssm_hbm, d_hbm, mem_hbm, wq_hbm, wk_hbm, wv_hbm,
            wo_hbm, gw_hbm, f_hbm, g_hbm, out_hbm,
            wn_ref, wo_ref, x_ref, xr_ref, xb_ref, pre_ref, k_ref, v_ref, ssm_ref, u_ref,
            fu_ref, fk_ref, kraw_ref, one_ref, f_ref, g_ref, fill_ref, shift_ref, wt_ref,
            d_ref, gw_ref, mem_ref, gate_ref, ost_ref, sems):
    w_hbm = (wq_hbm, wk_hbm, wv_hbm)

    def cp(src, dst, sem):
        return pltpu.make_async_copy(src, dst, sems.at[sem])

    def start_col_blocks(src_hbm, dst_ref, i0, i1, sem, row0=0):
        src = src_hbm.bitcast(u32)
        for i in range(i0, i1):
            cp(src.at[:, i * 128:(i + 1) * 128], dst_ref.at[i, row0:], sem).start()

    def start_ssm(r0, r1, sem):
        src = ssm_hbm.bitcast(u32)
        for a in range(NCH):
            cp(src.at[r0:r1, a * C:(a + 1) * C], ssm_ref.at[a, r0:r1], sem).start()

    def wait_all(dst, sem):
        cp(dst, dst, sem).wait()

    def even(p):
        return pltpu.bitcast(p << 16, f32)

    def odd(p):
        return pltpu.bitcast(p & jnp.uint32(0xFFFF0000), f32)

    def conv_prep(cb, i, dep=None):
        r0 = KPAD + 8 * i
        p0 = k_ref[cb, r0:r0 + 8, :]
        if dep is not None:
            p0 = jnp.where(one_ref[...] == 1, p0, dep)
        p1 = k_ref[cb, r0 - 1:r0 + 7, :]
        p2 = k_ref[cb, r0 - 2:r0 + 6, :]
        pv = v_ref[cb, 8 * i:8 * i + 8, :]
        w = wt_ref[cb]
        w0, w1, w2, w3 = w[0:1, :], w[1:2, :], w[2:3, :], w[3:4, :]
        e0, o0, e1, o1, o2 = even(p0), odd(p0), even(p1), odd(p1), odd(p2)
        ke = ((e0 * w0 + o1 * w1) + e1 * w2) + o2 * w3
        ko = ((o0 * w0 + e0 * w1) + o1 * w2) + e1 * w3
        re = pltpu.bitcast((ke * even(pv)).astype(bf16).astype(f32), u32)
        ro = pltpu.bitcast((ko * odd(pv)).astype(bf16).astype(f32), u32)
        kv = (re >> 16) | ro
        u_ref[cb, 8 * i:8 * i + 8, :] = kv
        return kv

    def combine(kf, prev):
        out = []
        for g in range(8):
            o = 32 * g
            out += [kf[o:o + 8] + prev[o + 8:o + 16], kf[o + 8:o + 16] - prev[o:o + 8],
                    kf[o + 16:o + 24] - prev[o + 24:o + 32], kf[o + 24:o + 32] + prev[o + 16:o + 24]]
        return jnp.concatenate(out, axis=0)

    def conv_fwd(cb, r):
        slot = cb % 2
        rows = pl.ds(pl.multiple_of(cb * 64, 64), 64)
        f = f_ref[...]
        kfs = []
        for a in (2 * r, 2 * r + 1):
            fu_ref[slot, NZ + a] = _dot(f, _as_bf16(u_ref[cb, pl.ds(pl.multiple_of(a * 64, 64), 64), :]))
            kfs.append(_dot_nt(f, _as_bf16(ssm_ref[a, rows, :])))
        fk_ref[slot, 2 * r] = combine(kfs[0], jnp.where(r > 0, kraw_ref[...], 0.0))
        fk_ref[slot, 2 * r + 1] = combine(kfs[1], kfs[0])
        kraw_ref[...] = kfs[1]

    def conv_mac(slot, a, nterms, pos, dep=None):
        rows = slice(pos * 16, pos * 16 + 16)
        p = q = None
        for c in range(nterms):
            u = fu_ref[slot, NZ + a - c, rows, :]
            k = fk_ref[slot, c, rows, :]
            ua, ub, kc, kd = u[0:8], u[8:16], k[0:8], k[8:16]
            if c == 0 and dep is not None:
                ua = jnp.where(one_ref[...] == 1, ua, pltpu.bitcast(dep, f32))
            p = (ua * kc if p is None else p + ua * kc) - ub * kd
            q = (ua * kd if q is None else q + ua * kd) + ub * kc
        return pltpu.bitcast(jnp.concatenate([p, q], axis=0).astype(bf16), u32)

    def conv_inv(a_ref, cb, dst, a, zs):
        rows = pl.ds(pl.multiple_of(a * 64, 64), 64)
        y = _dot(g_ref[...], _as_bf16(jnp.concatenate(zs, axis=0)))
        kv = _as_bf16(u_ref[cb, rows, :]).astype(f32)
        q = _as_bf16(x_ref[cb, rows, :]).astype(f32)
        a_ref[dst, pl.ds(pl.multiple_of(a * C, C), C), :] = q * (y + kv * wt_ref[cb, KS:KS + 1, :])

    def after(w, tok):
        if tok is None:
            return w
        return jnp.concatenate([jnp.where(one_ref[...] == 1, w[0:8], tok), w[8:]], axis=0)

    def prologue(stage_ref, acc_ref):
        st3 = stage_ref.reshape(NG * D, 8, E)

        def start_w(g):
            r0 = (g % 2) * 8
            cp(w_hbm[g // 2].bitcast(u32).at[:, r0:r0 + 8, :], st3.at[g * D:(g + 1) * D], SEM_W + g - 1).start()

        def slice_copies(q):
            cols = pl.ds(pl.multiple_of(q * DQ, DQ), DQ)
            return (cp(x3_hbm.at[:, NT:SEG, cols], xr_ref.at[q], SEM_Q + q),
                    cp(wq_hbm.bitcast(u32).at[cols, 0:8, :], st3.at[cols], SEM_Q + q))

        small = [cp(shift_hbm, shift_ref, SEM_SMALL), cp(d_hbm, d_ref, SEM_SMALL), cp(gw_hbm, gw_ref, SEM_SMALL),
                 cp(mem_hbm, mem_ref, SEM_SMALL), cp(f_hbm, f_ref, SEM_SMALL), cp(g_hbm, g_ref, SEM_SMALL)]
        for q in range(NQ):
            for c in slice_copies(q):
                c.start()
        for c in small:
            c.start()
        for g in range(1, NG):
            start_w(g)
            if g >= 2:
                start_col_blocks(k_hbm, k_ref, 2 * g - 4, 2 * g - 2, SEM_K + g - 2, row0=KPAD)
                start_col_blocks(v_hbm, v_ref, 2 * g - 4, 2 * g - 2, SEM_V + g - 2)
        start_col_blocks(wo_hbm, wo_ref, 0, NCB, SEM_WO)
        fill_ref[...] = _fill_matrix()
        one_ref[...] = jnp.ones((8, 128), jnp.int32)
        k_ref[:, KPAD - 8:KPAD, :] = jnp.zeros((NCB + 1, 8, 128), u32)
        wt_ref[...] = jnp.zeros(wt_ref.shape, f32)
        kraw_ref[...] = jnp.zeros(kraw_ref.shape, f32)
        fu_ref[0, NZ - 1] = jnp.zeros((256, 128), f32)

        def clear(a, c):
            rows = pl.ds(pl.multiple_of(a * 64, 64), 64)
            k_ref[NCB, pl.ds(pl.multiple_of(KPAD + a * 64, 32), 64), :] = jnp.zeros((64, 128), u32)
            v_ref[NCB, rows, :] = jnp.zeros((64, 128), u32)
            acc_ref[a] = jnp.zeros((NSEG * M, E), f32)
            return c
        lax.fori_loop(0, 16, clear, 0)

        def unpack_pair(w):
            return pltpu.bitcast(even(w).astype(bf16), u32), pltpu.bitcast(odd(w).astype(bf16), u32)

        def store_pre(idx, r1, r2):
            cc = jnp.concatenate([r1.reshape(NSEG, 8, E), r2.reshape(NSEG, 8, E)], axis=1).astype(bf16)
            pre_ref[:, idx] = pltpu.bitcast(cc, u32)

        def first(q, c):
            for cc in slice_copies(q):
                cc.wait()
            xq = pltpu.bitcast(xr_ref[q].astype(f32).reshape(NSEG * M, DQ).astype(bf16), u32)
            xb_ref[q] = xq
            sub = stage_ref.at[pl.ds(pl.multiple_of(q * (8 * DQ), 8 * DQ), 8 * DQ), :]
            rows = pl.ds(pl.multiple_of(q * (DQ // 2), DQ // 2), DQ // 2)
            for j in range(8):
                rs = []
                for h, w in zip((2 * j, 2 * j + 1), unpack_pair(sub[pl.ds(j, DQ, stride=8), :])):
                    wn_ref[h, rows, :] = w
                    r = _dot(_as_bf16(xq), _as_bf16(w)) + acc_ref[h]
                    acc_ref[h] = r
                    rs.append(r)
                store_pre(j, *rs)
            return c
        lax.fori_loop(0, NQ, first, 0)

        start_col_blocks(x_hbm, x_ref, 0, NCB, SEM_X)
        start_ssm(0, 64, SEM_SSM0)
        for c in small:
            c.wait()
        sh = shift_ref[...].astype(f32)
        dv = d_ref[...].astype(f32)
        for n in range(NCB):
            wt_ref[n, 0:KS, :] = sh[:, n * 128:(n + 1) * 128]
            wt_ref[n, KS:KS + 1, :] = dv[n:n + 1, :]

        def group(g, c):
            wait_all(st3.at[pl.ds(g * D, D)], SEM_W + g - 1)

            @pl.when(g >= 2)
            def _():
                wait_all(k_ref.at[pl.ds(2 * g - 4, 2), KPAD:], SEM_K + g - 2)
                wait_all(v_ref.at[pl.ds(2 * g - 4, 2)], SEM_V + g - 2)

            cbs = [jnp.where(g >= 2, 2 * g - 4 + i, NCB) for i in range(2)]
            npt = CFG["npt"]
            toks = [None] * 32
            for k in range(npt):
                t = None
                for i in range(k * 256 // npt, (k + 1) * 256 // npt):
                    t = conv_prep(cbs[i // 128], i % 128, t)
                    zero = pltpu.bitcast(jnp.where(one_ref[...] == 1, jnp.uint32(0), t), f32)
                    for v in range(i, 288, 256):
                        rows = slice(8 * (v % 32), 8 * (v % 32) + 8)
                        if v < 160:
                            fu_ref[1, jnp.minimum((g - 1) * 5 + v // 32, NZ + NCH - 1), rows, :] = zero
                        else:
                            fk_ref[1, jnp.minimum((g - 1) * 4 + v // 32 - 5, NCH - 1), rows, :] = zero
                toks[32 - npt + k] = t
            sub = stage_ref.at[pl.ds(pl.multiple_of(g * (8 * D), 8 * D), 8 * D), :]
            for j in range(8):
                ws = [unpack_pair(sub[pl.ds(blk * 2048 + j, 256, stride=8), :]) for blk in range(D // 256)]
                xb = _as_bf16(jnp.concatenate([xb_ref[q] for q in range(NQ)], axis=1))
                rs = [None, None]
                for i in range(2):
                    wn_ref[g * 16 + 2 * j + i] = jnp.concatenate([wb[i] for wb in ws], axis=0)
                if j == 0 and CFG["kq0"]:
                    for blk in range(D // 256):
                        for i in range(2):
                            d = _dot(xb[:, blk * 256:(blk + 1) * 256], _as_bf16(ws[blk][i]))
                            rs[i] = d if rs[i] is None else d + rs[i]
                else:
                    for i in range(2):
                        tk = toks[4 * j + 2 * i:4 * j + 2 * i + 2]
                        w = jnp.concatenate([after(ws[0][i], tk[0]), ws[1][i], after(ws[2][i], tk[1]), ws[3][i]], axis=0)
                        rs[i] = _dot(xb, _as_bf16(w))
                store_pre(g * 8 + j, *rs)
            return c
        lax.fori_loop(1, NG, group, 0)

    pl.run_scoped(prologue, pltpu.VMEM((NG * 8 * D, E), u32), pltpu.VMEM((16, NSEG * M, E), f32))

    start_ssm(64, D // 2, SEM_SSM1)
    wait_all(wo_ref, SEM_WO)
    wait_all(x_ref, SEM_X)
    wait_all(ssm_ref.at[:, 0:64], SEM_SSM0)

    scale = E ** -0.5

    def main(odef_ref, b_ref, a_ref):
        def step(s, mem, t):
            cfg = CFG
            cb = s // 8
            r = s % 8
            icb = jnp.maximum(cb - 1, 0)
            idst = jnp.where(cb >= 1, cb - 1, NCB)
            mslot = (cb + 1) % 2
            nh = 8 // UNROLL
            chunks = ((nh * t + r // UNROLL, nh * t + nh), (NCH - 1 - nh * t - r // UNROLL, NCH - nh * t))
            zs = ({}, {})

            xrows = pl.ds(pl.multiple_of(s * 16, 16), 16)
            xs = [_as_bf16(x_ref[n, xrows, :]).astype(f32) for n in range(NCB)]
            h32 = jnp.concatenate([jnp.concatenate(xs, axis=1)[0:NT], mem], axis=0).astype(bf16)
            r0 = pl.multiple_of(s * 8, 8)

            def gate(dep):
                gw = gw_ref[...].astype(f32)
                gl = None
                for n in range(NCB):
                    xg = _as_bf16(x_ref[n, xrows, :]).astype(f32) * gw[n:n + 1, :]
                    gl = xg if gl is None else gl + xg
                g = jnp.broadcast_to(jax.nn.sigmoid(jnp.sum(gl, axis=-1, keepdims=True)), (SEG, 128))
                gate_ref[s] = g
                g = pltpu.bitcast(g, u32)
                return (g[0:8] | g[8:16]) | (g[16:24] | g[24:32])

            jobs = []

            def mac_job(dep, w, pos):
                zs[w][pos] = conv_mac(mslot, chunks[w][0], chunks[w][1], pos, dep)
                return zs[w][pos]

            for i in range(32):
                due = cfg["dues"][i]
                start = max(due - cfg["maclag"], 0)
                jobs.append((start, due - start, False, functools.partial(mac_job, w=i % 2, pos=i // 2)))
            jobs.append((cfg["gate"], 4, False, gate))
            state = dict(count=0, due={})

            def sdot(lhs, w, acc=None, weight=1):
                c = state["count"]
                toks = [t for cc in range(c, c + weight) for t in state["due"].pop(cc, [])]
                nt = w.shape[0] // 64
                if toks:
                    tiles = [w[64 * i:64 * (i + 1)] for i in range(nt)]
                    for i, t in enumerate(toks):
                        tiles[i % nt] = after(tiles[i % nt], t)
                    w = jnp.concatenate(tiles, axis=0)
                d = _dot(lhs, _as_bf16(w))
                d = d if acc is None else d + acc
                for (st, lag, rel, fn) in jobs:
                    if c <= st < c + weight:
                        tok = fn(pltpu.bitcast(d[0:8], u32) if rel else None)
                        state["due"].setdefault(max(st + lag, c + weight), []).append(tok)
                state["count"] = c + weight
                return d

            def proj(m, j):
                r1 = sdot(h32, wn_ref[m * H + 2 * j], weight=4)
                r2 = sdot(h32, wn_ref[m * H + 2 * j + 1], weight=4)
                p = _as_bf16(pre_ref[s, m * NP + j]).astype(f32)
                if m == 0:
                    return jnp.concatenate([r1, r2, p], axis=0)
                return jnp.concatenate([r1, r2, p, jnp.zeros((48, E), f32)], axis=0).astype(bf16)

            def split_rows(dot, lhs, rhs, split):
                if not split:
                    return dot(lhs.astype(bf16), rhs)
                return jnp.concatenate([dot(lhs[0:split].astype(bf16), rhs), dot(lhs[split:].astype(bf16), rhs)], axis=0)

            def qk(q80, k80, split=False):
                fill = fill_ref[...]
                sc = jnp.where(fill == 0.0, split_rows(_dot_nt, q80, k80, split), fill)
                p = jnp.exp2((sc - jnp.max(sc, axis=-1, keepdims=True)) * (scale * LOG2E))
                den = jnp.sum(p, axis=-1, keepdims=True)
                rc = pl.reciprocal(den, approx=True)
                return p * (rc * (2.0 - den * rc))

            def pv(j, p, v80, split=False):
                o80 = split_rows(_dot, p, v80, split)
                odef_ref[pl.ds(r0, 8), (2 * j) * E:(2 * j + 1) * E] = o80[64:72]
                odef_ref[pl.ds(r0, 8), (2 * j + 1) * E:(2 * j + 2) * E] = o80[72:80]
                return jnp.concatenate([o80[0:32], o80[32:64]], axis=1).astype(bf16)

            def wo_part(o, j0, j1, n, acc=None):
                for j in range(j0, j1):
                    acc = sdot(o[j], wo_ref[n, j * 128:(j + 1) * 128, :], acc)
                return acc

            qs, ks, vs, ps, os_ = {}, {}, {}, {}, {}
            for j in range(0, NP, 2):
                for m, jj in cfg["order"]:
                    (qs, ks, vs)[m][j + jj] = proj(m, j + jj)
                ps[j] = qk(qs[j], ks[j], j == 0 and cfg["split"][t][0])
                ps[j + 1] = qk(qs[j + 1], ks[j + 1], j == 0 and cfg["split"][t][1])
                if j >= 2:
                    os_[j - 2] = pv(j - 2, ps[j - 2], vs[j - 2])
                    os_[j - 1] = pv(j - 1, ps[j - 1], vs[j - 1])
            na = NP - 2
            acc = {}
            nw = cfg["nw"]
            for n in range(nw):
                acc[n] = wo_part(os_, 0, na, n)
            os_[NP - 2] = pv(NP - 2, ps[NP - 2], vs[NP - 2], cfg["split"][t][2])
            os_[NP - 1] = pv(NP - 1, ps[NP - 1], vs[NP - 1], cfg["split"][t][3])
            acc[nw] = wo_part(os_, 0, na, nw)
            for n in range(nw + 1):
                acc[n] = wo_part(os_, na, NP, n, acc[n])
            for n in range(nw + 1, 8):
                acc[n] = wo_part(os_, 0, NP, n)
            assert state["count"] == 512 and not state["due"], state
            for w in range(2):
                conv_inv(a_ref, icb, idst, chunks[w][0], [zs[w][pos] for pos in range(16)])
            if t == UNROLL - 1:
                for tt in range(UNROLL):
                    conv_fwd(cb, r - t + tt)
            for n in range(NCB):
                b_ref[n, s, 0:NT, :] = acc[n][0:NT]
            return jnp.concatenate([acc[n][NT:SEG] for n in range(NCB)], axis=1).astype(bf16).astype(f32)

        def steps(i, mem):
            @pl.when(i == 8 // UNROLL)
            def _():
                wait_all(ssm_ref.at[:, 64:], SEM_SSM1)
            for t in range(UNROLL):
                mem = step(i * UNROLL + t, mem, t)
            return mem

        lax.fori_loop(0, _DBG_STEPS // UNROLL, steps, mem_ref[...].astype(f32))

        def out_copy(n):
            slot = n % 2
            return pltpu.make_async_copy(
                ost_ref.at[slot], out_hbm.at[:, :, pl.ds(pl.multiple_of(n * 128, 128), 128)],
                sems.at[SEM_OUT + slot])

        def fin(n, c):
            @pl.when(n >= 2)
            def _():
                out_copy(n - 2).wait()
            zs, toks, t = ([], []), [], None
            for pos in range(16):
                if pos % CFG["fgrp"] == 0:
                    t = None
                for w in range(2):
                    t = conv_mac((NCB - 1) % 2, n + 8 * w, 8 + 8 * w, pos, t)
                    zs[w].append(t)
                if pos % CFG["fgrp"] == CFG["fgrp"] - 1:
                    toks.append(t)
            bd = None
            for kb in range(8):
                if kb == CFG["finv"]:
                    for w in range(2):
                        conv_inv(a_ref, NCB - 1, NCB - 1, n + 8 * w, zs[w])
                w = after(wo_ref[n, kb * 256:(kb + 1) * 256, :], toks[kb - 1] if 0 < kb <= len(toks) else None)
                d = _dot(odef_ref[:, kb * 512:(kb + 1) * 512].astype(bf16), _as_bf16(w))
                bd = d if bd is None else d + bd
            b_ref[n, :, NT:SEG, :] = bd.reshape(NSEG, 8, 128)
            for blk in range(8):
                sg = slice(blk * 8, (blk + 1) * 8)
                b = b_ref[n, sg]
                a = a_ref[n, blk * 256:(blk + 1) * 256, :].reshape(8, SEG, 128)
                g = gate_ref[sg]
                ost_ref[n % 2, sg] = (g * a + (1.0 - g) * b).astype(bf16)
            out_copy(n).start()
            return c
        lax.fori_loop(0, NCB, fin, 0)
        out_copy(NCB - 2).wait()
        out_copy(NCB - 1).wait()

    pl.run_scoped(main, pltpu.VMEM((NSEG * 8, H * E), f32), pltpu.VMEM((NCB, NSEG, SEG, 128), f32),
                  pltpu.VMEM((NCB + 1, S, 128), f32))


@jax.jit
def pallas_gated_mix__ssm_conv_h3__memory_aug_recurrent_mem_tr__prompt_kernel(
    A_q: jax.Array,
    A_k: jax.Array,
    A_v: jax.Array,
    A_shift_k: jax.Array,
    A_ssm_k: jax.Array,
    A_ssm_D: jax.Array,
    B_x: jax.Array,
    B_mem0: jax.Array,
    B_Wq: jax.Array,
    B_Wk: jax.Array,
    B_Wv: jax.Array,
    B_Wo: jax.Array,
    B_seg_len: jax.Array,
    gate_w: jax.Array,
):
    del B_x, B_seg_len
    f_tab, g_tab = _dft_tables()
    out = pl.pallas_call(
        _kernel,
        out_shape=jax.ShapeDtypeStruct((NSEG, SEG, D), bf16),
        in_specs=[pl.BlockSpec(memory_space=pl.ANY)] * 15,
        out_specs=pl.BlockSpec(memory_space=pl.ANY),
        scratch_shapes=[
            pltpu.VMEM((3 * H, D // 2, E), u32),
            pltpu.VMEM((NCB, H * E // 2, 128), u32),
            pltpu.VMEM((NCB, S // 2, 128), u32),
            pltpu.VMEM((NQ, NSEG, M, DQ), bf16),
            pltpu.VMEM((NQ, NSEG * 4, DQ), u32),
            pltpu.VMEM((NSEG, 3 * NP, 8, E), u32),
            pltpu.VMEM((NCB + 1, KPAD + S // 2, 128), u32),
            pltpu.VMEM((NCB + 1, S // 2, 128), u32),
            pltpu.VMEM((NCH, D // 2, 128), u32),
            pltpu.VMEM((NCB + 1, S // 2, 128), u32),
            pltpu.VMEM((2, NZ + NCH, 256, 128), f32),
            pltpu.VMEM((2, NCH, 256, 128), f32),
            pltpu.VMEM((256, 128), f32),
            pltpu.VMEM((8, 128), jnp.int32),
            pltpu.VMEM((256, 128), bf16),
            pltpu.VMEM((128, 256), bf16),
            pltpu.VMEM((80, 128), f32),
            pltpu.VMEM((KS, D), bf16),
            pltpu.VMEM((NCB + 1, 8, 128), f32),
            pltpu.VMEM((NCB, 128), bf16),
            pltpu.VMEM((NCB, 128), bf16),
            pltpu.VMEM((M, D), bf16),
            pltpu.VMEM((NSEG, SEG, 128), f32),
            pltpu.VMEM((2, NSEG, SEG, 128), bf16),
            pltpu.SemaphoreType.DMA((NSEM,)),
        ],
        compiler_params=pltpu.CompilerParams(vmem_limit_bytes=120 * 2**20),
    )(A_q.reshape(NSEG, SEG, D), A_q.reshape(S, D), A_k.reshape(S, D), A_v.reshape(S, D), A_shift_k.T,
      A_ssm_k, A_ssm_D.reshape(NCB, 128), B_mem0.reshape(M, D), B_Wq, B_Wk, B_Wv,
      B_Wo.reshape(H * E, D), gate_w.reshape(NCB, 128), f_tab, g_tab)
    return out.reshape(1, S, D)
```

```python
import functools

import numpy as np
import jax
import jax.numpy as jnp
from jax import lax
import jax.experimental.pallas as pl
import jax.experimental.pallas.tpu as pltpu

S, D, H, E, M, SEG = 2048, 1024, 32, 128, 8, 32
NSEG = S // SEG
NT = SEG - M
NP = H // 2
NCB = D // 128
C = 128
NCH = S // C
LOG2E = 1.4426950408889634
KS = 4
NZ = 8
KPAD = 32
NG = 6
NQ = 8
DQ = D // NQ
UNROLL = 4
CFG = dict(
    dues=[12, 16, 20, 24, 28, 32, 36, 40, 44] + [48 * p + 40 for p in range(1, 8)] + [444 + 4 * i for i in range(16)],
    gate=440, split=((32, 32, 32, 32),) * 4, nw=3, order=((0, 0), (1, 0), (0, 1), (1, 1), (2, 0), (2, 1)),
    npt=28, fgrp=4, finv=4)
_DBG_STEPS = NSEG
bf16, f32, u32 = jnp.bfloat16, jnp.float32, jnp.uint32


def _dft_tables():
    t = np.arange(C, dtype=np.float64)
    rows = []
    for r in range(8):
        ev = 16 * r + np.arange(0, 16, 2)
        od = ev + 1
        for fn, fs in ((np.cos, ev), (np.sin, ev), (np.cos, od), (np.sin, od)):
            rows.append(fn(np.pi * (2 * fs[:, None] + 1) * t[None, :] / (2 * C)))
    f = np.concatenate(rows, axis=0)
    return f.astype(bf16), (f.T / C).astype(bf16)


def _fill_matrix():
    r = lax.broadcasted_iota(jnp.int32, (80, 128), 0)
    c = lax.broadcasted_iota(jnp.int32, (80, 128), 1)

    def head(i):
        return jnp.where(i < 64, i // 32, (i - 64) // 8)

    def idx(i):
        lo = i % 32
        main = jnp.where(lo < NT, lo + M, lo - NT)
        return jnp.where(i < 64, main, (i - 64) % 8 + NT + M)

    same = (head(r) == head(c)) & (c < 80)
    ok = (idx(r) < M) | (idx(r) >= idx(c))
    return jnp.where(same, jnp.where(ok, 0.0, -1e9 * E ** 0.5), -jnp.inf).astype(f32)


def _as_bf16(v):
    return pltpu.bitcast(v, bf16)


def _dot(a, b):
    return jnp.dot(a, b, preferred_element_type=f32)


def _dot_nt(a, b):
    return lax.dot_general(a, b, (((1,), (1,)), ((), ())), preferred_element_type=f32)


SEM_SMALL, SEM_WO, SEM_X, SEM_SSM0, SEM_SSM1 = range(5)
SEM_Q = 5
SEM_K = SEM_Q + NQ
SEM_V = SEM_K + 4
SEM_W = SEM_V + 4
SEM_OUT = SEM_W + NG - 1
NSEM = SEM_OUT + 2


def _kernel(x3_hbm, x_hbm, k_hbm, v_hbm, shift_hbm, ssm_hbm, d_hbm, mem_hbm, wq_hbm, wk_hbm, wv_hbm,
            wo_hbm, gw_hbm, f_hbm, g_hbm, out_hbm,
            wn_ref, wo_ref, x_ref, xr_ref, xb_ref, pre_ref, k_ref, v_ref, ssm_ref, u_ref,
            fu_ref, fk_ref, kraw_ref, one_ref, f_ref, g_ref, fill_ref, shift_ref, wt_ref,
            d_ref, gw_ref, mem_ref, gate_ref, ost_ref, sems):
    w_hbm = (wq_hbm, wk_hbm, wv_hbm)

    def cp(src, dst, sem):
        return pltpu.make_async_copy(src, dst, sems.at[sem])

    def start_col_blocks(src_hbm, dst_ref, i0, i1, sem, row0=0):
        src = src_hbm.bitcast(u32)
        for i in range(i0, i1):
            cp(src.at[:, i * 128:(i + 1) * 128], dst_ref.at[i, row0:], sem).start()

    def start_ssm(r0, r1, sem):
        src = ssm_hbm.bitcast(u32)
        for a in range(NCH):
            cp(src.at[r0:r1, a * C:(a + 1) * C], ssm_ref.at[a, r0:r1], sem).start()

    def wait_all(dst, sem):
        cp(dst, dst, sem).wait()

    def even(p):
        return pltpu.bitcast(p << 16, f32)

    def odd(p):
        return pltpu.bitcast(p & jnp.uint32(0xFFFF0000), f32)

    def conv_prep(cb, i, dep=None):
        r0 = KPAD + 8 * i
        p0 = k_ref[cb, r0:r0 + 8, :]
        if dep is not None:
            p0 = jnp.where(one_ref[...] == 1, p0, dep)
        p1 = k_ref[cb, r0 - 1:r0 + 7, :]
        p2 = k_ref[cb, r0 - 2:r0 + 6, :]
        pv = v_ref[cb, 8 * i:8 * i + 8, :]
        w = wt_ref[cb]
        w0, w1, w2, w3 = w[0:1, :], w[1:2, :], w[2:3, :], w[3:4, :]
        e0, o0, e1, o1, o2 = even(p0), odd(p0), even(p1), odd(p1), odd(p2)
        ke = ((e0 * w0 + o1 * w1) + e1 * w2) + o2 * w3
        ko = ((o0 * w0 + e0 * w1) + o1 * w2) + e1 * w3
        re = pltpu.bitcast((ke * even(pv)).astype(bf16).astype(f32), u32)
        ro = pltpu.bitcast((ko * odd(pv)).astype(bf16).astype(f32), u32)
        kv = (re >> 16) | (ro & jnp.uint32(0xFFFF0000))
        u_ref[cb, 8 * i:8 * i + 8, :] = kv
        return kv

    def combine(kf, prev):
        out = []
        for g in range(8):
            o = 32 * g
            out += [kf[o:o + 8] + prev[o + 8:o + 16], kf[o + 8:o + 16] - prev[o:o + 8],
                    kf[o + 16:o + 24] - prev[o + 24:o + 32], kf[o + 24:o + 32] + prev[o + 16:o + 24]]
        return jnp.concatenate(out, axis=0)

    def conv_fwd(cb, r):
        slot = cb % 2
        rows = pl.ds(pl.multiple_of(cb * 64, 64), 64)
        f = f_ref[...]
        kfs = []
        for a in (2 * r, 2 * r + 1):
            fu_ref[slot, NZ + a] = _dot(f, _as_bf16(u_ref[cb, pl.ds(pl.multiple_of(a * 64, 64), 64), :]))
            kfs.append(_dot_nt(f, _as_bf16(ssm_ref[a, rows, :])))
        fk_ref[slot, 2 * r] = combine(kfs[0], jnp.where(r > 0, kraw_ref[...], 0.0))
        fk_ref[slot, 2 * r + 1] = combine(kfs[1], kfs[0])
        kraw_ref[...] = kfs[1]

    def conv_mac(slot, a, nterms, pos, dep=None):
        rows = slice(pos * 16, pos * 16 + 16)
        p = q = None
        for c in range(nterms):
            u = fu_ref[slot, NZ + a - c, rows, :]
            k = fk_ref[slot, c, rows, :]
            ua, ub, kc, kd = u[0:8], u[8:16], k[0:8], k[8:16]
            if c == 0 and dep is not None:
                ua = jnp.where(one_ref[...] == 1, ua, pltpu.bitcast(dep, f32))
            p = (ua * kc if p is None else p + ua * kc) - ub * kd
            q = (ua * kd if q is None else q + ua * kd) + ub * kc
        return pltpu.bitcast(jnp.concatenate([p, q], axis=0).astype(bf16), u32)

    def conv_inv(a_ref, cb, dst, a, zs):
        rows = pl.ds(pl.multiple_of(a * 64, 64), 64)
        y = _dot(g_ref[...], _as_bf16(jnp.concatenate(zs, axis=0)))
        kv = _as_bf16(u_ref[cb, rows, :]).astype(f32)
        q = _as_bf16(x_ref[cb, rows, :]).astype(f32)
        a_ref[dst, pl.ds(pl.multiple_of(a * C, C), C), :] = q * (y + kv * wt_ref[cb, KS:KS + 1, :])

    def after(w, tok):
        if tok is None:
            return w
        return jnp.concatenate([jnp.where(one_ref[...] == 1, w[0:8], tok), w[8:]], axis=0)

    def prologue(stage_ref, acc_ref):
        st3 = stage_ref.reshape(NG * D, 8, E)

        def start_w(g):
            r0 = (g % 2) * 8
            cp(w_hbm[g // 2].bitcast(u32).at[:, r0:r0 + 8, :], st3.at[g * D:(g + 1) * D], SEM_W + g - 1).start()

        def slice_copies(q):
            cols = pl.ds(pl.multiple_of(q * DQ, DQ), DQ)
            return (cp(x3_hbm.at[:, NT:SEG, cols], xr_ref.at[q], SEM_Q + q),
                    cp(wq_hbm.bitcast(u32).at[cols, 0:8, :], st3.at[cols], SEM_Q + q))

        small = [cp(shift_hbm, shift_ref, SEM_SMALL), cp(d_hbm, d_ref, SEM_SMALL), cp(gw_hbm, gw_ref, SEM_SMALL),
                 cp(mem_hbm, mem_ref, SEM_SMALL), cp(f_hbm, f_ref, SEM_SMALL), cp(g_hbm, g_ref, SEM_SMALL)]
        for q in range(NQ):
            for c in slice_copies(q):
                c.start()
        for c in small:
            c.start()
        for g in range(1, NG):
            start_w(g)
            if g >= 2:
                start_col_blocks(k_hbm, k_ref, 2 * g - 4, 2 * g - 2, SEM_K + g - 2, row0=KPAD)
                start_col_blocks(v_hbm, v_ref, 2 * g - 4, 2 * g - 2, SEM_V + g - 2)
        start_col_blocks(wo_hbm, wo_ref, 0, NCB, SEM_WO)
        fill_ref[...] = _fill_matrix()
        one_ref[...] = jnp.ones((8, 128), jnp.int32)
        k_ref[:, KPAD - 8:KPAD, :] = jnp.zeros((NCB + 1, 8, 128), u32)
        wt_ref[...] = jnp.zeros(wt_ref.shape, f32)
        kraw_ref[...] = jnp.zeros(kraw_ref.shape, f32)
        fu_ref[0, NZ - 1] = jnp.zeros((256, 128), f32)

        def clear(a, c):
            rows = pl.ds(pl.multiple_of(a * 64, 64), 64)
            k_ref[NCB, pl.ds(pl.multiple_of(KPAD + a * 64, 32), 64), :] = jnp.zeros((64, 128), u32)
            v_ref[NCB, rows, :] = jnp.zeros((64, 128), u32)
            acc_ref[a] = jnp.zeros((NSEG * M, E), f32)
            return c
        lax.fori_loop(0, 16, clear, 0)

        def unpack_pair(w):
            return pltpu.bitcast(even(w).astype(bf16), u32), pltpu.bitcast(odd(w).astype(bf16), u32)

        def store_pre(idx, r1, r2):
            cc = jnp.concatenate([r1.reshape(NSEG, 8, E), r2.reshape(NSEG, 8, E)], axis=1).astype(bf16)
            pre_ref[:, idx] = pltpu.bitcast(cc, u32)

        def first(q, c):
            for cc in slice_copies(q):
                cc.wait()
            xq = pltpu.bitcast(xr_ref[q].astype(f32).reshape(NSEG * M, DQ).astype(bf16), u32)
            xb_ref[q] = xq
            sub = stage_ref.at[pl.ds(pl.multiple_of(q * (8 * DQ), 8 * DQ), 8 * DQ), :]
            rows = pl.ds(pl.multiple_of(q * (DQ // 2), DQ // 2), DQ // 2)
            for j in range(8):
                rs = []
                for h, w in zip((2 * j, 2 * j + 1), unpack_pair(sub[pl.ds(j, DQ, stride=8), :])):
                    wn_ref[h, rows, :] = w
                    r = _dot(_as_bf16(xq), _as_bf16(w)) + acc_ref[h]
                    acc_ref[h] = r
                    rs.append(r)
                store_pre(j, *rs)
            return c
        lax.fori_loop(0, NQ, first, 0)

        start_col_blocks(x_hbm, x_ref, 0, NCB, SEM_X)
        start_ssm(0, 64, SEM_SSM0)
        for c in small:
            c.wait()
        sh = shift_ref[...].astype(f32)
        dv = d_ref[...].astype(f32)
        for n in range(NCB):
            wt_ref[n, 0:KS, :] = sh[:, n * 128:(n + 1) * 128]
            wt_ref[n, KS:KS + 1, :] = dv[n:n + 1, :]

        def group(g, c):
            wait_all(st3.at[pl.ds(g * D, D)], SEM_W + g - 1)

            @pl.when(g >= 2)
            def _():
                wait_all(k_ref.at[pl.ds(2 * g - 4, 2), KPAD:], SEM_K + g - 2)
                wait_all(v_ref.at[pl.ds(2 * g - 4, 2)], SEM_V + g - 2)

            cbs = [jnp.where(g >= 2, 2 * g - 4 + i, NCB) for i in range(2)]
            npt = CFG["npt"]
            toks = [None] * 32
            for k in range(npt):
                t = None
                for i in range(k * 256 // npt, (k + 1) * 256 // npt):
                    t = conv_prep(cbs[i // 128], i % 128, t)
                    zero = pltpu.bitcast(jnp.where(one_ref[...] == 1, jnp.uint32(0), t), f32)
                    for v in range(i, 288, 256):
                        rows = slice(8 * (v % 32), 8 * (v % 32) + 8)
                        if v < 160:
                            fu_ref[1, jnp.minimum((g - 1) * 5 + v // 32, NZ + NCH - 1), rows, :] = zero
                        else:
                            fk_ref[1, jnp.minimum((g - 1) * 4 + v // 32 - 5, NCH - 1), rows, :] = zero
                toks[32 - npt + k] = t
            sub = stage_ref.at[pl.ds(pl.multiple_of(g * (8 * D), 8 * D), 8 * D), :]
            for j in range(8):
                ws = [unpack_pair(sub[pl.ds(blk * 2048 + j, 256, stride=8), :]) for blk in range(D // 256)]
                xb = _as_bf16(jnp.concatenate([xb_ref[q] for q in range(NQ)], axis=1))
                rs = [None, None]
                for i in range(2):
                    wn_ref[g * 16 + 2 * j + i] = jnp.concatenate([wb[i] for wb in ws], axis=0)
                if j == 0:
                    for blk in range(D // 256):
                        for i in range(2):
                            d = _dot(xb[:, blk * 256:(blk + 1) * 256], _as_bf16(ws[blk][i]))
                            rs[i] = d if rs[i] is None else d + rs[i]
                else:
                    for i in range(2):
                        tk = toks[4 * j + 2 * i:4 * j + 2 * i + 2]
                        w = jnp.concatenate([after(ws[0][i], tk[0]), ws[1][i], after(ws[2][i], tk[1]), ws[3][i]], axis=0)
                        rs[i] = _dot(xb, _as_bf16(w))
                store_pre(g * 8 + j, *rs)
            return c
        lax.fori_loop(1, NG, group, 0)

    pl.run_scoped(prologue, pltpu.VMEM((NG * 8 * D, E), u32), pltpu.VMEM((16, NSEG * M, E), f32))

    start_ssm(64, D // 2, SEM_SSM1)
    wait_all(wo_ref, SEM_WO)
    wait_all(x_ref, SEM_X)
    wait_all(ssm_ref.at[:, 0:64], SEM_SSM0)

    scale = E ** -0.5

    def main(odef_ref, b_ref, a_ref):
        def step(s, mem, t):
            cfg = CFG
            cb = s // 8
            r = s % 8
            icb = jnp.maximum(cb - 1, 0)
            idst = jnp.where(cb >= 1, cb - 1, NCB)
            mslot = (cb + 1) % 2
            nh = 8 // UNROLL
            chunks = ((nh * t + r // UNROLL, nh * t + nh), (NCH - 1 - nh * t - r // UNROLL, NCH - nh * t))
            zs = ({}, {})

            xrows = pl.ds(pl.multiple_of(s * 16, 16), 16)
            xs = [_as_bf16(x_ref[n, xrows, :]).astype(f32) for n in range(NCB)]
            h32 = jnp.concatenate([jnp.concatenate(xs, axis=1)[0:NT], mem], axis=0).astype(bf16)
            r0 = pl.multiple_of(s * 8, 8)

            def gate():
                gw = gw_ref[...].astype(f32)
                gl = None
                for n in range(NCB):
                    xg = _as_bf16(x_ref[n, xrows, :]).astype(f32) * gw[n:n + 1, :]
                    gl = xg if gl is None else gl + xg
                g = jnp.broadcast_to(jax.nn.sigmoid(jnp.sum(gl, axis=-1, keepdims=True)), (SEG, 128))
                gate_ref[s] = g
                g = pltpu.bitcast(g, u32)
                return (g[0:8] | g[8:16]) | (g[16:24] | g[24:32])

            def mac_job(w, pos):
                zs[w][pos] = conv_mac(mslot, chunks[w][0], chunks[w][1], pos)
                return zs[w][pos]

            jobs = [(cfg["dues"][i], functools.partial(mac_job, i % 2, i // 2)) for i in range(32)]
            jobs.append((cfg["gate"], gate))
            state = dict(count=0, due={})

            def sdot(lhs, w, acc=None, weight=1):
                c = state["count"]
                toks = [t for cc in range(c, c + weight) for t in state["due"].pop(cc, [])]
                nt = w.shape[0] // 64
                if toks:
                    tiles = [w[64 * i:64 * (i + 1)] for i in range(nt)]
                    for i, t in enumerate(toks):
                        tiles[i % nt] = after(tiles[i % nt], t)
                    w = jnp.concatenate(tiles, axis=0)
                d = _dot(lhs, _as_bf16(w))
                d = d if acc is None else d + acc
                for due, fn in jobs:
                    if c <= due - 4 < c + weight:
                        state["due"].setdefault(due, []).append(fn())
                state["count"] = c + weight
                return d

            def proj(m, j):
                r1 = sdot(h32, wn_ref[m * H + 2 * j], weight=4)
                r2 = sdot(h32, wn_ref[m * H + 2 * j + 1], weight=4)
                p = _as_bf16(pre_ref[s, m * NP + j]).astype(f32)
                if m == 0:
                    return jnp.concatenate([r1, r2, p], axis=0)
                return jnp.concatenate([r1, r2, p, jnp.zeros((48, E), f32)], axis=0).astype(bf16)

            def split_rows(dot, lhs, rhs, split):
                if not split:
                    return dot(lhs.astype(bf16), rhs)
                return jnp.concatenate([dot(lhs[0:split].astype(bf16), rhs), dot(lhs[split:].astype(bf16), rhs)], axis=0)

            def qk(q80, k80, split=False):
                fill = fill_ref[...]
                sc = jnp.where(fill == 0.0, split_rows(_dot_nt, q80, k80, split), fill)
                p = jnp.exp2((sc - jnp.max(sc, axis=-1, keepdims=True)) * (scale * LOG2E))
                den = jnp.sum(p, axis=-1, keepdims=True)
                rc = pl.reciprocal(den, approx=True)
                return p * (rc * (2.0 - den * rc))

            def pv(j, p, v80, split=False):
                o80 = split_rows(_dot, p, v80, split)
                odef_ref[pl.ds(r0, 8), (2 * j) * E:(2 * j + 1) * E] = o80[64:72]
                odef_ref[pl.ds(r0, 8), (2 * j + 1) * E:(2 * j + 2) * E] = o80[72:80]
                return jnp.concatenate([o80[0:32], o80[32:64]], axis=1).astype(bf16)

            def wo_part(o, j0, j1, n, acc=None):
                for j in range(j0, j1):
                    acc = sdot(o[j], wo_ref[n, j * 128:(j + 1) * 128, :], acc)
                return acc

            qs, ks, vs, ps, os_ = {}, {}, {}, {}, {}
            for j in range(0, NP, 2):
                for m, jj in cfg["order"]:
                    (qs, ks, vs)[m][j + jj] = proj(m, j + jj)
                ps[j] = qk(qs[j], ks[j], j == 0 and cfg["split"][t][0])
                ps[j + 1] = qk(qs[j + 1], ks[j + 1], j == 0 and cfg["split"][t][1])
                if j >= 2:
                    os_[j - 2] = pv(j - 2, ps[j - 2], vs[j - 2])
                    os_[j - 1] = pv(j - 1, ps[j - 1], vs[j - 1])
            na = NP - 2
            acc = {}
            nw = cfg["nw"]
            for n in range(nw):
                acc[n] = wo_part(os_, 0, na, n)
            os_[NP - 2] = pv(NP - 2, ps[NP - 2], vs[NP - 2], cfg["split"][t][2])
            os_[NP - 1] = pv(NP - 1, ps[NP - 1], vs[NP - 1], cfg["split"][t][3])
            acc[nw] = wo_part(os_, 0, na, nw)
            for n in range(nw + 1):
                acc[n] = wo_part(os_, na, NP, n, acc[n])
            for n in range(nw + 1, 8):
                acc[n] = wo_part(os_, 0, NP, n)
            assert state["count"] == 512 and not state["due"], state
            for w in range(2):
                conv_inv(a_ref, icb, idst, chunks[w][0], [zs[w][pos] for pos in range(16)])
            if t == UNROLL - 1:
                for tt in range(UNROLL):
                    conv_fwd(cb, r - t + tt)
            for n in range(NCB):
                b_ref[n, s, 0:NT, :] = acc[n][0:NT]
            return jnp.concatenate([acc[n][NT:SEG] for n in range(NCB)], axis=1).astype(bf16).astype(f32)

        def steps(i, mem):
            @pl.when(i == 8 // UNROLL)
            def _():
                wait_all(ssm_ref.at[:, 64:], SEM_SSM1)
            for t in range(UNROLL):
                mem = step(i * UNROLL + t, mem, t)
            return mem

        lax.fori_loop(0, _DBG_STEPS // UNROLL, steps, mem_ref[...].astype(f32))

        def out_copy(n):
            slot = n % 2
            return pltpu.make_async_copy(
                ost_ref.at[slot], out_hbm.at[:, :, pl.ds(pl.multiple_of(n * 128, 128), 128)],
                sems.at[SEM_OUT + slot])

        def fin(n, c):
            @pl.when(n >= 2)
            def _():
                out_copy(n - 2).wait()
            zs, toks, t = ([], []), [], None
            for pos in range(16):
                if pos % CFG["fgrp"] == 0:
                    t = None
                for w in range(2):
                    t = conv_mac((NCB - 1) % 2, n + 8 * w, 8 + 8 * w, pos, t)
                    zs[w].append(t)
                if pos % CFG["fgrp"] == CFG["fgrp"] - 1:
                    toks.append(t)
            bd = None
            for kb in range(8):
                if kb == CFG["finv"]:
                    for w in range(2):
                        conv_inv(a_ref, NCB - 1, NCB - 1, n + 8 * w, zs[w])
                w = after(wo_ref[n, kb * 256:(kb + 1) * 256, :], toks[kb - 1] if 0 < kb <= len(toks) else None)
                d = _dot(odef_ref[:, kb * 512:(kb + 1) * 512].astype(bf16), _as_bf16(w))
                bd = d if bd is None else d + bd
            b_ref[n, :, NT:SEG, :] = bd.reshape(NSEG, 8, 128)
            for blk in range(8):
                sg = slice(blk * 8, (blk + 1) * 8)
                b = b_ref[n, sg]
                a = a_ref[n, blk * 256:(blk + 1) * 256, :].reshape(8, SEG, 128)
                g = gate_ref[sg]
                ost_ref[n % 2, sg] = (g * a + (1.0 - g) * b).astype(bf16)
            out_copy(n).start()
            return c
        lax.fori_loop(0, NCB, fin, 0)
        out_copy(NCB - 2).wait()
        out_copy(NCB - 1).wait()

    pl.run_scoped(main, pltpu.VMEM((NSEG * 8, H * E), f32), pltpu.VMEM((NCB, NSEG, SEG, 128), f32),
                  pltpu.VMEM((NCB + 1, S, 128), f32))


@jax.jit
def pallas_gated_mix__ssm_conv_h3__memory_aug_recurrent_mem_tr__prompt_kernel(
    A_q: jax.Array,
    A_k: jax.Array,
    A_v: jax.Array,
    A_shift_k: jax.Array,
    A_ssm_k: jax.Array,
    A_ssm_D: jax.Array,
    B_x: jax.Array,
    B_mem0: jax.Array,
    B_Wq: jax.Array,
    B_Wk: jax.Array,
    B_Wv: jax.Array,
    B_Wo: jax.Array,
    B_seg_len: jax.Array,
    gate_w: jax.Array,
):
    del B_x, B_seg_len
    f_tab, g_tab = _dft_tables()
    out = pl.pallas_call(
        _kernel,
        out_shape=jax.ShapeDtypeStruct((NSEG, SEG, D), bf16),
        in_specs=[pl.BlockSpec(memory_space=pl.ANY)] * 15,
        out_specs=pl.BlockSpec(memory_space=pl.ANY),
        scratch_shapes=[
            pltpu.VMEM((3 * H, D // 2, E), u32),
            pltpu.VMEM((NCB, H * E // 2, 128), u32),
            pltpu.VMEM((NCB, S // 2, 128), u32),
            pltpu.VMEM((NQ, NSEG, M, DQ), bf16),
            pltpu.VMEM((NQ, NSEG * 4, DQ), u32),
            pltpu.VMEM((NSEG, 3 * NP, 8, E), u32),
            pltpu.VMEM((NCB + 1, KPAD + S // 2, 128), u32),
            pltpu.VMEM((NCB + 1, S // 2, 128), u32),
            pltpu.VMEM((NCH, D // 2, 128), u32),
            pltpu.VMEM((NCB + 1, S // 2, 128), u32),
            pltpu.VMEM((2, NZ + NCH, 256, 128), f32),
            pltpu.VMEM((2, NCH, 256, 128), f32),
            pltpu.VMEM((256, 128), f32),
            pltpu.VMEM((8, 128), jnp.int32),
            pltpu.VMEM((256, 128), bf16),
            pltpu.VMEM((128, 256), bf16),
            pltpu.VMEM((80, 128), f32),
            pltpu.VMEM((KS, D), bf16),
            pltpu.VMEM((NCB + 1, 8, 128), f32),
            pltpu.VMEM((NCB, 128), bf16),
            pltpu.VMEM((NCB, 128), bf16),
            pltpu.VMEM((M, D), bf16),
            pltpu.VMEM((NSEG, SEG, 128), f32),
            pltpu.VMEM((2, NSEG, SEG, 128), bf16),
            pltpu.SemaphoreType.DMA((NSEM,)),
        ],
        compiler_params=pltpu.CompilerParams(vmem_limit_bytes=120 * 2**20),
    )(A_q.reshape(NSEG, SEG, D), A_q.reshape(S, D), A_k.reshape(S, D), A_v.reshape(S, D), A_shift_k.T,
      A_ssm_k, A_ssm_D.reshape(NCB, 128), B_mem0.reshape(M, D), B_Wq, B_Wk, B_Wv,
      B_Wo.reshape(H * E, D), gate_w.reshape(NCB, 128), f_tab, g_tab)
    return out.reshape(1, S, D)
```

```python
import functools

import numpy as np
import jax
import jax.numpy as jnp
from jax import lax
import jax.experimental.pallas as pl
import jax.experimental.pallas.tpu as pltpu

S, D, H, E, M, SEG = 2048, 1024, 32, 128, 8, 32
NSEG = S // SEG
NT = SEG - M
NP = H // 2
NCB = D // 128
C = 128
NCH = S // C
LOG2E = 1.4426950408889634
KS = 4
NZ = 8
KPAD = 32
NG = 6
NQ = 8
DQ = D // NQ
UNROLL = 4
CFG = dict(npt=28, fgrp=4, finv=4, steps=[
    dict(dues=[12, 16, 20, 24, 28, 32, 36, 40, 44, 88, 136, 184, 232, 280, 328, 376, 444, 448, 452, 456, 460, 464,
               468, 472, 476, 480, 484, 488, 492, 496, 500, 504],
         gate=440, split=(32, 32, 32, 32), nw=3, order=((0, 0), (1, 0), (0, 1), (1, 1), (2, 0), (2, 1))),
    dict(dues=[12, 16, 20, 24, 28, 32, 36, 40, 490, 88, 136, 464, 232, 280, 328, 376, 444, 448, 452, 456, 460, 184,
               468, 472, 476, 480, 484, 488, 492, 496, 500, 504],
         gate=434, split=(32, 32, 32, 32), nw=4, order=((0, 0), (1, 0), (0, 1), (1, 1), (2, 0), (2, 1))),
    dict(dues=[12, 16, 20, 468, 496, 32, 220, 40, 188, 88, 136, 184, 232, 280, 450, 506, 444, 448, 452, 456, 460,
               464, 24, 472, 476, 480, 20, 488, 492, 28, 500, 504],
         gate=440, split=(32, 32, 32, 32), nw=3, order=((0, 0), (1, 0), (0, 1), (1, 1), (2, 0), (2, 1))),
    dict(dues=[12, 16, 20, 24, 28, 32, 36, 40, 220, 88, 136, 184, 232, 280, 328, 376, 444, 448, 452, 456, 460, 464,
               468, 472, 476, 480, 484, 488, 492, 496, 500, 504],
         gate=272, split=(32, 32, 32, 32), nw=3, order=((0, 0), (1, 0), (0, 1), (1, 1), (2, 0), (2, 1))),
])
_DBG_STEPS = NSEG
bf16, f32, u32 = jnp.bfloat16, jnp.float32, jnp.uint32


def _dft_tables():
    t = np.arange(C, dtype=np.float64)
    rows = []
    for r in range(8):
        ev = 16 * r + np.arange(0, 16, 2)
        od = ev + 1
        for fn, fs in ((np.cos, ev), (np.sin, ev), (np.cos, od), (np.sin, od)):
            rows.append(fn(np.pi * (2 * fs[:, None] + 1) * t[None, :] / (2 * C)))
    f = np.concatenate(rows, axis=0)
    return f.astype(bf16), (f.T / C).astype(bf16)


def _fill_matrix():
    r = lax.broadcasted_iota(jnp.int32, (80, 128), 0)
    c = lax.broadcasted_iota(jnp.int32, (80, 128), 1)

    def head(i):
        return jnp.where(i < 64, i // 32, (i - 64) // 8)

    def idx(i):
        lo = i % 32
        main = jnp.where(lo < NT, lo + M, lo - NT)
        return jnp.where(i < 64, main, (i - 64) % 8 + NT + M)

    same = (head(r) == head(c)) & (c < 80)
    ok = (idx(r) < M) | (idx(r) >= idx(c))
    return jnp.where(same, jnp.where(ok, 0.0, -1e9 * E ** 0.5), -jnp.inf).astype(f32)


def _as_bf16(v):
    return pltpu.bitcast(v, bf16)


def _dot(a, b):
    return jnp.dot(a, b, preferred_element_type=f32)


def _dot_nt(a, b):
    return lax.dot_general(a, b, (((1,), (1,)), ((), ())), preferred_element_type=f32)


SEM_SMALL, SEM_WO, SEM_X, SEM_SSM0, SEM_SSM1 = range(5)
SEM_Q = 5
SEM_K = SEM_Q + NQ
SEM_V = SEM_K + 4
SEM_W = SEM_V + 4
SEM_OUT = SEM_W + NG - 1
NSEM = SEM_OUT + 2


def _kernel(x3_hbm, x_hbm, k_hbm, v_hbm, shift_hbm, ssm_hbm, d_hbm, mem_hbm, wq_hbm, wk_hbm, wv_hbm,
            wo_hbm, gw_hbm, f_hbm, g_hbm, out_hbm,
            wn_ref, wo_ref, x_ref, xr_ref, xb_ref, pre_ref, k_ref, v_ref, ssm_ref, u_ref,
            fu_ref, fk_ref, kraw_ref, one_ref, f_ref, g_ref, fill_ref, shift_ref, wt_ref,
            d_ref, gw_ref, mem_ref, gate_ref, ost_ref, sems):
    w_hbm = (wq_hbm, wk_hbm, wv_hbm)

    def cp(src, dst, sem):
        return pltpu.make_async_copy(src, dst, sems.at[sem])

    def start_col_blocks(src_hbm, dst_ref, i0, i1, sem, row0=0):
        src = src_hbm.bitcast(u32)
        for i in range(i0, i1):
            cp(src.at[:, i * 128:(i + 1) * 128], dst_ref.at[i, row0:], sem).start()

    def start_ssm(r0, r1, sem):
        src = ssm_hbm.bitcast(u32)
        for a in range(NCH):
            cp(src.at[r0:r1, a * C:(a + 1) * C], ssm_ref.at[a, r0:r1], sem).start()

    def wait_all(dst, sem):
        cp(dst, dst, sem).wait()

    def even(p):
        return pltpu.bitcast(p << 16, f32)

    def odd(p):
        return pltpu.bitcast(p & jnp.uint32(0xFFFF0000), f32)

    def conv_prep(cb, i, dep=None):
        r0 = KPAD + 8 * i
        p0 = k_ref[cb, r0:r0 + 8, :]
        if dep is not None:
            p0 = jnp.where(one_ref[...] == 1, p0, dep)
        p1 = k_ref[cb, r0 - 1:r0 + 7, :]
        p2 = k_ref[cb, r0 - 2:r0 + 6, :]
        pv = v_ref[cb, 8 * i:8 * i + 8, :]
        w = wt_ref[cb]
        w0, w1, w2, w3 = w[0:1, :], w[1:2, :], w[2:3, :], w[3:4, :]
        e0, o0, e1, o1, o2 = even(p0), odd(p0), even(p1), odd(p1), odd(p2)
        ke = ((e0 * w0 + o1 * w1) + e1 * w2) + o2 * w3
        ko = ((o0 * w0 + e0 * w1) + o1 * w2) + e1 * w3
        re = pltpu.bitcast((ke * even(pv)).astype(bf16).astype(f32), u32)
        ro = pltpu.bitcast((ko * odd(pv)).astype(bf16).astype(f32), u32)
        kv = (re >> 16) | (ro & jnp.uint32(0xFFFF0000))
        u_ref[cb, 8 * i:8 * i + 8, :] = kv
        return kv

    def combine(kf, prev):
        out = []
        for g in range(8):
            o = 32 * g
            out += [kf[o:o + 8] + prev[o + 8:o + 16], kf[o + 8:o + 16] - prev[o:o + 8],
                    kf[o + 16:o + 24] - prev[o + 24:o + 32], kf[o + 24:o + 32] + prev[o + 16:o + 24]]
        return jnp.concatenate(out, axis=0)

    def conv_fwd(cb, r):
        slot = cb % 2
        rows = pl.ds(pl.multiple_of(cb * 64, 64), 64)
        f = f_ref[...]
        kfs = []
        for a in (2 * r, 2 * r + 1):
            fu_ref[slot, NZ + a] = _dot(f, _as_bf16(u_ref[cb, pl.ds(pl.multiple_of(a * 64, 64), 64), :]))
            kfs.append(_dot_nt(f, _as_bf16(ssm_ref[a, rows, :])))
        fk_ref[slot, 2 * r] = combine(kfs[0], jnp.where(r > 0, kraw_ref[...], 0.0))
        fk_ref[slot, 2 * r + 1] = combine(kfs[1], kfs[0])
        kraw_ref[...] = kfs[1]

    def conv_mac(slot, a, nterms, pos, dep=None):
        rows = slice(pos * 16, pos * 16 + 16)
        p = q = None
        for c in range(nterms):
            u = fu_ref[slot, NZ + a - c, rows, :]
            k = fk_ref[slot, c, rows, :]
            ua, ub, kc, kd = u[0:8], u[8:16], k[0:8], k[8:16]
            if c == 0 and dep is not None:
                ua = jnp.where(one_ref[...] == 1, ua, pltpu.bitcast(dep, f32))
            p = (ua * kc if p is None else p + ua * kc) - ub * kd
            q = (ua * kd if q is None else q + ua * kd) + ub * kc
        return pltpu.bitcast(jnp.concatenate([p, q], axis=0).astype(bf16), u32)

    def conv_inv(a_ref, cb, dst, a, zs):
        rows = pl.ds(pl.multiple_of(a * 64, 64), 64)
        y = _dot(g_ref[...], _as_bf16(jnp.concatenate(zs, axis=0)))
        kv = _as_bf16(u_ref[cb, rows, :]).astype(f32)
        q = _as_bf16(x_ref[cb, rows, :]).astype(f32)
        a_ref[dst, pl.ds(pl.multiple_of(a * C, C), C), :] = q * (y + kv * wt_ref[cb, KS:KS + 1, :])

    def after(w, tok):
        if tok is None:
            return w
        return jnp.concatenate([jnp.where(one_ref[...] == 1, w[0:8], tok), w[8:]], axis=0)

    def prologue(stage_ref, acc_ref):
        st3 = stage_ref.reshape(NG * D, 8, E)

        def start_w(g):
            r0 = (g % 2) * 8
            cp(w_hbm[g // 2].bitcast(u32).at[:, r0:r0 + 8, :], st3.at[g * D:(g + 1) * D], SEM_W + g - 1).start()

        def slice_copies(q):
            cols = pl.ds(pl.multiple_of(q * DQ, DQ), DQ)
            return (cp(x3_hbm.at[:, NT:SEG, cols], xr_ref.at[q], SEM_Q + q),
                    cp(wq_hbm.bitcast(u32).at[cols, 0:8, :], st3.at[cols], SEM_Q + q))

        small = [cp(shift_hbm, shift_ref, SEM_SMALL), cp(d_hbm, d_ref, SEM_SMALL), cp(gw_hbm, gw_ref, SEM_SMALL),
                 cp(mem_hbm, mem_ref, SEM_SMALL), cp(f_hbm, f_ref, SEM_SMALL), cp(g_hbm, g_ref, SEM_SMALL)]
        for q in range(NQ):
            for c in slice_copies(q):
                c.start()
        for c in small:
            c.start()
        for g in range(1, NG):
            start_w(g)
            if g >= 2:
                start_col_blocks(k_hbm, k_ref, 2 * g - 4, 2 * g - 2, SEM_K + g - 2, row0=KPAD)
                start_col_blocks(v_hbm, v_ref, 2 * g - 4, 2 * g - 2, SEM_V + g - 2)
        start_col_blocks(wo_hbm, wo_ref, 0, NCB, SEM_WO)
        fill_ref[...] = _fill_matrix()
        one_ref[...] = jnp.ones((8, 128), jnp.int32)
        k_ref[:, KPAD - 8:KPAD, :] = jnp.zeros((NCB + 1, 8, 128), u32)
        wt_ref[...] = jnp.zeros(wt_ref.shape, f32)
        kraw_ref[...] = jnp.zeros(kraw_ref.shape, f32)
        fu_ref[0, NZ - 1] = jnp.zeros((256, 128), f32)

        def clear(a, c):
            rows = pl.ds(pl.multiple_of(a * 64, 64), 64)
            k_ref[NCB, pl.ds(pl.multiple_of(KPAD + a * 64, 32), 64), :] = jnp.zeros((64, 128), u32)
            v_ref[NCB, rows, :] = jnp.zeros((64, 128), u32)
            acc_ref[a] = jnp.zeros((NSEG * M, E), f32)
            return c
        lax.fori_loop(0, 16, clear, 0)

        def unpack_pair(w):
            return pltpu.bitcast(even(w).astype(bf16), u32), pltpu.bitcast(odd(w).astype(bf16), u32)

        def store_pre(idx, r1, r2):
            cc = jnp.concatenate([r1.reshape(NSEG, 8, E), r2.reshape(NSEG, 8, E)], axis=1).astype(bf16)
            pre_ref[:, idx] = pltpu.bitcast(cc, u32)

        def first(q, c):
            for cc in slice_copies(q):
                cc.wait()
            xq = pltpu.bitcast(xr_ref[q].astype(f32).reshape(NSEG * M, DQ).astype(bf16), u32)
            xb_ref[q] = xq
            sub = stage_ref.at[pl.ds(pl.multiple_of(q * (8 * DQ), 8 * DQ), 8 * DQ), :]
            rows = pl.ds(pl.multiple_of(q * (DQ // 2), DQ // 2), DQ // 2)
            for j in range(8):
                rs = []
                for h, w in zip((2 * j, 2 * j + 1), unpack_pair(sub[pl.ds(j, DQ, stride=8), :])):
                    wn_ref[h, rows, :] = w
                    r = _dot(_as_bf16(xq), _as_bf16(w)) + acc_ref[h]
                    acc_ref[h] = r
                    rs.append(r)
                store_pre(j, *rs)
            return c
        lax.fori_loop(0, NQ, first, 0)

        start_col_blocks(x_hbm, x_ref, 0, NCB, SEM_X)
        start_ssm(0, 64, SEM_SSM0)
        for c in small:
            c.wait()
        sh = shift_ref[...].astype(f32)
        dv = d_ref[...].astype(f32)
        for n in range(NCB):
            wt_ref[n, 0:KS, :] = sh[:, n * 128:(n + 1) * 128]
            wt_ref[n, KS:KS + 1, :] = dv[n:n + 1, :]

        def group(g, c):
            wait_all(st3.at[pl.ds(g * D, D)], SEM_W + g - 1)

            @pl.when(g >= 2)
            def _():
                wait_all(k_ref.at[pl.ds(2 * g - 4, 2), KPAD:], SEM_K + g - 2)
                wait_all(v_ref.at[pl.ds(2 * g - 4, 2)], SEM_V + g - 2)

            cbs = [jnp.where(g >= 2, 2 * g - 4 + i, NCB) for i in range(2)]
            npt = CFG["npt"]
            toks = [None] * 32
            for k in range(npt):
                t = None
                for i in range(k * 256 // npt, (k + 1) * 256 // npt):
                    t = conv_prep(cbs[i // 128], i % 128, t)
                    zero = pltpu.bitcast(jnp.where(one_ref[...] == 1, jnp.uint32(0), t), f32)
                    for v in range(i, 288, 256):
                        rows = slice(8 * (v % 32), 8 * (v % 32) + 8)
                        if v < 160:
                            fu_ref[1, jnp.minimum((g - 1) * 5 + v // 32, NZ + NCH - 1), rows, :] = zero
                        else:
                            fk_ref[1, jnp.minimum((g - 1) * 4 + v // 32 - 5, NCH - 1), rows, :] = zero
                toks[32 - npt + k] = t
            sub = stage_ref.at[pl.ds(pl.multiple_of(g * (8 * D), 8 * D), 8 * D), :]
            for j in range(8):
                ws = [unpack_pair(sub[pl.ds(blk * 2048 + j, 256, stride=8), :]) for blk in range(D // 256)]
                xb = _as_bf16(jnp.concatenate([xb_ref[q] for q in range(NQ)], axis=1))
                rs = [None, None]
                for i in range(2):
                    wn_ref[g * 16 + 2 * j + i] = jnp.concatenate([wb[i] for wb in ws], axis=0)
                if j == 0:
                    for blk in range(D // 256):
                        for i in range(2):
                            d = _dot(xb[:, blk * 256:(blk + 1) * 256], _as_bf16(ws[blk][i]))
                            rs[i] = d if rs[i] is None else d + rs[i]
                else:
                    for i in range(2):
                        tk = toks[4 * j + 2 * i:4 * j + 2 * i + 2]
                        w = jnp.concatenate([after(ws[0][i], tk[0]), ws[1][i], after(ws[2][i], tk[1]), ws[3][i]], axis=0)
                        rs[i] = _dot(xb, _as_bf16(w))
                store_pre(g * 8 + j, *rs)
            return c
        lax.fori_loop(1, NG, group, 0)

    pl.run_scoped(prologue, pltpu.VMEM((NG * 8 * D, E), u32), pltpu.VMEM((16, NSEG * M, E), f32))

    start_ssm(64, D // 2, SEM_SSM1)
    wait_all(wo_ref, SEM_WO)
    wait_all(x_ref, SEM_X)
    wait_all(ssm_ref.at[:, 0:64], SEM_SSM0)

    scale = E ** -0.5

    def main(odef_ref, b_ref, a_ref):
        def step(s, mem, t):
            cfg = CFG["steps"][t]
            cb = s // 8
            r = s % 8
            icb = jnp.maximum(cb - 1, 0)
            idst = jnp.where(cb >= 1, cb - 1, NCB)
            mslot = (cb + 1) % 2
            nh = 8 // UNROLL
            chunks = ((nh * t + r // UNROLL, nh * t + nh), (NCH - 1 - nh * t - r // UNROLL, NCH - nh * t))
            zs = ({}, {})

            xrows = pl.ds(pl.multiple_of(s * 16, 16), 16)
            xs = [_as_bf16(x_ref[n, xrows, :]).astype(f32) for n in range(NCB)]
            h32 = jnp.concatenate([jnp.concatenate(xs, axis=1)[0:NT], mem], axis=0).astype(bf16)
            r0 = pl.multiple_of(s * 8, 8)

            def gate():
                gw = gw_ref[...].astype(f32)
                gl = None
                for n in range(NCB):
                    xg = _as_bf16(x_ref[n, xrows, :]).astype(f32) * gw[n:n + 1, :]
                    gl = xg if gl is None else gl + xg
                g = jnp.broadcast_to(jax.nn.sigmoid(jnp.sum(gl, axis=-1, keepdims=True)), (SEG, 128))
                gate_ref[s] = g
                g = pltpu.bitcast(g, u32)
                return (g[0:8] | g[8:16]) | (g[16:24] | g[24:32])

            def mac_job(w, pos):
                zs[w][pos] = conv_mac(mslot, chunks[w][0], chunks[w][1], pos)
                return zs[w][pos]

            jobs = [(cfg["dues"][i], functools.partial(mac_job, i % 2, i // 2)) for i in range(32)]
            jobs.append((cfg["gate"], gate))
            state = dict(count=0, due={})

            def sdot(lhs, w, acc=None, weight=1):
                c = state["count"]
                toks = [t for cc in range(c, c + weight) for t in state["due"].pop(cc, [])]
                nt = w.shape[0] // 64
                if toks:
                    tiles = [w[64 * i:64 * (i + 1)] for i in range(nt)]
                    for i, t in enumerate(toks):
                        tiles[i % nt] = after(tiles[i % nt], t)
                    w = jnp.concatenate(tiles, axis=0)
                d = _dot(lhs, _as_bf16(w))
                d = d if acc is None else d + acc
                for due, fn in jobs:
                    if c <= due - 4 < c + weight:
                        state["due"].setdefault(due, []).append(fn())
                state["count"] = c + weight
                return d

            def proj(m, j):
                r1 = sdot(h32, wn_ref[m * H + 2 * j], weight=4)
                r2 = sdot(h32, wn_ref[m * H + 2 * j + 1], weight=4)
                p = _as_bf16(pre_ref[s, m * NP + j]).astype(f32)
                if m == 0:
                    return jnp.concatenate([r1, r2, p], axis=0)
                return jnp.concatenate([r1, r2, p, jnp.zeros((48, E), f32)], axis=0).astype(bf16)

            def split_rows(dot, lhs, rhs, split):
                if not split:
                    return dot(lhs.astype(bf16), rhs)
                return jnp.concatenate([dot(lhs[0:split].astype(bf16), rhs), dot(lhs[split:].astype(bf16), rhs)], axis=0)

            def qk(q80, k80, split=False):
                fill = fill_ref[...]
                sc = jnp.where(fill == 0.0, split_rows(_dot_nt, q80, k80, split), fill)
                p = jnp.exp2((sc - jnp.max(sc, axis=-1, keepdims=True)) * (scale * LOG2E))
                den = jnp.sum(p, axis=-1, keepdims=True)
                rc = pl.reciprocal(den, approx=True)
                return p * (rc * (2.0 - den * rc))

            def pv(j, p, v80, split=False):
                o80 = split_rows(_dot, p, v80, split)
                odef_ref[pl.ds(r0, 8), (2 * j) * E:(2 * j + 1) * E] = o80[64:72]
                odef_ref[pl.ds(r0, 8), (2 * j + 1) * E:(2 * j + 2) * E] = o80[72:80]
                return jnp.concatenate([o80[0:32], o80[32:64]], axis=1).astype(bf16)

            def wo_part(o, j0, j1, n, acc=None):
                for j in range(j0, j1):
                    acc = sdot(o[j], wo_ref[n, j * 128:(j + 1) * 128, :], acc)
                return acc

            qs, ks, vs, ps, os_ = {}, {}, {}, {}, {}
            for j in range(0, NP, 2):
                for m, jj in cfg["order"]:
                    (qs, ks, vs)[m][j + jj] = proj(m, j + jj)
                ps[j] = qk(qs[j], ks[j], j == 0 and cfg["split"][0])
                ps[j + 1] = qk(qs[j + 1], ks[j + 1], j == 0 and cfg["split"][1])
                if j >= 2:
                    os_[j - 2] = pv(j - 2, ps[j - 2], vs[j - 2])
                    os_[j - 1] = pv(j - 1, ps[j - 1], vs[j - 1])
            na = NP - 2
            acc = {}
            nw = cfg["nw"]
            for n in range(nw):
                acc[n] = wo_part(os_, 0, na, n)
            os_[NP - 2] = pv(NP - 2, ps[NP - 2], vs[NP - 2], cfg["split"][2])
            os_[NP - 1] = pv(NP - 1, ps[NP - 1], vs[NP - 1], cfg["split"][3])
            acc[nw] = wo_part(os_, 0, na, nw)
            for n in range(nw + 1):
                acc[n] = wo_part(os_, na, NP, n, acc[n])
            for n in range(nw + 1, 8):
                acc[n] = wo_part(os_, 0, NP, n)
            assert state["count"] == 512 and not state["due"], state
            for w in range(2):
                conv_inv(a_ref, icb, idst, chunks[w][0], [zs[w][pos] for pos in range(16)])
            if t == UNROLL - 1:
                for tt in range(UNROLL):
                    conv_fwd(cb, r - t + tt)
            for n in range(NCB):
                b_ref[n, s, 0:NT, :] = acc[n][0:NT]
            return jnp.concatenate([acc[n][NT:SEG] for n in range(NCB)], axis=1).astype(bf16).astype(f32)

        def steps(i, mem):
            @pl.when(i == 8 // UNROLL)
            def _():
                wait_all(ssm_ref.at[:, 64:], SEM_SSM1)
            for t in range(UNROLL):
                mem = step(i * UNROLL + t, mem, t)
            return mem

        lax.fori_loop(0, _DBG_STEPS // UNROLL, steps, mem_ref[...].astype(f32))

        def out_copy(n):
            slot = n % 2
            return pltpu.make_async_copy(
                ost_ref.at[slot], out_hbm.at[:, :, pl.ds(pl.multiple_of(n * 128, 128), 128)],
                sems.at[SEM_OUT + slot])

        def fin(n, c):
            @pl.when(n >= 2)
            def _():
                out_copy(n - 2).wait()
            zs, toks, t = ([], []), [], None
            for pos in range(16):
                if pos % CFG["fgrp"] == 0:
                    t = None
                for w in range(2):
                    t = conv_mac((NCB - 1) % 2, n + 8 * w, 8 + 8 * w, pos, t)
                    zs[w].append(t)
                if pos % CFG["fgrp"] == CFG["fgrp"] - 1:
                    toks.append(t)
            bd = None
            for kb in range(8):
                if kb == CFG["finv"]:
                    for w in range(2):
                        conv_inv(a_ref, NCB - 1, NCB - 1, n + 8 * w, zs[w])
                w = after(wo_ref[n, kb * 256:(kb + 1) * 256, :], toks[kb - 1] if 0 < kb <= len(toks) else None)
                d = _dot(odef_ref[:, kb * 512:(kb + 1) * 512].astype(bf16), _as_bf16(w))
                bd = d if bd is None else d + bd
            b_ref[n, :, NT:SEG, :] = bd.reshape(NSEG, 8, 128)
            for blk in range(8):
                sg = slice(blk * 8, (blk + 1) * 8)
                b = b_ref[n, sg]
                a = a_ref[n, blk * 256:(blk + 1) * 256, :].reshape(8, SEG, 128)
                g = gate_ref[sg]
                ost_ref[n % 2, sg] = (g * a + (1.0 - g) * b).astype(bf16)
            out_copy(n).start()
            return c
        lax.fori_loop(0, NCB, fin, 0)
        out_copy(NCB - 2).wait()
        out_copy(NCB - 1).wait()

    pl.run_scoped(main, pltpu.VMEM((NSEG * 8, H * E), f32), pltpu.VMEM((NCB, NSEG, SEG, 128), f32),
                  pltpu.VMEM((NCB + 1, S, 128), f32))


@jax.jit
def pallas_gated_mix__ssm_conv_h3__memory_aug_recurrent_mem_tr__prompt_kernel(
    A_q: jax.Array,
    A_k: jax.Array,
    A_v: jax.Array,
    A_shift_k: jax.Array,
    A_ssm_k: jax.Array,
    A_ssm_D: jax.Array,
    B_x: jax.Array,
    B_mem0: jax.Array,
    B_Wq: jax.Array,
    B_Wk: jax.Array,
    B_Wv: jax.Array,
    B_Wo: jax.Array,
    B_seg_len: jax.Array,
    gate_w: jax.Array,
):
    del B_x, B_seg_len
    f_tab, g_tab = _dft_tables()
    out = pl.pallas_call(
        _kernel,
        out_shape=jax.ShapeDtypeStruct((NSEG, SEG, D), bf16),
        in_specs=[pl.BlockSpec(memory_space=pl.ANY)] * 15,
        out_specs=pl.BlockSpec(memory_space=pl.ANY),
        scratch_shapes=[
            pltpu.VMEM((3 * H, D // 2, E), u32),
            pltpu.VMEM((NCB, H * E // 2, 128), u32),
            pltpu.VMEM((NCB, S // 2, 128), u32),
            pltpu.VMEM((NQ, NSEG, M, DQ), bf16),
            pltpu.VMEM((NQ, NSEG * 4, DQ), u32),
            pltpu.VMEM((NSEG, 3 * NP, 8, E), u32),
            pltpu.VMEM((NCB + 1, KPAD + S // 2, 128), u32),
            pltpu.VMEM((NCB + 1, S // 2, 128), u32),
            pltpu.VMEM((NCH, D // 2, 128), u32),
            pltpu.VMEM((NCB + 1, S // 2, 128), u32),
            pltpu.VMEM((2, NZ + NCH, 256, 128), f32),
            pltpu.VMEM((2, NCH, 256, 128), f32),
            pltpu.VMEM((256, 128), f32),
            pltpu.VMEM((8, 128), jnp.int32),
            pltpu.VMEM((256, 128), bf16),
            pltpu.VMEM((128, 256), bf16),
            pltpu.VMEM((80, 128), f32),
            pltpu.VMEM((KS, D), bf16),
            pltpu.VMEM((NCB + 1, 8, 128), f32),
            pltpu.VMEM((NCB, 128), bf16),
            pltpu.VMEM((NCB, 128), bf16),
            pltpu.VMEM((M, D), bf16),
            pltpu.VMEM((NSEG, SEG, 128), f32),
            pltpu.VMEM((2, NSEG, SEG, 128), bf16),
            pltpu.SemaphoreType.DMA((NSEM,)),
        ],
        compiler_params=pltpu.CompilerParams(vmem_limit_bytes=120 * 2**20),
    )(A_q.reshape(NSEG, SEG, D), A_q.reshape(S, D), A_k.reshape(S, D), A_v.reshape(S, D), A_shift_k.T,
      A_ssm_k, A_ssm_D.reshape(NCB, 128), B_mem0.reshape(M, D), B_Wq, B_Wk, B_Wv,
      B_Wo.reshape(H * E, D), gate_w.reshape(NCB, 128), f_tab, g_tab)
    return out.reshape(1, S, D)
```

```python
import functools

import numpy as np
import jax
import jax.numpy as jnp
from jax import lax
import jax.experimental.pallas as pl
import jax.experimental.pallas.tpu as pltpu

S, D, H, E, M, SEG = 2048, 1024, 32, 128, 8, 32
NSEG = S // SEG
NT = SEG - M
NP = H // 2
NCB = D // 128
C = 128
NCH = S // C
LOG2E = 1.4426950408889634
KS = 4
NZ = 8
KPAD = 32
NG = 6
NQ = 8
DQ = D // NQ
UNROLL = 4
CFG = dict(npt=28, fgrp=4, finv=4, steps=[
    dict(dues=[12, 16, 20, 24, 28, 32, 36, 40, 44, 88, 136, 184, 232, 280, 328, 376, 444, 172, 452, 456, 460, 464,
               468, 472, 476, 480, 484, 488, 200, 496, 500, 504],
         sm=[124, 140, 164, 188, 212, 236, 260, 284, 308, 332, 356, 380, None, None, None, None],
         gate=440, nw=3, order=((0, 0), (1, 0), (0, 1), (1, 1), (2, 0), (2, 1))),
    dict(dues=[464, 16, 20, 24, 28, 32, 36, 40, 44, 88, 136, 184, 232, 280, 328, 376, 444, 448, 452, 456, 460, 84,
               468, 472, 476, 436, 484, 488, 492, 496, 500, 504],
         sm=[124, 140, 164, 188, 212, 236, 260, 284, 308, 332, 356, 380, None, None, None, None],
         gate=440, nw=3, order=((1, 0), (0, 0), (1, 1), (0, 1), (2, 1), (2, 0))),
    dict(dues=[12, 16, 20, 24, 28, 32, 36, 40, 44, 88, 136, 184, 232, 280, 328, 376, 444, 448, 452, 456, 460, 464,
               468, 472, 476, 480, 484, 488, 492, 496, 500, 504],
         sm=[124, 140, 164, 188, 212, 236, 260, 284, 308, 332, 356, 380, None, None, None, None],
         gate=92, nw=4, order=((0, 0), (1, 0), (0, 1), (1, 1), (2, 0), (2, 1))),
    dict(dues=[12, 16, 20, 24, 28, 32, 36, 40, 44, 88, 136, 184, 232, 244, 328, 376, 444, 448, 452, 456, 460, 464,
               468, 472, 476, 480, 484, 488, 492, 496, 500, 136],
         sm=[124, 140, 128, 188, 212, 212, 260, 284, 308, 332, 356, 380, None, None, None, None],
         gate=440, nw=3, order=((0, 0), (1, 0), (0, 1), (1, 1), (2, 0), (2, 1))),
])
_DBG_STEPS = NSEG
bf16, f32, u32 = jnp.bfloat16, jnp.float32, jnp.uint32


def _dft_tables():
    t = np.arange(C, dtype=np.float64)
    rows = []
    for r in range(8):
        ev = 16 * r + np.arange(0, 16, 2)
        od = ev + 1
        for fn, fs in ((np.cos, ev), (np.sin, ev), (np.cos, od), (np.sin, od)):
            rows.append(fn(np.pi * (2 * fs[:, None] + 1) * t[None, :] / (2 * C)))
    f = np.concatenate(rows, axis=0)
    return f.astype(bf16), (f.T / C).astype(bf16)


def _fill_matrix():
    r = lax.broadcasted_iota(jnp.int32, (80, 128), 0)
    c = lax.broadcasted_iota(jnp.int32, (80, 128), 1)

    def head(i):
        return jnp.where(i < 64, i // 32, (i - 64) // 8)

    def idx(i):
        lo = i % 32
        main = jnp.where(lo < NT, lo + M, lo - NT)
        return jnp.where(i < 64, main, (i - 64) % 8 + NT + M)

    same = (head(r) == head(c)) & (c < 80)
    ok = (idx(r) < M) | (idx(r) >= idx(c))
    return jnp.where(same, jnp.where(ok, 0.0, -1e9 * E ** 0.5), -jnp.inf).astype(f32)


def _as_bf16(v):
    return pltpu.bitcast(v, bf16)


def _dot(a, b):
    return jnp.dot(a, b, preferred_element_type=f32)


def _dot_nt(a, b):
    return lax.dot_general(a, b, (((1,), (1,)), ((), ())), preferred_element_type=f32)


SEM_SMALL, SEM_WO, SEM_X, SEM_SSM0, SEM_SSM1 = range(5)
SEM_Q = 5
SEM_K = SEM_Q + NQ
SEM_V = SEM_K + 4
SEM_W = SEM_V + 4
SEM_OUT = SEM_W + NG - 1
NSEM = SEM_OUT + 2


def _kernel(x3_hbm, x_hbm, k_hbm, v_hbm, shift_hbm, ssm_hbm, d_hbm, mem_hbm, wq_hbm, wk_hbm, wv_hbm,
            wo_hbm, gw_hbm, f_hbm, g_hbm, out_hbm,
            wn_ref, wo_ref, x_ref, xr_ref, xb_ref, pre_ref, k_ref, v_ref, ssm_ref, u_ref,
            fu_ref, fk_ref, kraw_ref, one_ref, f_ref, g_ref, fill_ref, shift_ref, wt_ref,
            d_ref, gw_ref, mem_ref, gate_ref, ost_ref, sems):
    w_hbm = (wq_hbm, wk_hbm, wv_hbm)

    def cp(src, dst, sem):
        return pltpu.make_async_copy(src, dst, sems.at[sem])

    def start_col_blocks(src_hbm, dst_ref, i0, i1, sem, row0=0):
        src = src_hbm.bitcast(u32)
        for i in range(i0, i1):
            cp(src.at[:, i * 128:(i + 1) * 128], dst_ref.at[i, row0:], sem).start()

    def start_ssm(r0, r1, sem):
        src = ssm_hbm.bitcast(u32)
        for a in range(NCH):
            cp(src.at[r0:r1, a * C:(a + 1) * C], ssm_ref.at[a, r0:r1], sem).start()

    def wait_all(dst, sem):
        cp(dst, dst, sem).wait()

    def even(p):
        return pltpu.bitcast(p << 16, f32)

    def odd(p):
        return pltpu.bitcast(p & jnp.uint32(0xFFFF0000), f32)

    def conv_prep(cb, i, dep=None):
        r0 = KPAD + 8 * i
        p0 = k_ref[cb, r0:r0 + 8, :]
        if dep is not None:
            p0 = jnp.where(one_ref[...] == 1, p0, dep)
        p1 = k_ref[cb, r0 - 1:r0 + 7, :]
        p2 = k_ref[cb, r0 - 2:r0 + 6, :]
        pv = v_ref[cb, 8 * i:8 * i + 8, :]
        w = wt_ref[cb]
        w0, w1, w2, w3 = w[0:1, :], w[1:2, :], w[2:3, :], w[3:4, :]
        e0, o0, e1, o1, o2 = even(p0), odd(p0), even(p1), odd(p1), odd(p2)
        ke = ((e0 * w0 + o1 * w1) + e1 * w2) + o2 * w3
        ko = ((o0 * w0 + e0 * w1) + o1 * w2) + e1 * w3
        re = pltpu.bitcast((ke * even(pv)).astype(bf16).astype(f32), u32)
        ro = pltpu.bitcast((ko * odd(pv)).astype(bf16).astype(f32), u32)
        kv = (re >> 16) | (ro & jnp.uint32(0xFFFF0000))
        u_ref[cb, 8 * i:8 * i + 8, :] = kv
        return kv

    def combine(kf, prev):
        out = []
        for g in range(8):
            o = 32 * g
            out += [kf[o:o + 8] + prev[o + 8:o + 16], kf[o + 8:o + 16] - prev[o:o + 8],
                    kf[o + 16:o + 24] - prev[o + 24:o + 32], kf[o + 24:o + 32] + prev[o + 16:o + 24]]
        return jnp.concatenate(out, axis=0)

    def conv_fwd(cb, r):
        slot = cb % 2
        rows = pl.ds(pl.multiple_of(cb * 64, 64), 64)
        f = f_ref[...]
        kfs = []
        for a in (2 * r, 2 * r + 1):
            fu_ref[slot, NZ + a] = _dot(f, _as_bf16(u_ref[cb, pl.ds(pl.multiple_of(a * 64, 64), 64), :]))
            kfs.append(_dot_nt(f, _as_bf16(ssm_ref[a, rows, :])))
        fk_ref[slot, 2 * r] = combine(kfs[0], jnp.where(r > 0, kraw_ref[...], 0.0))
        fk_ref[slot, 2 * r + 1] = combine(kfs[1], kfs[0])
        kraw_ref[...] = kfs[1]

    def conv_mac(slot, a, nterms, pos, dep=None):
        rows = slice(pos * 16, pos * 16 + 16)
        p = q = None
        for c in range(nterms):
            u = fu_ref[slot, NZ + a - c, rows, :]
            k = fk_ref[slot, c, rows, :]
            ua, ub, kc, kd = u[0:8], u[8:16], k[0:8], k[8:16]
            if c == 0 and dep is not None:
                ua = jnp.where(one_ref[...] == 1, ua, pltpu.bitcast(dep, f32))
            p = (ua * kc if p is None else p + ua * kc) - ub * kd
            q = (ua * kd if q is None else q + ua * kd) + ub * kc
        return pltpu.bitcast(jnp.concatenate([p, q], axis=0).astype(bf16), u32)

    def conv_inv(a_ref, cb, dst, a, zs):
        rows = pl.ds(pl.multiple_of(a * 64, 64), 64)
        y = _dot(g_ref[...], _as_bf16(jnp.concatenate(zs, axis=0)))
        kv = _as_bf16(u_ref[cb, rows, :]).astype(f32)
        q = _as_bf16(x_ref[cb, rows, :]).astype(f32)
        a_ref[dst, pl.ds(pl.multiple_of(a * C, C), C), :] = q * (y + kv * wt_ref[cb, KS:KS + 1, :])

    def after(w, tok):
        if tok is None:
            return w
        return jnp.concatenate([jnp.where(one_ref[...] == 1, w[0:8], tok), w[8:]], axis=0)

    def prologue(stage_ref, acc_ref):
        st3 = stage_ref.reshape(NG * D, 8, E)

        def start_w(g):
            r0 = (g % 2) * 8
            cp(w_hbm[g // 2].bitcast(u32).at[:, r0:r0 + 8, :], st3.at[g * D:(g + 1) * D], SEM_W + g - 1).start()

        def slice_copies(q):
            cols = pl.ds(pl.multiple_of(q * DQ, DQ), DQ)
            return (cp(x3_hbm.at[:, NT:SEG, cols], xr_ref.at[q], SEM_Q + q),
                    cp(wq_hbm.bitcast(u32).at[cols, 0:8, :], st3.at[cols], SEM_Q + q))

        small = [cp(shift_hbm, shift_ref, SEM_SMALL), cp(d_hbm, d_ref, SEM_SMALL), cp(gw_hbm, gw_ref, SEM_SMALL),
                 cp(mem_hbm, mem_ref, SEM_SMALL), cp(f_hbm, f_ref, SEM_SMALL), cp(g_hbm, g_ref, SEM_SMALL)]
        for q in range(NQ):
            for c in slice_copies(q):
                c.start()
        for c in small:
            c.start()
        for g in range(1, NG):
            start_w(g)
            if g >= 2:
                start_col_blocks(k_hbm, k_ref, 2 * g - 4, 2 * g - 2, SEM_K + g - 2, row0=KPAD)
                start_col_blocks(v_hbm, v_ref, 2 * g - 4, 2 * g - 2, SEM_V + g - 2)
        start_col_blocks(wo_hbm, wo_ref, 0, NCB, SEM_WO)
        fill_ref[...] = _fill_matrix()
        one_ref[...] = jnp.ones((8, 128), jnp.int32)
        k_ref[:, KPAD - 8:KPAD, :] = jnp.zeros((NCB + 1, 8, 128), u32)
        wt_ref[...] = jnp.zeros(wt_ref.shape, f32)
        kraw_ref[...] = jnp.zeros(kraw_ref.shape, f32)
        fu_ref[0, NZ - 1] = jnp.zeros((256, 128), f32)

        def clear(a, c):
            rows = pl.ds(pl.multiple_of(a * 64, 64), 64)
            k_ref[NCB, pl.ds(pl.multiple_of(KPAD + a * 64, 32), 64), :] = jnp.zeros((64, 128), u32)
            v_ref[NCB, rows, :] = jnp.zeros((64, 128), u32)
            acc_ref[a] = jnp.zeros((NSEG * M, E), f32)
            return c
        lax.fori_loop(0, 16, clear, 0)

        def unpack_pair(w):
            return pltpu.bitcast(even(w).astype(bf16), u32), pltpu.bitcast(odd(w).astype(bf16), u32)

        def store_pre(idx, r1, r2):
            cc = jnp.concatenate([r1.reshape(NSEG, 8, E), r2.reshape(NSEG, 8, E)], axis=1).astype(bf16)
            pre_ref[:, idx] = pltpu.bitcast(cc, u32)

        def first(q, c):
            for cc in slice_copies(q):
                cc.wait()
            xq = pltpu.bitcast(xr_ref[q].astype(f32).reshape(NSEG * M, DQ).astype(bf16), u32)
            xb_ref[q] = xq
            sub = stage_ref.at[pl.ds(pl.multiple_of(q * (8 * DQ), 8 * DQ), 8 * DQ), :]
            rows = pl.ds(pl.multiple_of(q * (DQ // 2), DQ // 2), DQ // 2)
            for j in range(8):
                rs = []
                for h, w in zip((2 * j, 2 * j + 1), unpack_pair(sub[pl.ds(j, DQ, stride=8), :])):
                    wn_ref[h, rows, :] = w
                    r = _dot(_as_bf16(xq), _as_bf16(w)) + acc_ref[h]
                    acc_ref[h] = r
                    rs.append(r)
                store_pre(j, *rs)
            return c
        lax.fori_loop(0, NQ, first, 0)

        start_col_blocks(x_hbm, x_ref, 0, NCB, SEM_X)
        start_ssm(0, 64, SEM_SSM0)
        for c in small:
            c.wait()
        sh = shift_ref[...].astype(f32)
        dv = d_ref[...].astype(f32)
        for n in range(NCB):
            wt_ref[n, 0:KS, :] = sh[:, n * 128:(n + 1) * 128]
            wt_ref[n, KS:KS + 1, :] = dv[n:n + 1, :]

        def group(g, c):
            wait_all(st3.at[pl.ds(g * D, D)], SEM_W + g - 1)

            @pl.when(g >= 2)
            def _():
                wait_all(k_ref.at[pl.ds(2 * g - 4, 2), KPAD:], SEM_K + g - 2)
                wait_all(v_ref.at[pl.ds(2 * g - 4, 2)], SEM_V + g - 2)

            cbs = [jnp.where(g >= 2, 2 * g - 4 + i, NCB) for i in range(2)]
            npt = CFG["npt"]
            toks = [None] * 32
            for k in range(npt):
                t = None
                for i in range(k * 256 // npt, (k + 1) * 256 // npt):
                    t = conv_prep(cbs[i // 128], i % 128, t)
                    zero = pltpu.bitcast(jnp.where(one_ref[...] == 1, jnp.uint32(0), t), f32)
                    for v in range(i, 288, 256):
                        rows = slice(8 * (v % 32), 8 * (v % 32) + 8)
                        if v < 160:
                            fu_ref[1, jnp.minimum((g - 1) * 5 + v // 32, NZ + NCH - 1), rows, :] = zero
                        else:
                            fk_ref[1, jnp.minimum((g - 1) * 4 + v // 32 - 5, NCH - 1), rows, :] = zero
                toks[32 - npt + k] = t
            sub = stage_ref.at[pl.ds(pl.multiple_of(g * (8 * D), 8 * D), 8 * D), :]
            for j in range(8):
                ws = [unpack_pair(sub[pl.ds(blk * 2048 + j, 256, stride=8), :]) for blk in range(D // 256)]
                xb = _as_bf16(jnp.concatenate([xb_ref[q] for q in range(NQ)], axis=1))
                rs = [None, None]
                for i in range(2):
                    wn_ref[g * 16 + 2 * j + i] = jnp.concatenate([wb[i] for wb in ws], axis=0)
                if j == 0:
                    for blk in range(D // 256):
                        for i in range(2):
                            d = _dot(xb[:, blk * 256:(blk + 1) * 256], _as_bf16(ws[blk][i]))
                            rs[i] = d if rs[i] is None else d + rs[i]
                else:
                    for i in range(2):
                        tk = toks[4 * j + 2 * i:4 * j + 2 * i + 2]
                        w = jnp.concatenate([after(ws[0][i], tk[0]), ws[1][i], after(ws[2][i], tk[1]), ws[3][i]], axis=0)
                        rs[i] = _dot(xb, _as_bf16(w))
                store_pre(g * 8 + j, *rs)
            return c
        lax.fori_loop(1, NG, group, 0)

    pl.run_scoped(prologue, pltpu.VMEM((NG * 8 * D, E), u32), pltpu.VMEM((16, NSEG * M, E), f32))

    start_ssm(64, D // 2, SEM_SSM1)
    wait_all(wo_ref, SEM_WO)
    wait_all(x_ref, SEM_X)
    wait_all(ssm_ref.at[:, 0:64], SEM_SSM0)

    scale = E ** -0.5

    def main(odef_ref, b_ref, a_ref):
        def step(s, mem, t):
            cfg = CFG["steps"][t]
            cb = s // 8
            r = s % 8
            icb = jnp.maximum(cb - 1, 0)
            idst = jnp.where(cb >= 1, cb - 1, NCB)
            mslot = (cb + 1) % 2
            nh = 8 // UNROLL
            chunks = ((nh * t + r // UNROLL, nh * t + nh), (NCH - 1 - nh * t - r // UNROLL, NCH - nh * t))
            zs = ({}, {})

            xrows = pl.ds(pl.multiple_of(s * 16, 16), 16)
            xs = [_as_bf16(x_ref[n, xrows, :]).astype(f32) for n in range(NCB)]
            h32 = jnp.concatenate([jnp.concatenate(xs, axis=1)[0:NT], mem], axis=0).astype(bf16)
            r0 = pl.multiple_of(s * 8, 8)

            def gate():
                gw = gw_ref[...].astype(f32)
                gl = None
                for n in range(NCB):
                    xg = _as_bf16(x_ref[n, xrows, :]).astype(f32) * gw[n:n + 1, :]
                    gl = xg if gl is None else gl + xg
                g = jnp.broadcast_to(jax.nn.sigmoid(jnp.sum(gl, axis=-1, keepdims=True)), (SEG, 128))
                gate_ref[s] = g
                g = pltpu.bitcast(g, u32)
                return (g[0:8] | g[8:16]) | (g[16:24] | g[24:32])

            def mac_job(w, pos):
                zs[w][pos] = conv_mac(mslot, chunks[w][0], chunks[w][1], pos)
                return zs[w][pos]

            jobs = [(cfg["dues"][i], functools.partial(mac_job, i % 2, i // 2)) for i in range(32)]
            jobs.append((cfg["gate"], gate))
            state = dict(count=0, due={})

            def sdot(lhs, w, acc=None, weight=1):
                c = state["count"]
                toks = [t for cc in range(c, c + weight) for t in state["due"].pop(cc, [])]
                nt = w.shape[0] // 64
                if toks:
                    tiles = [w[64 * i:64 * (i + 1)] for i in range(nt)]
                    for i, t in enumerate(toks):
                        tiles[i % nt] = after(tiles[i % nt], t)
                    w = jnp.concatenate(tiles, axis=0)
                d = _dot(lhs, _as_bf16(w))
                d = d if acc is None else d + acc
                for due, fn in jobs:
                    if c <= due - 4 < c + weight:
                        state["due"].setdefault(due, []).append(fn())
                state["count"] = c + weight
                return d

            def proj(m, j):
                r1 = sdot(h32, wn_ref[m * H + 2 * j], weight=4)
                r2 = sdot(h32, wn_ref[m * H + 2 * j + 1], weight=4)
                p = _as_bf16(pre_ref[s, m * NP + j]).astype(f32)
                if m == 0:
                    return jnp.concatenate([r1, r2, p], axis=0)
                return jnp.concatenate([r1, r2, p, jnp.zeros((48, E), f32)], axis=0).astype(bf16)

            def qk(q80, k80, due):
                fill = fill_ref[...]
                sc = jnp.where(fill == 0.0, _dot_nt(q80.astype(bf16), k80), fill)
                p = jnp.exp2((sc - jnp.max(sc, axis=-1, keepdims=True)) * (scale * LOG2E))
                den = jnp.sum(p, axis=-1, keepdims=True)
                rc = pl.reciprocal(den, approx=True)
                p = p * (rc * (2.0 - den * rc))
                if due is not None:
                    pb = pltpu.bitcast(p, u32)
                    tok = pb[0:8]
                    for i in range(1, 10):
                        tok = tok | pb[8 * i:8 * i + 8]
                    state["due"].setdefault(due, []).append(tok)
                return p

            def pv(j, p, v80):
                o80 = _dot(p.astype(bf16), v80)
                odef_ref[pl.ds(r0, 8), (2 * j) * E:(2 * j + 1) * E] = o80[64:72]
                odef_ref[pl.ds(r0, 8), (2 * j + 1) * E:(2 * j + 2) * E] = o80[72:80]
                return jnp.concatenate([o80[0:32], o80[32:64]], axis=1).astype(bf16)

            def wo_part(o, j0, j1, n, acc=None):
                for j in range(j0, j1):
                    acc = sdot(o[j], wo_ref[n, j * 128:(j + 1) * 128, :], acc)
                return acc

            qs, ks, vs, ps, os_ = {}, {}, {}, {}, {}
            for j in range(0, NP, 2):
                for m, jj in cfg["order"]:
                    (qs, ks, vs)[m][j + jj] = proj(m, j + jj)
                if j == 2:
                    for jj in range(4):
                        ps[jj] = qk(qs[jj], ks[jj], cfg["sm"][jj])
                elif j > 2:
                    ps[j] = qk(qs[j], ks[j], cfg["sm"][j])
                    ps[j + 1] = qk(qs[j + 1], ks[j + 1], cfg["sm"][j + 1])
                    os_[j - 4] = pv(j - 4, ps[j - 4], vs[j - 4])
                    os_[j - 3] = pv(j - 3, ps[j - 3], vs[j - 3])
            na = NP - 4
            acc = {}
            nw = cfg["nw"]
            for n in range(nw):
                acc[n] = wo_part(os_, 0, na, n)
            for jj in range(na, NP):
                os_[jj] = pv(jj, ps[jj], vs[jj])
            acc[nw] = wo_part(os_, 0, na, nw)
            for n in range(nw + 1):
                acc[n] = wo_part(os_, na, NP, n, acc[n])
            for n in range(nw + 1, 8):
                acc[n] = wo_part(os_, 0, NP, n)
            assert state["count"] == 512 and not state["due"], state
            for w in range(2):
                conv_inv(a_ref, icb, idst, chunks[w][0], [zs[w][pos] for pos in range(16)])
            if t == UNROLL - 1:
                for tt in range(UNROLL):
                    conv_fwd(cb, r - t + tt)
            for n in range(NCB):
                b_ref[n, s, 0:NT, :] = acc[n][0:NT]
            return jnp.concatenate([acc[n][NT:SEG] for n in range(NCB)], axis=1).astype(bf16).astype(f32)

        def steps(i, mem):
            @pl.when(i == 8 // UNROLL)
            def _():
                wait_all(ssm_ref.at[:, 64:], SEM_SSM1)
            for t in range(UNROLL):
                mem = step(i * UNROLL + t, mem, t)
            return mem

        lax.fori_loop(0, _DBG_STEPS // UNROLL, steps, mem_ref[...].astype(f32))

        def out_copy(n):
            slot = n % 2
            return pltpu.make_async_copy(
                ost_ref.at[slot], out_hbm.at[:, :, pl.ds(pl.multiple_of(n * 128, 128), 128)],
                sems.at[SEM_OUT + slot])

        def fin(n, c):
            @pl.when(n >= 2)
            def _():
                out_copy(n - 2).wait()
            zs, toks, t = ([], []), [], None
            for pos in range(16):
                if pos % CFG["fgrp"] == 0:
                    t = None
                for w in range(2):
                    t = conv_mac((NCB - 1) % 2, n + 8 * w, 8 + 8 * w, pos, t)
                    zs[w].append(t)
                if pos % CFG["fgrp"] == CFG["fgrp"] - 1:
                    toks.append(t)
            bd = None
            for kb in range(8):
                if kb == CFG["finv"]:
                    for w in range(2):
                        conv_inv(a_ref, NCB - 1, NCB - 1, n + 8 * w, zs[w])
                w = after(wo_ref[n, kb * 256:(kb + 1) * 256, :], toks[kb - 1] if 0 < kb <= len(toks) else None)
                d = _dot(odef_ref[:, kb * 512:(kb + 1) * 512].astype(bf16), _as_bf16(w))
                bd = d if bd is None else d + bd
            b_ref[n, :, NT:SEG, :] = bd.reshape(NSEG, 8, 128)
            for blk in range(8):
                sg = slice(blk * 8, (blk + 1) * 8)
                b = b_ref[n, sg]
                a = a_ref[n, blk * 256:(blk + 1) * 256, :].reshape(8, SEG, 128)
                g = gate_ref[sg]
                ost_ref[n % 2, sg] = (g * a + (1.0 - g) * b).astype(bf16)
            out_copy(n).start()
            return c
        lax.fori_loop(0, NCB, fin, 0)
        out_copy(NCB - 2).wait()
        out_copy(NCB - 1).wait()

    pl.run_scoped(main, pltpu.VMEM((NSEG * 8, H * E), f32), pltpu.VMEM((NCB, NSEG, SEG, 128), f32),
                  pltpu.VMEM((NCB + 1, S, 128), f32))


@jax.jit
def pallas_gated_mix__ssm_conv_h3__memory_aug_recurrent_mem_tr__prompt_kernel(
    A_q: jax.Array,
    A_k: jax.Array,
    A_v: jax.Array,
    A_shift_k: jax.Array,
    A_ssm_k: jax.Array,
    A_ssm_D: jax.Array,
    B_x: jax.Array,
    B_mem0: jax.Array,
    B_Wq: jax.Array,
    B_Wk: jax.Array,
    B_Wv: jax.Array,
    B_Wo: jax.Array,
    B_seg_len: jax.Array,
    gate_w: jax.Array,
):
    del B_x, B_seg_len
    f_tab, g_tab = _dft_tables()
    out = pl.pallas_call(
        _kernel,
        out_shape=jax.ShapeDtypeStruct((NSEG, SEG, D), bf16),
        in_specs=[pl.BlockSpec(memory_space=pl.ANY)] * 15,
        out_specs=pl.BlockSpec(memory_space=pl.ANY),
        scratch_shapes=[
            pltpu.VMEM((3 * H, D // 2, E), u32),
            pltpu.VMEM((NCB, H * E // 2, 128), u32),
            pltpu.VMEM((NCB, S // 2, 128), u32),
            pltpu.VMEM((NQ, NSEG, M, DQ), bf16),
            pltpu.VMEM((NQ, NSEG * 4, DQ), u32),
            pltpu.VMEM((NSEG, 3 * NP, 8, E), u32),
            pltpu.VMEM((NCB + 1, KPAD + S // 2, 128), u32),
            pltpu.VMEM((NCB + 1, S // 2, 128), u32),
            pltpu.VMEM((NCH, D // 2, 128), u32),
            pltpu.VMEM((NCB + 1, S // 2, 128), u32),
            pltpu.VMEM((2, NZ + NCH, 256, 128), f32),
            pltpu.VMEM((2, NCH, 256, 128), f32),
            pltpu.VMEM((256, 128), f32),
            pltpu.VMEM((8, 128), jnp.int32),
            pltpu.VMEM((256, 128), bf16),
            pltpu.VMEM((128, 256), bf16),
            pltpu.VMEM((80, 128), f32),
            pltpu.VMEM((KS, D), bf16),
            pltpu.VMEM((NCB + 1, 8, 128), f32),
            pltpu.VMEM((NCB, 128), bf16),
            pltpu.VMEM((NCB, 128), bf16),
            pltpu.VMEM((M, D), bf16),
            pltpu.VMEM((NSEG, SEG, 128), f32),
            pltpu.VMEM((2, NSEG, SEG, 128), bf16),
            pltpu.SemaphoreType.DMA((NSEM,)),
        ],
        compiler_params=pltpu.CompilerParams(vmem_limit_bytes=120 * 2**20),
    )(A_q.reshape(NSEG, SEG, D), A_q.reshape(S, D), A_k.reshape(S, D), A_v.reshape(S, D), A_shift_k.T,
      A_ssm_k, A_ssm_D.reshape(NCB, 128), B_mem0.reshape(M, D), B_Wq, B_Wk, B_Wv,
      B_Wo.reshape(H * E, D), gate_w.reshape(NCB, 128), f_tab, g_tab)
    return out.reshape(1, S, D)
```

```python
import functools

import numpy as np
import jax
import jax.numpy as jnp
from jax import lax
import jax.experimental.pallas as pl
import jax.experimental.pallas.tpu as pltpu

S, D, H, E, M, SEG = 2048, 1024, 32, 128, 8, 32
NSEG = S // SEG
NT = SEG - M
NP = H // 2
NCB = D // 128
C = 128
NCH = S // C
LOG2E = 1.4426950408889634
KS = 4
NZ = 8
KPAD = 32
NG = 6
NQ = 8
DQ = D // NQ
UNROLL = 4
CFG = dict(npt=28, fgrp=4, finv=4, steps=[
    dict(dues=[12, 16, 20, 24, 28, 32, 36, 40, 44, 88, 136, 184, 232, 280, 328, 376, 444, 172, 452, 456, 460, 464,
               468, 472, 476, 480, 484, 488, 200, 496, 500, 504],
         sm=[124, 140, 164, 188, 212, 236, 260, 284, 308, 332, 356, 380, None, None, None, None],
         gate=440, nw=3, order=((0, 0), (1, 0), (0, 1), (1, 1), (2, 0), (2, 1))),
    dict(dues=[464, 16, 20, 24, 28, 32, 36, 40, 44, 88, 136, 184, 232, 280, 328, 376, 444, 448, 452, 456, 460, 84,
               468, 472, 476, 436, 484, 488, 492, 496, 500, 504],
         sm=[124, 140, 164, 188, 212, 236, 260, 284, 308, 332, 356, 380, None, None, None, None],
         gate=440, nw=3, order=((1, 0), (0, 0), (1, 1), (0, 1), (2, 1), (2, 0))),
    dict(dues=[12, 16, 20, 24, 28, 32, 36, 40, 44, 88, 136, 184, 232, 280, 328, 376, 444, 448, 452, 456, 460, 464,
               468, 472, 476, 480, 484, 488, 492, 496, 500, 504],
         sm=[124, 140, 164, 188, 212, 236, 260, 284, 308, 332, 356, 380, None, None, None, None],
         gate=92, nw=4, order=((0, 0), (1, 0), (0, 1), (1, 1), (2, 0), (2, 1))),
    dict(dues=[12, 16, 20, 24, 28, 32, 36, 40, 44, 88, 136, 184, 232, 244, 328, 376, 444, 448, 452, 456, 460, 464,
               468, 472, 476, 480, 484, 488, 492, 496, 500, 136],
         sm=[124, 140, 128, 188, 212, 212, 260, 284, 308, 332, 356, 380, None, None, None, None],
         gate=440, nw=3, order=((0, 0), (1, 0), (0, 1), (1, 1), (2, 0), (2, 1))),
])
_DBG_STEPS = NSEG
bf16, f32, u32 = jnp.bfloat16, jnp.float32, jnp.uint32


def _dft_tables():
    t = np.arange(C, dtype=np.float64)
    rows = []
    for r in range(8):
        ev = 16 * r + np.arange(0, 16, 2)
        od = ev + 1
        for fn, fs in ((np.cos, ev), (np.sin, ev), (np.cos, od), (np.sin, od)):
            rows.append(fn(np.pi * (2 * fs[:, None] + 1) * t[None, :] / (2 * C)))
    f = np.concatenate(rows, axis=0)
    return f.astype(bf16), (f.T / C).astype(bf16)


def _fill_matrix():
    r = lax.broadcasted_iota(jnp.int32, (80, 128), 0)
    c = lax.broadcasted_iota(jnp.int32, (80, 128), 1)

    def head(i):
        return jnp.where(i < 64, i // 32, (i - 64) // 8)

    def idx(i):
        lo = i % 32
        main = jnp.where(lo < NT, lo + M, lo - NT)
        return jnp.where(i < 64, main, (i - 64) % 8 + NT + M)

    same = (head(r) == head(c)) & (c < 80)
    ok = (idx(r) < M) | (idx(r) >= idx(c))
    return jnp.where(same, jnp.where(ok, 0.0, -1e9 * E ** 0.5), -jnp.inf).astype(f32)


def _as_bf16(v):
    return pltpu.bitcast(v, bf16)


def _dot(a, b):
    return jnp.dot(a, b, preferred_element_type=f32)


def _dot_nt(a, b):
    return lax.dot_general(a, b, (((1,), (1,)), ((), ())), preferred_element_type=f32)


SEM_SMALL, SEM_WO = range(2)
SEM_Q = 2
SEM_K = SEM_Q + NQ
SEM_V = SEM_K + 4
SEM_W = SEM_V + 4
NSEM = SEM_W + NG - 1
SEM_X, SEM_SSM0, SEM_SSM1, SEM_OUT = SEM_Q, SEM_Q + 1, SEM_Q + 2, SEM_Q + 3


def _kernel(x3_hbm, x_hbm, k_hbm, v_hbm, shift_hbm, ssm_hbm, d_hbm, mem_hbm, wq_hbm, wk_hbm, wv_hbm,
            wo_hbm, gw_hbm, f_hbm, g_hbm, out_hbm,
            wn_ref, wo_ref, x_ref, xr_ref, xb_ref, pre_ref, k_ref, v_ref, ssm_ref, u_ref,
            fu_ref, fk_ref, kraw_ref, one_ref, f_ref, g_ref, fill_ref, shift_ref, wt_ref,
            d_ref, gw_ref, mem_ref, gate_ref, ost_ref, sems):
    w_hbm = (wq_hbm, wk_hbm, wv_hbm)

    def cp(src, dst, sem):
        return pltpu.make_async_copy(src, dst, sems.at[sem])

    def start_col_blocks(src_hbm, dst_ref, i0, i1, sem, row0=0):
        src = src_hbm.bitcast(u32)
        for i in range(i0, i1):
            cp(src.at[:, i * 128:(i + 1) * 128], dst_ref.at[i, row0:], sem).start()

    def start_ssm(r0, r1, sem):
        src = ssm_hbm.bitcast(u32)
        for a in range(NCH):
            cp(src.at[r0:r1, a * C:(a + 1) * C], ssm_ref.at[a, r0:r1], sem).start()

    def wait_all(dst, sem):
        cp(dst, dst, sem).wait()

    def even(p):
        return pltpu.bitcast(p << 16, f32)

    def odd(p):
        return pltpu.bitcast(p & jnp.uint32(0xFFFF0000), f32)

    def conv_prep(cb, i, dep=None):
        r0 = KPAD + 8 * i
        p0 = k_ref[cb, r0:r0 + 8, :]
        if dep is not None:
            p0 = jnp.where(one_ref[...] == 1, p0, dep)
        p1 = k_ref[cb, r0 - 1:r0 + 7, :]
        p2 = k_ref[cb, r0 - 2:r0 + 6, :]
        pv = v_ref[cb, 8 * i:8 * i + 8, :]
        w = wt_ref[cb]
        w0, w1, w2, w3 = w[0:1, :], w[1:2, :], w[2:3, :], w[3:4, :]
        e0, o0, e1, o1, o2 = even(p0), odd(p0), even(p1), odd(p1), odd(p2)
        ke = ((e0 * w0 + o1 * w1) + e1 * w2) + o2 * w3
        ko = ((o0 * w0 + e0 * w1) + o1 * w2) + e1 * w3
        re = pltpu.bitcast((ke * even(pv)).astype(bf16).astype(f32), u32)
        ro = pltpu.bitcast((ko * odd(pv)).astype(bf16).astype(f32), u32)
        kv = (re >> 16) | (ro & jnp.uint32(0xFFFF0000))
        u_ref[cb, 8 * i:8 * i + 8, :] = kv
        return kv

    def combine(kf, prev):
        out = []
        for g in range(8):
            o = 32 * g
            out += [kf[o:o + 8] + prev[o + 8:o + 16], kf[o + 8:o + 16] - prev[o:o + 8],
                    kf[o + 16:o + 24] - prev[o + 24:o + 32], kf[o + 24:o + 32] + prev[o + 16:o + 24]]
        return jnp.concatenate(out, axis=0)

    def conv_fwd(cb, r):
        slot = cb % 2
        rows = pl.ds(pl.multiple_of(cb * 64, 64), 64)
        f = f_ref[...]
        kfs = []
        for a in (2 * r, 2 * r + 1):
            fu_ref[slot, NZ + a] = _dot(f, _as_bf16(u_ref[cb, pl.ds(pl.multiple_of(a * 64, 64), 64), :]))
            kfs.append(_dot_nt(f, _as_bf16(ssm_ref[a, rows, :])))
        fk_ref[slot, 2 * r] = combine(kfs[0], jnp.where(r > 0, kraw_ref[...], 0.0))
        fk_ref[slot, 2 * r + 1] = combine(kfs[1], kfs[0])
        kraw_ref[...] = kfs[1]

    def conv_mac(slot, a, nterms, pos, dep=None):
        rows = slice(pos * 16, pos * 16 + 16)
        p = q = None
        for c in range(nterms):
            u = fu_ref[slot, NZ + a - c, rows, :]
            k = fk_ref[slot, c, rows, :]
            ua, ub, kc, kd = u[0:8], u[8:16], k[0:8], k[8:16]
            if c == 0 and dep is not None:
                ua = jnp.where(one_ref[...] == 1, ua, pltpu.bitcast(dep, f32))
            p = (ua * kc if p is None else p + ua * kc) - ub * kd
            q = (ua * kd if q is None else q + ua * kd) + ub * kc
        return pltpu.bitcast(jnp.concatenate([p, q], axis=0).astype(bf16), u32)

    def conv_inv(a_ref, cb, dst, a, zs):
        rows = pl.ds(pl.multiple_of(a * 64, 64), 64)
        y = _dot(g_ref[...], _as_bf16(jnp.concatenate(zs, axis=0)))
        kv = _as_bf16(u_ref[cb, rows, :]).astype(f32)
        q = _as_bf16(x_ref[cb, rows, :]).astype(f32)
        a_ref[dst, pl.ds(pl.multiple_of(a * C, C), C), :] = q * (y + kv * wt_ref[cb, KS:KS + 1, :])

    def after(w, tok):
        if tok is None:
            return w
        return jnp.concatenate([jnp.where(one_ref[...] == 1, w[0:8], tok), w[8:]], axis=0)

    def prologue(stage_ref, acc_ref):
        st3 = stage_ref.reshape(NG * D, 8, E)

        def start_w(g):
            r0 = (g % 2) * 8
            cp(w_hbm[g // 2].bitcast(u32).at[:, r0:r0 + 8, :], st3.at[g * D:(g + 1) * D], SEM_W + g - 1).start()

        def slice_copies(q):
            cols = pl.ds(pl.multiple_of(q * DQ, DQ), DQ)
            return (cp(x3_hbm.at[:, NT:SEG, cols], xr_ref.at[q], SEM_Q + q),
                    cp(wq_hbm.bitcast(u32).at[cols, 0:8, :], st3.at[cols], SEM_Q + q))

        small = [cp(shift_hbm, shift_ref, SEM_SMALL), cp(d_hbm, d_ref, SEM_SMALL), cp(gw_hbm, gw_ref, SEM_SMALL),
                 cp(mem_hbm, mem_ref, SEM_SMALL), cp(f_hbm, f_ref, SEM_SMALL), cp(g_hbm, g_ref, SEM_SMALL)]
        for q in range(NQ):
            for c in slice_copies(q):
                c.start()
        for c in small:
            c.start()
        for g in range(1, NG):
            start_w(g)
            if g >= 2:
                start_col_blocks(k_hbm, k_ref, 2 * g - 4, 2 * g - 2, SEM_K + g - 2, row0=KPAD)
                start_col_blocks(v_hbm, v_ref, 2 * g - 4, 2 * g - 2, SEM_V + g - 2)
        start_col_blocks(wo_hbm, wo_ref, 0, NCB, SEM_WO)
        fill_ref[...] = _fill_matrix()
        one_ref[...] = jnp.ones((8, 128), jnp.int32)
        k_ref[:, KPAD - 8:KPAD, :] = jnp.zeros((NCB + 1, 8, 128), u32)
        wt_ref[...] = jnp.zeros(wt_ref.shape, f32)
        kraw_ref[...] = jnp.zeros(kraw_ref.shape, f32)
        fu_ref[0, NZ - 1] = jnp.zeros((256, 128), f32)

        def clear(a, c):
            rows = pl.ds(pl.multiple_of(a * 64, 64), 64)
            k_ref[NCB, pl.ds(pl.multiple_of(KPAD + a * 64, 32), 64), :] = jnp.zeros((64, 128), u32)
            v_ref[NCB, rows, :] = jnp.zeros((64, 128), u32)
            acc_ref[a] = jnp.zeros((NSEG * M, E), f32)
            return c
        lax.fori_loop(0, 16, clear, 0)

        def unpack_pair(w):
            return pltpu.bitcast(even(w).astype(bf16), u32), pltpu.bitcast(odd(w).astype(bf16), u32)

        def store_pre(idx, r1, r2):
            cc = jnp.concatenate([r1.reshape(NSEG, 8, E), r2.reshape(NSEG, 8, E)], axis=1).astype(bf16)
            pre_ref[:, idx] = pltpu.bitcast(cc, u32)

        def first(q, c):
            for cc in slice_copies(q):
                cc.wait()
            xq = pltpu.bitcast(xr_ref[q].astype(f32).reshape(NSEG * M, DQ).astype(bf16), u32)
            xb_ref[q] = xq
            sub = stage_ref.at[pl.ds(pl.multiple_of(q * (8 * DQ), 8 * DQ), 8 * DQ), :]
            rows = pl.ds(pl.multiple_of(q * (DQ // 2), DQ // 2), DQ // 2)
            for j in range(8):
                rs = []
                for h, w in zip((2 * j, 2 * j + 1), unpack_pair(sub[pl.ds(j, DQ, stride=8), :])):
                    wn_ref[h, rows, :] = w
                    r = _dot(_as_bf16(xq), _as_bf16(w)) + acc_ref[h]
                    acc_ref[h] = r
                    rs.append(r)
                store_pre(j, *rs)
            return c
        lax.fori_loop(0, NQ, first, 0)

        start_col_blocks(x_hbm, x_ref, 0, NCB, SEM_X)
        start_ssm(0, 64, SEM_SSM0)
        for c in small:
            c.wait()
        sh = shift_ref[...].astype(f32)
        dv = d_ref[...].astype(f32)
        for n in range(NCB):
            wt_ref[n, 0:KS, :] = sh[:, n * 128:(n + 1) * 128]
            wt_ref[n, KS:KS + 1, :] = dv[n:n + 1, :]

        def group(g, c):
            wait_all(st3.at[pl.ds(g * D, D)], SEM_W + g - 1)

            @pl.when(g >= 2)
            def _():
                wait_all(k_ref.at[pl.ds(2 * g - 4, 2), KPAD:], SEM_K + g - 2)
                wait_all(v_ref.at[pl.ds(2 * g - 4, 2)], SEM_V + g - 2)

            cbs = [jnp.where(g >= 2, 2 * g - 4 + i, NCB) for i in range(2)]
            npt = CFG["npt"]
            toks = [None] * 32
            for k in range(npt):
                t = None
                for i in range(k * 256 // npt, (k + 1) * 256 // npt):
                    t = conv_prep(cbs[i // 128], i % 128, t)
                    zero = pltpu.bitcast(jnp.where(one_ref[...] == 1, jnp.uint32(0), t), f32)
                    for v in range(i, 288, 256):
                        rows = slice(8 * (v % 32), 8 * (v % 32) + 8)
                        if v < 160:
                            fu_ref[1, jnp.minimum((g - 1) * 5 + v // 32, NZ + NCH - 1), rows, :] = zero
                        else:
                            fk_ref[1, jnp.minimum((g - 1) * 4 + v // 32 - 5, NCH - 1), rows, :] = zero
                toks[32 - npt + k] = t
            sub = stage_ref.at[pl.ds(pl.multiple_of(g * (8 * D), 8 * D), 8 * D), :]
            for j in range(8):
                ws = [unpack_pair(sub[pl.ds(blk * 2048 + j, 256, stride=8), :]) for blk in range(D // 256)]
                xb = _as_bf16(jnp.concatenate([xb_ref[q] for q in range(NQ)], axis=1))
                rs = [None, None]
                for i in range(2):
                    wn_ref[g * 16 + 2 * j + i] = jnp.concatenate([wb[i] for wb in ws], axis=0)
                if j == 0:
                    for blk in range(D // 256):
                        for i in range(2):
                            d = _dot(xb[:, blk * 256:(blk + 1) * 256], _as_bf16(ws[blk][i]))
                            rs[i] = d if rs[i] is None else d + rs[i]
                else:
                    for i in range(2):
                        tk = toks[4 * j + 2 * i:4 * j + 2 * i + 2]
                        w = jnp.concatenate([after(ws[0][i], tk[0]), ws[1][i], after(ws[2][i], tk[1]), ws[3][i]], axis=0)
                        rs[i] = _dot(xb, _as_bf16(w))
                store_pre(g * 8 + j, *rs)
            return c
        lax.fori_loop(1, NG, group, 0)

    pl.run_scoped(prologue, pltpu.VMEM((NG * 8 * D, E), u32), pltpu.VMEM((16, NSEG * M, E), f32))

    start_ssm(64, D // 2, SEM_SSM1)
    wait_all(wo_ref, SEM_WO)
    wait_all(x_ref, SEM_X)
    wait_all(ssm_ref.at[:, 0:64], SEM_SSM0)

    scale = E ** -0.5

    def main(odef_ref, b_ref, a_ref):
        def step(s, mem, t):
            cfg = CFG["steps"][t]
            cb = s // 8
            r = s % 8
            icb = jnp.maximum(cb - 1, 0)
            idst = jnp.where(cb >= 1, cb - 1, NCB)
            mslot = (cb + 1) % 2
            nh = 8 // UNROLL
            chunks = ((nh * t + r // UNROLL, nh * t + nh), (NCH - 1 - nh * t - r // UNROLL, NCH - nh * t))
            zs = ({}, {})

            xrows = pl.ds(pl.multiple_of(s * 16, 16), 16)
            xs = [_as_bf16(x_ref[n, xrows, :]).astype(f32) for n in range(NCB)]
            h32 = jnp.concatenate([jnp.concatenate(xs, axis=1)[0:NT], mem], axis=0).astype(bf16)
            r0 = pl.multiple_of(s * 8, 8)

            def gate():
                gw = gw_ref[...].astype(f32)
                gl = None
                for n in range(NCB):
                    xg = _as_bf16(x_ref[n, xrows, :]).astype(f32) * gw[n:n + 1, :]
                    gl = xg if gl is None else gl + xg
                g = jnp.broadcast_to(jax.nn.sigmoid(jnp.sum(gl, axis=-1, keepdims=True)), (SEG, 128))
                gate_ref[s] = g
                g = pltpu.bitcast(g, u32)
                return (g[0:8] | g[8:16]) | (g[16:24] | g[24:32])

            def mac_job(w, pos):
                zs[w][pos] = conv_mac(mslot, chunks[w][0], chunks[w][1], pos)
                return zs[w][pos]

            jobs = [(cfg["dues"][i], functools.partial(mac_job, i % 2, i // 2)) for i in range(32)]
            jobs.append((cfg["gate"], gate))
            state = dict(count=0, due={})

            def sdot(lhs, w, acc=None, weight=1):
                c = state["count"]
                toks = [t for cc in range(c, c + weight) for t in state["due"].pop(cc, [])]
                nt = w.shape[0] // 64
                if toks:
                    tiles = [w[64 * i:64 * (i + 1)] for i in range(nt)]
                    for i, t in enumerate(toks):
                        tiles[i % nt] = after(tiles[i % nt], t)
                    w = jnp.concatenate(tiles, axis=0)
                d = _dot(lhs, _as_bf16(w))
                d = d if acc is None else d + acc
                for due, fn in jobs:
                    if c <= due - 4 < c + weight:
                        state["due"].setdefault(due, []).append(fn())
                state["count"] = c + weight
                return d

            def proj(m, j):
                r1 = sdot(h32, wn_ref[m * H + 2 * j], weight=4)
                r2 = sdot(h32, wn_ref[m * H + 2 * j + 1], weight=4)
                p = _as_bf16(pre_ref[s, m * NP + j]).astype(f32)
                if m == 0:
                    return jnp.concatenate([r1, r2, p], axis=0)
                return jnp.concatenate([r1, r2, p, jnp.zeros((48, E), f32)], axis=0).astype(bf16)

            def qk(q80, k80, due):
                fill = fill_ref[...]
                sc = jnp.where(fill == 0.0, _dot_nt(q80.astype(bf16), k80), fill)
                p = jnp.exp2((sc - jnp.max(sc, axis=-1, keepdims=True)) * (scale * LOG2E))
                den = jnp.sum(p, axis=-1, keepdims=True)
                rc = pl.reciprocal(den, approx=True)
                p = p * (rc * (2.0 - den * rc))
                if due is not None:
                    pb = pltpu.bitcast(p, u32)
                    tok = pb[0:8]
                    for i in range(1, 10):
                        tok = tok | pb[8 * i:8 * i + 8]
                    state["due"].setdefault(due, []).append(tok)
                return p

            def pv(j, p, v80):
                o80 = _dot(p.astype(bf16), v80)
                odef_ref[pl.ds(r0, 8), (2 * j) * E:(2 * j + 1) * E] = o80[64:72]
                odef_ref[pl.ds(r0, 8), (2 * j + 1) * E:(2 * j + 2) * E] = o80[72:80]
                return jnp.concatenate([o80[0:32], o80[32:64]], axis=1).astype(bf16)

            def wo_part(o, j0, j1, n, acc=None):
                for j in range(j0, j1):
                    acc = sdot(o[j], wo_ref[n, j * 128:(j + 1) * 128, :], acc)
                return acc

            qs, ks, vs, ps, os_ = {}, {}, {}, {}, {}
            for j in range(0, NP, 2):
                for m, jj in cfg["order"]:
                    (qs, ks, vs)[m][j + jj] = proj(m, j + jj)
                if j == 2:
                    for jj in range(4):
                        ps[jj] = qk(qs[jj], ks[jj], cfg["sm"][jj])
                elif j > 2:
                    ps[j] = qk(qs[j], ks[j], cfg["sm"][j])
                    ps[j + 1] = qk(qs[j + 1], ks[j + 1], cfg["sm"][j + 1])
                    os_[j - 4] = pv(j - 4, ps[j - 4], vs[j - 4])
                    os_[j - 3] = pv(j - 3, ps[j - 3], vs[j - 3])
            na = NP - 4
            acc = {}
            nw = cfg["nw"]
            for n in range(nw):
                acc[n] = wo_part(os_, 0, na, n)
            for jj in range(na, NP):
                os_[jj] = pv(jj, ps[jj], vs[jj])
            acc[nw] = wo_part(os_, 0, na, nw)
            for n in range(nw + 1):
                acc[n] = wo_part(os_, na, NP, n, acc[n])
            for n in range(nw + 1, 8):
                acc[n] = wo_part(os_, 0, NP, n)
            assert state["count"] == 512 and not state["due"], state
            for w in range(2):
                conv_inv(a_ref, icb, idst, chunks[w][0], [zs[w][pos] for pos in range(16)])
            if t == UNROLL - 1:
                for tt in range(UNROLL):
                    conv_fwd(cb, r - t + tt)
            for n in range(NCB):
                b_ref[n, s, 0:NT, :] = acc[n][0:NT]
            return jnp.concatenate([acc[n][NT:SEG] for n in range(NCB)], axis=1).astype(bf16).astype(f32)

        def steps(i, mem):
            @pl.when(i == 8 // UNROLL)
            def _():
                wait_all(ssm_ref.at[:, 64:], SEM_SSM1)
            for t in range(UNROLL):
                mem = step(i * UNROLL + t, mem, t)
            return mem

        lax.fori_loop(0, _DBG_STEPS // UNROLL, steps, mem_ref[...].astype(f32))

        def out_copy(n):
            slot = n % 2
            return pltpu.make_async_copy(
                ost_ref.at[slot], out_hbm.at[:, :, pl.ds(pl.multiple_of(n * 128, 128), 128)],
                sems.at[SEM_OUT + slot])

        def fin(n, c):
            @pl.when(n >= 2)
            def _():
                out_copy(n - 2).wait()
            zs, toks, t = ([], []), [], None
            for pos in range(16):
                if pos % CFG["fgrp"] == 0:
                    t = None
                for w in range(2):
                    t = conv_mac((NCB - 1) % 2, n + 8 * w, 8 + 8 * w, pos, t)
                    zs[w].append(t)
                if pos % CFG["fgrp"] == CFG["fgrp"] - 1:
                    toks.append(t)
            bd = None
            for kb in range(8):
                if kb == CFG["finv"]:
                    for w in range(2):
                        conv_inv(a_ref, NCB - 1, NCB - 1, n + 8 * w, zs[w])
                w = after(wo_ref[n, kb * 256:(kb + 1) * 256, :], toks[kb - 1] if 0 < kb <= len(toks) else None)
                d = _dot(odef_ref[:, kb * 512:(kb + 1) * 512].astype(bf16), _as_bf16(w))
                bd = d if bd is None else d + bd
            b_ref[n, :, NT:SEG, :] = bd.reshape(NSEG, 8, 128)
            for blk in range(8):
                sg = slice(blk * 8, (blk + 1) * 8)
                b = b_ref[n, sg]
                a = a_ref[n, blk * 256:(blk + 1) * 256, :].reshape(8, SEG, 128)
                g = gate_ref[sg]
                ost_ref[n % 2, sg] = (g * a + (1.0 - g) * b).astype(bf16)
            out_copy(n).start()
            return c
        lax.fori_loop(0, NCB, fin, 0)
        out_copy(NCB - 2).wait()
        out_copy(NCB - 1).wait()

    pl.run_scoped(main, pltpu.VMEM((NSEG * 8, H * E), f32), pltpu.VMEM((NCB, NSEG, SEG, 128), f32),
                  pltpu.VMEM((NCB + 1, S, 128), f32))


@jax.jit
def pallas_gated_mix__ssm_conv_h3__memory_aug_recurrent_mem_tr__prompt_kernel(
    A_q: jax.Array,
    A_k: jax.Array,
    A_v: jax.Array,
    A_shift_k: jax.Array,
    A_ssm_k: jax.Array,
    A_ssm_D: jax.Array,
    B_x: jax.Array,
    B_mem0: jax.Array,
    B_Wq: jax.Array,
    B_Wk: jax.Array,
    B_Wv: jax.Array,
    B_Wo: jax.Array,
    B_seg_len: jax.Array,
    gate_w: jax.Array,
):
    del B_x, B_seg_len
    f_tab, g_tab = _dft_tables()
    out = pl.pallas_call(
        _kernel,
        out_shape=jax.ShapeDtypeStruct((NSEG, SEG, D), bf16),
        in_specs=[pl.BlockSpec(memory_space=pl.ANY)] * 15,
        out_specs=pl.BlockSpec(memory_space=pl.ANY),
        scratch_shapes=[
            pltpu.VMEM((3 * H, D // 2, E), u32),
            pltpu.VMEM((NCB, H * E // 2, 128), u32),
            pltpu.VMEM((NCB, S // 2, 128), u32),
            pltpu.VMEM((NQ, NSEG, M, DQ), bf16),
            pltpu.VMEM((NQ, NSEG * 4, DQ), u32),
            pltpu.VMEM((NSEG, 3 * NP, 8, E), u32),
            pltpu.VMEM((NCB + 1, KPAD + S // 2, 128), u32),
            pltpu.VMEM((NCB + 1, S // 2, 128), u32),
            pltpu.VMEM((NCH, D // 2, 128), u32),
            pltpu.VMEM((NCB + 1, S // 2, 128), u32),
            pltpu.VMEM((2, NZ + NCH, 256, 128), f32),
            pltpu.VMEM((2, NCH, 256, 128), f32),
            pltpu.VMEM((256, 128), f32),
            pltpu.VMEM((8, 128), jnp.int32),
            pltpu.VMEM((256, 128), bf16),
            pltpu.VMEM((128, 256), bf16),
            pltpu.VMEM((80, 128), f32),
            pltpu.VMEM((KS, D), bf16),
            pltpu.VMEM((NCB + 1, 8, 128), f32),
            pltpu.VMEM((NCB, 128), bf16),
            pltpu.VMEM((NCB, 128), bf16),
            pltpu.VMEM((M, D), bf16),
            pltpu.VMEM((NSEG, SEG, 128), f32),
            pltpu.VMEM((2, NSEG, SEG, 128), bf16),
            pltpu.SemaphoreType.DMA((NSEM,)),
        ],
        compiler_params=pltpu.CompilerParams(vmem_limit_bytes=120 * 2**20),
    )(A_q.reshape(NSEG, SEG, D), A_q.reshape(S, D), A_k.reshape(S, D), A_v.reshape(S, D), A_shift_k.T,
      A_ssm_k, A_ssm_D.reshape(NCB, 128), B_mem0.reshape(M, D), B_Wq, B_Wk, B_Wv,
      B_Wo.reshape(H * E, D), gate_w.reshape(NCB, 128), f_tab, g_tab)
    return out.reshape(1, S, D)
```

```python
import functools

import numpy as np
import jax
import jax.numpy as jnp
from jax import lax
import jax.experimental.pallas as pl
import jax.experimental.pallas.tpu as pltpu

S, D, H, E, M, SEG = 2048, 1024, 32, 128, 8, 32
NSEG = S // SEG
NT = SEG - M
NP = H // 2
NCB = D // 128
C = 128
NCH = S // C
LOG2E = 1.4426950408889634
KS = 4
NZ = 8
KPAD = 32
NG = 6
NQ = 8
DQ = D // NQ
UNROLL = 4
CFG = dict(fout=5, npt=28, fgrp=4, finv=4, steps=[
    dict(dues=[12, 16, 20, 24, 28, 32, 36, 40, 44, 88, 136, 184, 232, 280, 328, 376, 444, 172, 452, 456, 460, 464,
               468, 472, 476, 480, 484, 488, 200, 496, 500, 504],
         sm=[124, 140, 164, 188, 212, 236, 260, 284, 308, 332, 356, 380, None, None, None, None],
         gate=440, nw=3, order=((0, 0), (1, 0), (0, 1), (1, 1), (2, 0), (2, 1))),
    dict(dues=[464, 16, 20, 24, 28, 32, 36, 40, 44, 88, 136, 184, 232, 280, 328, 376, 444, 448, 452, 456, 460, 84,
               468, 472, 476, 436, 484, 488, 492, 496, 500, 504],
         sm=[124, 140, 164, 188, 212, 236, 260, 284, 308, 332, 356, 380, None, None, None, None],
         gate=440, nw=3, order=((1, 0), (0, 0), (1, 1), (0, 1), (2, 1), (2, 0))),
    dict(dues=[12, 16, 20, 24, 28, 32, 36, 40, 44, 88, 136, 184, 232, 280, 328, 376, 444, 448, 452, 456, 460, 464,
               468, 472, 476, 480, 484, 488, 492, 496, 500, 504],
         sm=[124, 140, 164, 188, 212, 236, 260, 284, 308, 332, 356, 380, None, None, None, None],
         gate=92, nw=4, order=((0, 0), (1, 0), (0, 1), (1, 1), (2, 0), (2, 1))),
    dict(dues=[12, 16, 20, 24, 28, 32, 36, 40, 44, 88, 136, 184, 232, 244, 328, 376, 444, 448, 452, 456, 460, 464,
               468, 472, 476, 480, 484, 488, 492, 496, 500, 136],
         sm=[124, 140, 128, 188, 212, 212, 260, 284, 308, 332, 356, 380, None, None, None, None],
         gate=440, nw=3, order=((0, 0), (1, 0), (0, 1), (1, 1), (2, 0), (2, 1))),
])
_DBG_STEPS = NSEG
bf16, f32, u32 = jnp.bfloat16, jnp.float32, jnp.uint32


def _dft_tables():
    t = np.arange(C, dtype=np.float64)
    rows = []
    for r in range(8):
        ev = 16 * r + np.arange(0, 16, 2)
        od = ev + 1
        for fn, fs in ((np.cos, ev), (np.sin, ev), (np.cos, od), (np.sin, od)):
            rows.append(fn(np.pi * (2 * fs[:, None] + 1) * t[None, :] / (2 * C)))
    f = np.concatenate(rows, axis=0)
    return f.astype(bf16), (f.T / C).astype(bf16)


def _fill_matrix():
    r = lax.broadcasted_iota(jnp.int32, (80, 128), 0)
    c = lax.broadcasted_iota(jnp.int32, (80, 128), 1)

    def head(i):
        return jnp.where(i < 64, i // 32, (i - 64) // 8)

    def idx(i):
        lo = i % 32
        main = jnp.where(lo < NT, lo + M, lo - NT)
        return jnp.where(i < 64, main, (i - 64) % 8 + NT + M)

    same = (head(r) == head(c)) & (c < 80)
    ok = (idx(r) < M) | (idx(r) >= idx(c))
    return jnp.where(same, jnp.where(ok, 0.0, -1e9 * E ** 0.5), -jnp.inf).astype(f32)


def _as_bf16(v):
    return pltpu.bitcast(v, bf16)


def _dot(a, b):
    return jnp.dot(a, b, preferred_element_type=f32)


def _dot_nt(a, b):
    return lax.dot_general(a, b, (((1,), (1,)), ((), ())), preferred_element_type=f32)


SEM_SMALL, SEM_WO = range(2)
SEM_Q = 2
SEM_K = SEM_Q + NQ
SEM_V = SEM_K + 4
SEM_W = SEM_V + 4
NSEM = SEM_W + NG - 1
SEM_X, SEM_SSM0, SEM_SSM1, SEM_OUT = SEM_Q, SEM_Q + 1, SEM_Q + 2, SEM_Q + 3


def _kernel(x3_hbm, x_hbm, k_hbm, v_hbm, shift_hbm, ssm_hbm, d_hbm, mem_hbm, wq_hbm, wk_hbm, wv_hbm,
            wo_hbm, gw_hbm, f_hbm, g_hbm, out_hbm,
            wn_ref, wo_ref, x_ref, xr_ref, xb_ref, pre_ref, k_ref, v_ref, ssm_ref, u_ref,
            fu_ref, fk_ref, kraw_ref, one_ref, f_ref, g_ref, fill_ref, shift_ref, wt_ref,
            d_ref, gw_ref, mem_ref, gate_ref, ost_ref, sems):
    w_hbm = (wq_hbm, wk_hbm, wv_hbm)

    def cp(src, dst, sem):
        return pltpu.make_async_copy(src, dst, sems.at[sem])

    def start_col_blocks(src_hbm, dst_ref, i0, i1, sem, row0=0):
        src = src_hbm.bitcast(u32)
        for i in range(i0, i1):
            cp(src.at[:, i * 128:(i + 1) * 128], dst_ref.at[i, row0:], sem).start()

    def start_ssm(r0, r1, sem):
        src = ssm_hbm.bitcast(u32)
        for a in range(NCH):
            cp(src.at[r0:r1, a * C:(a + 1) * C], ssm_ref.at[a, r0:r1], sem).start()

    def wait_all(dst, sem):
        cp(dst, dst, sem).wait()

    def even(p):
        return pltpu.bitcast(p << 16, f32)

    def odd(p):
        return pltpu.bitcast(p & jnp.uint32(0xFFFF0000), f32)

    def conv_prep(cb, i, dep=None):
        r0 = KPAD + 8 * i
        p0 = k_ref[cb, r0:r0 + 8, :]
        if dep is not None:
            p0 = jnp.where(one_ref[...] == 1, p0, dep)
        p1 = k_ref[cb, r0 - 1:r0 + 7, :]
        p2 = k_ref[cb, r0 - 2:r0 + 6, :]
        pv = v_ref[cb, 8 * i:8 * i + 8, :]
        w = wt_ref[cb]
        w0, w1, w2, w3 = w[0:1, :], w[1:2, :], w[2:3, :], w[3:4, :]
        e0, o0, e1, o1, o2 = even(p0), odd(p0), even(p1), odd(p1), odd(p2)
        ke = ((e0 * w0 + o1 * w1) + e1 * w2) + o2 * w3
        ko = ((o0 * w0 + e0 * w1) + o1 * w2) + e1 * w3
        re = pltpu.bitcast((ke * even(pv)).astype(bf16).astype(f32), u32)
        ro = pltpu.bitcast((ko * odd(pv)).astype(bf16).astype(f32), u32)
        kv = (re >> 16) | (ro & jnp.uint32(0xFFFF0000))
        u_ref[cb, 8 * i:8 * i + 8, :] = kv
        return kv

    def combine(kf, prev):
        out = []
        for g in range(8):
            o = 32 * g
            out += [kf[o:o + 8] + prev[o + 8:o + 16], kf[o + 8:o + 16] - prev[o:o + 8],
                    kf[o + 16:o + 24] - prev[o + 24:o + 32], kf[o + 24:o + 32] + prev[o + 16:o + 24]]
        return jnp.concatenate(out, axis=0)

    def conv_fwd(cb, r):
        slot = cb % 2
        rows = pl.ds(pl.multiple_of(cb * 64, 64), 64)
        f = f_ref[...]
        kfs = []
        for a in (2 * r, 2 * r + 1):
            fu_ref[slot, NZ + a] = _dot(f, _as_bf16(u_ref[cb, pl.ds(pl.multiple_of(a * 64, 64), 64), :]))
            kfs.append(_dot_nt(f, _as_bf16(ssm_ref[a, rows, :])))
        fk_ref[slot, 2 * r] = combine(kfs[0], jnp.where(r > 0, kraw_ref[...], 0.0))
        fk_ref[slot, 2 * r + 1] = combine(kfs[1], kfs[0])
        kraw_ref[...] = kfs[1]

    def conv_mac(slot, a, nterms, pos, dep=None):
        rows = slice(pos * 16, pos * 16 + 16)
        p = q = None
        for c in range(nterms):
            u = fu_ref[slot, NZ + a - c, rows, :]
            k = fk_ref[slot, c, rows, :]
            ua, ub, kc, kd = u[0:8], u[8:16], k[0:8], k[8:16]
            if c == 0 and dep is not None:
                ua = jnp.where(one_ref[...] == 1, ua, pltpu.bitcast(dep, f32))
            p = (ua * kc if p is None else p + ua * kc) - ub * kd
            q = (ua * kd if q is None else q + ua * kd) + ub * kc
        return pltpu.bitcast(jnp.concatenate([p, q], axis=0).astype(bf16), u32)

    def conv_inv(a_ref, cb, dst, a, zs):
        rows = pl.ds(pl.multiple_of(a * 64, 64), 64)
        y = _dot(g_ref[...], _as_bf16(jnp.concatenate(zs, axis=0)))
        kv = _as_bf16(u_ref[cb, rows, :]).astype(f32)
        q = _as_bf16(x_ref[cb, rows, :]).astype(f32)
        a_ref[dst, pl.ds(pl.multiple_of(a * C, C), C), :] = q * (y + kv * wt_ref[cb, KS:KS + 1, :])

    def after(w, tok):
        if tok is None:
            return w
        return jnp.concatenate([jnp.where(one_ref[...] == 1, w[0:8], tok), w[8:]], axis=0)

    def prologue(stage_ref, acc_ref):
        st3 = stage_ref.reshape(NG * D, 8, E)

        def start_w(g):
            r0 = (g % 2) * 8
            cp(w_hbm[g // 2].bitcast(u32).at[:, r0:r0 + 8, :], st3.at[g * D:(g + 1) * D], SEM_W + g - 1).start()

        def slice_copies(q):
            cols = pl.ds(pl.multiple_of(q * DQ, DQ), DQ)
            return (cp(x3_hbm.at[:, NT:SEG, cols], xr_ref.at[q], SEM_Q + q),
                    cp(wq_hbm.bitcast(u32).at[cols, 0:8, :], st3.at[cols], SEM_Q + q))

        small = [cp(shift_hbm, shift_ref, SEM_SMALL), cp(d_hbm, d_ref, SEM_SMALL), cp(gw_hbm, gw_ref, SEM_SMALL),
                 cp(mem_hbm, mem_ref, SEM_SMALL), cp(f_hbm, f_ref, SEM_SMALL), cp(g_hbm, g_ref, SEM_SMALL)]
        for q in range(NQ):
            for c in slice_copies(q):
                c.start()
        for c in small:
            c.start()
        for g in range(1, NG):
            start_w(g)
            if g >= 2:
                start_col_blocks(k_hbm, k_ref, 2 * g - 4, 2 * g - 2, SEM_K + g - 2, row0=KPAD)
                start_col_blocks(v_hbm, v_ref, 2 * g - 4, 2 * g - 2, SEM_V + g - 2)
        start_col_blocks(wo_hbm, wo_ref, 0, NCB, SEM_WO)
        fill_ref[...] = _fill_matrix()
        one_ref[...] = jnp.ones((8, 128), jnp.int32)
        k_ref[:, KPAD - 8:KPAD, :] = jnp.zeros((NCB + 1, 8, 128), u32)
        wt_ref[...] = jnp.zeros(wt_ref.shape, f32)
        kraw_ref[...] = jnp.zeros(kraw_ref.shape, f32)
        fu_ref[0, NZ - 1] = jnp.zeros((256, 128), f32)

        def clear(a, c):
            rows = pl.ds(pl.multiple_of(a * 64, 64), 64)
            k_ref[NCB, pl.ds(pl.multiple_of(KPAD + a * 64, 32), 64), :] = jnp.zeros((64, 128), u32)
            v_ref[NCB, rows, :] = jnp.zeros((64, 128), u32)
            acc_ref[a] = jnp.zeros((NSEG * M, E), f32)
            return c
        lax.fori_loop(0, 16, clear, 0)

        def unpack_pair(w):
            return pltpu.bitcast(even(w).astype(bf16), u32), pltpu.bitcast(odd(w).astype(bf16), u32)

        def store_pre(idx, r1, r2):
            cc = jnp.concatenate([r1.reshape(NSEG, 8, E), r2.reshape(NSEG, 8, E)], axis=1).astype(bf16)
            pre_ref[:, idx] = pltpu.bitcast(cc, u32)

        def first(q, c):
            for cc in slice_copies(q):
                cc.wait()
            xq = pltpu.bitcast(xr_ref[q].astype(f32).reshape(NSEG * M, DQ).astype(bf16), u32)
            xb_ref[q] = xq
            sub = stage_ref.at[pl.ds(pl.multiple_of(q * (8 * DQ), 8 * DQ), 8 * DQ), :]
            rows = pl.ds(pl.multiple_of(q * (DQ // 2), DQ // 2), DQ // 2)
            for j in range(8):
                rs = []
                for h, w in zip((2 * j, 2 * j + 1), unpack_pair(sub[pl.ds(j, DQ, stride=8), :])):
                    wn_ref[h, rows, :] = w
                    r = _dot(_as_bf16(xq), _as_bf16(w)) + acc_ref[h]
                    acc_ref[h] = r
                    rs.append(r)
                store_pre(j, *rs)
            return c
        lax.fori_loop(0, NQ, first, 0)

        start_col_blocks(x_hbm, x_ref, 0, NCB, SEM_X)
        start_ssm(0, 64, SEM_SSM0)
        for c in small:
            c.wait()
        sh = shift_ref[...].astype(f32)
        dv = d_ref[...].astype(f32)
        for n in range(NCB):
            wt_ref[n, 0:KS, :] = sh[:, n * 128:(n + 1) * 128]
            wt_ref[n, KS:KS + 1, :] = dv[n:n + 1, :]

        def group(g, c):
            wait_all(st3.at[pl.ds(g * D, D)], SEM_W + g - 1)

            @pl.when(g >= 2)
            def _():
                wait_all(k_ref.at[pl.ds(2 * g - 4, 2), KPAD:], SEM_K + g - 2)
                wait_all(v_ref.at[pl.ds(2 * g - 4, 2)], SEM_V + g - 2)

            cbs = [jnp.where(g >= 2, 2 * g - 4 + i, NCB) for i in range(2)]
            npt = CFG["npt"]
            toks = [None] * 32
            for k in range(npt):
                t = None
                for i in range(k * 256 // npt, (k + 1) * 256 // npt):
                    t = conv_prep(cbs[i // 128], i % 128, t)
                    zero = pltpu.bitcast(jnp.where(one_ref[...] == 1, jnp.uint32(0), t), f32)
                    for v in range(i, 288, 256):
                        rows = slice(8 * (v % 32), 8 * (v % 32) + 8)
                        if v < 160:
                            fu_ref[1, jnp.minimum((g - 1) * 5 + v // 32, NZ + NCH - 1), rows, :] = zero
                        else:
                            fk_ref[1, jnp.minimum((g - 1) * 4 + v // 32 - 5, NCH - 1), rows, :] = zero
                toks[32 - npt + k] = t
            sub = stage_ref.at[pl.ds(pl.multiple_of(g * (8 * D), 8 * D), 8 * D), :]
            for j in range(8):
                ws = [unpack_pair(sub[pl.ds(blk * 2048 + j, 256, stride=8), :]) for blk in range(D // 256)]
                xb = _as_bf16(jnp.concatenate([xb_ref[q] for q in range(NQ)], axis=1))
                rs = [None, None]
                for i in range(2):
                    wn_ref[g * 16 + 2 * j + i] = jnp.concatenate([wb[i] for wb in ws], axis=0)
                if j == 0:
                    for blk in range(D // 256):
                        for i in range(2):
                            d = _dot(xb[:, blk * 256:(blk + 1) * 256], _as_bf16(ws[blk][i]))
                            rs[i] = d if rs[i] is None else d + rs[i]
                else:
                    for i in range(2):
                        tk = toks[4 * j + 2 * i:4 * j + 2 * i + 2]
                        w = jnp.concatenate([after(ws[0][i], tk[0]), ws[1][i], after(ws[2][i], tk[1]), ws[3][i]], axis=0)
                        rs[i] = _dot(xb, _as_bf16(w))
                store_pre(g * 8 + j, *rs)
            return c
        lax.fori_loop(1, NG, group, 0)

    pl.run_scoped(prologue, pltpu.VMEM((NG * 8 * D, E), u32), pltpu.VMEM((16, NSEG * M, E), f32))

    start_ssm(64, D // 2, SEM_SSM1)
    wait_all(wo_ref, SEM_WO)
    wait_all(x_ref, SEM_X)
    wait_all(ssm_ref.at[:, 0:64], SEM_SSM0)

    scale = E ** -0.5

    def main(odef_ref, b_ref, a_ref):
        def step(s, mem, t):
            cfg = CFG["steps"][t]
            cb = s // 8
            r = s % 8
            icb = jnp.maximum(cb - 1, 0)
            idst = jnp.where(cb >= 1, cb - 1, NCB)
            mslot = (cb + 1) % 2
            nh = 8 // UNROLL
            chunks = ((nh * t + r // UNROLL, nh * t + nh), (NCH - 1 - nh * t - r // UNROLL, NCH - nh * t))
            zs = ({}, {})

            xrows = pl.ds(pl.multiple_of(s * 16, 16), 16)
            xs = [_as_bf16(x_ref[n, xrows, :]).astype(f32) for n in range(NCB)]
            h32 = jnp.concatenate([jnp.concatenate(xs, axis=1)[0:NT], mem], axis=0).astype(bf16)
            r0 = pl.multiple_of(s * 8, 8)

            def gate():
                gw = gw_ref[...].astype(f32)
                gl = None
                for n in range(NCB):
                    xg = _as_bf16(x_ref[n, xrows, :]).astype(f32) * gw[n:n + 1, :]
                    gl = xg if gl is None else gl + xg
                g = jnp.broadcast_to(jax.nn.sigmoid(jnp.sum(gl, axis=-1, keepdims=True)), (SEG, 128))
                gate_ref[s] = g
                g = pltpu.bitcast(g, u32)
                return (g[0:8] | g[8:16]) | (g[16:24] | g[24:32])

            def mac_job(w, pos):
                zs[w][pos] = conv_mac(mslot, chunks[w][0], chunks[w][1], pos)
                return zs[w][pos]

            jobs = [(cfg["dues"][i], functools.partial(mac_job, i % 2, i // 2)) for i in range(32)]
            jobs.append((cfg["gate"], gate))
            state = dict(count=0, due={})

            def sdot(lhs, w, acc=None, weight=1):
                c = state["count"]
                toks = [t for cc in range(c, c + weight) for t in state["due"].pop(cc, [])]
                nt = w.shape[0] // 64
                if toks:
                    tiles = [w[64 * i:64 * (i + 1)] for i in range(nt)]
                    for i, t in enumerate(toks):
                        tiles[i % nt] = after(tiles[i % nt], t)
                    w = jnp.concatenate(tiles, axis=0)
                d = _dot(lhs, _as_bf16(w))
                d = d if acc is None else d + acc
                for due, fn in jobs:
                    if c <= due - 4 < c + weight:
                        state["due"].setdefault(due, []).append(fn())
                state["count"] = c + weight
                return d

            def proj(m, j):
                r1 = sdot(h32, wn_ref[m * H + 2 * j], weight=4)
                r2 = sdot(h32, wn_ref[m * H + 2 * j + 1], weight=4)
                p = _as_bf16(pre_ref[s, m * NP + j]).astype(f32)
                if m == 0:
                    return jnp.concatenate([r1, r2, p], axis=0)
                return jnp.concatenate([r1, r2, p, jnp.zeros((48, E), f32)], axis=0).astype(bf16)

            def qk(q80, k80, due):
                fill = fill_ref[...]
                sc = jnp.where(fill == 0.0, _dot_nt(q80.astype(bf16), k80), fill)
                p = jnp.exp2((sc - jnp.max(sc, axis=-1, keepdims=True)) * (scale * LOG2E))
                den = jnp.sum(p, axis=-1, keepdims=True)
                rc = pl.reciprocal(den, approx=True)
                p = p * (rc * (2.0 - den * rc))
                if due is not None:
                    pb = pltpu.bitcast(p, u32)
                    tok = pb[0:8]
                    for i in range(1, 10):
                        tok = tok | pb[8 * i:8 * i + 8]
                    state["due"].setdefault(due, []).append(tok)
                return p

            def pv(j, p, v80):
                o80 = _dot(p.astype(bf16), v80)
                odef_ref[pl.ds(r0, 8), (2 * j) * E:(2 * j + 1) * E] = o80[64:72]
                odef_ref[pl.ds(r0, 8), (2 * j + 1) * E:(2 * j + 2) * E] = o80[72:80]
                return jnp.concatenate([o80[0:32], o80[32:64]], axis=1).astype(bf16)

            def wo_part(o, j0, j1, n, acc=None):
                for j in range(j0, j1):
                    acc = sdot(o[j], wo_ref[n, j * 128:(j + 1) * 128, :], acc)
                return acc

            qs, ks, vs, ps, os_ = {}, {}, {}, {}, {}
            for j in range(0, NP, 2):
                for m, jj in cfg["order"]:
                    (qs, ks, vs)[m][j + jj] = proj(m, j + jj)
                if j == 2:
                    for jj in range(4):
                        ps[jj] = qk(qs[jj], ks[jj], cfg["sm"][jj])
                elif j > 2:
                    ps[j] = qk(qs[j], ks[j], cfg["sm"][j])
                    ps[j + 1] = qk(qs[j + 1], ks[j + 1], cfg["sm"][j + 1])
                    os_[j - 4] = pv(j - 4, ps[j - 4], vs[j - 4])
                    os_[j - 3] = pv(j - 3, ps[j - 3], vs[j - 3])
            na = NP - 4
            acc = {}
            nw = cfg["nw"]
            for n in range(nw):
                acc[n] = wo_part(os_, 0, na, n)
            for jj in range(na, NP):
                os_[jj] = pv(jj, ps[jj], vs[jj])
            acc[nw] = wo_part(os_, 0, na, nw)
            for n in range(nw + 1):
                acc[n] = wo_part(os_, na, NP, n, acc[n])
            for n in range(nw + 1, 8):
                acc[n] = wo_part(os_, 0, NP, n)
            assert state["count"] == 512 and not state["due"], state
            for w in range(2):
                conv_inv(a_ref, icb, idst, chunks[w][0], [zs[w][pos] for pos in range(16)])
            if t == UNROLL - 1:
                for tt in range(UNROLL):
                    conv_fwd(cb, r - t + tt)
            for n in range(NCB):
                b_ref[n, s, 0:NT, :] = acc[n][0:NT]
            return jnp.concatenate([acc[n][NT:SEG] for n in range(NCB)], axis=1).astype(bf16).astype(f32)

        def steps(i, mem):
            @pl.when(i == 8 // UNROLL)
            def _():
                wait_all(ssm_ref.at[:, 64:], SEM_SSM1)
            for t in range(UNROLL):
                mem = step(i * UNROLL + t, mem, t)
            return mem

        lax.fori_loop(0, _DBG_STEPS // UNROLL, steps, mem_ref[...].astype(f32))

        def out_copy(n, r0=0, r1=SEG, sem=None):
            slot = n % 2
            return pltpu.make_async_copy(
                ost_ref.at[slot, :, r0:r1], out_hbm.at[:, r0:r1, pl.ds(pl.multiple_of(n * 128, 128), 128)],
                sems.at[SEM_OUT + (slot if sem is None else sem)])

        def fin(n, last):
            def mix(r0, r1):
                for blk in range(8):
                    sg = slice(blk * 8, (blk + 1) * 8)
                    b = b_ref[n, sg, r0:r1]
                    a = a_ref[n, blk * 256:(blk + 1) * 256, :].reshape(8, SEG, 128)[:, r0:r1]
                    g = gate_ref[sg, r0:r1]
                    ost_ref[n % 2, sg, r0:r1] = (g * a + (1.0 - g) * b).astype(bf16)

            zs, toks, t = ([], []), [], None
            for pos in range(16):
                if pos % CFG["fgrp"] == 0:
                    t = None
                for w in range(2):
                    t = conv_mac((NCB - 1) % 2, n + 8 * w, 8 + 8 * w, pos, t)
                    zs[w].append(t)
                if pos % CFG["fgrp"] == CFG["fgrp"] - 1:
                    toks.append(t)
            bd = None
            for kb in range(8):
                if kb == CFG["finv"]:
                    for w in range(2):
                        conv_inv(a_ref, NCB - 1, NCB - 1, n + 8 * w, zs[w])
                if last and kb == CFG["fout"]:
                    mix(0, NT)
                    out_copy(n, 0, NT, 2).start()
                w = after(wo_ref[n, kb * 256:(kb + 1) * 256, :], toks[kb - 1] if 0 < kb <= len(toks) else None)
                d = _dot(odef_ref[:, kb * 512:(kb + 1) * 512].astype(bf16), _as_bf16(w))
                bd = d if bd is None else d + bd
            b_ref[n, :, NT:SEG, :] = bd.reshape(NSEG, 8, 128)
            mix(NT if last else 0, SEG)
            out_copy(n, NT if last else 0, SEG).start()

        def fin_loop(n, c):
            @pl.when(n >= 2)
            def _():
                out_copy(n - 2).wait()
            fin(n, False)
            return c
        lax.fori_loop(0, NCB - 1, fin_loop, 0)
        out_copy(NCB - 3).wait()
        fin(NCB - 1, True)
        out_copy(NCB - 2).wait()
        out_copy(NCB - 1, 0, NT, 2).wait()
        out_copy(NCB - 1, NT, SEG).wait()

    pl.run_scoped(main, pltpu.VMEM((NSEG * 8, H * E), f32), pltpu.VMEM((NCB, NSEG, SEG, 128), f32),
                  pltpu.VMEM((NCB + 1, S, 128), f32))


@jax.jit
def pallas_gated_mix__ssm_conv_h3__memory_aug_recurrent_mem_tr__prompt_kernel(
    A_q: jax.Array,
    A_k: jax.Array,
    A_v: jax.Array,
    A_shift_k: jax.Array,
    A_ssm_k: jax.Array,
    A_ssm_D: jax.Array,
    B_x: jax.Array,
    B_mem0: jax.Array,
    B_Wq: jax.Array,
    B_Wk: jax.Array,
    B_Wv: jax.Array,
    B_Wo: jax.Array,
    B_seg_len: jax.Array,
    gate_w: jax.Array,
):
    del B_x, B_seg_len
    f_tab, g_tab = _dft_tables()
    out = pl.pallas_call(
        _kernel,
        out_shape=jax.ShapeDtypeStruct((NSEG, SEG, D), bf16),
        in_specs=[pl.BlockSpec(memory_space=pl.ANY)] * 15,
        out_specs=pl.BlockSpec(memory_space=pl.ANY),
        scratch_shapes=[
            pltpu.VMEM((3 * H, D // 2, E), u32),
            pltpu.VMEM((NCB, H * E // 2, 128), u32),
            pltpu.VMEM((NCB, S // 2, 128), u32),
            pltpu.VMEM((NQ, NSEG, M, DQ), bf16),
            pltpu.VMEM((NQ, NSEG * 4, DQ), u32),
            pltpu.VMEM((NSEG, 3 * NP, 8, E), u32),
            pltpu.VMEM((NCB + 1, KPAD + S // 2, 128), u32),
            pltpu.VMEM((NCB + 1, S // 2, 128), u32),
            pltpu.VMEM((NCH, D // 2, 128), u32),
            pltpu.VMEM((NCB + 1, S // 2, 128), u32),
            pltpu.VMEM((2, NZ + NCH, 256, 128), f32),
            pltpu.VMEM((2, NCH, 256, 128), f32),
            pltpu.VMEM((256, 128), f32),
            pltpu.VMEM((8, 128), jnp.int32),
            pltpu.VMEM((256, 128), bf16),
            pltpu.VMEM((128, 256), bf16),
            pltpu.VMEM((80, 128), f32),
            pltpu.VMEM((KS, D), bf16),
            pltpu.VMEM((NCB + 1, 8, 128), f32),
            pltpu.VMEM((NCB, 128), bf16),
            pltpu.VMEM((NCB, 128), bf16),
            pltpu.VMEM((M, D), bf16),
            pltpu.VMEM((NSEG, SEG, 128), f32),
            pltpu.VMEM((2, NSEG, SEG, 128), bf16),
            pltpu.SemaphoreType.DMA((NSEM,)),
        ],
        compiler_params=pltpu.CompilerParams(vmem_limit_bytes=120 * 2**20),
    )(A_q.reshape(NSEG, SEG, D), A_q.reshape(S, D), A_k.reshape(S, D), A_v.reshape(S, D), A_shift_k.T,
      A_ssm_k, A_ssm_D.reshape(NCB, 128), B_mem0.reshape(M, D), B_Wq, B_Wk, B_Wv,
      B_Wo.reshape(H * E, D), gate_w.reshape(NCB, 128), f_tab, g_tab)
    return out.reshape(1, S, D)
```

```python
import functools

import numpy as np
import jax
import jax.numpy as jnp
from jax import lax
import jax.experimental.pallas as pl
import jax.experimental.pallas.tpu as pltpu

S, D, H, E, M, SEG = 2048, 1024, 32, 128, 8, 32
NSEG = S // SEG
NT = SEG - M
NP = H // 2
NCB = D // 128
C = 128
NCH = S // C
LOG2E = 1.4426950408889634
KS = 4
NZ = 8
KPAD = 32
NG = 6
NQ = 8
DQ = D // NQ
UNROLL = 4
CFG = dict(fout=5, npt=28, fgrp=4, finv=4, steps=[
    dict(dues=[12, 16, 20, 24, 28, 32, 36, 40, 44, 88, 136, 184, 232, 280, 328, 376, 444, 172, 452, 456, 460, 464,
               468, 472, 476, 480, 484, 488, 200, 496, 500, 504],
         sm=[124, 140, 164, 188, 212, 236, 260, 284, 308, 332, 356, 380, None, None, None, None],
         gate=440, nw=3, order=((0, 0), (1, 0), (0, 1), (1, 1), (2, 0), (2, 1))),
    dict(dues=[464, 16, 20, 24, 28, 32, 36, 40, 44, 88, 136, 184, 232, 280, 328, 376, 444, 448, 452, 456, 460, 84,
               468, 472, 476, 436, 484, 488, 492, 496, 500, 504],
         sm=[124, 140, 164, 188, 212, 236, 260, 284, 308, 332, 356, 380, None, None, None, None],
         gate=440, nw=3, order=((1, 0), (0, 0), (1, 1), (0, 1), (2, 1), (2, 0))),
    dict(dues=[12, 16, 20, 24, 28, 32, 36, 40, 44, 88, 136, 184, 232, 280, 328, 376, 444, 448, 452, 456, 460, 464,
               468, 472, 476, 480, 484, 488, 492, 496, 500, 504],
         sm=[124, 140, 164, 188, 212, 236, 260, 284, 308, 332, 356, 380, None, None, None, None],
         gate=92, nw=4, order=((0, 0), (1, 0), (0, 1), (1, 1), (2, 0), (2, 1))),
    dict(dues=[12, 16, 20, 24, 28, 32, 36, 40, 44, 88, 136, 184, 232, 244, 328, 376, 444, 448, 452, 456, 460, 464,
               468, 472, 476, 480, 484, 488, 492, 496, 500, 136],
         sm=[124, 140, 128, 188, 212, 212, 260, 284, 308, 332, 356, 380, None, None, None, None],
         gate=440, nw=3, order=((0, 0), (1, 0), (0, 1), (1, 1), (2, 0), (2, 1))),
])
_DBG_STEPS = NSEG
bf16, f32, u32 = jnp.bfloat16, jnp.float32, jnp.uint32


def _dft_tables():
    t = np.arange(C, dtype=np.float64)
    rows = []
    for r in range(8):
        ev = 16 * r + np.arange(0, 16, 2)
        od = ev + 1
        for fn, fs in ((np.cos, ev), (np.sin, ev), (np.cos, od), (np.sin, od)):
            rows.append(fn(np.pi * (2 * fs[:, None] + 1) * t[None, :] / (2 * C)))
    f = np.concatenate(rows, axis=0)
    return f.astype(bf16), (f.T / C).astype(bf16)


def _fill_matrix():
    r = lax.broadcasted_iota(jnp.int32, (80, 128), 0)
    c = lax.broadcasted_iota(jnp.int32, (80, 128), 1)

    def head(i):
        return jnp.where(i < 64, i // 32, (i - 64) // 8)

    def idx(i):
        lo = i % 32
        main = jnp.where(lo < NT, lo + M, lo - NT)
        return jnp.where(i < 64, main, (i - 64) % 8 + NT + M)

    same = (head(r) == head(c)) & (c < 80)
    ok = (idx(r) < M) | (idx(r) >= idx(c))
    return jnp.where(same, jnp.where(ok, 0.0, -1e9 * E ** 0.5), -jnp.inf).astype(f32)


def _as_bf16(v):
    return pltpu.bitcast(v, bf16)


def _dot(a, b):
    return jnp.dot(a, b, preferred_element_type=f32)


def _dot_nt(a, b):
    return lax.dot_general(a, b, (((1,), (1,)), ((), ())), preferred_element_type=f32)


SEM_SMALL, SEM_WO = range(2)
SEM_Q = 2
SEM_K = SEM_Q + NQ
SEM_V = SEM_K + 4
SEM_W = SEM_V + 4
NSEM = SEM_W + NG - 1
SEM_X, SEM_SSM0, SEM_SSM1, SEM_OUT = SEM_Q, SEM_Q + 1, SEM_Q + 2, SEM_Q + 3


def _kernel(x3_hbm, x_hbm, k_hbm, v_hbm, shift_hbm, ssm_hbm, d_hbm, mem_hbm, wq_hbm, wk_hbm, wv_hbm,
            wo_hbm, gw_hbm, f_hbm, g_hbm, out_hbm,
            wn_ref, wo_ref, x_ref, xr_ref, xb_ref, pre_ref, k_ref, v_ref, ssm_ref, u_ref,
            fu_ref, fk_ref, kraw_ref, one_ref, f_ref, g_ref, fill_ref, shift_ref, wt_ref,
            d_ref, gw_ref, mem_ref, gate_ref, ost_ref, tail_ref, sems):
    w_hbm = (wq_hbm, wk_hbm, wv_hbm)

    def cp(src, dst, sem):
        return pltpu.make_async_copy(src, dst, sems.at[sem])

    def start_col_blocks(src_hbm, dst_ref, i0, i1, sem, row0=0):
        src = src_hbm.bitcast(u32)
        for i in range(i0, i1):
            cp(src.at[:, i * 128:(i + 1) * 128], dst_ref.at[i, row0:], sem).start()

    def start_ssm(r0, r1, sem):
        src = ssm_hbm.bitcast(u32)
        for a in range(NCH):
            cp(src.at[r0:r1, a * C:(a + 1) * C], ssm_ref.at[a, r0:r1], sem).start()

    def wait_all(dst, sem):
        cp(dst, dst, sem).wait()

    def even(p):
        return pltpu.bitcast(p << 16, f32)

    def odd(p):
        return pltpu.bitcast(p & jnp.uint32(0xFFFF0000), f32)

    def conv_prep(cb, i, dep=None):
        r0 = KPAD + 8 * i
        p0 = k_ref[cb, r0:r0 + 8, :]
        if dep is not None:
            p0 = jnp.where(one_ref[...] == 1, p0, dep)
        p1 = k_ref[cb, r0 - 1:r0 + 7, :]
        p2 = k_ref[cb, r0 - 2:r0 + 6, :]
        pv = v_ref[cb, 8 * i:8 * i + 8, :]
        w = wt_ref[cb]
        w0, w1, w2, w3 = w[0:1, :], w[1:2, :], w[2:3, :], w[3:4, :]
        e0, o0, e1, o1, o2 = even(p0), odd(p0), even(p1), odd(p1), odd(p2)
        ke = ((e0 * w0 + o1 * w1) + e1 * w2) + o2 * w3
        ko = ((o0 * w0 + e0 * w1) + o1 * w2) + e1 * w3
        re = pltpu.bitcast((ke * even(pv)).astype(bf16).astype(f32), u32)
        ro = pltpu.bitcast((ko * odd(pv)).astype(bf16).astype(f32), u32)
        kv = (re >> 16) | (ro & jnp.uint32(0xFFFF0000))
        u_ref[cb, 8 * i:8 * i + 8, :] = kv
        return kv

    def combine(kf, prev):
        out = []
        for g in range(8):
            o = 32 * g
            out += [kf[o:o + 8] + prev[o + 8:o + 16], kf[o + 8:o + 16] - prev[o:o + 8],
                    kf[o + 16:o + 24] - prev[o + 24:o + 32], kf[o + 24:o + 32] + prev[o + 16:o + 24]]
        return jnp.concatenate(out, axis=0)

    def conv_fwd(cb, r):
        slot = cb % 2
        rows = pl.ds(pl.multiple_of(cb * 64, 64), 64)
        f = f_ref[...]
        kfs = []
        for a in (2 * r, 2 * r + 1):
            fu_ref[slot, NZ + a] = _dot(f, _as_bf16(u_ref[cb, pl.ds(pl.multiple_of(a * 64, 64), 64), :]))
            kfs.append(_dot_nt(f, _as_bf16(ssm_ref[a, rows, :])))
        fk_ref[slot, 2 * r] = combine(kfs[0], jnp.where(r > 0, kraw_ref[...], 0.0))
        fk_ref[slot, 2 * r + 1] = combine(kfs[1], kfs[0])
        kraw_ref[...] = kfs[1]

    def conv_mac(slot, a, nterms, pos, dep=None):
        rows = slice(pos * 16, pos * 16 + 16)
        p = q = None
        for c in range(nterms):
            u = fu_ref[slot, NZ + a - c, rows, :]
            k = fk_ref[slot, c, rows, :]
            ua, ub, kc, kd = u[0:8], u[8:16], k[0:8], k[8:16]
            if c == 0 and dep is not None:
                ua = jnp.where(one_ref[...] == 1, ua, pltpu.bitcast(dep, f32))
            p = (ua * kc if p is None else p + ua * kc) - ub * kd
            q = (ua * kd if q is None else q + ua * kd) + ub * kc
        return pltpu.bitcast(jnp.concatenate([p, q], axis=0).astype(bf16), u32)

    def conv_inv(a_ref, cb, dst, a, zs):
        rows = pl.ds(pl.multiple_of(a * 64, 64), 64)
        y = _dot(g_ref[...], _as_bf16(jnp.concatenate(zs, axis=0)))
        kv = _as_bf16(u_ref[cb, rows, :]).astype(f32)
        q = _as_bf16(x_ref[cb, rows, :]).astype(f32)
        a_ref[dst, pl.ds(pl.multiple_of(a * C, C), C), :] = q * (y + kv * wt_ref[cb, KS:KS + 1, :])

    def after(w, tok):
        if tok is None:
            return w
        return jnp.concatenate([jnp.where(one_ref[...] == 1, w[0:8], tok), w[8:]], axis=0)

    def prologue(stage_ref, acc_ref):
        st3 = stage_ref.reshape(NG * D, 8, E)

        def start_w(g):
            r0 = (g % 2) * 8
            cp(w_hbm[g // 2].bitcast(u32).at[:, r0:r0 + 8, :], st3.at[g * D:(g + 1) * D], SEM_W + g - 1).start()

        def slice_copies(q):
            cols = pl.ds(pl.multiple_of(q * DQ, DQ), DQ)
            return (cp(x3_hbm.at[:, NT:SEG, cols], xr_ref.at[q], SEM_Q + q),
                    cp(wq_hbm.bitcast(u32).at[cols, 0:8, :], st3.at[cols], SEM_Q + q))

        small = [cp(shift_hbm, shift_ref, SEM_SMALL), cp(d_hbm, d_ref, SEM_SMALL), cp(gw_hbm, gw_ref, SEM_SMALL),
                 cp(mem_hbm, mem_ref, SEM_SMALL), cp(f_hbm, f_ref, SEM_SMALL), cp(g_hbm, g_ref, SEM_SMALL)]
        for q in range(NQ):
            for c in slice_copies(q):
                c.start()
        for c in small:
            c.start()
        for g in range(1, NG):
            start_w(g)
            if g >= 2:
                start_col_blocks(k_hbm, k_ref, 2 * g - 4, 2 * g - 2, SEM_K + g - 2, row0=KPAD)
                start_col_blocks(v_hbm, v_ref, 2 * g - 4, 2 * g - 2, SEM_V + g - 2)
        start_col_blocks(wo_hbm, wo_ref, 0, NCB, SEM_WO)
        fill_ref[...] = _fill_matrix()
        one_ref[...] = jnp.ones((8, 128), jnp.int32)
        k_ref[:, KPAD - 8:KPAD, :] = jnp.zeros((NCB + 1, 8, 128), u32)
        wt_ref[...] = jnp.zeros(wt_ref.shape, f32)
        kraw_ref[...] = jnp.zeros(kraw_ref.shape, f32)
        fu_ref[0, NZ - 1] = jnp.zeros((256, 128), f32)

        def clear(a, c):
            rows = pl.ds(pl.multiple_of(a * 64, 64), 64)
            k_ref[NCB, pl.ds(pl.multiple_of(KPAD + a * 64, 32), 64), :] = jnp.zeros((64, 128), u32)
            v_ref[NCB, rows, :] = jnp.zeros((64, 128), u32)
            acc_ref[a] = jnp.zeros((NSEG * M, E), f32)
            return c
        lax.fori_loop(0, 16, clear, 0)

        def unpack_pair(w):
            return pltpu.bitcast(even(w).astype(bf16), u32), pltpu.bitcast(odd(w).astype(bf16), u32)

        def store_pre(idx, r1, r2):
            cc = jnp.concatenate([r1.reshape(NSEG, 8, E), r2.reshape(NSEG, 8, E)], axis=1).astype(bf16)
            pre_ref[:, idx] = pltpu.bitcast(cc, u32)

        def first(q, c):
            for cc in slice_copies(q):
                cc.wait()
            xq = pltpu.bitcast(xr_ref[q].astype(f32).reshape(NSEG * M, DQ).astype(bf16), u32)
            xb_ref[q] = xq
            sub = stage_ref.at[pl.ds(pl.multiple_of(q * (8 * DQ), 8 * DQ), 8 * DQ), :]
            rows = pl.ds(pl.multiple_of(q * (DQ // 2), DQ // 2), DQ // 2)
            for j in range(8):
                rs = []
                for h, w in zip((2 * j, 2 * j + 1), unpack_pair(sub[pl.ds(j, DQ, stride=8), :])):
                    wn_ref[h, rows, :] = w
                    r = _dot(_as_bf16(xq), _as_bf16(w)) + acc_ref[h]
                    acc_ref[h] = r
                    rs.append(r)
                store_pre(j, *rs)
            return c
        lax.fori_loop(0, NQ, first, 0)

        start_col_blocks(x_hbm, x_ref, 0, NCB, SEM_X)
        start_ssm(0, 64, SEM_SSM0)
        for c in small:
            c.wait()
        sh = shift_ref[...].astype(f32)
        dv = d_ref[...].astype(f32)
        for n in range(NCB):
            wt_ref[n, 0:KS, :] = sh[:, n * 128:(n + 1) * 128]
            wt_ref[n, KS:KS + 1, :] = dv[n:n + 1, :]

        def group(g, c):
            wait_all(st3.at[pl.ds(g * D, D)], SEM_W + g - 1)

            @pl.when(g >= 2)
            def _():
                wait_all(k_ref.at[pl.ds(2 * g - 4, 2), KPAD:], SEM_K + g - 2)
                wait_all(v_ref.at[pl.ds(2 * g - 4, 2)], SEM_V + g - 2)

            cbs = [jnp.where(g >= 2, 2 * g - 4 + i, NCB) for i in range(2)]
            npt = CFG["npt"]
            toks = [None] * 32
            for k in range(npt):
                t = None
                for i in range(k * 256 // npt, (k + 1) * 256 // npt):
                    t = conv_prep(cbs[i // 128], i % 128, t)
                    zero = pltpu.bitcast(jnp.where(one_ref[...] == 1, jnp.uint32(0), t), f32)
                    for v in range(i, 288, 256):
                        rows = slice(8 * (v % 32), 8 * (v % 32) + 8)
                        if v < 160:
                            fu_ref[1, jnp.minimum((g - 1) * 5 + v // 32, NZ + NCH - 1), rows, :] = zero
                        else:
                            fk_ref[1, jnp.minimum((g - 1) * 4 + v // 32 - 5, NCH - 1), rows, :] = zero
                toks[32 - npt + k] = t
            sub = stage_ref.at[pl.ds(pl.multiple_of(g * (8 * D), 8 * D), 8 * D), :]
            for j in range(8):
                ws = [unpack_pair(sub[pl.ds(blk * 2048 + j, 256, stride=8), :]) for blk in range(D // 256)]
                xb = _as_bf16(jnp.concatenate([xb_ref[q] for q in range(NQ)], axis=1))
                rs = [None, None]
                for i in range(2):
                    wn_ref[g * 16 + 2 * j + i] = jnp.concatenate([wb[i] for wb in ws], axis=0)
                if j == 0:
                    for blk in range(D // 256):
                        for i in range(2):
                            d = _dot(xb[:, blk * 256:(blk + 1) * 256], _as_bf16(ws[blk][i]))
                            rs[i] = d if rs[i] is None else d + rs[i]
                else:
                    for i in range(2):
                        tk = toks[4 * j + 2 * i:4 * j + 2 * i + 2]
                        w = jnp.concatenate([after(ws[0][i], tk[0]), ws[1][i], after(ws[2][i], tk[1]), ws[3][i]], axis=0)
                        rs[i] = _dot(xb, _as_bf16(w))
                store_pre(g * 8 + j, *rs)
            return c
        lax.fori_loop(1, NG, group, 0)

    pl.run_scoped(prologue, pltpu.VMEM((NG * 8 * D, E), u32), pltpu.VMEM((16, NSEG * M, E), f32))

    start_ssm(64, D // 2, SEM_SSM1)
    wait_all(wo_ref, SEM_WO)
    wait_all(x_ref, SEM_X)
    wait_all(ssm_ref.at[:, 0:64], SEM_SSM0)

    scale = E ** -0.5

    def main(odef_ref, b_ref, a_ref):
        def step(s, mem, t):
            cfg = CFG["steps"][t]
            cb = s // 8
            r = s % 8
            icb = jnp.maximum(cb - 1, 0)
            idst = jnp.where(cb >= 1, cb - 1, NCB)
            mslot = (cb + 1) % 2
            nh = 8 // UNROLL
            chunks = ((nh * t + r // UNROLL, nh * t + nh), (NCH - 1 - nh * t - r // UNROLL, NCH - nh * t))
            zs = ({}, {})

            xrows = pl.ds(pl.multiple_of(s * 16, 16), 16)
            xs = [_as_bf16(x_ref[n, xrows, :]).astype(f32) for n in range(NCB)]
            h32 = jnp.concatenate([jnp.concatenate(xs, axis=1)[0:NT], mem], axis=0).astype(bf16)
            r0 = pl.multiple_of(s * 8, 8)

            def gate():
                gw = gw_ref[...].astype(f32)
                gl = None
                for n in range(NCB):
                    xg = _as_bf16(x_ref[n, xrows, :]).astype(f32) * gw[n:n + 1, :]
                    gl = xg if gl is None else gl + xg
                g = jnp.broadcast_to(jax.nn.sigmoid(jnp.sum(gl, axis=-1, keepdims=True)), (SEG, 128))
                gate_ref[s] = g
                g = pltpu.bitcast(g, u32)
                return (g[0:8] | g[8:16]) | (g[16:24] | g[24:32])

            def mac_job(w, pos):
                zs[w][pos] = conv_mac(mslot, chunks[w][0], chunks[w][1], pos)
                return zs[w][pos]

            jobs = [(cfg["dues"][i], functools.partial(mac_job, i % 2, i // 2)) for i in range(32)]
            jobs.append((cfg["gate"], gate))
            state = dict(count=0, due={})

            def sdot(lhs, w, acc=None, weight=1):
                c = state["count"]
                toks = [t for cc in range(c, c + weight) for t in state["due"].pop(cc, [])]
                nt = w.shape[0] // 64
                if toks:
                    tiles = [w[64 * i:64 * (i + 1)] for i in range(nt)]
                    for i, t in enumerate(toks):
                        tiles[i % nt] = after(tiles[i % nt], t)
                    w = jnp.concatenate(tiles, axis=0)
                d = _dot(lhs, _as_bf16(w))
                d = d if acc is None else d + acc
                for due, fn in jobs:
                    if c <= due - 4 < c + weight:
                        state["due"].setdefault(due, []).append(fn())
                state["count"] = c + weight
                return d

            def proj(m, j):
                r1 = sdot(h32, wn_ref[m * H + 2 * j], weight=4)
                r2 = sdot(h32, wn_ref[m * H + 2 * j + 1], weight=4)
                p = _as_bf16(pre_ref[s, m * NP + j]).astype(f32)
                if m == 0:
                    return jnp.concatenate([r1, r2, p], axis=0)
                return jnp.concatenate([r1, r2, p, jnp.zeros((48, E), f32)], axis=0).astype(bf16)

            def qk(q80, k80, due):
                fill = fill_ref[...]
                sc = jnp.where(fill == 0.0, _dot_nt(q80.astype(bf16), k80), fill)
                p = jnp.exp2((sc - jnp.max(sc, axis=-1, keepdims=True)) * (scale * LOG2E))
                den = jnp.sum(p, axis=-1, keepdims=True)
                rc = pl.reciprocal(den, approx=True)
                p = p * (rc * (2.0 - den * rc))
                if due is not None:
                    pb = pltpu.bitcast(p, u32)
                    tok = pb[0:8]
                    for i in range(1, 10):
                        tok = tok | pb[8 * i:8 * i + 8]
                    state["due"].setdefault(due, []).append(tok)
                return p

            def pv(j, p, v80):
                o80 = _dot(p.astype(bf16), v80)
                odef_ref[pl.ds(r0, 8), (2 * j) * E:(2 * j + 1) * E] = o80[64:72]
                odef_ref[pl.ds(r0, 8), (2 * j + 1) * E:(2 * j + 2) * E] = o80[72:80]
                return jnp.concatenate([o80[0:32], o80[32:64]], axis=1).astype(bf16)

            def wo_part(o, j0, j1, n, acc=None):
                for j in range(j0, j1):
                    acc = sdot(o[j], wo_ref[n, j * 128:(j + 1) * 128, :], acc)
                return acc

            qs, ks, vs, ps, os_ = {}, {}, {}, {}, {}
            for j in range(0, NP, 2):
                for m, jj in cfg["order"]:
                    (qs, ks, vs)[m][j + jj] = proj(m, j + jj)
                if j == 2:
                    for jj in range(4):
                        ps[jj] = qk(qs[jj], ks[jj], cfg["sm"][jj])
                elif j > 2:
                    ps[j] = qk(qs[j], ks[j], cfg["sm"][j])
                    ps[j + 1] = qk(qs[j + 1], ks[j + 1], cfg["sm"][j + 1])
                    os_[j - 4] = pv(j - 4, ps[j - 4], vs[j - 4])
                    os_[j - 3] = pv(j - 3, ps[j - 3], vs[j - 3])
            na = NP - 4
            acc = {}
            nw = cfg["nw"]
            for n in range(nw):
                acc[n] = wo_part(os_, 0, na, n)
            for jj in range(na, NP):
                os_[jj] = pv(jj, ps[jj], vs[jj])
            acc[nw] = wo_part(os_, 0, na, nw)
            for n in range(nw + 1):
                acc[n] = wo_part(os_, na, NP, n, acc[n])
            for n in range(nw + 1, 8):
                acc[n] = wo_part(os_, 0, NP, n)
            assert state["count"] == 512 and not state["due"], state
            for w in range(2):
                conv_inv(a_ref, icb, idst, chunks[w][0], [zs[w][pos] for pos in range(16)])
            if t == UNROLL - 1:
                for tt in range(UNROLL):
                    conv_fwd(cb, r - t + tt)
            for n in range(NCB):
                b_ref[n, s, 0:NT, :] = acc[n][0:NT]
            return jnp.concatenate([acc[n][NT:SEG] for n in range(NCB)], axis=1).astype(bf16).astype(f32)

        def steps(i, mem):
            @pl.when(i == 8 // UNROLL)
            def _():
                wait_all(ssm_ref.at[:, 64:], SEM_SSM1)
            for t in range(UNROLL):
                mem = step(i * UNROLL + t, mem, t)
            return mem

        lax.fori_loop(0, _DBG_STEPS // UNROLL, steps, mem_ref[...].astype(f32))

        def out_copy(n, rows=SEG):
            return cp(ost_ref.at[n % 2, :, 0:rows],
                      out_hbm.at[:, 0:rows, pl.ds(pl.multiple_of(n * 128, 128), 128)], SEM_OUT + n % 2)

        tail_copy = cp(tail_ref, out_hbm.at[:, NT:SEG, (NCB - 1) * 128:], SEM_OUT + 2)

        def fin(n, last):
            def mix(dst, r0, r1):
                for blk in range(8):
                    sg = slice(blk * 8, (blk + 1) * 8)
                    b = b_ref[n, sg, r0:r1]
                    a = a_ref[n, blk * 256:(blk + 1) * 256, :].reshape(8, SEG, 128)[:, r0:r1]
                    g = gate_ref[sg, r0:r1]
                    dst[sg, 0:r1 - r0] = (g * a + (1.0 - g) * b).astype(bf16)

            zs, toks, t = ([], []), [], None
            for pos in range(16):
                if pos % CFG["fgrp"] == 0:
                    t = None
                for w in range(2):
                    t = conv_mac((NCB - 1) % 2, n + 8 * w, 8 + 8 * w, pos, t)
                    zs[w].append(t)
                if pos % CFG["fgrp"] == CFG["fgrp"] - 1:
                    toks.append(t)
            bd = None
            for kb in range(8):
                if kb == CFG["finv"]:
                    for w in range(2):
                        conv_inv(a_ref, NCB - 1, NCB - 1, n + 8 * w, zs[w])
                if last and kb == CFG["fout"]:
                    mix(ost_ref.at[n % 2], 0, NT)
                    out_copy(n, NT).start()
                w = after(wo_ref[n, kb * 256:(kb + 1) * 256, :], toks[kb - 1] if 0 < kb <= len(toks) else None)
                d = _dot(odef_ref[:, kb * 512:(kb + 1) * 512].astype(bf16), _as_bf16(w))
                bd = d if bd is None else d + bd
            b_ref[n, :, NT:SEG, :] = bd.reshape(NSEG, 8, 128)
            if last:
                mix(tail_ref, NT, SEG)
                tail_copy.start()
            else:
                mix(ost_ref.at[n % 2], 0, SEG)
                out_copy(n).start()

        def fin_loop(n, c):
            @pl.when(n >= 2)
            def _():
                out_copy(n - 2).wait()
            fin(n, False)
            return c
        lax.fori_loop(0, NCB - 1, fin_loop, 0)
        out_copy(NCB - 3).wait()
        fin(NCB - 1, True)
        out_copy(NCB - 2).wait()
        out_copy(NCB - 1, NT).wait()
        tail_copy.wait()

    pl.run_scoped(main, pltpu.VMEM((NSEG * 8, H * E), f32), pltpu.VMEM((NCB, NSEG, SEG, 128), f32),
                  pltpu.VMEM((NCB + 1, S, 128), f32))


@jax.jit
def pallas_gated_mix__ssm_conv_h3__memory_aug_recurrent_mem_tr__prompt_kernel(
    A_q: jax.Array,
    A_k: jax.Array,
    A_v: jax.Array,
    A_shift_k: jax.Array,
    A_ssm_k: jax.Array,
    A_ssm_D: jax.Array,
    B_x: jax.Array,
    B_mem0: jax.Array,
    B_Wq: jax.Array,
    B_Wk: jax.Array,
    B_Wv: jax.Array,
    B_Wo: jax.Array,
    B_seg_len: jax.Array,
    gate_w: jax.Array,
):
    del B_x, B_seg_len
    f_tab, g_tab = _dft_tables()
    out = pl.pallas_call(
        _kernel,
        out_shape=jax.ShapeDtypeStruct((NSEG, SEG, D), bf16),
        in_specs=[pl.BlockSpec(memory_space=pl.ANY)] * 15,
        out_specs=pl.BlockSpec(memory_space=pl.ANY),
        scratch_shapes=[
            pltpu.VMEM((3 * H, D // 2, E), u32),
            pltpu.VMEM((NCB, H * E // 2, 128), u32),
            pltpu.VMEM((NCB, S // 2, 128), u32),
            pltpu.VMEM((NQ, NSEG, M, DQ), bf16),
            pltpu.VMEM((NQ, NSEG * 4, DQ), u32),
            pltpu.VMEM((NSEG, 3 * NP, 8, E), u32),
            pltpu.VMEM((NCB + 1, KPAD + S // 2, 128), u32),
            pltpu.VMEM((NCB + 1, S // 2, 128), u32),
            pltpu.VMEM((NCH, D // 2, 128), u32),
            pltpu.VMEM((NCB + 1, S // 2, 128), u32),
            pltpu.VMEM((2, NZ + NCH, 256, 128), f32),
            pltpu.VMEM((2, NCH, 256, 128), f32),
            pltpu.VMEM((256, 128), f32),
            pltpu.VMEM((8, 128), jnp.int32),
            pltpu.VMEM((256, 128), bf16),
            pltpu.VMEM((128, 256), bf16),
            pltpu.VMEM((80, 128), f32),
            pltpu.VMEM((KS, D), bf16),
            pltpu.VMEM((NCB + 1, 8, 128), f32),
            pltpu.VMEM((NCB, 128), bf16),
            pltpu.VMEM((NCB, 128), bf16),
            pltpu.VMEM((M, D), bf16),
            pltpu.VMEM((NSEG, SEG, 128), f32),
            pltpu.VMEM((2, NSEG, SEG, 128), bf16),
            pltpu.VMEM((NSEG, M, 128), bf16),
            pltpu.SemaphoreType.DMA((NSEM,)),
        ],
        compiler_params=pltpu.CompilerParams(vmem_limit_bytes=120 * 2**20),
    )(A_q.reshape(NSEG, SEG, D), A_q.reshape(S, D), A_k.reshape(S, D), A_v.reshape(S, D), A_shift_k.T,
      A_ssm_k, A_ssm_D.reshape(NCB, 128), B_mem0.reshape(M, D), B_Wq, B_Wk, B_Wv,
      B_Wo.reshape(H * E, D), gate_w.reshape(NCB, 128), f_tab, g_tab)
    return out.reshape(1, S, D)
```
